```python
import jax
import jax.numpy as jnp

def _softmax(x, axis=-1):
    return jax.nn.softmax(x, axis=axis)
def _gelu(x):
    return jax.nn.gelu(x, approximate=True)
def _silu(x):
    return jax.nn.silu(x)
def _sigmoid(x):
    return jax.nn.sigmoid(x)
def _layernorm(x, axis=-1, eps=1e-5):
    m = jnp.mean(x, axis=axis, keepdims=True)
    v = jnp.var(x, axis=axis, keepdims=True)
    return (x - m) / jnp.sqrt(v + eps)
def _scatter_add(tgt, idx, src, axis=0):
    return tgt.at[idx].add(src)
def _segment_sum(src, seg, n):
    return jax.ops.segment_sum(src, seg, n)
class _Rng:
    def __init__(self, key):
        self._k = key
    def _next(self):
        self._k, sub = jax.random.split(self._k)
        return sub
    def normal(self, shape):
        return jax.random.normal(self._next(), shape, dtype=jnp.bfloat16)
    def randint(self, lo, hi, shape):
        return jax.random.randint(self._next(), shape, lo, hi, dtype=jnp.int32)
    def uniform(self, shape, lo=0.0, hi=1.0):
        return jax.random.uniform(self._next(), shape, jnp.bfloat16, lo, hi)
    def permutation(self, n):
        return jax.random.permutation(self._next(), n)


kernel_name = 'concat_heads__gqa_block_cached__mha_block_cached__near_ridge'

def setup_inputs():
    _rng = _Rng(jax.random.key(int.from_bytes(__import__("os").urandom(4), "little")))
    _w = (lambda a: (lambda t: t.astype(jnp.bfloat16) if jnp.issubdtype(t.dtype, jnp.floating) else t)(jnp.asarray(a)))
    def _A_setup():
        B, Sq, D = 16, 160, 640
        Hq, Hkv, Sk, Dh = 32, 32, 512, 192
        assert Hq % Hkv == 0, (Hq, Hkv)
        return {
            "x": _w((lambda *s: _rng.normal(s) * 0.05)(B, Sq, D)),
            "k_cache": _w((lambda *s: _rng.normal(s) * 0.05)(B, Hkv, Sk, Dh)),
            "v_cache": _w((lambda *s: _rng.normal(s) * 0.05)(B, Hkv, Sk, Dh)),
            "wq": _w((lambda *s: _rng.normal(s) * 0.05)(D, Hq * Dh) * (D ** -0.5)),
            "wo": _w((lambda *s: _rng.normal(s) * 0.05)(Hq * Dh, D) * ((Hq * Dh) ** -0.5)),
        }
    _A_in = _A_setup()

    def _B_setup():
        B, Sq, D = 16, 160, 640
        H, Sk, Dh = 32, 512, 192
        return {
            "x": _w((lambda *s: _rng.normal(s) * 0.05)(B, Sq, D)),
            "k_cache": _w((lambda *s: _rng.normal(s) * 0.05)(B, H, Sk, Dh)),
            "v_cache": _w((lambda *s: _rng.normal(s) * 0.05)(B, H, Sk, Dh)),
            "wq": _w((lambda *s: _rng.normal(s) * 0.05)(D, H * Dh) * (D ** -0.5)),
            "wo": _w((lambda *s: _rng.normal(s) * 0.05)(H * Dh, D) * ((H * Dh) ** -0.5)),
        }
    _B_in = _B_setup()

    return {
        "A_x": _A_in["x"],
        "A_k_cache": _A_in["k_cache"],
        "A_v_cache": _A_in["v_cache"],
        "A_wq": _A_in["wq"],
        "A_wo": _A_in["wo"],
        "B_x": _B_in["x"],
        "B_k_cache": _B_in["k_cache"],
        "B_v_cache": _B_in["v_cache"],
        "B_wq": _B_in["wq"],
        "B_wo": _B_in["wo"],
    }

def reference(A_x, A_k_cache, A_v_cache, A_wq, A_wo, B_x, B_k_cache, B_v_cache, B_wq, B_wo):
    def _A_ref(x, k_cache, v_cache, wq, wo):
        B, Sq, D = x.shape
        Hq, Dh = 32, 192
        Hkv = k_cache.shape[1]
        rep = Hq // Hkv
        q = (lambda x, *d: x.transpose(*d))((x @ wq).reshape(B, Sq, Hq, Dh), 0, 2, 1, 3)
        k = jnp.repeat(k_cache, rep, axis=1)
        v = jnp.repeat(v_cache, rep, axis=1)
        scores = jnp.einsum("bhqd,bhkd->bhqk", q, k) * (Dh ** -0.5)
        p = _softmax(scores, axis=-1)
        o = jnp.einsum("bhqk,bhkd->bhqd", p, v)
        return (lambda x, *d: x.transpose(*d))(o, 0, 2, 1, 3).reshape(B, Sq, Hq * Dh) @ wo

    def _B_ref(x, k_cache, v_cache, wq, wo):
        B, Sq, D = x.shape
        H, Dh = 32, 192
        q = (lambda x, *d: x.transpose(*d))((x @ wq).reshape(B, Sq, H, Dh), 0, 2, 1, 3)
        scores = jnp.einsum("bhqd,bhkd->bhqk", q, k_cache) * (Dh ** -0.5)
        p = _softmax(scores, axis=-1)
        o = jnp.einsum("bhqk,bhkd->bhqd", p, v_cache)
        return (lambda x, *d: x.transpose(*d))(o, 0, 2, 1, 3).reshape(B, Sq, H * Dh) @ wo

    a = _A_ref(A_x, A_k_cache, A_v_cache, A_wq, A_wo)
    b = _B_ref(B_x, B_k_cache, B_v_cache, B_wq, B_wo)
    return jnp.concatenate([a, b], axis=-1)
```

```python
import functools
import jax
import jax.numpy as jnp
from jax import lax
import jax.experimental.pallas as pl
import jax.experimental.pallas.tpu as pltpu

BB = 4
LOG2E = 1.4426950408889634
bf16 = jnp.bfloat16
f32 = jnp.float32


def _qproj(x, wq, scale, lo):
    q = jnp.dot(x, wq, preferred_element_type=f32) * scale
    qm = q[:, 128:256]
    q0 = jnp.concatenate([q[:, 0:128], jnp.where(lo, qm, 0.0)], axis=1).astype(bf16)
    q1 = jnp.concatenate([jnp.where(lo, 0.0, qm), q[:, 256:384]], axis=1).astype(bf16)
    return q0, q1


def _score(qh, kt, h):
    s = jnp.dot(qh, kt[h * 128:h * 128 + 256, :], preferred_element_type=f32)
    m = jnp.max(s, axis=1, keepdims=True)
    p = jnp.exp2(s - m)
    l = jnp.sum(p, axis=1, keepdims=True)
    return p.astype(bf16), l


def _pv(p, l, vt, h):
    o = lax.dot_general(p, vt[h * 128:h * 128 + 256, :], (((1,), (1,)), ((), ())),
                        preferred_element_type=f32)
    return o * (1.0 / l)


def _oproj(o0, o1, wo, lo):
    op = jnp.concatenate([o0[:, 0:128], jnp.where(lo, o0[:, 128:256], o1[:, 0:128]), o1[:, 128:256]], axis=1)
    return jnp.dot(op.astype(bf16), wo, preferred_element_type=f32)


def _kernel(ax, ak, av, awq, awo, bx, bk, bv, bwq, bwo, o_ref, acc, *, scale, nhp):
    hp = pl.program_id(0)
    bi = pl.program_id(1)
    sq = ax.shape[1]
    d = ax.shape[2]

    @pl.when(hp == 0)
    def _():
        for j in range(BB):
            acc[bi * BB + j] = jnp.zeros(acc.shape[1:], f32)

    lo = lax.broadcasted_iota(jnp.int32, (sq, 128), 1) < 64
    units = []
    for j in range(BB):
        units.append((j, 0, ax, ak, av, awq, awo))
        units.append((j, 1, bx, bk, bv, bwq, bwo))
    U = len(units)
    Q = {}
    P = {}
    O = {}

    def q_(u):
        j, br, x, k, v, wq, wo = units[u]
        Q[u] = _qproj(x[bi * BB + j], wq[...], scale, lo)

    def s_(u, h):
        j, br, x, k, v, wq, wo = units[u]
        P[u, h] = _score(Q[u][h], k.at[j, 0], h)

    def pv_(u, h):
        j, br, x, k, v, wq, wo = units[u]
        O[u, h] = _pv(*P[u, h], v.at[j, 0], h)

    def o_(u):
        j, br, x, k, v, wq, wo = units[u]
        acc[bi * BB + j, :, br * d:(br + 1) * d] += _oproj(O[u, 0], O[u, 1], wo[...], lo)

    q_(0)
    q_(1)
    for u in range(U):
        s_(u, 0)
        s_(u, 1)
        if u >= 1:
            o_(u - 1)
        elif u + 2 < U:
            q_(u + 2)
        pv_(u, 0)
        if u >= 1 and u + 2 < U:
            q_(u + 2)
        pv_(u, 1)
    o_(U - 1)

    @pl.when(hp == nhp - 1)
    def _():
        for j in range(BB):
            o_ref[j] = acc[bi * BB + j].astype(o_ref.dtype)


@jax.jit
def pallas_concat_heads__gqa_block_cached__mha_block_cached__near_ridge_kernel(
    A_x, A_k_cache, A_v_cache, A_wq, A_wo, B_x, B_k_cache, B_v_cache, B_wq, B_wo):
    B, Sq, D = A_x.shape
    _, H, Sk, Dh = A_k_cache.shape
    nhp = H // 2

    def tr(c):
        return jnp.swapaxes(c, 2, 3).reshape(B, nhp, 2 * Dh, Sk)

    x_spec = pl.BlockSpec((B, Sq, D), lambda hp, bi: (0, 0, 0))
    kv_spec = pl.BlockSpec((BB, 1, 2 * Dh, Sk), lambda hp, bi: (bi, hp, 0, 0))
    wq_spec = pl.BlockSpec((D, 2 * Dh), lambda hp, bi: (0, hp))
    wo_spec = pl.BlockSpec((2 * Dh, D), lambda hp, bi: (hp, 0))
    out_spec = pl.BlockSpec((BB, Sq, 2 * D), lambda hp, bi: (jnp.where(hp == nhp - 1, bi, 0), 0, 0))
    return pl.pallas_call(
        functools.partial(_kernel, scale=Dh ** -0.5 * LOG2E, nhp=nhp),
        grid=(nhp, B // BB),
        in_specs=[x_spec, kv_spec, kv_spec, wq_spec, wo_spec] * 2,
        out_specs=out_spec,
        out_shape=jax.ShapeDtypeStruct((B, Sq, 2 * D), A_x.dtype),
        scratch_shapes=[pltpu.VMEM((B, Sq, 2 * D), jnp.float32)],
        compiler_params=pltpu.CompilerParams(
            dimension_semantics=("arbitrary", "arbitrary"),
            vmem_limit_bytes=100 * 1024 * 1024),
    )(A_x, tr(A_k_cache), tr(A_v_cache), A_wq, A_wo, B_x, tr(B_k_cache), tr(B_v_cache), B_wq, B_wo)
```

```python
import functools
import jax
import jax.numpy as jnp
from jax import lax
import jax.experimental.pallas as pl
import jax.experimental.pallas.tpu as pltpu

BB = 4
STARTPOS = 0
ALWAYS_OUT = 1
LOG2E = 1.4426950408889634
bf16 = jnp.bfloat16
f32 = jnp.float32
NT = (((1,), (1,)), ((), ()))


def _qproj(x, wq, scale, lo):
    q = jnp.dot(x, wq, preferred_element_type=f32) * scale
    qm = q[:, 128:256]
    q0 = jnp.concatenate([q[:, 0:128], jnp.where(lo, qm, 0.0)], axis=1).astype(bf16)
    q1 = jnp.concatenate([jnp.where(lo, 0.0, qm), q[:, 256:384]], axis=1).astype(bf16)
    return q0, q1


def _score(qh, kt, h):
    s = jnp.dot(qh, kt[h * 128:h * 128 + 256, :], preferred_element_type=f32)
    m = jnp.max(s, axis=1, keepdims=True)
    p = jnp.exp2(s - m)
    l = jnp.sum(p, axis=1, keepdims=True)
    return p.astype(bf16), 1.0 / l


def _schedule(U):
    order = [("q", 0), ("q", 1)]
    L = U - 1
    for u in range(U - 2):
        order += [("s", u, 0), ("s", u, 1)]
        if u >= 1:
            order += [("o", u - 1), ("pv", u, 0), ("q", u + 2), ("pv", u, 1), ("pvc", u)]
        else:
            order += [("q", u + 2), ("pv", u, 0), ("pv", u, 1), ("pvc", u)]
    order += [("s", L - 1, 0), ("s", L - 1, 1)]
    if L - 2 >= 0:
        order += [("o", L - 2)]
    order += [("s", L, 0), ("pv", L - 1, 0), ("s", L, 1), ("pv", L - 1, 1), ("pvc", L - 1),
              ("pv", L, 0), ("pv", L, 1), ("pvc", L), ("o", L - 1), ("o", L)]
    return order


def _kernel(ax, ak, av, awq, awo, bx, bk, bv, bwq, bwo, o_hbm,
            acc, xbuf, wqbuf, wobuf, kvbuf, obuf, kv_sem, x_sem, w_sem, o_sem, *, scale, nhp, nbg):
    step = pl.program_id(0)
    hp = step // nbg
    bi = step % nbg
    nsteps = nhp * nbg
    sq = xbuf.shape[2]
    d = xbuf.shape[3]
    hw = wqbuf.shape[3]
    U = 2 * BB
    slot = step % 2
    wslot = hp % 2

    def kv_copies(st):
        sl = st % 2
        return [pltpu.make_async_copy(src.at[pl.ds((st % nbg) * BB, BB), st // nbg],
                                      kvbuf.at[sl, i], kv_sem.at[sl])
                for i, src in enumerate((ak, av, bk, bv))]

    def x_copies(g):
        return [pltpu.make_async_copy(src.at[pl.ds(g * BB, BB)], xbuf.at[i, pl.ds(g * BB, BB)], x_sem.at[g % 2])
                for i, src in enumerate((ax, bx))]

    def w_copies(h):
        sl = h % 2
        off = pl.multiple_of(h * hw, 128)
        return ([pltpu.make_async_copy(src.at[:, pl.ds(off, hw)], wqbuf.at[sl, i], w_sem.at[sl])
                 for i, src in enumerate((awq, bwq))] +
                [pltpu.make_async_copy(src.at[pl.ds(off, hw), :], wobuf.at[sl, i], w_sem.at[sl])
                 for i, src in enumerate((awo, bwo))])

    def o_copy(g):
        return pltpu.make_async_copy(obuf.at[pl.ds(g * BB, BB)], o_hbm.at[pl.ds(g * BB, BB)], o_sem.at[g])

    @pl.when(step == 0)
    def _():
        for c in x_copies(0) + w_copies(0) + kv_copies(0):
            c.start()

    @pl.when(hp == 0)
    def _():
        for c in x_copies(bi):
            c.wait()

    @pl.when(bi == 0)
    def _():
        for c in w_copies(hp):
            c.wait()

    pltpu.make_async_copy(kvbuf.at[slot], kvbuf.at[slot], kv_sem.at[slot]).wait()

    def prefetch():
        @pl.when(step + 1 < nsteps)
        def _():
            for c in kv_copies(step + 1):
                c.start()

        @pl.when(step + 1 < nbg)
        def _():
            for c in x_copies(step + 1):
                c.start()

        @pl.when(jnp.logical_and(bi == 0, hp + 1 < nhp))
        def _():
            for c in w_copies(hp + 1):
                c.start()

    lo = lax.broadcasted_iota(jnp.int32, (sq, 128), 1) < 64
    Q = {}
    P = {}
    O = {}
    OT = {}
    OC = {}

    def q_(u):
        j, br = u // 2, u % 2
        Q[u] = _qproj(xbuf[br, bi * BB + j], wqbuf[wslot, br], scale, lo)

    def s_(u, h):
        j, br = u // 2, u % 2
        P[u, h] = _score(Q[u][h], kvbuf.at[slot, 2 * br, j], h)

    def pv_(u, h):
        j, br = u // 2, u % 2
        p, r = P[u, h]
        vt = kvbuf.at[slot, 2 * br + 1, j]
        O[u, h] = lax.dot_general(p, vt[h * 256:h * 256 + 128, :], NT, preferred_element_type=f32) * r
        OT[u, h] = lax.dot_general(vt[128 + h * 64:192 + h * 64, :], p[0:128, :], NT,
                                   preferred_element_type=f32)

    def pvc_(u):
        j, br = u // 2, u % 2
        vt = kvbuf.at[slot, 2 * br + 1, j]
        pc = jnp.concatenate([P[u, 0][0][128:sq, :], P[u, 1][0][128:sq, :]], axis=0)
        OC[u] = lax.dot_general(pc, vt[128:256, :], NT, preferred_element_type=f32)

    def o_(u):
        j, br = u // 2, u % 2
        n = sq - 128
        top = jnp.concatenate([OT[u, 0], OT[u, 1]], axis=0).T
        lo_n = lax.broadcasted_iota(jnp.int32, (n, 128), 1) < 64
        bot = jnp.where(lo_n, OC[u][0:n], OC[u][n:2 * n])
        mid = jnp.concatenate([top, bot], axis=0) * jnp.where(lo, P[u, 0][1], P[u, 1][1])
        op = jnp.concatenate([O[u, 0], mid, O[u, 1]], axis=1).astype(bf16)
        r = jnp.dot(op, wobuf[wslot, br], preferred_element_type=f32)
        b = bi * BB + j
        prev = acc[b, :, br * d:(br + 1) * d]
        new = jnp.where(hp == 0, 0.0, prev) + r
        acc[b, :, br * d:(br + 1) * d] = new
        if ALWAYS_OUT:
            obuf[b, :, br * d:(br + 1) * d] = new.astype(obuf.dtype)

    fns = {"q": q_, "s": s_, "pv": pv_, "pvc": pvc_, "o": o_}
    for i, item in enumerate(_schedule(U)):
        if i == STARTPOS:
            prefetch()
        fns[item[0]](*item[1:])

    @pl.when(hp == nhp - 1)
    def _():
        if not ALWAYS_OUT:
            for j in range(BB):
                obuf[bi * BB + j] = acc[bi * BB + j].astype(obuf.dtype)
        o_copy(bi).start()

    @pl.when(step == nsteps - 1)
    def _():
        for g in range(nbg):
            o_copy(g).wait()


@jax.jit
def pallas_concat_heads__gqa_block_cached__mha_block_cached__near_ridge_kernel(
    A_x, A_k_cache, A_v_cache, A_wq, A_wo, B_x, B_k_cache, B_v_cache, B_wq, B_wo):
    B, Sq, D = A_x.shape
    _, H, Sk, Dh = A_k_cache.shape
    nhp = H // 2
    nbg = B // BB

    def tr(c):
        return jnp.swapaxes(c, 2, 3).reshape(B, nhp, 2 * Dh, Sk)

    any_spec = pl.BlockSpec(memory_space=pl.ANY)
    return pl.pallas_call(
        functools.partial(_kernel, scale=Dh ** -0.5 * LOG2E, nhp=nhp, nbg=nbg),
        grid=(nhp * nbg,),
        in_specs=[any_spec] * 10,
        out_specs=any_spec,
        out_shape=jax.ShapeDtypeStruct((B, Sq, 2 * D), A_x.dtype),
        scratch_shapes=[pltpu.VMEM((B, Sq, 2 * D), f32),
                        pltpu.VMEM((2, B, Sq, D), bf16),
                        pltpu.VMEM((2, 2, D, 2 * Dh), bf16),
                        pltpu.VMEM((2, 2, 2 * Dh, D), bf16),
                        pltpu.VMEM((2, 4, BB, 2 * Dh, Sk), bf16),
                        pltpu.VMEM((B, Sq, 2 * D), bf16),
                        pltpu.SemaphoreType.DMA((2,)),
                        pltpu.SemaphoreType.DMA((2,)),
                        pltpu.SemaphoreType.DMA((2,)),
                        pltpu.SemaphoreType.DMA((nbg,))],
        compiler_params=pltpu.CompilerParams(
            dimension_semantics=("arbitrary",),
            disable_bounds_checks=True,
            vmem_limit_bytes=100 * 1024 * 1024),
    )(A_x, tr(A_k_cache), tr(A_v_cache), A_wq, A_wo, B_x, tr(B_k_cache), tr(B_v_cache), B_wq, B_wo)
```

```python
import functools
import jax
import jax.numpy as jnp
from jax import lax
import jax.experimental.pallas as pl
import jax.experimental.pallas.tpu as pltpu

BB = 8
SB = 1
G1 = 24
C0 = 2
RATE = 2
PFPOS = 1
PFSTEP = 3
PAT = "s0:0,p0:-1,q:2,s1:0,p1:-1,c:-1,o:-2"
SPAT = PAT
LOG2E = 1.4426950408889634
bf16 = jnp.bfloat16
f32 = jnp.float32
NT = (((1,), (1,)), ((), ()))


def _qproj(x, wq, scale, lo):
    q = jnp.dot(x, wq, preferred_element_type=f32) * scale
    qm = q[:, 128:256]
    q0 = jnp.concatenate([q[:, 0:128], jnp.where(lo, qm, 0.0)], axis=1).astype(bf16)
    q1 = jnp.concatenate([jnp.where(lo, 0.0, qm), q[:, 256:384]], axis=1).astype(bf16)
    return q0, q1


def _score(qh, kt, h):
    s = jnp.dot(qh, kt[h * 128:h * 128 + 256, :], preferred_element_type=f32)
    m = jnp.max(s, axis=1, keepdims=True)
    p = jnp.exp2(s - m)
    t = (p[:, 0:128] + p[:, 128:256]) + (p[:, 256:384] + p[:, 384:512])
    p = jnp.concatenate([p[:, 0:384], jnp.minimum(p[:, 384:512], t)], axis=1)
    l = jnp.sum(t, axis=1, keepdims=True)
    r = pl.reciprocal(l, approx=True)
    r = r * (2.0 - l * r)
    return p.astype(bf16), r, p[0:128].astype(bf16), p[128:].astype(bf16)


def _schedule(U, pat):
    pat = [(a.split(":")[0], int(a.split(":")[1])) for a in pat.split(",")]
    order = []
    for t in range(-4, U + 4):
        for name, lag in pat:
            u = t + lag
            if 0 <= u < U:
                order.append({"s0": ("s", u, 0), "s1": ("s", u, 1), "p0": ("pv", u, 0), "p1": ("pv", u, 1),
                              "c": ("pvc", u), "q": ("q", u), "o": ("o", u)}[name])
    return order


def _kernel(ax, ak, av, awq, awo, bx, bk, bv, bwq, bwo, o_hbm,
            acc, xbuf, wqbuf, wobuf, kvbuf, obuf, kv_sem, x_sem, w_sem, o_sem, *, scale, nhp, nb):
    sq = xbuf.shape[2]
    d = xbuf.shape[3]
    hw = wqbuf.shape[3]
    ng = nhp * nb
    lg = nb.bit_length() - 1
    assert nb == 1 << lg

    def kv_start(g):
        hp, b = g >> lg, g & (nb - 1)
        for i, src in enumerate((ak, av, bk, bv)):
            pltpu.make_async_copy(src.at[b, hp], kvbuf.at[b, i], kv_sem.at[b]).start()

    def kv_wait(b):
        pltpu.make_async_copy(kvbuf.at[b], kvbuf.at[b], kv_sem.at[b]).wait()

    def x_start(b):
        for i, src in enumerate((ax, bx)):
            pltpu.make_async_copy(src.at[b], xbuf.at[b, i], x_sem.at[b]).start()

    def x_wait(b):
        pltpu.make_async_copy(xbuf.at[b], xbuf.at[b], x_sem.at[b]).wait()

    def w_copies(h):
        sl = h & 1
        off = h * hw if isinstance(h, int) else pl.multiple_of(h * hw, 128)
        return ([pltpu.make_async_copy(src.at[:, pl.ds(off, hw)], wqbuf.at[sl, i], w_sem.at[0, sl])
                 for i, src in enumerate((awq, bwq))] +
                [pltpu.make_async_copy(src.at[pl.ds(off, hw), :], wobuf.at[sl, i], w_sem.at[1, sl])
                 for i, src in enumerate((awo, bwo))])

    def w_wait(sl):
        pltpu.make_async_copy(wqbuf.at[sl], wqbuf.at[sl], w_sem.at[0, sl]).wait()
        pltpu.make_async_copy(wobuf.at[sl], wobuf.at[sl], w_sem.at[1, sl]).wait()

    lo = lax.broadcasted_iota(jnp.int32, (sq, 128), 1) < 64

    def body(g0, nbat, prefetch, pat):
        hp = g0 >> lg
        b0 = g0 & (nb - 1)
        wslot = hp & 1
        U = 2 * nbat
        Q, P, O, OT, OC = {}, {}, {}, {}, {}

        def q_(u):
            j, br = u // 2, u % 2
            Q[u] = _qproj(xbuf[b0 + j, br], wqbuf[wslot, br], scale, lo)

        def s_(u, h):
            j, br = u // 2, u % 2
            P[u, h] = _score(Q[u][h], kvbuf.at[b0 + j, 2 * br], h)

        def pv_(u, h):
            j, br = u // 2, u % 2
            p, r, ptop, _ = P[u, h]
            vt = kvbuf.at[b0 + j, 2 * br + 1]
            O[u, h] = lax.dot_general(p, vt[h * 256:h * 256 + 128, :], NT, preferred_element_type=f32) * r
            OT[u, h] = lax.dot_general(vt[128 + h * 64:192 + h * 64, :], ptop, NT,
                                       preferred_element_type=f32)

        def pvc_(u):
            j, br = u // 2, u % 2
            vt = kvbuf.at[b0 + j, 2 * br + 1]
            pc = jnp.concatenate([P[u, 0][3], P[u, 1][3]], axis=0)
            OC[u] = lax.dot_general(pc, vt[128:256, :], NT, preferred_element_type=f32)

        def o_(u):
            j, br = u // 2, u % 2
            n = sq - 128
            top = jnp.concatenate([OT[u, 0], OT[u, 1]], axis=0).T
            lo_n = lax.broadcasted_iota(jnp.int32, (n, 128), 1) < 64
            bot = jnp.where(lo_n, OC[u][0:n], OC[u][n:2 * n])
            mid = jnp.concatenate([top, bot], axis=0) * jnp.where(lo, P[u, 0][1], P[u, 1][1])
            op = jnp.concatenate([O[u, 0], mid, O[u, 1]], axis=1).astype(bf16)
            r = jnp.dot(op, wobuf[wslot, br], preferred_element_type=f32)
            b = b0 + j
            prev = acc[b, :, br * d:(br + 1) * d]
            new = jnp.where(hp == 0, 0.0, prev) + r
            acc[b, :, br * d:(br + 1) * d] = new
            obuf[b, :, br * d:(br + 1) * d] = new.astype(obuf.dtype)
            if br == 1:
                @pl.when(hp == nhp - 1)
                def _():
                    pltpu.make_async_copy(obuf.at[b], o_hbm.at[b], o_sem).start()

        fns = {"q": q_, "s": s_, "pv": pv_, "pvc": pvc_, "o": o_}
        for i, item in enumerate(_schedule(U, pat)):
            if i >= PFPOS and (i - PFPOS) % PFSTEP == 0 and (i - PFPOS) // PFSTEP < len(prefetch):
                prefetch[(i - PFPOS) // PFSTEP]()
            fns[item[0]](*item[1:])

    w0 = w_copies(0)
    x_start(0)
    w0[0].start()
    w0[1].start()
    kv_start(0)
    w0[2].start()
    w0[3].start()
    for g in range(1, C0):
        x_start(g)
        kv_start(g)

    def issued(g):
        return jnp.minimum(jnp.minimum(RATE * (g + SB) + C0, g + nb), G1 + BB)

    def small(i, carry):
        g0 = i * SB
        hp = g0 >> lg
        b0 = g0 & (nb - 1)

        @pl.when(hp == 0)
        def _():
            for j in range(SB):
                x_wait(b0 + j)

        @pl.when(b0 == 0)
        def _():
            w_wait(hp & 1)

        for j in range(SB):
            kv_wait(b0 + j)

        def prefetch():
            hi = issued(g0)
            prev = jnp.where(i == 0, C0, issued(g0 - SB))
            for k in range(RATE * SB):
                n = prev + k

                @pl.when(n < hi)
                def _():
                    @pl.when(n < nb)
                    def _():
                        x_start(n)
                    kv_start(n)

            @pl.when(b0 == nb // 2)
            def _():
                for c in w_copies(hp + 1):
                    c.start()

        body(g0, SB, [prefetch], SPAT)
        return carry

    def big(i, carry):
        g0 = i * BB
        hp = g0 >> lg
        b0 = g0 & (nb - 1)

        @pl.when(b0 == 0)
        def _():
            w_wait(hp & 1)

        for j in range(BB):
            kv_wait(b0 + j)

        def pf_kv(j):
            @pl.when(g0 + BB + j < ng)
            def _():
                kv_start(g0 + BB + j)

        def pf_w():
            @pl.when(jnp.logical_and(b0 == nb // 2, hp + 1 < nhp))
            def _():
                for c in w_copies(hp + 1):
                    c.start()

        prefetch = [functools.partial(pf_kv, j) for j in range(BB)] + [pf_w]
        body(g0, BB, prefetch, PAT)
        return carry

    lax.fori_loop(0, G1 // SB, small, 0)
    lax.fori_loop(G1 // BB, ng // BB, big, 0)
    pltpu.make_async_copy(obuf, o_hbm, o_sem).wait()


@jax.jit
def pallas_concat_heads__gqa_block_cached__mha_block_cached__near_ridge_kernel(
    A_x, A_k_cache, A_v_cache, A_wq, A_wo, B_x, B_k_cache, B_v_cache, B_wq, B_wo):
    B, Sq, D = A_x.shape
    _, H, Sk, Dh = A_k_cache.shape
    nhp = H // 2
    assert G1 >= B and G1 % BB == 0 and 2 * BB <= B
    n_iss = C0
    for g0 in range(0, G1, SB):
        assert n_iss >= g0 + SB, (g0, n_iss)
        hi = min(RATE * (g0 + SB) + C0, g0 + B, G1 + BB)
        assert hi - n_iss <= RATE * SB and hi >= n_iss
        n_iss = hi
    assert n_iss == G1 + BB, n_iss
    assert C0 <= B and G1 % SB == 0

    def tr(c):
        return jnp.swapaxes(c, 2, 3).reshape(B, nhp, 2 * Dh, Sk)

    any_spec = pl.BlockSpec(memory_space=pl.ANY)
    return pl.pallas_call(
        functools.partial(_kernel, scale=Dh ** -0.5 * LOG2E, nhp=nhp, nb=B),
        in_specs=[any_spec] * 10,
        out_specs=any_spec,
        out_shape=jax.ShapeDtypeStruct((B, Sq, 2 * D), A_x.dtype),
        scratch_shapes=[pltpu.VMEM((B, Sq, 2 * D), f32),
                        pltpu.VMEM((B, 2, Sq, D), bf16),
                        pltpu.VMEM((2, 2, D, 2 * Dh), bf16),
                        pltpu.VMEM((2, 2, 2 * Dh, D), bf16),
                        pltpu.VMEM((B, 4, 2 * Dh, Sk), bf16),
                        pltpu.VMEM((B, Sq, 2 * D), bf16),
                        pltpu.SemaphoreType.DMA((B,)),
                        pltpu.SemaphoreType.DMA((B,)),
                        pltpu.SemaphoreType.DMA((2, 2)),
                        pltpu.SemaphoreType.DMA(())],
        compiler_params=pltpu.CompilerParams(
            disable_bounds_checks=True,
            vmem_limit_bytes=100 * 1024 * 1024),
    )(A_x, tr(A_k_cache), tr(A_v_cache), A_wq, A_wo, B_x, tr(B_k_cache), tr(B_v_cache), B_wq, B_wo)
```

```python
import functools
import jax
import jax.numpy as jnp
from jax import lax
import jax.experimental.pallas as pl
import jax.experimental.pallas.tpu as pltpu

BB = 8
SB = 1
G1 = 24
C0 = 2
RATE = 2
PFPOS = 1
PFSTEP = 3
PAT = "s0:0,p0:-1,q:2,s1:0,p1:-1,c:-1,o:-2"
SPAT = PAT
LOG2E = 1.4426950408889634
bf16 = jnp.bfloat16
f32 = jnp.float32
u32 = jnp.uint32
NT = (((1,), (1,)), ((), ()))


SMODE = 1


def _qproj(x, wq, scale, lo):
    q = jnp.dot(x, wq, preferred_element_type=f32) * scale
    if SMODE == 0:
        qm = q[:, 128:256]
        q0 = jnp.concatenate([q[:, 0:128], jnp.where(lo, qm, 0.0)], axis=1).astype(bf16)
        q1 = jnp.concatenate([jnp.where(lo, 0.0, qm), q[:, 256:384]], axis=1).astype(bf16)
        return q0, q1
    sq = q.shape[0]
    lane = lax.broadcasted_iota(jnp.int32, (sq // 2, 128), 1)
    t0, t1, t2 = q[:, 0:128], q[:, 128:256], q[:, 256:384]
    out = []
    for h in range(2):
        if h == 0:
            valid = lane < 96
            h1 = t0
            h2 = jnp.where(lo, t1, pltpu.roll(t0, 96, 1))
        else:
            valid = lane >= 32
            h1 = t2
            h2 = jnp.where(lo, pltpu.roll(t2, 32, 1), t1)
        a11, a21 = _split_rows(h1)
        a12, a22 = _split_rows(h2)
        out.append([a.astype(bf16) for a in
                    (a11 + a22, jnp.where(valid, a21 + a22, 0.0), a11, a22, a11 + a12, a21 - a11, a12 - a22)])
    return out


ILV = 1
NOCSE = 1


def _split_rows(a):
    n = a.shape[0]
    if not ILV:
        return a[:n // 2], a[n // 2:]
    a = a.reshape(n // 16, 16, a.shape[1])
    return a[:, 0:8, :].reshape(n // 2, -1), a[:, 8:16, :].reshape(n // 2, -1)


def _join_rows(a, b):
    if not ILV:
        return jnp.concatenate([a, b], axis=0)
    n = a.shape[0]
    return jnp.concatenate([a.reshape(n // 8, 8, -1), b.reshape(n // 8, 8, -1)], axis=1).reshape(2 * n, -1)


def _rows(ref, c, r0, r1):
    return pltpu.bitcast(ref[c, r0 // 2:r1 // 2, :], bf16)


def _wide(ref, r0, n):
    return jnp.concatenate([_rows(ref, c, r0, r0 + n) for c in range(ref.shape[0])], axis=1)


def _krows(h):
    if h == 0:
        return [(0, 96)], [(128, 192), (96, 128)]
    return [(288, 384)], [(256, 288), (192, 256)]


def _scores(qh, kts, h):
    kt = kts(0)
    if SMODE == 0:
        return jnp.dot(qh, kt[h * 128:h * 128 + 256, :], preferred_element_type=f32)
    r1, r2 = _krows(h)
    zf = jnp.zeros((32, 128), f32)

    def ldf(k, rs, c):
        return jnp.concatenate([k[a:b, c * 128:(c + 1) * 128].astype(f32) for a, b in rs], axis=0)

    def pk(f):
        return jnp.concatenate([f, zf] if h == 0 else [zf, f], axis=0).astype(bf16)

    cols = [None] * 4
    for j in range(2):
        def blk(i, name):
            k = kts(i if NOCSE else 0)
            return ldf(k, r1 if name[0] == "1" else r2, j if name[1] == "1" else j + 2)

        bs = [pk(blk(0, "11") + blk(0, "22")), None, pk(blk(1, "12") - blk(1, "22")),
              pk(blk(2, "21") - blk(2, "11")), pk(blk(3, "22")), pk(blk(4, "11") + blk(4, "12")),
              pk(blk(5, "21") + blk(5, "22"))]
        bs[1] = kts(6 if NOCSE else 0)[h * 256:h * 256 + 128, j * 128:(j + 1) * 128]
        m = [None] * 7
        for i in (0, 3, 4, 6, 1, 2, 5):
            m[i] = jnp.dot(qh[i], bs[i], preferred_element_type=f32)
        cols[j] = _join_rows((m[0] + m[3]) + (m[6] - m[4]), m[1] + m[3])
        cols[j + 2] = _join_rows(m[2] + m[4], (m[0] - m[1]) + (m[2] + m[5]))
    return jnp.concatenate(cols, axis=1)


PSCR = 1
QSCR = 1


def _score(qh, kt, h, pref):
    s = _scores(qh, kt, h)
    m = jnp.max(s, axis=1, keepdims=True)
    p = jnp.exp2(s - m)
    t = (p[:, 0:128] + p[:, 128:256]) + (p[:, 256:384] + p[:, 384:512])
    p = jnp.concatenate([p[:, 0:384], jnp.minimum(p[:, 384:512], t)], axis=1)
    l = jnp.sum(t, axis=1, keepdims=True)
    r = pl.reciprocal(l, approx=True)
    r = r * (2.0 - l * r)
    if PSCR:
        pref[...] = p.astype(bf16)
        return None, r, None, None
    return p.astype(bf16), r, p[0:128].astype(bf16), p[128:].astype(bf16)


def _schedule(U, pat):
    pat = [(a.split(":")[0], int(a.split(":")[1])) for a in pat.split(",")]
    order = []
    for t in range(-4, U + 4):
        for name, lag in pat:
            u = t + lag
            if 0 <= u < U:
                order.append({"s0": ("s", u, 0), "s1": ("s", u, 1), "p0": ("pv", u, 0), "p1": ("pv", u, 1),
                              "c": ("pvc", u), "q": ("q", u), "o": ("o", u)}[name])
    return order


def _kernel(ax, ak, av, awq, awo, bx, bk, bv, bwq, bwo, o_hbm,
            acc, xbuf, wqbuf, wobuf, kvbuf, obuf, pbuf, qbuf, kv_sem, x_sem, w_sem, o_sem, *, scale, nhp, nb):
    x32, wq32, wo32 = xbuf, wqbuf, wobuf
    xbuf, wqbuf, wobuf = (r.bitcast(bf16) for r in (xbuf, wqbuf, wobuf))
    pbuf = pbuf.bitcast(bf16)
    qbuf = qbuf.bitcast(bf16)
    sq = xbuf.shape[3]
    d = wqbuf.shape[3]
    hw = wobuf.shape[3]
    ng = nhp * nb
    lg = nb.bit_length() - 1
    assert nb == 1 << lg

    def kv_start(g, which=(0, 1, 2, 3)):
        hp, b = (g >> lg) & (nhp - 1), g & (nb - 1)
        for i, src in enumerate((ak, av, bk, bv)):
            if i in which:
                pltpu.make_async_copy(src.at[b, hp], kvbuf.at[b, i], kv_sem.at[b]).start()

    def kv_wait(b):
        pltpu.make_async_copy(kvbuf.at[b], kvbuf.at[b], kv_sem.at[b]).wait()

    def x_start(b, which=(0, 1)):
        for i, src in enumerate((ax, bx)):
            if i in which:
                for c in range(xbuf.shape[2]):
                    pltpu.make_async_copy(src.at[b, :, pl.ds(c * 128, 128)], xbuf.at[b, i, c], x_sem.at[b]).start()

    def x_wait(b):
        pltpu.make_async_copy(xbuf.at[b], xbuf.at[b], x_sem.at[b]).wait()

    def w_start(h, k):
        sl = h & 1
        off = h * hw if isinstance(h, int) else pl.multiple_of(h * hw, 128)
        if k < 2:
            for c in range(wqbuf.shape[2]):
                pltpu.make_async_copy((awq, bwq)[k].at[:, pl.ds(off + c * 128, 128)], wqbuf.at[sl, k, c],
                                      w_sem.at[0, sl]).start()
        else:
            for c in range(wobuf.shape[2]):
                pltpu.make_async_copy((awo, bwo)[k - 2].at[pl.ds(off, hw), pl.ds(c * 128, 128)],
                                      wobuf.at[sl, k - 2, c], w_sem.at[1, sl]).start()

    def w_wait(sl):
        pltpu.make_async_copy(wqbuf.at[sl], wqbuf.at[sl], w_sem.at[0, sl]).wait()
        pltpu.make_async_copy(wobuf.at[sl], wobuf.at[sl], w_sem.at[1, sl]).wait()

    lo = lax.broadcasted_iota(jnp.int32, (sq, 128), 1) < 64

    def body(g0, nbat, prefetch, pat):
        hp = g0 >> lg
        b0 = g0 & (nb - 1)
        wslot = hp & 1
        U = 2 * nbat
        Q, P, O, OT, OC = {}, {}, {}, {}, {}

        def q_(u):
            j, br = u // 2, u % 2
            Q[u] = _qproj(_wide(x32.at[b0 + j, br], 0, sq), _wide(wq32.at[wslot, br], 0, d), scale, lo)
            if QSCR and SMODE:
                for h in range(2):
                    for i in range(7):
                        qbuf[u, :, (7 * h + i) * 128:(7 * h + i + 1) * 128] = Q[u][h][i]

        def s_(u, h):
            j, br = u // 2, u % 2
            if QSCR and SMODE:
                qh = [qbuf[u, :, (7 * h + i) * 128:(7 * h + i + 1) * 128] for i in range(7)]
            else:
                qh = Q[u][h]
            P[u, h] = _score(qh, lambda i: kvbuf.at[b0 + j + (g0 >> (16 + i)), 2 * br], h, pbuf.at[u, h])

        def pv_(u, h):
            j, br = u // 2, u % 2
            p, r, ptop, _ = P[u, h]
            if PSCR:
                p = pbuf[u, h]
                ptop = pbuf[u, h, 0:128, :]
            vt = kvbuf.at[b0 + j, 2 * br + 1]
            O[u, h] = lax.dot_general(p, vt[h * 256:h * 256 + 128, :], NT, preferred_element_type=f32) * r
            OT[u, h] = lax.dot_general(vt[128 + h * 64:192 + h * 64, :], ptop, NT,
                                       preferred_element_type=f32)

        def pvc_(u):
            j, br = u // 2, u % 2
            vt = kvbuf.at[b0 + j, 2 * br + 1]
            if PSCR:
                pc = jnp.concatenate([pbuf[u, 0, 128:sq, :], pbuf[u, 1, 128:sq, :]], axis=0)
            else:
                pc = jnp.concatenate([P[u, 0][3], P[u, 1][3]], axis=0)
            OC[u] = lax.dot_general(pc, vt[128:256, :], NT, preferred_element_type=f32)

        def o_(u):
            j, br = u // 2, u % 2
            n = sq - 128
            top = jnp.concatenate([OT[u, 0], OT[u, 1]], axis=0).T
            lo_n = lax.broadcasted_iota(jnp.int32, (n, 128), 1) < 64
            bot = jnp.where(lo_n, OC[u][0:n], OC[u][n:2 * n])
            mid = jnp.concatenate([top, bot], axis=0) * jnp.where(lo, P[u, 0][1], P[u, 1][1])
            op = jnp.concatenate([O[u, 0], mid, O[u, 1]], axis=1).astype(bf16)
            r = jnp.dot(op, _wide(wo32.at[wslot, br], 0, hw), preferred_element_type=f32)
            b = b0 + j
            prev = acc[b, :, br * d:(br + 1) * d]
            new = jnp.where(hp == 0, 0.0, prev) + r
            acc[b, :, br * d:(br + 1) * d] = new
            obuf[b, :, br * d:(br + 1) * d] = new.astype(obuf.dtype)
            if br == 1:
                @pl.when(hp == nhp - 1)
                def _():
                    pltpu.make_async_copy(obuf.at[b], o_hbm.at[b], o_sem).start()

        fns = {"q": q_, "s": s_, "pv": pv_, "pvc": pvc_, "o": o_}
        sched = _schedule(U, pat)
        slots = list(range(PFPOS, len(sched), PFSTEP if nbat > 1 else 1))
        per = -(-len(prefetch) // len(slots))
        for i, item in enumerate(sched):
            if i in slots:
                k = slots.index(i)
                for f in prefetch[k * per:(k + 1) * per]:
                    f()
            fns[item[0]](*item[1:])

    x_start(0)
    w_start(0, 0)
    w_start(0, 1)
    kv_start(0)
    w_start(0, 2)
    w_start(0, 3)
    for g in range(1, C0):
        x_start(g)
        kv_start(g)

    def issued(g):
        return jnp.minimum(jnp.minimum(RATE * (g + SB) + C0, g + nb), G1 + BB)

    def small(i, carry):
        g0 = i * SB
        hp = g0 >> lg
        b0 = g0 & (nb - 1)

        @pl.when(hp == 0)
        def _():
            for j in range(SB):
                x_wait(b0 + j)

        @pl.when(b0 == 0)
        def _():
            w_wait(hp & 1)

        for j in range(SB):
            kv_wait(b0 + j)

        hi = issued(g0)
        prev = jnp.where(i == 0, C0, issued(g0 - SB))

        def pf_x(k, w):
            @pl.when(jnp.logical_and(prev + k < hi, prev + k < nb))
            def _():
                x_start(prev + k, (w,))

        def pf_kv(k, w):
            @pl.when(prev + k < hi)
            def _():
                kv_start(prev + k, (w,))

        def pf_w(k):
            @pl.when(b0 == nb // 2)
            def _():
                w_start(hp + 1, k)

        prefetch = []
        for k in range(RATE * SB):
            prefetch += [functools.partial(pf_x, k, w) for w in range(2)]
            prefetch += [functools.partial(pf_kv, k, w) for w in range(4)]
        prefetch += [functools.partial(pf_w, k) for k in range(4)]
        body(g0, SB, prefetch, SPAT)
        return carry

    def big(i, carry):
        g0 = i * BB
        hp = g0 >> lg
        b0 = g0 & (nb - 1)

        @pl.when(b0 == 0)
        def _():
            w_wait(hp & 1)

        for j in range(BB):
            kv_wait(b0 + j)

        def pf_w(k):
            @pl.when(jnp.logical_and(b0 == nb // 2, hp + 1 < nhp))
            def _():
                w_start(hp + 1, k)

        prefetch = [functools.partial(kv_start, g0 + BB + j) for j in range(BB)]
        prefetch += [functools.partial(pf_w, k) for k in range(4)]
        body(g0, BB, prefetch, PAT)
        return carry

    lax.fori_loop(0, G1 // SB, small, 0)
    lax.fori_loop(G1 // BB, ng // BB, big, 0)
    for j in range(BB):
        kv_wait(j)
    pltpu.make_async_copy(obuf, o_hbm, o_sem).wait()


@jax.jit
def pallas_concat_heads__gqa_block_cached__mha_block_cached__near_ridge_kernel(
    A_x, A_k_cache, A_v_cache, A_wq, A_wo, B_x, B_k_cache, B_v_cache, B_wq, B_wo):
    B, Sq, D = A_x.shape
    _, H, Sk, Dh = A_k_cache.shape
    nhp = H // 2
    assert G1 >= B and G1 % BB == 0 and 2 * BB <= B
    n_iss = C0
    for g0 in range(0, G1, SB):
        assert n_iss >= g0 + SB, (g0, n_iss)
        hi = min(RATE * (g0 + SB) + C0, g0 + B, G1 + BB)
        assert hi - n_iss <= RATE * SB and hi >= n_iss
        n_iss = hi
    assert n_iss == G1 + BB, n_iss
    assert C0 <= B and G1 % SB == 0

    def tr(c):
        return jnp.swapaxes(c, 2, 3).reshape(B, nhp, 2 * Dh, Sk)

    any_spec = pl.BlockSpec(memory_space=pl.ANY)
    return pl.pallas_call(
        functools.partial(_kernel, scale=Dh ** -0.5 * LOG2E, nhp=nhp, nb=B),
        in_specs=[any_spec] * 10,
        out_specs=any_spec,
        out_shape=jax.ShapeDtypeStruct((B, Sq, 2 * D), A_x.dtype),
        scratch_shapes=[pltpu.VMEM((B, Sq, 2 * D), f32),
                        pltpu.VMEM((B, 2, D // 128, Sq // 2, 128), u32),
                        pltpu.VMEM((2, 2, 2 * Dh // 128, D // 2, 128), u32),
                        pltpu.VMEM((2, 2, D // 128, Dh, 128), u32),
                        pltpu.VMEM((B, 4, 2 * Dh, Sk), bf16),
                        pltpu.VMEM((B, Sq, 2 * D), bf16),
                        pltpu.VMEM((2 * BB, 2, Sq // 2, Sk), u32),
                        pltpu.VMEM((2 * BB, Sq // 4, 14 * 128), u32),
                        pltpu.SemaphoreType.DMA((B,)),
                        pltpu.SemaphoreType.DMA((B,)),
                        pltpu.SemaphoreType.DMA((2, 2)),
                        pltpu.SemaphoreType.DMA(())],
        compiler_params=pltpu.CompilerParams(
            disable_bounds_checks=True,
            vmem_limit_bytes=100 * 1024 * 1024),
    )(A_x, tr(A_k_cache), tr(A_v_cache), A_wq, A_wo, B_x, tr(B_k_cache), tr(B_v_cache), B_wq, B_wo)
```

```python
import functools
import jax
import jax.numpy as jnp
from jax import lax
import jax.experimental.pallas as pl
import jax.experimental.pallas.tpu as pltpu

BB = 4
G1 = 32
C0 = 2
RATE = 2
PFPOS = 1
PFSTEP = 3
PSKIP = 2
OBUF = 1
SKIP_SMALL = 0
KVTOP = 8
NOCSE = 1
PAT = "s00:0,qa:2,s01:0,t0:-1,m1:-1,m0:-2,c:-1,oa:-2,qb:2,s11:0,t1:-1,s10:1,ob:-2"
SPAT = PAT
LOG2E = 1.4426950408889634
bf16 = jnp.bfloat16
f32 = jnp.float32
u32 = jnp.uint32
NT = (((1,), (1,)), ((), ()))

E1, E2, SS, DD = (1, 0), (0, 1), (1, 1), (1, -1)


def _neg(v):
    return (-v[0], -v[1])


_TYPES = [[(E1, E1), (E2, E2)], [(SS, E1), (E2, _neg(DD))], [(E1, DD), (SS, E2)]]
_PAIRS = {
    (1, 2): ([(E2, E1, E1, E2), (E1, _neg(E1), E1, E1), (E2, _neg(E2), E2, E2)],
             (1, 1, (-1, 0), (1, 0)), (1, -1, (0, 1), (0, -1))),
    (0, 1): ([(E1, SS, E2, DD), (SS, SS, E2, _neg(E2)), (E1, E1, DD, _neg(DD))],
             (1, -1, (0, 1), (-1, 0)), (1, 1, (-1, 0), (0, 1))),
    (0, 2): ([(E2, SS, E1, DD), (SS, SS, E1, E1), (E2, E2, DD, DD)],
             (-1, 1, (-1, 0), (0, -1)), (1, -1, (0, -1), (-1, 0))),
}


def _scheme(ks, ns, types):
    prods = {}
    for i, t in enumerate(types):
        for m, (f, g) in enumerate(_TYPES[t]):
            prods["d", i, m] = dict(f=[(ks[i], f)], g=[(ns[i], g)], w={(ks[i], ns[i]): 1})
    for i in range(len(types)):
        for j in range(i + 1, len(types)):
            ms, (x0, x1, ci, cj), (y0, y1, di, dj) = _PAIRS[types[i], types[j]]
            for name, (a, ap, b, bp) in zip("abc", ms):
                prods[name, i, j] = dict(f=[(ks[i], a), (ks[j], ap)], g=[(ns[i], b), (ns[j], bp)], w={})
            cij, cji = (ks[i], ns[j]), (ks[j], ns[i])
            prods["a", i, j]["w"].update({cij: x0, cji: y0})
            prods["b", i, j]["w"][cij] = x1
            prods["c", i, j]["w"][cji] = y1
            for m in range(2):
                for idx, out, cf in ((i, cij, ci[m]), (j, cij, cj[m]), (i, cji, di[m]), (j, cji, dj[m])):
                    if cf:
                        prods["d", idx, m]["w"][out] = cf
    return prods


def _plain(k, n):
    return [dict(f=[(k, e)], g=[(n, e)], w={(k, n): 1}) for e in (E1, E2)]


_CYC = [("d", 1, 0), ("a", 1, 2), ("d", 2, 1), ("c", 1, 2), ("b", 0, 1), ("d", 0, 1), ("a", 0, 1), ("d", 1, 1),
        ("c", 0, 1), ("c", 0, 2), ("d", 2, 0), ("a", 0, 2), ("d", 0, 0), ("b", 0, 2), ("b", 1, 2)]
_STR = [("d", 0, 0), ("a", 0, 1), ("d", 1, 1), ("c", 0, 1), ("d", 0, 1), ("b", 0, 1), ("d", 1, 0)]


def _prods(kind):
    big = _scheme([0, 1, 2], [0, 1, 2], [0, 1, 2])
    out = [big[k] for k in _CYC]
    if kind == "o":
        st, p0, p1 = _scheme([1, 2], [3, 4], [1, 2]), _plain(0, 3), _plain(0, 4)
        s = [st[k] for k in _STR]
        out += [p0[0], s[0], s[1], s[2], p1[1], s[3], s[4], p0[1], s[5], s[6], p1[0]]
    else:
        st, p0, p1 = _scheme([3, 4], [1, 2], [1, 2]), _plain(3, 0), _plain(4, 0)
        out += [st[k] for k in _STR] + [p0[0], p1[0], p0[1], p1[1]]
    for p in out:
        if next(iter(p["w"].values())) < 0:
            p["w"] = {k: -c for k, c in p["w"].items()}
            p["g"] = [(n, _neg(v)) for n, v in p["g"]]
        p["f"] = tuple(p["f"])
    return out


O_PRODS = _prods("o")
Q_PRODS = _prods("q")
O_WC = [r for r, p in enumerate(O_PRODS) if len(p["w"]) > 1]
Q_WC = [r for r, p in enumerate(Q_PRODS) if len(p["w"]) > 1]


def _is_raw(f):
    return len(f) == 1 and f[0][1] in (E1, E2)


def _uniq(xs):
    out = []
    for x in xs:
        if x not in out:
            out.append(x)
    return out


O_LHS = _uniq([p["f"] for p in O_PRODS])
Q_LHS = [f for f in _uniq([p["f"] for p in Q_PRODS]) if not _is_raw(f)]


def _make_lhs(block, keys):
    cache = {}

    def form(k, v):
        sgn = -1 if min(v) < 0 else 1
        v = (abs(v[0]), abs(v[1]))
        if (k, v) not in cache:
            cache[k, v] = form(k, E1)[1] + form(k, E2)[1] if v == SS else block(v[1], k)
        return sgn, cache[k, v]

    out = []
    for key in keys:
        terms = [form(k, v) for k, v in key]
        assert terms[0][0] == 1
        val = terms[0][1]
        if len(terms) == 2:
            val = val + terms[1][1] if terms[1][0] > 0 else val - terms[1][1]
        out.append(val)
    return out


def _bilinear_run(accs, prods, lo, hi, lhs_of, w_of):
    for r in range(lo, hi):
        p = prods[r]
        m = jnp.dot(lhs_of(p["f"]), w_of(r), preferred_element_type=f32)
        for n, v in p["g"]:
            sgn = -1 if (v[0] < 0 or (v[0] == 0 and v[1] < 0)) else 1
            key = (n, (v[0] * sgn, v[1] * sgn))
            if key not in accs:
                accs[key] = (sgn, m)
            else:
                s0, a = accs[key]
                accs[key] = (s0, a + m if s0 == sgn else a - m)


def _bilinear_out(accs, i, n):
    s, a = accs[n, (E1, E2)[i]]
    if (n, DD) in accs:
        sd, dd = accs[n, DD]
        a = a + dd if s == (sd if i == 0 else -sd) else a - dd
    return s, a


def _mul(i, n):
    return i * n if isinstance(i, int) else pl.multiple_of(i * n, 16)


def _as_bf16(packed):
    return pltpu.bitcast(packed, bf16)


def _as_f32(packed):
    return pltpu.bitcast(packed, bf16).astype(f32)


def _q_operands(c, scale):
    t = [[a * (s * scale) for s, a in row] for row in c]
    lane = lax.broadcasted_iota(jnp.int32, t[0][0].shape, 1)
    lo = lane < 64
    out = []
    for h in range(2):
        if h == 0:
            valid = lane < 96
            h1 = [t[i][0] for i in range(2)]
            h2 = [jnp.where(lo, t[i][1], pltpu.roll(t[i][0], 96, 1)) for i in range(2)]
        else:
            valid = lane >= 32
            h1 = [t[i][2] for i in range(2)]
            h2 = [jnp.where(lo, pltpu.roll(t[i][2], 32, 1), t[i][1]) for i in range(2)]
        (a11, a21), (a12, a22) = h1, h2
        out.append([a11 + a22, jnp.where(valid, a21 + a22, 0.0), a11, a22, a11 + a12, a21 - a11, a12 - a22])
    return out


def _scores_half(qh, kts, h, j):
    r1, r2 = ([(0, 96)], [(128, 192), (96, 128)]) if h == 0 else ([(288, 384)], [(256, 288), (192, 256)])
    zf = jnp.zeros((32, 128), f32)

    def pk(f):
        return jnp.concatenate([f, zf] if h == 0 else [zf, f], axis=0).astype(bf16)

    def blk(i, name):
        k = kts(i if NOCSE else 0)
        c = j if name[1] == "1" else j + 2
        return jnp.concatenate([k[a:b, c * 128:(c + 1) * 128].astype(f32)
                                for a, b in (r1 if name[0] == "1" else r2)], axis=0)

    bs = [pk(blk(0, "11") + blk(0, "22")),
          kts(6 if NOCSE else 0)[h * 256:h * 256 + 128, j * 128:(j + 1) * 128],
          pk(blk(1, "12") - blk(1, "22")), pk(blk(2, "21") - blk(2, "11")), pk(blk(3, "22")),
          pk(blk(4, "11") + blk(4, "12")), pk(blk(5, "21") + blk(5, "22"))]
    m = [None] * 7
    for i in (0, 3, 4, 6, 1, 2, 5):
        m[i] = jnp.dot(qh[i], bs[i], preferred_element_type=f32)
    return (jnp.concatenate([(m[0] + m[3]) + (m[6] - m[4]), m[1] + m[3]], axis=0),
            jnp.concatenate([m[2] + m[4], (m[0] - m[1]) + (m[2] + m[5])], axis=0))


def _softmax(s):
    m = jnp.max(s, axis=1, keepdims=True)
    p = jnp.exp2(s - m)
    t = (p[:, 0:128] + p[:, 128:256]) + (p[:, 256:384] + p[:, 384:512])
    p = jnp.concatenate([p[:, 0:384], jnp.minimum(p[:, 384:512], t)], axis=1)
    l = jnp.sum(t, axis=1, keepdims=True)
    r = pl.reciprocal(l, approx=True)
    r = r * (2.0 - l * r)
    return p.astype(bf16), r


def _schedule(nu, pat):
    pat = [(a.split(":")[0], int(a.split(":")[1])) for a in pat.split(",")]
    order = []
    for t in range(-6, nu + 6):
        for name, lag in pat:
            u = t + lag
            if 0 <= u < nu:
                order.append((name, u))
    return order


def _kernel(ax, ak, av, awq, awo, bx, bk, bv, bwq, bwo, o_hbm,
            acc, x32, wq32, wo32, kvbuf, obuf, pbuf, qbuf, xc32, wqc0, wqc1, woc0, woc1,
            kv_sem, x_sem, w_sem, o_sem, *, scale, nhp, nb):
    xbuf, wqbuf, wobuf = (r.bitcast(bf16) for r in (x32, wq32, wo32))
    pbuf, qbuf, xc = (r.bitcast(bf16) for r in (pbuf, qbuf, xc32))
    wqc = [r.bitcast(bf16) for r in (wqc0, wqc1)]
    woc = [r.bitcast(bf16) for r in (woc0, woc1)]
    sq = xbuf.shape[3]
    hq = sq // 2
    d = wqbuf.shape[3]
    hw = wobuf.shape[3]
    ng = nhp * nb
    lg = nb.bit_length() - 1
    assert nb == 1 << lg

    def kv_start(g, which=(0, 1, 2, 3)):
        hp, b = (g >> lg) & (nhp - 1), g & (nb - 1)
        for i, src in enumerate((ak, av, bk, bv)):
            if i in which:
                pltpu.make_async_copy(src.at[b, hp], kvbuf.at[b, i], kv_sem.at[b]).start()

    def kv_wait(b):
        pltpu.make_async_copy(kvbuf.at[b], kvbuf.at[b], kv_sem.at[b]).wait()

    def x_start(b, which=(0, 1)):
        for i, src in enumerate((ax, bx)):
            if i in which:
                for c in range(xbuf.shape[2]):
                    pltpu.make_async_copy(src.at[b, :, pl.ds(c * 128, 128)], xbuf.at[b, i, c], x_sem.at[b]).start()

    def x_wait(b):
        pltpu.make_async_copy(xbuf.at[b], xbuf.at[b], x_sem.at[b]).wait()

    def wslot(h):
        return h % 3 if isinstance(h, int) else lax.rem(h, 3)

    def w_start(h, k):
        sl = wslot(h)
        off = h * hw if isinstance(h, int) else pl.multiple_of(h * hw, 128)
        if k < 2:
            for c in range(wqbuf.shape[2]):
                pltpu.make_async_copy((awq, bwq)[k].at[:, pl.ds(off + c * 128, 128)], wqbuf.at[sl, k, c],
                                      w_sem.at[0, sl]).start()
        else:
            for c in range(wobuf.shape[2]):
                pltpu.make_async_copy((awo, bwo)[k - 2].at[pl.ds(off, hw), pl.ds(c * 128, 128)],
                                      wobuf.at[sl, k - 2, c], w_sem.at[1, sl]).start()

    def w_wait(h):
        sl = wslot(h)
        pltpu.make_async_copy(wqbuf.at[sl], wqbuf.at[sl], w_sem.at[0, sl]).wait()
        pltpu.make_async_copy(wobuf.at[sl], wobuf.at[sl], w_sem.at[1, sl]).wait()

    def prep_w(src_slot, dst_slot, row, nrows, br, which):
        raw, dst, prods, idx = ((wq32, wqc, Q_PRODS, Q_WC), (wo32, woc, O_PRODS, O_WC))[which]
        r8 = row * 8 if isinstance(row, int) else pl.multiple_of(row * 8, 8)
        r16 = row * 16 if isinstance(row, int) else pl.multiple_of(row * 16, 16)
        for slot, r in enumerate(idx):
            val = None
            for (k, n), c in prods[r]["w"].items():
                t = _as_f32(raw[src_slot, br, n, pl.ds(k * 64 + r8, nrows * 8), :])
                val = t if val is None else (val + t if c > 0 else val - t)
            dst[dst_slot][pl.ds(br * 128 + r16, nrows * 16), slot * 128:(slot + 1) * 128] = val.astype(bf16)

    def prep_x(b, br):
        vals = _make_lhs(lambda i, k: _as_f32(x32[b, br, k, i * (hq // 2):(i + 1) * (hq // 2), :]), Q_LHS)
        for i, v in enumerate(vals):
            xc[pl.ds(_mul(b * 2 + br, hq), hq), i * 128:(i + 1) * 128] = v.astype(bf16)

    def body(g0, nbat, extra, pat, cs, first_hp=False, last_hp=False):
        hp = g0 >> lg
        b0 = g0 & (nb - 1)
        rs = wslot(hp)
        R, O, OT, OC = {}, {}, {}, {}

        def prow(u, h):
            return (2 * u + h) * sq

        def weights(raw, comb, prods, idx, br):
            def w_of(r):
                if r in idx:
                    s = idx.index(r)
                    return comb[cs][br * 128:(br + 1) * 128, s * 128:(s + 1) * 128]
                (k, n), = prods[r]["w"]
                return _as_bf16(raw[rs, br, n, k * 64:(k + 1) * 64, :])
            return w_of

        QA, OA, SC, LH = {}, {}, {}, {}

        def q_(u, lo_, hi_):
            b, br = b0 + u // 2, u % 2

            def lhs_of(f):
                if _is_raw(f):
                    (k, v), = f
                    return _as_bf16(x32[b, br, k, v[1] * (hq // 2):(v[1] + 1) * (hq // 2), :])
                i = Q_LHS.index(f)
                return xc[pl.ds(_mul(b * 2 + br, hq), hq), i * 128:(i + 1) * 128]

            _bilinear_run(QA.setdefault(u, {}), Q_PRODS, lo_, hi_, lhs_of, weights(wq32, wqc, Q_PRODS, Q_WC, br))
            if hi_ == len(Q_PRODS):
                c = [[_bilinear_out(QA[u], i, n) for n in range(3)] for i in range(2)]
                for h, ops in enumerate(_q_operands(c, scale)):
                    for i, a in enumerate(ops):
                        qbuf[u * hq:(u + 1) * hq, (7 * h + i) * 128:(7 * h + i + 1) * 128] = a.astype(bf16)

        def s_(u, h, j):
            b, br = b0 + u // 2, u % 2
            qh = [qbuf[u * hq:(u + 1) * hq, (7 * h + i) * 128:(7 * h + i + 1) * 128] for i in range(7)]
            SC[u, h, j] = _scores_half(qh, lambda i: kvbuf.at[b + (g0 >> (16 + i)), 2 * br], h, j)
            if j == 1:
                s = jnp.concatenate([SC[u, h, 0][0], SC[u, h, 1][0], SC[u, h, 0][1], SC[u, h, 1][1]], axis=1)
                p, R[u, h] = _softmax(s)
                pbuf[prow(u, h):prow(u, h) + sq, :] = p

        def m_(u, h):
            vt = kvbuf.at[b0 + u // 2, 2 * (u % 2) + 1]
            O[u, h] = lax.dot_general(pbuf[prow(u, h):prow(u, h) + sq, :], vt[h * 256:h * 256 + 128, :], NT,
                                      preferred_element_type=f32) * R[u, h]

        def t_(u, h):
            vt = kvbuf.at[b0 + u // 2, 2 * (u % 2) + 1]
            OT[u, h] = lax.dot_general(vt[128 + h * 64:192 + h * 64, :], pbuf[prow(u, h):prow(u, h) + 128, :], NT,
                                       preferred_element_type=f32)

        def c_(u):
            vt = kvbuf.at[b0 + u // 2, 2 * (u % 2) + 1]
            pc = jnp.concatenate([pbuf[prow(u, h) + 128:prow(u, h) + sq, :] for h in range(2)], axis=0)
            OC[u] = lax.dot_general(pc, vt[128:256, :], NT, preferred_element_type=f32)

        def o_(u, lo_, hi_):
            b, br = b0 + u // 2, u % 2
            if lo_ == 0:
                n = sq - 128
                top = jnp.concatenate([OT[u, 0], OT[u, 1]], axis=0).T
                bot = jnp.where(lax.broadcasted_iota(jnp.int32, (n, 128), 1) < 64, OC[u][0:n], OC[u][n:2 * n])
                lo = lax.broadcasted_iota(jnp.int32, (sq, 128), 1) < 64
                mid = jnp.concatenate([top, bot], axis=0) * jnp.where(lo, R[u, 0], R[u, 1])
                tiles = (O[u, 0], mid, O[u, 1])
                LH[u] = [a.astype(bf16) for a in _make_lhs(lambda i, k: tiles[k][i * hq:(i + 1) * hq], O_LHS)]
            _bilinear_run(OA.setdefault(u, {}), O_PRODS, lo_, hi_, lambda f: LH[u][O_LHS.index(f)],
                          weights(wo32, woc, O_PRODS, O_WC, br))
            for n in (range(3) if lo_ == 0 else range(3, 5)):
                for i in range(2):
                    s, a = _bilinear_out(OA[u], i, n)
                    rows = slice(i * hq, (i + 1) * hq)
                    cols = slice(br * d + n * 128, br * d + (n + 1) * 128)
                    if first_hp:
                        new = a if s > 0 else -a
                    else:
                        new = acc[b, rows, cols] + a if s > 0 else acc[b, rows, cols] - a
                    if last_hp:
                        obuf[b, rows, cols] = new.astype(obuf.dtype)
                    else:
                        acc[b, rows, cols] = new
            if br == 1 and lo_ > 0 and last_hp:
                pltpu.make_async_copy(obuf.at[b], o_hbm.at[b], o_sem).start()

        fns = {"qa": lambda u: q_(u, 0, 15), "qb": lambda u: q_(u, 15, 26),
               "oa": lambda u: o_(u, 0, 15), "ob": lambda u: o_(u, 15, 26),
               "s00": lambda u: s_(u, 0, 0), "s01": lambda u: s_(u, 0, 1),
               "s10": lambda u: s_(u, 1, 0), "s11": lambda u: s_(u, 1, 1),
               "m0": lambda u: m_(u, 0), "m1": lambda u: m_(u, 1),
               "t0": lambda u: t_(u, 0), "t1": lambda u: t_(u, 1), "c": c_}
        sched = _schedule(2 * nbat, pat)
        first, dmas, preps = extra
        for f in first:
            f()
        slots = list(range(PFPOS, len(sched), PFSTEP if nbat > 1 else 1))
        per = max(1, -(-len(dmas) // len(slots)))
        pslots = [i + 1 for i in range(len(sched) - 1)
                  if sched[i][0][0] in "qo" and sched[i + 1][0][0] not in "qo"][PSKIP if nbat > 1 else 0:]
        pper = max(1, -(-len(preps) // len(pslots)))
        for i, item in enumerate(sched):
            if i in slots:
                k = slots.index(i)
                for f in dmas[k * per:(k + 1) * per]:
                    f()
            if i in pslots:
                k = pslots.index(i)
                for f in preps[k * pper:(k + 1) * pper]:
                    f()
            fns[item[0]](item[1])

    for k in range(4):
        w_start(0, k)
    x_start(0)
    kv_start(0)
    x_start(1)
    for g in range(1, C0):
        kv_start(g)
        x_start(g + 1)
    w_wait(0)
    for br in range(2):
        for which in range(2):
            prep_w(0, 0, 0, 8, br, which)
    x_wait(0)
    for br in range(2):
        prep_x(0, br)

    def issued(g):
        return jnp.minimum(jnp.minimum(RATE * (g + 1) + C0, g + nb), G1 + BB)

    def small(hp, b0, carry):
        g0 = hp * nb + b0

        if hp == 0:
            @pl.when(b0 + 1 < nb)
            def _():
                x_wait(b0 + 1)

        @pl.when(b0 == nb // 2)
        def _():
            w_wait(hp + 1)

        kv_wait(b0)

        hi = issued(g0)
        prev = jnp.where(g0 == 0, C0, issued(g0 - 1))

        def pf_x(k, w):
            @pl.when(jnp.logical_and(prev + k < hi, prev + k + 1 < nb))
            def _():
                x_start(prev + k + 1, (w,))

        def pf_kv(k):
            @pl.when(prev + k < hi)
            def _():
                kv_start(prev + k)

        def pf_w(h, at, k):
            @pl.when(b0 + k == at + k)
            def _():
                w_start(h, k)

        src = jnp.where(b0 >= nb // 2, wslot(hp + 1), wslot(hp))
        row = b0 & (nb // 2 - 1)
        first = [functools.partial(pf_w, hp + 2, 12, k) for k in range(4)]
        preps = []
        if hp == 0:
            first += [functools.partial(pf_w, 1, 3, k) for k in range(4)]
            first += [functools.partial(pf_x, k, w) for k in range(RATE) for w in range(2)]
            preps += [functools.partial(prep_x, jnp.minimum(b0 + 1, nb - 1), br) for br in range(2)]
        first += [functools.partial(pf_kv, k) for k in range(RATE)]
        preps += [functools.partial(prep_w, src, (hp + 1) & 1, row, 1, br, w) for br in range(2) for w in range(2)]
        body(g0, 1, (first, [], preps), SPAT, hp & 1, first_hp=hp == 0)
        return carry

    def big(par, last, i, carry):
        g0 = i * BB
        hp = g0 >> lg
        b0 = g0 & (nb - 1)
        nrows = 8 * BB // nb

        if not last:
            @pl.when(b0 == 0)
            def _():
                w_wait(hp + 1)

        for j in range(BB):
            kv_wait(b0 + j)

        def pf_w(k):
            @pl.when(jnp.logical_and(b0 + k == nb - BB + k, hp + 2 < nhp))
            def _():
                w_start(hp + 2, k)

        def pf_kv(j):
            @pl.when(g0 + BB + j < ng)
            def _():
                kv_start(g0 + BB + j)

        row = lax.div(b0, BB) * nrows
        if last:
            extra = ([functools.partial(pf_kv, j) for j in range(BB)], [], [])
        else:
            kvs = [functools.partial(kv_start, g0 + BB + j) for j in range(BB)]
            extra = ([functools.partial(pf_w, k) for k in range(4)] + kvs[:KVTOP], kvs[KVTOP:],
                     [functools.partial(prep_w, wslot(hp + 1), 1 - par, row + r, 1, br, w)
                      for r in range(nrows) for br in range(2) for w in range(2)])
        body(g0, BB, extra, PAT, par, last_hp=last)
        return carry

    nsm = G1 // nb
    spb = nb // BB
    if not SKIP_SMALL:
        for hp in range(nsm):
            lax.fori_loop(0, nb, functools.partial(small, hp), 0)

    def pair(t, carry):
        lax.fori_loop(2 * t * spb, (2 * t + 1) * spb, functools.partial(big, 0, False), 0)
        lax.fori_loop((2 * t + 1) * spb, jnp.minimum(2 * t + 2, nhp - 1) * spb, functools.partial(big, 1, False), 0)
        return carry

    assert nsm % 2 == 0
    lax.fori_loop(nsm // 2, nhp // 2, pair, 0)
    if not SKIP_SMALL:
        lax.fori_loop((nhp - 1) * spb, nhp * spb, functools.partial(big, 1, True), 0)
    pltpu.make_async_copy(obuf, o_hbm, o_sem).wait()


@jax.jit
def pallas_concat_heads__gqa_block_cached__mha_block_cached__near_ridge_kernel(
    A_x, A_k_cache, A_v_cache, A_wq, A_wo, B_x, B_k_cache, B_v_cache, B_wq, B_wo):
    B, Sq, D = A_x.shape
    _, H, Sk, Dh = A_k_cache.shape
    nhp = H // 2
    assert B == 16 and G1 % B == 0 and 2 * BB <= B and C0 >= 1
    n_iss = C0
    for g0 in range(G1):
        assert n_iss >= min(g0 + 2, G1 + BB), (g0, n_iss)
        hi = min(RATE * (g0 + 1) + C0, g0 + B, G1 + BB)
        assert 0 <= hi - n_iss <= RATE
        n_iss = hi
    assert n_iss == G1 + BB, n_iss

    def tr(c):
        return jnp.swapaxes(c, 2, 3).reshape(B, nhp, 2 * Dh, Sk)

    any_spec = pl.BlockSpec(memory_space=pl.ANY)
    return pl.pallas_call(
        functools.partial(_kernel, scale=Dh ** -0.5 * LOG2E, nhp=nhp, nb=B),
        in_specs=[any_spec] * 10,
        out_specs=any_spec,
        out_shape=jax.ShapeDtypeStruct((B, Sq, 2 * D), A_x.dtype),
        scratch_shapes=[pltpu.VMEM((B, Sq, 2 * D), f32),
                        pltpu.VMEM((B, 2, D // 128, Sq // 2, 128), u32),
                        pltpu.VMEM((3, 2, 2 * Dh // 128, D // 2, 128), u32),
                        pltpu.VMEM((3, 2, D // 128, Dh, 128), u32),
                        pltpu.VMEM((B, 4, 2 * Dh, Sk), bf16),
                        pltpu.VMEM((B, Sq, 2 * D), bf16),
                        pltpu.VMEM((2 * BB * Sq, Sk), u32),
                        pltpu.VMEM((2 * BB * Sq // 4, 14 * 128), u32),
                        pltpu.VMEM((B * 2 * Sq // 4, len(Q_LHS) * 128), u32),
                        pltpu.VMEM((2 * 64, len(Q_WC) * 128), u32),
                        pltpu.VMEM((2 * 64, len(Q_WC) * 128), u32),
                        pltpu.VMEM((2 * 64, len(O_WC) * 128), u32),
                        pltpu.VMEM((2 * 64, len(O_WC) * 128), u32),
                        pltpu.SemaphoreType.DMA((B,)),
                        pltpu.SemaphoreType.DMA((B,)),
                        pltpu.SemaphoreType.DMA((2, 3)),
                        pltpu.SemaphoreType.DMA(())],
        compiler_params=pltpu.CompilerParams(
            disable_bounds_checks=True,
            vmem_limit_bytes=110 * 1024 * 1024),
    )(A_x, tr(A_k_cache), tr(A_v_cache), A_wq, A_wo, B_x, tr(B_k_cache), tr(B_v_cache), B_wq, B_wo)
```

```python
import functools
import jax
import jax.numpy as jnp
from jax import lax
import jax.experimental.pallas as pl
import jax.experimental.pallas.tpu as pltpu

BB = 4
G1 = 16
C0 = 2
RATE = 2
PFPOS = 1
PFSTEP = 3
PSKIP = 2
OBUF = 1
SKIP_SMALL = 0
KVTOP = 8
NOCSE = 1
PAT = "s00:0,qa:2,s01:0,t0:-1,m1:-1,m0:-2,c:-1,oa:-2,s11:0,s10:1,t1:-1,ob:-2,qb:2"
SPAT = "qa@0,qb@0,qa@1,s10@0,qb@1,s00@0,s11@0,s10@1,s00@1,s01@0,m1@0,t1@0,s11@1,t0@0,c@0,m0@0,m1@1,s01@1,oa@0,t1@1,c@1,t0@1,m0@1,ob@0,oa@1,ob@1"
LOG2E = 1.4426950408889634
bf16 = jnp.bfloat16
f32 = jnp.float32
u32 = jnp.uint32
NT = (((1,), (1,)), ((), ()))

E1, E2, SS, DD = (1, 0), (0, 1), (1, 1), (1, -1)


def _neg(v):
    return (-v[0], -v[1])


_TYPES = [[(E1, E1), (E2, E2)], [(SS, E1), (E2, _neg(DD))], [(E1, DD), (SS, E2)]]
_PAIRS = {
    (1, 2): ([(E2, E1, E1, E2), (E1, _neg(E1), E1, E1), (E2, _neg(E2), E2, E2)],
             (1, 1, (-1, 0), (1, 0)), (1, -1, (0, 1), (0, -1))),
    (0, 1): ([(E1, SS, E2, DD), (SS, SS, E2, _neg(E2)), (E1, E1, DD, _neg(DD))],
             (1, -1, (0, 1), (-1, 0)), (1, 1, (-1, 0), (0, 1))),
    (0, 2): ([(E2, SS, E1, DD), (SS, SS, E1, E1), (E2, E2, DD, DD)],
             (-1, 1, (-1, 0), (0, -1)), (1, -1, (0, -1), (-1, 0))),
}


def _scheme(ks, ns, types):
    prods = {}
    for i, t in enumerate(types):
        for m, (f, g) in enumerate(_TYPES[t]):
            prods["d", i, m] = dict(f=[(ks[i], f)], g=[(ns[i], g)], w={(ks[i], ns[i]): 1})
    for i in range(len(types)):
        for j in range(i + 1, len(types)):
            ms, (x0, x1, ci, cj), (y0, y1, di, dj) = _PAIRS[types[i], types[j]]
            for name, (a, ap, b, bp) in zip("abc", ms):
                prods[name, i, j] = dict(f=[(ks[i], a), (ks[j], ap)], g=[(ns[i], b), (ns[j], bp)], w={})
            cij, cji = (ks[i], ns[j]), (ks[j], ns[i])
            prods["a", i, j]["w"].update({cij: x0, cji: y0})
            prods["b", i, j]["w"][cij] = x1
            prods["c", i, j]["w"][cji] = y1
            for m in range(2):
                for idx, out, cf in ((i, cij, ci[m]), (j, cij, cj[m]), (i, cji, di[m]), (j, cji, dj[m])):
                    if cf:
                        prods["d", idx, m]["w"][out] = cf
    return prods


def _plain(k, n):
    return [dict(f=[(k, e)], g=[(n, e)], w={(k, n): 1}) for e in (E1, E2)]


_CYC = [("d", 1, 0), ("a", 1, 2), ("d", 2, 1), ("c", 1, 2), ("b", 0, 1), ("d", 0, 1), ("a", 0, 1), ("d", 1, 1),
        ("c", 0, 1), ("c", 0, 2), ("d", 2, 0), ("a", 0, 2), ("d", 0, 0), ("b", 0, 2), ("b", 1, 2)]
_STR = [("d", 0, 0), ("a", 0, 1), ("d", 1, 1), ("c", 0, 1), ("d", 0, 1), ("b", 0, 1), ("d", 1, 0)]


def _prods(kind):
    big = _scheme([0, 1, 2], [0, 1, 2], [0, 1, 2])
    out = [big[k] for k in _CYC]
    if kind == "o":
        st, p0, p1 = _scheme([1, 2], [3, 4], [1, 2]), _plain(0, 3), _plain(0, 4)
        s = [st[k] for k in _STR]
        out += [p0[0], s[0], s[1], s[2], p1[1], s[3], s[4], p0[1], s[5], s[6], p1[0]]
    else:
        st, p0, p1 = _scheme([3, 4], [1, 2], [1, 2]), _plain(3, 0), _plain(4, 0)
        out += [st[k] for k in _STR] + [p0[0], p1[0], p0[1], p1[1]]
    for p in out:
        if next(iter(p["w"].values())) < 0:
            p["w"] = {k: -c for k, c in p["w"].items()}
            p["g"] = [(n, _neg(v)) for n, v in p["g"]]
        p["f"] = tuple(p["f"])
    return out


O_PRODS = _prods("o")
Q_PRODS = _prods("q")
O_WC = [r for r, p in enumerate(O_PRODS) if len(p["w"]) > 1]
Q_WC = [r for r, p in enumerate(Q_PRODS) if len(p["w"]) > 1]


def _is_raw(f):
    return len(f) == 1 and f[0][1] in (E1, E2)


def _uniq(xs):
    out = []
    for x in xs:
        if x not in out:
            out.append(x)
    return out


O_LHS = _uniq([p["f"] for p in O_PRODS])
Q_LHS = [f for f in _uniq([p["f"] for p in Q_PRODS]) if not _is_raw(f)]


def _make_lhs(block, keys):
    cache = {}

    def form(k, v):
        sgn = -1 if min(v) < 0 else 1
        v = (abs(v[0]), abs(v[1]))
        if (k, v) not in cache:
            cache[k, v] = form(k, E1)[1] + form(k, E2)[1] if v == SS else block(v[1], k)
        return sgn, cache[k, v]

    out = []
    for key in keys:
        terms = [form(k, v) for k, v in key]
        assert terms[0][0] == 1
        val = terms[0][1]
        if len(terms) == 2:
            val = val + terms[1][1] if terms[1][0] > 0 else val - terms[1][1]
        out.append(val)
    return out


def _bilinear_run(accs, prods, lo, hi, lhs_of, w_of):
    for r in range(lo, hi):
        p = prods[r]
        m = jnp.dot(lhs_of(p["f"]), w_of(r), preferred_element_type=f32)
        for n, v in p["g"]:
            sgn = -1 if (v[0] < 0 or (v[0] == 0 and v[1] < 0)) else 1
            key = (n, (v[0] * sgn, v[1] * sgn))
            if key not in accs:
                accs[key] = (sgn, m)
            else:
                s0, a = accs[key]
                accs[key] = (s0, a + m if s0 == sgn else a - m)


def _bilinear_out(accs, i, n):
    s, a = accs[n, (E1, E2)[i]]
    if (n, DD) in accs:
        sd, dd = accs[n, DD]
        a = a + dd if s == (sd if i == 0 else -sd) else a - dd
    return s, a


def _mul(i, n):
    return i * n if isinstance(i, int) else pl.multiple_of(i * n, 16)


def _as_bf16(packed):
    return pltpu.bitcast(packed, bf16)


def _as_f32(packed):
    return pltpu.bitcast(packed, bf16).astype(f32)


def _q_operands(c, scale):
    t = [[a * (s * scale) for s, a in row] for row in c]
    lane = lax.broadcasted_iota(jnp.int32, t[0][0].shape, 1)
    lo = lane < 64
    out = []
    for h in range(2):
        if h == 0:
            valid = lane < 96
            h1 = [t[i][0] for i in range(2)]
            h2 = [jnp.where(lo, t[i][1], pltpu.roll(t[i][0], 96, 1)) for i in range(2)]
        else:
            valid = lane >= 32
            h1 = [t[i][2] for i in range(2)]
            h2 = [jnp.where(lo, pltpu.roll(t[i][2], 32, 1), t[i][1]) for i in range(2)]
        (a11, a21), (a12, a22) = h1, h2
        out.append([a11 + a22, jnp.where(valid, a21 + a22, 0.0), a11, a22, a11 + a12, a21 - a11, a12 - a22])
    return out


def _scores_half(qh, kts, h, j):
    r1, r2 = ([(0, 96)], [(128, 192), (96, 128)]) if h == 0 else ([(288, 384)], [(256, 288), (192, 256)])
    zf = jnp.zeros((32, 128), f32)

    def pk(f):
        return jnp.concatenate([f, zf] if h == 0 else [zf, f], axis=0).astype(bf16)

    def blk(i, name):
        k = kts(i if NOCSE else 0)
        c = j if name[1] == "1" else j + 2
        return jnp.concatenate([k[a:b, c * 128:(c + 1) * 128].astype(f32)
                                for a, b in (r1 if name[0] == "1" else r2)], axis=0)

    bs = [pk(blk(0, "11") + blk(0, "22")),
          kts(6 if NOCSE else 0)[h * 256:h * 256 + 128, j * 128:(j + 1) * 128],
          pk(blk(1, "12") - blk(1, "22")), pk(blk(2, "21") - blk(2, "11")), pk(blk(3, "22")),
          pk(blk(4, "11") + blk(4, "12")), pk(blk(5, "21") + blk(5, "22"))]
    m = [None] * 7
    for i in (0, 3, 4, 6, 1, 2, 5):
        m[i] = jnp.dot(qh[i], bs[i], preferred_element_type=f32)
    return (jnp.concatenate([(m[0] + m[3]) + (m[6] - m[4]), m[1] + m[3]], axis=0),
            jnp.concatenate([m[2] + m[4], (m[0] - m[1]) + (m[2] + m[5])], axis=0))


def _softmax(s):
    m = jnp.max(s, axis=1, keepdims=True)
    p = jnp.exp2(s - m)
    t = (p[:, 0:128] + p[:, 128:256]) + (p[:, 256:384] + p[:, 384:512])
    p = jnp.concatenate([p[:, 0:384], jnp.minimum(p[:, 384:512], t)], axis=1)
    l = jnp.sum(t, axis=1, keepdims=True)
    r = pl.reciprocal(l, approx=True)
    r = r * (2.0 - l * r)
    return p.astype(bf16), r


def _schedule(nu, pat):
    if "@" in pat:
        return [(a.split("@")[0], int(a.split("@")[1])) for a in pat.split(",")]
    pat = [(a.split(":")[0], int(a.split(":")[1])) for a in pat.split(",")]
    order = []
    for t in range(-6, nu + 6):
        for name, lag in pat:
            u = t + lag
            if 0 <= u < nu:
                order.append((name, u))
    return order


def _kernel(ax, ak, av, awq, awo, bx, bk, bv, bwq, bwo, o_hbm,
            acc, x32, wq32, wo32, kvbuf, obuf, pbuf, qbuf, xc32, wqc0, wqc1, woc0, woc1,
            kv_sem, x_sem, w_sem, o_sem, *, scale, nhp, nb):
    xbuf, wqbuf, wobuf = (r.bitcast(bf16) for r in (x32, wq32, wo32))
    pbuf, qbuf, xc = (r.bitcast(bf16) for r in (pbuf, qbuf, xc32))
    wqc = [r.bitcast(bf16) for r in (wqc0, wqc1)]
    woc = [r.bitcast(bf16) for r in (woc0, woc1)]
    sq = xbuf.shape[3]
    hq = sq // 2
    d = wqbuf.shape[3]
    hw = wobuf.shape[3]
    ng = nhp * nb
    lg = nb.bit_length() - 1
    assert nb == 1 << lg

    def kv_start(g, which=(0, 1, 2, 3)):
        hp, b = (g >> lg) & (nhp - 1), g & (nb - 1)
        for i, src in enumerate((ak, av, bk, bv)):
            if i in which:
                pltpu.make_async_copy(src.at[b, hp], kvbuf.at[b, i], kv_sem.at[b]).start()

    def kv_wait(b):
        pltpu.make_async_copy(kvbuf.at[b], kvbuf.at[b], kv_sem.at[b]).wait()

    def x_start(b, which=(0, 1)):
        for i, src in enumerate((ax, bx)):
            if i in which:
                for c in range(xbuf.shape[2]):
                    pltpu.make_async_copy(src.at[b, :, pl.ds(c * 128, 128)], xbuf.at[b, i, c], x_sem.at[b]).start()

    def x_wait(b):
        pltpu.make_async_copy(xbuf.at[b], xbuf.at[b], x_sem.at[b]).wait()

    def wslot(h):
        return h % 3 if isinstance(h, int) else lax.rem(h, 3)

    def w_start(h, k):
        sl = wslot(h)
        off = h * hw if isinstance(h, int) else pl.multiple_of(h * hw, 128)
        if k < 2:
            for c in range(wqbuf.shape[2]):
                pltpu.make_async_copy((awq, bwq)[k].at[:, pl.ds(off + c * 128, 128)], wqbuf.at[sl, k, c],
                                      w_sem.at[0, sl]).start()
        else:
            for c in range(wobuf.shape[2]):
                pltpu.make_async_copy((awo, bwo)[k - 2].at[pl.ds(off, hw), pl.ds(c * 128, 128)],
                                      wobuf.at[sl, k - 2, c], w_sem.at[1, sl]).start()

    def w_wait(h):
        sl = wslot(h)
        pltpu.make_async_copy(wqbuf.at[sl], wqbuf.at[sl], w_sem.at[0, sl]).wait()
        pltpu.make_async_copy(wobuf.at[sl], wobuf.at[sl], w_sem.at[1, sl]).wait()

    def prep_w(src_slot, dst_slot, row, nrows, br, which):
        raw, dst, prods, idx = ((wq32, wqc, Q_PRODS, Q_WC), (wo32, woc, O_PRODS, O_WC))[which]
        r8 = row * 8 if isinstance(row, int) else pl.multiple_of(row * 8, 8)
        r16 = row * 16 if isinstance(row, int) else pl.multiple_of(row * 16, 16)
        for slot, r in enumerate(idx):
            val = None
            for (k, n), c in prods[r]["w"].items():
                t = _as_f32(raw[src_slot, br, n, pl.ds(k * 64 + r8, nrows * 8), :])
                val = t if val is None else (val + t if c > 0 else val - t)
            dst[dst_slot][pl.ds(br * 128 + r16, nrows * 16), slot * 128:(slot + 1) * 128] = val.astype(bf16)

    def prep_x(b, br):
        vals = _make_lhs(lambda i, k: _as_f32(x32[b, br, k, i * (hq // 2):(i + 1) * (hq // 2), :]), Q_LHS)
        for i, v in enumerate(vals):
            xc[pl.ds(_mul(b * 2 + br, hq), hq), i * 128:(i + 1) * 128] = v.astype(bf16)

    def body(g0, nbat, extra, pat, cs, first_hp=False, last_hp=False):
        hp = g0 >> lg
        b0 = g0 & (nb - 1)
        rs = wslot(hp)
        R, O, OT, OC = {}, {}, {}, {}

        def prow(u, h):
            return (2 * u + h) * sq

        def weights(raw, comb, prods, idx, br):
            def w_of(r):
                if r in idx:
                    s = idx.index(r)
                    return comb[cs][br * 128:(br + 1) * 128, s * 128:(s + 1) * 128]
                (k, n), = prods[r]["w"]
                return _as_bf16(raw[rs, br, n, k * 64:(k + 1) * 64, :])
            return w_of

        QA, OA, SC, LH = {}, {}, {}, {}

        def q_(u, lo_, hi_):
            b, br = b0 + u // 2, u % 2

            def lhs_of(f):
                if _is_raw(f):
                    (k, v), = f
                    return _as_bf16(x32[b, br, k, v[1] * (hq // 2):(v[1] + 1) * (hq // 2), :])
                i = Q_LHS.index(f)
                return xc[pl.ds(_mul(b * 2 + br, hq), hq), i * 128:(i + 1) * 128]

            _bilinear_run(QA.setdefault(u, {}), Q_PRODS, lo_, hi_, lhs_of, weights(wq32, wqc, Q_PRODS, Q_WC, br))
            if hi_ == len(Q_PRODS):
                c = [[_bilinear_out(QA[u], i, n) for n in range(3)] for i in range(2)]
                for h, ops in enumerate(_q_operands(c, scale)):
                    for i, a in enumerate(ops):
                        qbuf[u * hq:(u + 1) * hq, (7 * h + i) * 128:(7 * h + i + 1) * 128] = a.astype(bf16)

        def s_(u, h, j):
            b, br = b0 + u // 2, u % 2
            qh = [qbuf[u * hq:(u + 1) * hq, (7 * h + i) * 128:(7 * h + i + 1) * 128] for i in range(7)]
            SC[u, h, j] = _scores_half(qh, lambda i: kvbuf.at[b + (g0 >> (16 + i)), 2 * br], h, j)
            if j == 1:
                s = jnp.concatenate([SC[u, h, 0][0], SC[u, h, 1][0], SC[u, h, 0][1], SC[u, h, 1][1]], axis=1)
                p, R[u, h] = _softmax(s)
                pbuf[prow(u, h):prow(u, h) + sq, :] = p

        def m_(u, h):
            vt = kvbuf.at[b0 + u // 2, 2 * (u % 2) + 1]
            O[u, h] = lax.dot_general(pbuf[prow(u, h):prow(u, h) + sq, :], vt[h * 256:h * 256 + 128, :], NT,
                                      preferred_element_type=f32) * R[u, h]

        def t_(u, h):
            vt = kvbuf.at[b0 + u // 2, 2 * (u % 2) + 1]
            OT[u, h] = lax.dot_general(vt[128 + h * 64:192 + h * 64, :], pbuf[prow(u, h):prow(u, h) + 128, :], NT,
                                       preferred_element_type=f32)

        def c_(u):
            vt = kvbuf.at[b0 + u // 2, 2 * (u % 2) + 1]
            pc = jnp.concatenate([pbuf[prow(u, h) + 128:prow(u, h) + sq, :] for h in range(2)], axis=0)
            OC[u] = lax.dot_general(pc, vt[128:256, :], NT, preferred_element_type=f32)

        def o_(u, lo_, hi_):
            b, br = b0 + u // 2, u % 2
            if lo_ == 0:
                n = sq - 128
                top = jnp.concatenate([OT[u, 0], OT[u, 1]], axis=0).T
                bot = jnp.where(lax.broadcasted_iota(jnp.int32, (n, 128), 1) < 64, OC[u][0:n], OC[u][n:2 * n])
                lo = lax.broadcasted_iota(jnp.int32, (sq, 128), 1) < 64
                mid = jnp.concatenate([top, bot], axis=0) * jnp.where(lo, R[u, 0], R[u, 1])
                tiles = (O[u, 0], mid, O[u, 1])
                LH[u] = [a.astype(bf16) for a in _make_lhs(lambda i, k: tiles[k][i * hq:(i + 1) * hq], O_LHS)]
            _bilinear_run(OA.setdefault(u, {}), O_PRODS, lo_, hi_, lambda f: LH[u][O_LHS.index(f)],
                          weights(wo32, woc, O_PRODS, O_WC, br))
            for n in (range(3) if lo_ == 0 else range(3, 5)):
                for i in range(2):
                    s, a = _bilinear_out(OA[u], i, n)
                    rows = slice(i * hq, (i + 1) * hq)
                    cols = slice(br * d + n * 128, br * d + (n + 1) * 128)
                    if first_hp:
                        new = a if s > 0 else -a
                    else:
                        new = acc[b, rows, cols] + a if s > 0 else acc[b, rows, cols] - a
                    if last_hp:
                        obuf[b, rows, cols] = new.astype(obuf.dtype)
                    else:
                        acc[b, rows, cols] = new
            if br == 1 and lo_ > 0 and last_hp:
                pltpu.make_async_copy(obuf.at[b], o_hbm.at[b], o_sem).start()

        fns = {"qa": lambda u: q_(u, 0, 15), "qb": lambda u: q_(u, 15, 26),
               "oa": lambda u: o_(u, 0, 15), "ob": lambda u: o_(u, 15, 26),
               "s00": lambda u: s_(u, 0, 0), "s01": lambda u: s_(u, 0, 1),
               "s10": lambda u: s_(u, 1, 0), "s11": lambda u: s_(u, 1, 1),
               "m0": lambda u: m_(u, 0), "m1": lambda u: m_(u, 1),
               "t0": lambda u: t_(u, 0), "t1": lambda u: t_(u, 1), "c": c_}
        sched = _schedule(2 * nbat, pat)
        first, dmas, preps = extra
        for f in first:
            f()
        slots = list(range(PFPOS, len(sched), PFSTEP if nbat > 1 else 1))
        per = max(1, -(-len(dmas) // len(slots)))
        pslots = [i + 1 for i in range(len(sched) - 1)
                  if sched[i][0][0] in "qo" and sched[i + 1][0][0] not in "qo"][PSKIP if nbat > 1 else 0:]
        pper = max(1, -(-len(preps) // len(pslots)))
        for i, item in enumerate(sched):
            if i in slots:
                k = slots.index(i)
                for f in dmas[k * per:(k + 1) * per]:
                    f()
            if i in pslots:
                k = pslots.index(i)
                for f in preps[k * pper:(k + 1) * pper]:
                    f()
            fns[item[0]](item[1])

    for k in range(4):
        w_start(0, k)
    x_start(0)
    kv_start(0)
    x_start(1)
    for g in range(1, C0):
        kv_start(g)
        x_start(g + 1)
    w_wait(0)
    for br in range(2):
        for which in range(2):
            prep_w(0, 0, 0, 8, br, which)
    x_wait(0)
    for br in range(2):
        prep_x(0, br)

    def issued(g):
        return jnp.minimum(jnp.minimum(RATE * (g + 1) + C0, g + nb), G1 + BB)

    def small(hp, b0, carry):
        g0 = hp * nb + b0

        if hp == 0:
            @pl.when(b0 + 1 < nb)
            def _():
                x_wait(b0 + 1)

        @pl.when(b0 == nb // 2)
        def _():
            w_wait(hp + 1)

        kv_wait(b0)

        hi = issued(g0)
        prev = jnp.where(g0 == 0, C0, issued(g0 - 1))

        def pf_x(k, w):
            @pl.when(jnp.logical_and(prev + k < hi, prev + k + 1 < nb))
            def _():
                x_start(prev + k + 1, (w,))

        def pf_kv(k):
            @pl.when(prev + k < hi)
            def _():
                kv_start(prev + k)

        def pf_w(h, at, k):
            @pl.when(b0 + k == at + k)
            def _():
                w_start(h, k)

        src = jnp.where(b0 >= nb // 2, wslot(hp + 1), wslot(hp))
        row = b0 & (nb // 2 - 1)
        first = [functools.partial(pf_w, hp + 2, 12, k) for k in range(4)]
        preps = []
        if hp == 0:
            first += [functools.partial(pf_w, 1, 3, k) for k in range(4)]
            first += [functools.partial(pf_x, k, w) for k in range(RATE) for w in range(2)]
            preps += [functools.partial(prep_x, jnp.minimum(b0 + 1, nb - 1), br) for br in range(2)]
        first += [functools.partial(pf_kv, k) for k in range(RATE)]
        preps += [functools.partial(prep_w, src, (hp + 1) & 1, row, 1, br, w) for br in range(2) for w in range(2)]
        body(g0, 1, (first, [], preps), SPAT, hp & 1, first_hp=hp == 0)
        return carry

    def big(par, last, i, carry):
        g0 = i * BB
        hp = g0 >> lg
        b0 = g0 & (nb - 1)
        nrows = 8 * BB // nb

        if not last:
            @pl.when(b0 == 0)
            def _():
                w_wait(hp + 1)

        for j in range(BB):
            kv_wait(b0 + j)

        def pf_w(k):
            @pl.when(jnp.logical_and(b0 + k == nb - BB + k, hp + 2 < nhp))
            def _():
                w_start(hp + 2, k)

        def pf_kv(j):
            @pl.when(g0 + BB + j < ng)
            def _():
                kv_start(g0 + BB + j)

        row = lax.div(b0, BB) * nrows
        if last:
            extra = ([functools.partial(pf_kv, j) for j in range(BB)], [], [])
        else:
            kvs = [functools.partial(kv_start, g0 + BB + j) for j in range(BB)]
            extra = ([functools.partial(pf_w, k) for k in range(4)] + kvs[:KVTOP], kvs[KVTOP:],
                     [functools.partial(prep_w, wslot(hp + 1), 1 - par, row + r, 1, br, w)
                      for r in range(nrows) for br in range(2) for w in range(2)])
        body(g0, BB, extra, PAT, par, last_hp=last)
        return carry

    nsm = G1 // nb
    spb = nb // BB
    if SKIP_SMALL in (0, 2):
        for hp in range(nsm):
            lax.fori_loop(0, nb, functools.partial(small, hp), 0)
    if SKIP_SMALL == 2:
        prep_x(0, 0)
        acc[0, 0:128, 0:128] = (wqc[1][0:128, 0:128] + woc[1][0:128, 0:128]).astype(f32)
        pltpu.make_async_copy(obuf, o_hbm, o_sem).start()
        pltpu.make_async_copy(obuf, o_hbm, o_sem).wait()
        return

    def pair(t, carry):
        lax.fori_loop(jnp.maximum(2 * t, nsm) * spb, (2 * t + 1) * spb, functools.partial(big, 0, False), 0)
        lax.fori_loop((2 * t + 1) * spb, jnp.minimum(2 * t + 2, nhp - 1) * spb, functools.partial(big, 1, False), 0)
        return carry

    lax.fori_loop(nsm // 2, nhp // 2, pair, 0)
    if not SKIP_SMALL:
        lax.fori_loop((nhp - 1) * spb, nhp * spb, functools.partial(big, 1, True), 0)
    pltpu.make_async_copy(obuf, o_hbm, o_sem).wait()


@jax.jit
def pallas_concat_heads__gqa_block_cached__mha_block_cached__near_ridge_kernel(
    A_x, A_k_cache, A_v_cache, A_wq, A_wo, B_x, B_k_cache, B_v_cache, B_wq, B_wo):
    B, Sq, D = A_x.shape
    _, H, Sk, Dh = A_k_cache.shape
    nhp = H // 2
    assert B == 16 and G1 % B == 0 and 2 * BB <= B and C0 >= 1
    n_iss = C0
    for g0 in range(G1):
        assert n_iss >= min(g0 + 2, G1 + BB), (g0, n_iss)
        hi = min(RATE * (g0 + 1) + C0, g0 + B, G1 + BB)
        assert 0 <= hi - n_iss <= RATE
        n_iss = hi
    assert n_iss == G1 + BB, n_iss

    def tr(c):
        return jnp.swapaxes(c, 2, 3).reshape(B, nhp, 2 * Dh, Sk)

    any_spec = pl.BlockSpec(memory_space=pl.ANY)
    return pl.pallas_call(
        functools.partial(_kernel, scale=Dh ** -0.5 * LOG2E, nhp=nhp, nb=B),
        in_specs=[any_spec] * 10,
        out_specs=any_spec,
        out_shape=jax.ShapeDtypeStruct((B, Sq, 2 * D), A_x.dtype),
        scratch_shapes=[pltpu.VMEM((B, Sq, 2 * D), f32),
                        pltpu.VMEM((B, 2, D // 128, Sq // 2, 128), u32),
                        pltpu.VMEM((3, 2, 2 * Dh // 128, D // 2, 128), u32),
                        pltpu.VMEM((3, 2, D // 128, Dh, 128), u32),
                        pltpu.VMEM((B, 4, 2 * Dh, Sk), bf16),
                        pltpu.VMEM((B, Sq, 2 * D), bf16),
                        pltpu.VMEM((2 * BB * Sq, Sk), u32),
                        pltpu.VMEM((2 * BB * Sq // 4, 14 * 128), u32),
                        pltpu.VMEM((B * 2 * Sq // 4, len(Q_LHS) * 128), u32),
                        pltpu.VMEM((2 * 64, len(Q_WC) * 128), u32),
                        pltpu.VMEM((2 * 64, len(Q_WC) * 128), u32),
                        pltpu.VMEM((2 * 64, len(O_WC) * 128), u32),
                        pltpu.VMEM((2 * 64, len(O_WC) * 128), u32),
                        pltpu.SemaphoreType.DMA((B,)),
                        pltpu.SemaphoreType.DMA((B,)),
                        pltpu.SemaphoreType.DMA((2, 3)),
                        pltpu.SemaphoreType.DMA(())],
        compiler_params=pltpu.CompilerParams(
            disable_bounds_checks=True,
            vmem_limit_bytes=110 * 1024 * 1024),
    )(A_x, tr(A_k_cache), tr(A_v_cache), A_wq, A_wo, B_x, tr(B_k_cache), tr(B_v_cache), B_wq, B_wo)
```

```python
import functools
import jax
import jax.numpy as jnp
from jax import lax
import jax.experimental.pallas as pl
import jax.experimental.pallas.tpu as pltpu

BB = 4
G1 = 16
C0 = 2
RATE = 2
PFPOS = 1
PFSTEP = 3
PSKIP = 2
OBUF = 1
SKIP_SMALL = 0
KVTOP = 8
QSPLIT = 13
OSPLIT = 13
PPARTS = 8
PEND = 10
XCW = 32
WCW = 40
ACCR = 160
WQT = 3
WOT = 5
MERGE = 0
TOK = 1
W2AT = 11
LA = 6
NOCSE = 1
PAT = "s00:0,s01:0,m0:-1,qb:2,qa:3,s10:0,s11:0,m1:-1,t1:-1,t0:-1,oa:-2,c:-1,ob:-2"
SPAT = "qa@0,qb@0,qa@1,qb@1,s00@0,s10@0,s11@0,s00@1,s10@1,s01@0,t1@0,m1@0,s11@1,m0@0,t0@0,c@0,m1@1,s01@1,oa@0,t1@1,c@1,t0@1,m0@1,ob@0,oa@1,ob@1"
LOG2E = 1.4426950408889634
bf16 = jnp.bfloat16
f32 = jnp.float32
u32 = jnp.uint32
NT = (((1,), (1,)), ((), ()))

O_LHS_PROG = [(100, 4, 5, 1), (101, 0, 1, -1), (102, 3, 101, 1), (103, 2, 100, 1), (104, 0, 3, 1), (105, 2, 3, -1), (106, 0, 2, 1), (107, 2, 101, -1), (108, 3, 5, 1), (109, 1, 103, 1), (110, 2, 5, 1), (111, 3, 100, -1), (112, 5, 101, 1), (113, 4, 102, -1), (114, 0, 100, 1)]
O_OUT_PROG = [(100, 5, 8, -1), (101, 3, 100, 1), (102, 2, 7, -1), (103, 0, 102, 1)]
O_PRODS = [((101, 1), [(2, 1), (5, 1), (10, -1), (12, 1)], [(102, 1)]), ((104, 1), [(3, 1)], [(100, -1)]), ((111, 1), [(0, 1), (3, 1)], [(5, 1)]), ((5, 1), [(5, 1), (10, -1)], [(5, -1), (103, 1)]), ((112, 1), [(5, 1), (10, -1), (12, 1)], [(103, -1)]), ((114, 1), [(0, 1), (3, 1), (5, 1)], [(101, 1)]), ((0, 1), [(0, 1), (5, 1)], [(0, 1), (101, -1)]), ((107, -1), [(10, 1), (12, -1)], [(0, -1)]), ((110, 1), [(12, 1)], [(0, 1), (2, 1)]), ((1, 1), [(2, 1), (7, 1)], [(2, 1), (4, -1)]), ((104, 1), [(1, 1), (2, 1), (4, 1), (7, 1), (9, 1)], [(4, 1)]), ((106, 1), [(1, 1)], [(1, 1), (4, -1)]), ((1, 1), [(6, 1)], [(1, 1), (3, -1)]), ((109, 1), [(6, 1), (8, 1)], [(3, 1)]), ((2, 1), [(1, 1), (11, -1)], [(1, -1), (6, 1)]), ((103, 1), [(6, 1), (8, 1), (13, -1)], [(3, -1), (6, 1)]), ((100, 1), [(0, 1), (3, 1), (5, 1), (13, 1)], [(3, -1), (8, 1)]), ((4, 1), [(8, 1), (13, -1)], [(6, -1), (8, 1)]), ((110, 1), [(6, 1), (8, 1), (11, -1), (13, -1), (14, -1)], [(6, -1)]), ((105, 1), [(1, 1), (14, 1)], [(4, 1), (6, -1)]), ((108, 1), [(14, 1)], [(6, -1), (9, 1)]), ((3, 1), [(4, 1), (14, -1)], [(4, -1), (9, 1)]), ((4, 1), [(9, 1)], [(7, -1), (9, 1)]), ((102, 1), [(2, 1), (7, 1), (9, 1)], [(4, -1), (7, 1)]), ((113, -1), [(7, 1), (9, 1)], [(7, -1)])]
Q_LHS_PROG = [(100, 3, 8, -1), (101, 0, 2, 1), (102, 7, 101, -1), (103, 5, 100, 1), (104, 4, 6, -1), (105, 4, 9, -1), (106, 7, 9, -1), (107, 0, 103, -1), (108, 6, 8, -1), (109, 5, 102, 1), (110, 1, 4, -1), (111, 5, 8, -1), (112, 6, 9, -1), (113, 4, 7, -1), (114, 2, 4, -1), (115, 1, 6, -1), (116, 2, 7, -1), (117, 1, 3, -1), (118, 3, 6, -1)]
Q_OUT_PROG = [(100, 0, 3, 1), (101, 4, 5, 1), (102, 0, 1, -1), (103, 2, 101, 1), (104, 2, 5, 1), (105, 1, 100, -1)]
Q_PRODS = [((6, -1), [(6, 1), (8, 1), (11, -1), (13, -1), (14, -1)], [(104, 1)]), ((101, 1), [(12, 1)], [(104, 1)]), ((4, 1), [(1, 1), (2, 1), (4, 1), (7, 1), (9, 1)], [(100, 1)]), ((111, -1), [(3, 1)], [(100, 1)]), ((118, -1), [(6, 1), (8, 1), (13, -1)], [(103, 1)]), ((3, 1), [(6, 1), (8, 1)], [(1, 1), (103, 1)]), ((114, 1), [(2, 1), (7, 1)], [(1, 1)]), ((117, 1), [(6, 1)], [(1, 1)]), ((115, -1), [(1, 1), (11, -1)], [(2, 1)]), ((0, -1), [(10, 1), (12, -1)], [(2, -1), (102, 1)]), ((116, 1), [(2, 1), (5, 1), (10, -1), (12, 1)], [(102, 1)]), ((102, 1), [(5, 1), (10, -1), (12, 1)], [(5, 1), (102, 1)]), ((109, -1), [(5, 1), (10, -1)], [(5, 1)]), ((112, -1), [(14, 1)], [(3, 1), (5, 1)]), ((104, 1), [(1, 1), (14, 1)], [(2, 1), (3, -1)]), ((105, -1), [(4, 1), (14, -1)], [(3, 1)]), ((5, 1), [(0, 1), (3, 1)], [(3, 1), (101, -1)]), ((100, -1), [(0, 1), (3, 1), (5, 1), (13, 1)], [(101, 1)]), ((103, 1), [(0, 1), (3, 1), (5, 1)], [(0, 1), (101, 1)]), ((110, 1), [(1, 1)], [(0, 1), (2, 1)]), ((107, 1), [(0, 1), (5, 1)], [(0, 1)]), ((113, -1), [(2, 1), (7, 1), (9, 1)], [(105, -1)]), ((7, -1), [(7, 1), (9, 1)], [(4, -1), (105, -1)]), ((106, -1), [(9, 1)], [(4, 1)]), ((108, -1), [(8, 1), (13, -1)], [(4, 1)])]
NPROD = len(O_PRODS)


def _normalize(prods):
    out = []
    for (var, sgn), w, g in prods:
        sgn *= w[0][1]
        out.append((var, [(y, c * w[0][1]) for y, c in w], [(z, c * sgn) for z, c in g]))
    return out


OORD = "1.0.3.2.5.6.8.9.4.24.11.12.10.14.13.15.16.17.18.19.20.21.22.23.7"
QORD = "14.15.16.17.18.19.20.21.22.24.23.0.1.6.2.7.3.4.5.8.9.10.11.12.13"
SOORD = "7.23.22.21.20.19.18.16.17.15.13.12.10.11.14.9.8.24.6.5.2.3.4.0.1"
SQORD = "14.15.16.17.18.10.20.21.22.24.1.23.6.2.7.0.3.8.4.5.9.19.11.12.13"
LOORD = OORD
LQORD = QORD
LPAT = PAT
O_PRODS = _normalize(O_PRODS)
Q_PRODS = _normalize(Q_PRODS)
W_FORMS = [p[1] for p in O_PRODS]


def _positive_outputs(prods, prog):
    for flips in range(1 << 6):
        sg = [(-1 if (flips >> (r % 6)) & 1 else 1) for r in range(len(prods))]
        pos = {}
        for r, p in enumerate(prods):
            for z, c in p[2]:
                pos[z] = max(pos.get(z, -1), c * sg[r])
        for t, a, b, s in reversed(prog):
            st = pos.pop(t)
            pos[a] = max(pos.get(a, -1), st)
            pos[b] = max(pos.get(b, -1), st * s)
        if min(pos.values()) > 0:
            return sg
    raise AssertionError


Q_SIGN = _positive_outputs(Q_PRODS, Q_OUT_PROG)
Q_PRODS = [(v, w, [(z, c * s) for z, c in g]) for (v, w, g), s in zip(Q_PRODS, Q_SIGN)]


def _make_lhs(block, prog):
    vals = {}

    def get(v):
        if v not in vals:
            vals[v] = block(v)
        return vals[v]

    for t, a, b, s in prog:
        vals[t] = get(a) + get(b) if s > 0 else get(a) - get(b)
    return get


def _acc_add(accs, z, sgn, m):
    if z not in accs:
        accs[z] = (sgn, m)
    else:
        s0, a = accs[z]
        accs[z] = (s0, a + m) if s0 == sgn else ((1, a - m) if s0 > 0 else (1, m - a))


def _bilinear_run(accs, prods, which, lhs_of, w_of):
    for r in which:
        m = jnp.dot(lhs_of(r), w_of(r), preferred_element_type=f32)
        for z, c in prods[r][2]:
            _acc_add(accs, z, c, m)


def _bilinear_finish(accs, prog):
    for t, a, b, s in reversed(prog):
        st, v = accs.pop(t)
        _acc_add(accs, a, st, v)
        _acc_add(accs, b, st * s, v)
    return accs


def _mul(i, n):
    return i * n if isinstance(i, int) else pl.multiple_of(i * n, 16)


def _as_bf16(packed):
    return pltpu.bitcast(packed, bf16)


def _as_f32(packed):
    return pltpu.bitcast(packed, bf16).astype(f32)


def _q_operands(c):
    assert all(s > 0 for row in c for s, _ in row)
    t = [[a for _, a in row] for row in c]
    lane = lax.broadcasted_iota(jnp.int32, t[0][0].shape, 1)
    lo = lane < 64
    out = []
    for h in range(2):
        if h == 0:
            valid = lane < 96
            h1 = [t[i][0] for i in range(2)]
            h2 = [jnp.where(lo, t[i][1], pltpu.roll(t[i][0], 96, 1)) for i in range(2)]
        else:
            valid = lane >= 32
            h1 = [t[i][2] for i in range(2)]
            h2 = [jnp.where(lo, pltpu.roll(t[i][2], 32, 1), t[i][1]) for i in range(2)]
        (a11, a21), (a12, a22) = h1, h2
        out.append([a11 + a22, jnp.where(valid, a21 + a22, 0.0), a11, a22, a11 + a12, a21 - a11, a12 - a22])
    return out


def _scores_half(qh, kts, h, j):
    r1, r2 = ([(0, 96)], [(128, 192), (96, 128)]) if h == 0 else ([(288, 384)], [(256, 288), (192, 256)])
    zf = jnp.zeros((32, 128), f32)

    def pk(f):
        return jnp.concatenate([f, zf] if h == 0 else [zf, f], axis=0).astype(bf16)

    def blk(i, name):
        k = kts(i if NOCSE else 0)
        c = j if name[1] == "1" else j + 2
        return jnp.concatenate([k[a:b, c * 128:(c + 1) * 128].astype(f32)
                                for a, b in (r1 if name[0] == "1" else r2)], axis=0)

    bs = [pk(blk(0, "11") + blk(0, "22")),
          kts(6 if NOCSE else 0)[h * 256:h * 256 + 128, j * 128:(j + 1) * 128],
          pk(blk(1, "12") - blk(1, "22")), pk(blk(2, "21") - blk(2, "11")), pk(blk(3, "22")),
          pk(blk(4, "11") + blk(4, "12")), pk(blk(5, "21") + blk(5, "22"))]
    m = [None] * 7
    for i in (0, 3, 4, 6, 1, 2, 5):
        m[i] = jnp.dot(qh[i], bs[i], preferred_element_type=f32)
    return (jnp.concatenate([(m[0] + m[3]) + (m[6] - m[4]), m[1] + m[3]], axis=0),
            jnp.concatenate([m[2] + m[4], (m[0] - m[1]) + (m[2] + m[5])], axis=0))


def _softmax(s):
    m = jnp.max(s, axis=1, keepdims=True)
    p = jnp.exp2(s - m)
    t = (p[:, 0:128] + p[:, 128:256]) + (p[:, 256:384] + p[:, 384:512])
    p = jnp.concatenate([p[:, 0:384], jnp.minimum(p[:, 384:512], t)], axis=1)
    l = jnp.sum(t, axis=1, keepdims=True)
    r = pl.reciprocal(l, approx=True)
    r = r * (2.0 - l * r)
    return p.astype(bf16), r


def _schedule(nu, pat):
    if "@" in pat:
        return [(a.split("@")[0], int(a.split("@")[1])) for a in pat.split(",")]
    pat = [(a.split(":")[0], int(a.split(":")[1])) for a in pat.split(",")]
    order = []
    for t in range(-6, nu + 6):
        for name, lag in pat:
            u = t + lag
            if 0 <= u < nu:
                order.append((name, u))
    return order


def _kernel(ax, ak, av, awq, awo, bx, bk, bv, bwq, bwo, o_hbm,
            acc, x32, w32, kvbuf, obuf, pbuf, qbuf, xc32, wc0, wc1,
            kv_sem, x_sem, w_sem, o_sem, *, scale, nhp, nb):
    xbuf, wbuf = (r.bitcast(bf16) for r in (x32, w32))
    pbuf, qbuf, xc = (r.bitcast(bf16) for r in (pbuf, qbuf, xc32))
    wc = [r.bitcast(bf16) for r in (wc0, wc1)]
    sq = xbuf.shape[3]
    hq = sq // 2
    d = awq.shape[0]
    hw = kvbuf.shape[2]
    wrows = wbuf.shape[0] // 4
    ng = nhp * nb
    lg = nb.bit_length() - 1
    assert nb == 1 << lg

    def kv_start(g, which=(0, 1, 2, 3)):
        hp, b = (g >> lg) & (nhp - 1), g & (nb - 1)
        for i, src in enumerate((ak, av, bk, bv)):
            if i in which:
                pltpu.make_async_copy(src.at[b, hp], kvbuf.at[b, i], kv_sem.at[b]).start()

    def kv_wait(b):
        pltpu.make_async_copy(kvbuf.at[b], kvbuf.at[b], kv_sem.at[b]).wait()

    def x_start(b, which=(0, 1)):
        for i, src in enumerate((ax, bx)):
            if i in which:
                for c in range(xbuf.shape[2]):
                    pltpu.make_async_copy(src.at[b, :, pl.ds(c * 128, 128)], xbuf.at[b, i, c], x_sem.at[b]).start()

    def x_wait(b):
        pltpu.make_async_copy(xbuf.at[b], xbuf.at[b], x_sem.at[b]).wait()

    def w_start(h, m):
        off = h * hw if isinstance(h, int) else pl.multiple_of(h * hw, 128)
        if m < 2:
            for c in range(hw // 128):
                pltpu.make_async_copy((awq, bwq)[m].at[:, pl.ds(off + c * 128, 128)],
                                      wbuf.at[pl.ds(m * wrows + c * d, d)], w_sem.at[m]).start()
        else:
            for c in range(d // 128):
                pltpu.make_async_copy((awo, bwo)[m - 2].at[pl.ds(off, hw), pl.ds(c * 128, 128)],
                                      wbuf.at[pl.ds(m * wrows + c * hw, hw)], w_sem.at[m]).start()

    def w_start_dyn(h, m, valid):
        for k in range(4):
            @pl.when(jnp.logical_and(m == k, valid))
            def _():
                w_start(h, k)

    def w_wait(m):
        v = wbuf.at[pl.ds(_mul(m, wrows), wrows)]
        pltpu.make_async_copy(v, v, w_sem.at[m]).wait()

    def prep_w(dst, msrc, mdst, row, nrows, part=None, zero=None):
        if isinstance(msrc, int):
            sa, sc = (5, 1) if msrc < 2 else (1, 3)
            off = [(msrc * 15 + (y // 5) * sa + (y % 5) * sc) * 64 + row * 8 for y in range(15)]
        else:
            sa, sc = jnp.where(msrc < 2, 5, 1), jnp.where(msrc < 2, 1, 3)
            off = [pl.multiple_of((msrc * 15 + (y // 5) * sa + (y % 5) * sc) * 64 + row * 8, 64 if isinstance(row, int) and row == 0 else 32)
                   for y in range(15)]
        r16 = _mul(mdst * 8 + row, 16)
        if not isinstance(r16, int):
            r16 = pl.multiple_of(r16, 128 if isinstance(row, int) and row == 0 else 64)
        for r, form in enumerate(W_FORMS):
            if part is not None and r % PPARTS != part:
                continue
            if len(form) == 1:
                val = _as_bf16(w32[pl.ds(off[form[0][0]], nrows * 8), :])
            else:
                val = None
                for y, c in form:
                    t = _as_f32(w32[pl.ds(off[y], nrows * 8), :])
                    val = t if val is None else (val + t if c > 0 else val - t)
                val = val.astype(bf16)
            wc[dst][pl.ds(r16, nrows * 16), r * 128:(r + 1) * 128] = val
        if zero is not None:
            c0 = (part or 0) * 128
            return wc[dst][pl.ds(pl.multiple_of(r16 + zero * 16, 16), 16), c0:c0 + 128].astype(f32)[0:8]

    def prep_x(b, br, zero=None):
        get = _make_lhs(
            lambda z: _as_f32(x32[b, br, z % 5, (z // 5) * (hq // 2):(z // 5 + 1) * (hq // 2), :]) * scale,
            Q_LHS_PROG)
        for r, p in enumerate(Q_PRODS):
            xc[pl.ds(_mul(b * 2 + br, hq), hq), r * 128:(r + 1) * 128] = (get(p[0]) * Q_SIGN[r]).astype(bf16)
        if zero is not None:
            return xc[pl.ds(_mul(b * 2 + br + zero, hq), 16), 0:128].astype(f32)[0:8]

    def body(g0, nbat, extra, pat, cs, first_hp=False, last_hp=False):
        hp = g0 >> lg
        b0 = g0 & (nb - 1)
        R, O, OT, OC = {}, {}, {}, {}

        def prow(u, h):
            return (2 * u + h) * sq

        def weights(m, prods):
            def w_of(r):
                s = W_FORMS.index(prods[r][1])
                return wc[cs][m * 128:(m + 1) * 128, s * 128:(s + 1) * 128]
            return w_of

        QA, OA, SC, LH = {}, {}, {}, {}
        tokens = []
        pat, qord, oord = pat
        qord = [int(i) for i in qord.split(".")]
        oord = [int(i) for i in oord.split(".")]

        def q_(u, lo_, hi_):
            b, br = b0 + u // 2, u % 2

            def lhs_of(r):
                return xc[pl.ds(_mul(b * 2 + br, hq), hq), r * 128:(r + 1) * 128]

            _bilinear_run(QA.setdefault(u, {}), Q_PRODS, qord[lo_:hi_], lhs_of, weights(br, Q_PRODS))
            if hi_ == len(Q_PRODS):
                fin = _bilinear_finish(QA[u], Q_OUT_PROG)
                c = [[fin[i * 3 + n] for n in range(3)] for i in range(2)]
                for h, ops in enumerate(_q_operands(c)):
                    for i, a in enumerate(ops):
                        qbuf[u * hq:(u + 1) * hq, (7 * h + i) * 128:(7 * h + i + 1) * 128] = a.astype(bf16)

        def s_(u, h, j):
            b, br = b0 + u // 2, u % 2
            qh = [qbuf[u * hq:(u + 1) * hq, (7 * h + i) * 128:(7 * h + i + 1) * 128] for i in range(7)]
            SC[u, h, j] = _scores_half(qh, lambda i: kvbuf.at[b + (g0 >> (16 + i)), 2 * br], h, j)
            if j == 1:
                s = jnp.concatenate([SC[u, h, 0][0], SC[u, h, 1][0], SC[u, h, 0][1], SC[u, h, 1][1]], axis=1)
                p, R[u, h] = _softmax(s)
                pbuf[prow(u, h):prow(u, h) + sq, :] = p

        def m_(u, h):
            vt = kvbuf.at[b0 + u // 2, 2 * (u % 2) + 1]
            o = lax.dot_general(pbuf[prow(u, h):prow(u, h) + sq, :], vt[h * 256:h * 256 + 128, :], NT,
                                preferred_element_type=f32)
            while tokens:
                o = jnp.concatenate([jnp.minimum(o[0:8], jnp.maximum(o[0:8], tokens.pop())), o[8:]], axis=0)
            O[u, h] = o * R[u, h]

        def t_(u, h):
            vt = kvbuf.at[b0 + u // 2, 2 * (u % 2) + 1]
            OT[u, h] = lax.dot_general(vt[128 + h * 64:192 + h * 64, :], pbuf[prow(u, h):prow(u, h) + 128, :], NT,
                                       preferred_element_type=f32)

        def c_(u):
            vt = kvbuf.at[b0 + u // 2, 2 * (u % 2) + 1]
            pc = jnp.concatenate([pbuf[prow(u, h) + 128:prow(u, h) + sq, :] for h in range(2)], axis=0)
            OC[u] = lax.dot_general(pc, vt[128:256, :], NT, preferred_element_type=f32)

        def o_(u, lo_, hi_):
            b, br = b0 + u // 2, u % 2
            if lo_ == 0:
                n = sq - 128
                top = jnp.concatenate([OT[u, 0], OT[u, 1]], axis=0).T
                bot = jnp.where(lax.broadcasted_iota(jnp.int32, (n, 128), 1) < 64, OC[u][0:n], OC[u][n:2 * n])
                lo = lax.broadcasted_iota(jnp.int32, (sq, 128), 1) < 64
                mid = jnp.concatenate([top, bot], axis=0) * jnp.where(lo, R[u, 0], R[u, 1])
                tiles = (O[u, 0], mid, O[u, 1])
                get = _make_lhs(lambda x: tiles[x % 3][(x // 3) * hq:(x // 3 + 1) * hq], O_LHS_PROG)
                LH[u] = {p[0]: get(p[0]).astype(bf16) for p in O_PRODS}
            _bilinear_run(OA.setdefault(u, {}), O_PRODS, oord[lo_:hi_], lambda r: LH[u][O_PRODS[r][0]],
                          weights(2 + br, O_PRODS))
            fin = _bilinear_finish(OA[u], O_OUT_PROG) if hi_ == NPROD else {}
            for n in (range(5) if fin else ()):
                for i in range(2):
                    s, a = fin[i * 5 + n]
                    rows = slice(i * hq, (i + 1) * hq)
                    cols = slice(br * d + n * 128, br * d + (n + 1) * 128)
                    if first_hp:
                        new = a if s > 0 else -a
                    else:
                        new = acc[b, rows, cols] + a if s > 0 else acc[b, rows, cols] - a
                    if last_hp:
                        obuf[b, rows, cols] = new.astype(obuf.dtype)
                    if not last_hp:
                        acc[b, rows, cols] = new
            if br == 1 and lo_ > 0 and last_hp:
                pltpu.make_async_copy(obuf.at[b], o_hbm.at[b], o_sem).start()

        fns = {"qa": lambda u: q_(u, 0, QSPLIT), "qb": lambda u: q_(u, QSPLIT, NPROD),
               "oa": lambda u: o_(u, 0, OSPLIT), "ob": lambda u: o_(u, OSPLIT, NPROD),
               "s00": lambda u: s_(u, 0, 0), "s01": lambda u: s_(u, 0, 1),
               "s10": lambda u: s_(u, 1, 0), "s11": lambda u: s_(u, 1, 1),
               "m0": lambda u: m_(u, 0), "m1": lambda u: m_(u, 1),
               "t0": lambda u: t_(u, 0), "t1": lambda u: t_(u, 1), "c": c_}
        sched = _schedule(2 * nbat, pat)
        first, dmas, preps = extra
        for f in first:
            f()
        slots = list(range(PFPOS, len(sched), PFSTEP if nbat > 1 else 1))
        per = max(1, -(-len(dmas) // len(slots)))
        if nbat > 1:
            lo_, hi_ = PSKIP, len(sched) - PEND
            where = [lo_ + (k * (hi_ - lo_)) // max(len(preps), 1) for k in range(len(preps))]
        else:
            pslots = [i + 1 for i in range(len(sched) - 1)
                      if sched[i][0][0] in "qo" and sched[i + 1][0][0] not in "qo"]
            pper = max(1, -(-len(preps) // len(pslots)))
            where = [pslots[k // pper] for k in range(len(preps))]
        for i, item in enumerate(sched):
            if i in slots:
                k = slots.index(i)
                for f in dmas[k * per:(k + 1) * per]:
                    f()
            for k, f in enumerate(preps):
                if where[k] == i:
                    tok = f(zero=(g0 >> (24 - k)) if TOK else None)
                    if tok is not None:
                        tokens.append(tok)
            fns[item[0]](item[1])

    for k in range(4):
        w_start(0, k)
    x_start(0)
    kv_start(0)
    x_start(1)
    for g in range(1, C0):
        kv_start(g)
        x_start(g + 1)
    for m in range(4):
        w_wait(m)
        prep_w(0, m, m, 0, 8)
    x_wait(0)
    for br in range(2):
        prep_x(0, br)

    def issued(g):
        return jnp.minimum(jnp.minimum(RATE * (g + 1) + C0, g + LA), G1 + BB)

    def small(b0, carry):
        half = nb // 2
        m = (b0 - half) >> 1

        @pl.when(b0 + 1 < nb)
        def _():
            x_wait(b0 + 1)

        @pl.when(jnp.logical_and(b0 >= half, (b0 & 1) == 0))
        def _():
            w_wait(m)

        kv_wait(b0)

        hi = issued(b0)
        prev = jnp.where(b0 == 0, C0, issued(b0 - 1))

        def pf_x(k, w):
            @pl.when(jnp.logical_and(prev + k < hi, prev + k + 1 < nb))
            def _():
                x_start(prev + k + 1, (w,))

        def pf_kv(k):
            @pl.when(prev + k < hi)
            def _():
                kv_start(prev + k)

        def pf_w():
            w_start_dyn(jnp.where(b0 == W2AT, 2, 1), jnp.where(b0 == W2AT, 0, (b0 >> 1) - 1),
                        jnp.logical_or(b0 == W2AT, jnp.logical_and(b0 <= half, (b0 & 1) == 0)))

        first = [pf_w] + [functools.partial(pf_x, k, w) for k in range(RATE) for w in range(2)]
        first += [functools.partial(pf_kv, k) for k in range(RATE)]
        preps = [functools.partial(prep_x, jnp.minimum(b0 + 1, nb - 1), br) for br in range(2)]
        preps += [functools.partial(prep_w, 1, jnp.where(b0 >= half, m, 3), jnp.maximum(m, 0), (b0 & 1) * 4, 4)]
        body(b0, 1, (first, [], preps), (SPAT, SQORD, SOORD), 0, first_hp=True)
        return carry

    def big(par, last, hp, i, carry):
        b0 = i * BB
        g0 = hp * nb + b0

        if not last:
            w_wait(i)

        for j in range(BB):
            kv_wait(b0 + j)

        def pf_kv(j):
            @pl.when(g0 + BB + j < ng)
            def _():
                kv_start(g0 + BB + j)

        if last:
            extra = ([functools.partial(pf_kv, j) for j in range(BB)], [], [])
        else:
            hn = jnp.where(i == 3, hp + 2, hp + 1)
            extra = ([lambda: w_start_dyn(hn, (i + 1) & 3, hn < nhp)] +
                     [functools.partial(kv_start, g0 + BB + j) for j in range(BB)], [],
                     [functools.partial(prep_w, 1 - par, i, i, 0, 8, part) for part in range(PPARTS)])
        body(g0, BB, extra, (LPAT, LQORD, LOORD) if last else (PAT, QORD, OORD), par, last_hp=last)
        return carry

    spb = nb // BB
    assert spb == 4 and G1 == nb
    if SKIP_SMALL in (0, 2):
        lax.fori_loop(0, nb, small, 0)
    if SKIP_SMALL == 2:
        prep_x(0, 0)
        acc[0, 0:128, 0:128] = wc[1][0:128, 0:128].astype(f32)
        pltpu.make_async_copy(obuf, o_hbm, o_sem).start()
        pltpu.make_async_copy(obuf, o_hbm, o_sem).wait()
        return

    def pair(t, carry):
        lax.fori_loop(jnp.where(t > 0, 0, spb), spb, functools.partial(big, 0, False, 2 * t), 0)
        lax.fori_loop(0, jnp.where(2 * t + 1 < nhp - 1, spb, 0), functools.partial(big, 1, False, 2 * t + 1), 0)
        return carry

    if SKIP_SMALL != 3:
        lax.fori_loop(0, nhp // 2, pair, 0)
    else:
        prep_w(1, 0, 0, 0, 8)
    if SKIP_SMALL in (0, 3):
        lax.fori_loop(0, spb, functools.partial(big, 1, True, nhp - 1), 0)
    pltpu.make_async_copy(obuf, o_hbm, o_sem).wait()


@jax.jit
def pallas_concat_heads__gqa_block_cached__mha_block_cached__near_ridge_kernel(
    A_x, A_k_cache, A_v_cache, A_wq, A_wo, B_x, B_k_cache, B_v_cache, B_wq, B_wo):
    B, Sq, D = A_x.shape
    _, H, Sk, Dh = A_k_cache.shape
    nhp = H // 2
    assert B == 16 and G1 % B == 0 and 2 * BB <= B and C0 >= 1
    n_iss = C0
    for g0 in range(G1):
        assert n_iss >= min(g0 + 2, G1 + BB), (g0, n_iss)
        hi = min(RATE * (g0 + 1) + C0, g0 + LA, G1 + BB)
        assert 0 <= hi - n_iss <= RATE
        n_iss = hi
    assert n_iss == G1 + BB, n_iss
    assert 10 <= W2AT <= 15 and 5 <= LA <= B

    def tr(c):
        return jnp.swapaxes(c, 2, 3).reshape(B, nhp, 2 * Dh, Sk)

    any_spec = pl.BlockSpec(memory_space=pl.ANY)
    return pl.pallas_call(
        functools.partial(_kernel, scale=Dh ** -0.5 * LOG2E, nhp=nhp, nb=B),
        in_specs=[any_spec] * 10,
        out_specs=any_spec,
        out_shape=jax.ShapeDtypeStruct((B, Sq, 2 * D), A_x.dtype),
        scratch_shapes=[pltpu.VMEM((B, ACCR, 2 * D), f32),
                        pltpu.VMEM((B, 2, D // 128, Sq // 2, 128), u32),
                        pltpu.VMEM((4 * 15 * 64, 128), u32),
                        pltpu.VMEM((B, 4, 2 * Dh, Sk), bf16),
                        pltpu.VMEM((B, Sq, 2 * D), bf16),
                        pltpu.VMEM((2 * BB * Sq, Sk), u32),
                        pltpu.VMEM((2 * BB * Sq // 4, 14 * 128), u32),
                        pltpu.VMEM((B * 2 * Sq // 4, XCW * 128), u32),
                        pltpu.VMEM((4 * 64, WCW * 128), u32),
                        pltpu.VMEM((4 * 64, WCW * 128), u32),
                        pltpu.SemaphoreType.DMA((B,)),
                        pltpu.SemaphoreType.DMA((B,)),
                        pltpu.SemaphoreType.DMA((4,)),
                        pltpu.SemaphoreType.DMA(())],
        compiler_params=pltpu.CompilerParams(
            disable_bounds_checks=True,
            vmem_limit_bytes=110 * 1024 * 1024),
    )(A_x, tr(A_k_cache), tr(A_v_cache), A_wq, A_wo, B_x, tr(B_k_cache), tr(B_v_cache), B_wq, B_wo)
```

```python
import functools
import jax
import jax.numpy as jnp
from jax import lax
import jax.experimental.pallas as pl
import jax.experimental.pallas.tpu as pltpu

BB = 4
G1 = 16
C0 = 2
RATE = 2
PFPOS = 1
PFSTEP = 3
PSKIP = 2
OBUF = 1
SKIP_SMALL = 0
KVTOP = 8
QSPLIT = 13
OSPLIT = 13
PPARTS = 25
PEND = 10
XCW = 32
WCW = 40
ACCR = 160
WQT = 3
WOT = 5
MERGE = 0
TOK = 1
W2AT = 11
LA = 6
XPARTS = 25
SWPARTS = 12
QCH = 80
QD = 9999
QS = 60
PCH = 160
SD = 9999
SS = 40
PLO = 300
PHI = 600
SWLO = 100
SWHI = 1000
SXLO = 1800
SXHI = 100
NOCSE = 1
PAT = "s00:0,s01:0,m0:-1,qb:2,qa:3,s10:0,s11:0,m1:-1,t1:-1,t0:-1,oa:-2,c:-1,ob:-2"
SPAT = "qa@0,qb@0,qa@1,qb@1,s00@0,s10@0,s11@0,s00@1,s10@1,s01@0,t1@0,m1@0,s11@1,m0@0,t0@0,c@0,m1@1,s01@1,oa@0,t1@1,c@1,t0@1,m0@1,ob@0,oa@1,ob@1"
LOG2E = 1.4426950408889634
bf16 = jnp.bfloat16
f32 = jnp.float32
u32 = jnp.uint32
NT = (((1,), (1,)), ((), ()))

O_LHS_PROG = [(100, 4, 5, 1), (101, 0, 1, -1), (102, 3, 101, 1), (103, 2, 100, 1), (104, 0, 3, 1), (105, 2, 3, -1), (106, 0, 2, 1), (107, 2, 101, -1), (108, 3, 5, 1), (109, 1, 103, 1), (110, 2, 5, 1), (111, 3, 100, -1), (112, 5, 101, 1), (113, 4, 102, -1), (114, 0, 100, 1)]
O_OUT_PROG = [(100, 5, 8, -1), (101, 3, 100, 1), (102, 2, 7, -1), (103, 0, 102, 1)]
O_PRODS = [((101, 1), [(2, 1), (5, 1), (10, -1), (12, 1)], [(102, 1)]), ((104, 1), [(3, 1)], [(100, -1)]), ((111, 1), [(0, 1), (3, 1)], [(5, 1)]), ((5, 1), [(5, 1), (10, -1)], [(5, -1), (103, 1)]), ((112, 1), [(5, 1), (10, -1), (12, 1)], [(103, -1)]), ((114, 1), [(0, 1), (3, 1), (5, 1)], [(101, 1)]), ((0, 1), [(0, 1), (5, 1)], [(0, 1), (101, -1)]), ((107, -1), [(10, 1), (12, -1)], [(0, -1)]), ((110, 1), [(12, 1)], [(0, 1), (2, 1)]), ((1, 1), [(2, 1), (7, 1)], [(2, 1), (4, -1)]), ((104, 1), [(1, 1), (2, 1), (4, 1), (7, 1), (9, 1)], [(4, 1)]), ((106, 1), [(1, 1)], [(1, 1), (4, -1)]), ((1, 1), [(6, 1)], [(1, 1), (3, -1)]), ((109, 1), [(6, 1), (8, 1)], [(3, 1)]), ((2, 1), [(1, 1), (11, -1)], [(1, -1), (6, 1)]), ((103, 1), [(6, 1), (8, 1), (13, -1)], [(3, -1), (6, 1)]), ((100, 1), [(0, 1), (3, 1), (5, 1), (13, 1)], [(3, -1), (8, 1)]), ((4, 1), [(8, 1), (13, -1)], [(6, -1), (8, 1)]), ((110, 1), [(6, 1), (8, 1), (11, -1), (13, -1), (14, -1)], [(6, -1)]), ((105, 1), [(1, 1), (14, 1)], [(4, 1), (6, -1)]), ((108, 1), [(14, 1)], [(6, -1), (9, 1)]), ((3, 1), [(4, 1), (14, -1)], [(4, -1), (9, 1)]), ((4, 1), [(9, 1)], [(7, -1), (9, 1)]), ((102, 1), [(2, 1), (7, 1), (9, 1)], [(4, -1), (7, 1)]), ((113, -1), [(7, 1), (9, 1)], [(7, -1)])]
Q_LHS_PROG = [(100, 3, 8, -1), (101, 0, 2, 1), (102, 7, 101, -1), (103, 5, 100, 1), (104, 4, 6, -1), (105, 4, 9, -1), (106, 7, 9, -1), (107, 0, 103, -1), (108, 6, 8, -1), (109, 5, 102, 1), (110, 1, 4, -1), (111, 5, 8, -1), (112, 6, 9, -1), (113, 4, 7, -1), (114, 2, 4, -1), (115, 1, 6, -1), (116, 2, 7, -1), (117, 1, 3, -1), (118, 3, 6, -1)]
Q_OUT_PROG = [(100, 0, 3, 1), (101, 4, 5, 1), (102, 0, 1, -1), (103, 2, 101, 1), (104, 2, 5, 1), (105, 1, 100, -1)]
Q_PRODS = [((6, -1), [(6, 1), (8, 1), (11, -1), (13, -1), (14, -1)], [(104, 1)]), ((101, 1), [(12, 1)], [(104, 1)]), ((4, 1), [(1, 1), (2, 1), (4, 1), (7, 1), (9, 1)], [(100, 1)]), ((111, -1), [(3, 1)], [(100, 1)]), ((118, -1), [(6, 1), (8, 1), (13, -1)], [(103, 1)]), ((3, 1), [(6, 1), (8, 1)], [(1, 1), (103, 1)]), ((114, 1), [(2, 1), (7, 1)], [(1, 1)]), ((117, 1), [(6, 1)], [(1, 1)]), ((115, -1), [(1, 1), (11, -1)], [(2, 1)]), ((0, -1), [(10, 1), (12, -1)], [(2, -1), (102, 1)]), ((116, 1), [(2, 1), (5, 1), (10, -1), (12, 1)], [(102, 1)]), ((102, 1), [(5, 1), (10, -1), (12, 1)], [(5, 1), (102, 1)]), ((109, -1), [(5, 1), (10, -1)], [(5, 1)]), ((112, -1), [(14, 1)], [(3, 1), (5, 1)]), ((104, 1), [(1, 1), (14, 1)], [(2, 1), (3, -1)]), ((105, -1), [(4, 1), (14, -1)], [(3, 1)]), ((5, 1), [(0, 1), (3, 1)], [(3, 1), (101, -1)]), ((100, -1), [(0, 1), (3, 1), (5, 1), (13, 1)], [(101, 1)]), ((103, 1), [(0, 1), (3, 1), (5, 1)], [(0, 1), (101, 1)]), ((110, 1), [(1, 1)], [(0, 1), (2, 1)]), ((107, 1), [(0, 1), (5, 1)], [(0, 1)]), ((113, -1), [(2, 1), (7, 1), (9, 1)], [(105, -1)]), ((7, -1), [(7, 1), (9, 1)], [(4, -1), (105, -1)]), ((106, -1), [(9, 1)], [(4, 1)]), ((108, -1), [(8, 1), (13, -1)], [(4, 1)])]
NPROD = len(O_PRODS)


def _normalize(prods):
    out = []
    for (var, sgn), w, g in prods:
        sgn *= w[0][1]
        out.append((var, [(y, c * w[0][1]) for y, c in w], [(z, c * sgn) for z, c in g]))
    return out


OORD = "1.0.3.2.5.6.8.9.4.24.11.12.10.14.13.15.16.17.18.19.20.21.22.23.7"
QORD = "14.15.16.17.18.19.20.21.22.24.23.0.1.6.2.7.3.4.5.8.9.10.11.12.13"
SOORD = "7.23.22.21.20.19.18.16.17.15.13.12.10.11.14.9.8.24.6.5.2.3.4.0.1"
SQORD = "14.15.16.17.18.10.20.21.22.24.1.23.6.2.7.0.3.8.4.5.9.19.11.12.13"
LOORD = OORD
LQORD = QORD
LPAT = PAT
O_PRODS = _normalize(O_PRODS)
Q_PRODS = _normalize(Q_PRODS)
W_FORMS = [p[1] for p in O_PRODS]


def _positive_outputs(prods, prog):
    for flips in range(1 << 6):
        sg = [(-1 if (flips >> (r % 6)) & 1 else 1) for r in range(len(prods))]
        pos = {}
        for r, p in enumerate(prods):
            for z, c in p[2]:
                pos[z] = max(pos.get(z, -1), c * sg[r])
        for t, a, b, s in reversed(prog):
            st = pos.pop(t)
            pos[a] = max(pos.get(a, -1), st)
            pos[b] = max(pos.get(b, -1), st * s)
        if min(pos.values()) > 0:
            return sg
    raise AssertionError


Q_SIGN = _positive_outputs(Q_PRODS, Q_OUT_PROG)
Q_PRODS = [(v, w, [(z, c * s) for z, c in g]) for (v, w, g), s in zip(Q_PRODS, Q_SIGN)]


def _make_lhs(block, prog):
    vals = {}

    def get(v):
        if v not in vals:
            vals[v] = block(v)
        return vals[v]

    for t, a, b, s in prog:
        vals[t] = get(a) + get(b) if s > 0 else get(a) - get(b)
    return get


def _acc_add(accs, z, sgn, m):
    if z not in accs:
        accs[z] = (sgn, m)
    else:
        s0, a = accs[z]
        accs[z] = (s0, a + m) if s0 == sgn else ((1, a - m) if s0 > 0 else (1, m - a))


def _bilinear_run(accs, prods, which, lhs_of, w_of, tick):
    for r in which:
        m = tick(jnp.dot(lhs_of(r), w_of(r), preferred_element_type=f32), 20)
        for z, c in prods[r][2]:
            _acc_add(accs, z, c, m)


def _bilinear_finish(accs, prog):
    for t, a, b, s in reversed(prog):
        st, v = accs.pop(t)
        _acc_add(accs, a, st, v)
        _acc_add(accs, b, st * s, v)
    return accs


def _mul(i, n):
    return i * n if isinstance(i, int) else pl.multiple_of(i * n, 16)


def _as_bf16(packed):
    return pltpu.bitcast(packed, bf16)


def _as_f32(packed):
    return pltpu.bitcast(packed, bf16).astype(f32)


def _q_operands(c):
    assert all(s > 0 for row in c for s, _ in row)
    (t0, t1, t2), (b0, b1, b2) = [[a for _, a in row] for row in c]
    lo = lax.broadcasted_iota(jnp.int32, t0.shape, 1) < 64
    return [[jnp.where(lo, t0, b0), jnp.where(lo, t1, t0 - b0), jnp.where(lo, b0 - t0, pltpu.roll(b1, 64, 1))],
            [jnp.where(lo, t2, b2), jnp.where(lo, pltpu.roll(t1, 64, 1), t2 - b2), jnp.where(lo, b2 - t2, b1)]]


def _scores_half(qh, kt, h, j, tick):
    k0, k1, k2 = (0, 64, 128) if h == 0 else (256, 320, 192)
    out = []
    for c in (2 * j, 2 * j + 1):
        cs = slice(c * 128, (c + 1) * 128)
        w = [kt[k0:k0 + 128, cs],
             jnp.concatenate([kt[k2:k2 + 64, cs], kt[k1:k1 + 64, cs]], axis=0),
             jnp.concatenate([kt[k0:k0 + 64, cs], kt[k2:k2 + 64, cs]], axis=0)]
        m = [tick(jnp.dot(qh[i], w[i], preferred_element_type=f32), 20) for i in range(3)]
        out.append(jnp.concatenate([m[0] + m[1], m[0] + m[2]], axis=0))
    return out


def _softmax(s):
    m = jnp.max(s, axis=1, keepdims=True)
    p = jnp.exp2(s - m)
    t = (p[:, 0:128] + p[:, 128:256]) + (p[:, 256:384] + p[:, 384:512])
    p = jnp.concatenate([p[:, 0:384], jnp.minimum(p[:, 384:512], t)], axis=1)
    l = jnp.sum(t, axis=1, keepdims=True)
    r = pl.reciprocal(l, approx=True)
    r = r * (2.0 - l * r)
    return p.astype(bf16), r


def _schedule(nu, pat):
    if "@" in pat:
        return [(a.split("@")[0], int(a.split("@")[1])) for a in pat.split(",")]
    pat = [(a.split(":")[0], int(a.split(":")[1])) for a in pat.split(",")]
    order = []
    for t in range(-6, nu + 6):
        for name, lag in pat:
            u = t + lag
            if 0 <= u < nu:
                order.append((name, u))
    return order


def _kernel(ax, ak, av, awq, awo, bx, bk, bv, bwq, bwo, o_hbm,
            acc, x32, w32, kvbuf, obuf, pbuf, qbuf, xc32, wc0, wc1,
            kv_sem, x_sem, w_sem, o_sem, *, scale, nhp, nb):
    xbuf, wbuf = (r.bitcast(bf16) for r in (x32, w32))
    pbuf, qbuf, xc = (r.bitcast(bf16) for r in (pbuf, qbuf, xc32))
    wc = [r.bitcast(bf16) for r in (wc0, wc1)]
    sq = xbuf.shape[3]
    hq = sq // 2
    d = awq.shape[0]
    hw = kvbuf.shape[2]
    wrows = wbuf.shape[0] // 4
    ng = nhp * nb
    lg = nb.bit_length() - 1
    assert nb == 1 << lg

    def kv_start(g, which=(0, 1, 2, 3)):
        hp, b = (g >> lg) & (nhp - 1), g & (nb - 1)
        for i, src in enumerate((ak, av, bk, bv)):
            if i in which:
                sem = kv_sem.at[jnp.where(g < nb, b, nb + (b >> 2))]
                pltpu.make_async_copy(src.at[b, hp], kvbuf.at[b, i], sem).start()

    def kv_wait(b):
        pltpu.make_async_copy(kvbuf.at[b], kvbuf.at[b], kv_sem.at[b]).wait()

    def kvg_start(g):
        hp, i4 = g >> lg, (g >> 2) & 3
        b = pl.multiple_of(i4 * BB, BB)
        for i, src in enumerate((ak, av, bk, bv)):
            pltpu.make_async_copy(src.at[pl.ds(b, BB), hp], kvbuf.at[pl.ds(b, BB), i], kv_sem.at[nb + i4]).start()

    def kvg_wait(i4):
        v = kvbuf.at[pl.ds(i4 * BB, BB)]
        pltpu.make_async_copy(v, v, kv_sem.at[nb + i4]).wait()

    def x_start(b, which=(0, 1)):
        for i, src in enumerate((ax, bx)):
            if i in which:
                for c in range(xbuf.shape[2]):
                    pltpu.make_async_copy(src.at[b, :, pl.ds(c * 128, 128)], xbuf.at[b, i, c], x_sem.at[b]).start()

    def x_wait(b):
        pltpu.make_async_copy(xbuf.at[b], xbuf.at[b], x_sem.at[b]).wait()

    def w_start(h, m):
        off = h * hw if isinstance(h, int) else pl.multiple_of(h * hw, 128)
        if m < 2:
            for c in range(hw // 128):
                pltpu.make_async_copy((awq, bwq)[m].at[:, pl.ds(off + c * 128, 128)],
                                      wbuf.at[pl.ds(m * wrows + c * d, d)], w_sem.at[m]).start()
        else:
            for c in range(d // 128):
                pltpu.make_async_copy((awo, bwo)[m - 2].at[pl.ds(off, hw), pl.ds(c * 128, 128)],
                                      wbuf.at[pl.ds(m * wrows + c * hw, hw)], w_sem.at[m]).start()

    def w_start_dyn(h, m, valid):
        for k in range(4):
            @pl.when(jnp.logical_and(m == k, valid))
            def _():
                w_start(h, k)

    def w_wait(m):
        v = wbuf.at[pl.ds(_mul(m, wrows), wrows)]
        pltpu.make_async_copy(v, v, w_sem.at[m]).wait()

    def prep_w(dst, msrc, mdst, row, nrows, part=None, zero=None):
        if isinstance(msrc, int):
            sa, sc = (5, 1) if msrc < 2 else (1, 3)
            off = [(msrc * 15 + (y // 5) * sa + (y % 5) * sc) * 64 + row * 8 for y in range(15)]
        else:
            sa, sc = jnp.where(msrc < 2, 5, 1), jnp.where(msrc < 2, 1, 3)
            off = [pl.multiple_of((msrc * 15 + (y // 5) * sa + (y % 5) * sc) * 64 + row * 8, 64 if isinstance(row, int) and row == 0 else 32)
                   for y in range(15)]
        r16 = _mul(mdst * 8 + row, 16)
        if not isinstance(r16, int):
            r16 = pl.multiple_of(r16, 128 if isinstance(row, int) and row == 0 else 64)
        for r, form in enumerate(W_FORMS):
            if part is not None and r % part[1] != part[0]:
                continue
            if len(form) == 1:
                val = _as_bf16(w32[pl.ds(off[form[0][0]], nrows * 8), :])
            else:
                val = None
                for y, c in form:
                    t = _as_f32(w32[pl.ds(off[y], nrows * 8), :])
                    val = t if val is None else (val + t if c > 0 else val - t)
                val = val.astype(bf16)
            wc[dst][pl.ds(r16, nrows * 16), r * 128:(r + 1) * 128] = val
        if zero is not None:
            c0 = part[0] * 128
            return lambda: wc[dst][pl.ds(pl.multiple_of(r16 + zero * 16, 16), 16), c0:c0 + 128].astype(f32)[0:8]

    def prep_x(b, br, part=None, zero=None):
        get = _make_lhs(
            lambda z: _as_f32(x32[b, br, z % 5, (z // 5) * (hq // 2):(z // 5 + 1) * (hq // 2), :]) * scale,
            Q_LHS_PROG)
        for r, p in enumerate(Q_PRODS):
            if part is not None and r * XPARTS // NPROD != part:
                continue
            c0 = r * 128
            xc[pl.ds(_mul(b * 2 + br, hq), hq), r * 128:(r + 1) * 128] = (get(p[0]) * Q_SIGN[r]).astype(bf16)
        if zero is not None:
            return lambda: xc[pl.ds(_mul(b * 2 + br + zero, hq), 16), c0:c0 + 128].astype(f32)[0:8]

    def body(g0, nbat, extra, pat, cs, first_hp=False, last_hp=False):
        hp = g0 >> lg
        b0 = g0 & (nb - 1)
        R, O, OT, OC = {}, {}, {}, {}

        def prow(u, h):
            return (2 * u + h) * sq

        def weights(m, prods):
            def w_of(r):
                s = W_FORMS.index(prods[r][1])
                return wc[cs][m * 128:(m + 1) * 128, s * 128:(s + 1) * 128]
            return w_of

        QA, OA, SC, LH = {}, {}, {}, {}
        pending = []
        clock = [0]
        zero16 = pl.multiple_of((g0 >> 20) * 16, 16)

        def later(key, delay, emit):
            pending.append((clock[0] + delay, key, emit))
            pending.sort(key=lambda e: e[0])

        def flush(key):
            for e in [e for e in pending if e[1] == key]:
                pending.remove(e)
                e[2]()

        def tick(o, cycles):
            t0 = clock[0]
            clock[0] += cycles
            groups = o.shape[0] // 8
            rows = None
            while pending and pending[0][0] <= clock[0]:
                due, _, emit = pending.pop(0)
                tok = emit()
                if tok is None or not TOK:
                    continue
                g = min(max((due - t0) * groups // cycles, 0), groups - 1)
                rows = rows or [o[8 * i:8 * i + 8] for i in range(groups)]
                rows[g] = jnp.minimum(rows[g], jnp.maximum(rows[g], tok()))
            return o if rows is None else jnp.concatenate(rows, axis=0)

        pat, qord, oord = pat
        qord = [int(i) for i in qord.split(".")]
        oord = [int(i) for i in oord.split(".")]

        def q_(u, lo_, hi_):
            b, br = b0 + u // 2, u % 2

            def lhs_of(r):
                return xc[pl.ds(_mul(b * 2 + br, hq), hq), r * 128:(r + 1) * 128]

            _bilinear_run(QA.setdefault(u, {}), Q_PRODS, qord[lo_:hi_], lhs_of, weights(br, Q_PRODS), tick)
            if hi_ == len(Q_PRODS):
                fin = _bilinear_finish(QA[u], Q_OUT_PROG)
                c = [[fin[i * 3 + n] for n in range(3)] for i in range(2)]
                nch = hq // QCH

                def chunk(k):
                    ck = [[(s, a[k * QCH:(k + 1) * QCH]) for s, a in row] for row in c]
                    r0 = u * hq + k * QCH
                    for h, ops in enumerate(_q_operands(ck)):
                        for i, a in enumerate(ops):
                            qbuf[r0:r0 + QCH, (3 * h + i) * 128:(3 * h + i + 1) * 128] = a.astype(bf16)
                    return lambda: qbuf[pl.ds(r0 + zero16, 16), 0:128].astype(f32)[0:8]

                for k in range(nch):
                    later(("q", u), QD + k * QS, functools.partial(chunk, k))

        def s_(u, h, j):
            b, br = b0 + u // 2, u % 2
            flush(("q", u))
            qh = [qbuf[u * hq:(u + 1) * hq, (3 * h + i) * 128:(3 * h + i + 1) * 128] for i in range(3)]
            SC[u, h, j] = _scores_half(qh, kvbuf.at[b, 2 * br], h, j, tick)
            if j == 1:
                s = jnp.concatenate(SC[u, h, 0] + SC[u, h, 1], axis=1)
                R[u, h] = []

                def chunk(k):
                    p, r = _softmax(s[k * PCH:(k + 1) * PCH])
                    R[u, h].append(r)
                    r0 = prow(u, h) + k * PCH
                    pbuf[r0:r0 + PCH, :] = p
                    return lambda: pbuf[pl.ds(r0 + zero16, 16), 0:128].astype(f32)[0:8]

                for k in range(sq // PCH):
                    later(("p", u, h), SD + k * SS, functools.partial(chunk, k))

        def rinv(u, h):
            return jnp.concatenate(R[u, h], axis=0)

        def m_(u, h):
            flush(("p", u, h))
            vt = kvbuf.at[b0 + u // 2, 2 * (u % 2) + 1]
            o = lax.dot_general(pbuf[prow(u, h):prow(u, h) + sq, :], vt[h * 256:h * 256 + 128, :], NT,
                                preferred_element_type=f32)
            O[u, h] = tick(o, 160) * rinv(u, h)

        def t_(u, h):
            flush(("p", u, h))
            vt = kvbuf.at[b0 + u // 2, 2 * (u % 2) + 1]
            OT[u, h] = lax.dot_general(vt[128 + h * 64:192 + h * 64, :], pbuf[prow(u, h):prow(u, h) + 128, :], NT,
                                       preferred_element_type=f32)
            OT[u, h] = tick(OT[u, h], 64)

        def c_(u):
            flush(("p", u, 0))
            flush(("p", u, 1))
            vt = kvbuf.at[b0 + u // 2, 2 * (u % 2) + 1]
            pc = jnp.concatenate([pbuf[prow(u, h) + 128:prow(u, h) + sq, :] for h in range(2)], axis=0)
            OC[u] = lax.dot_general(pc, vt[128:256, :], NT, preferred_element_type=f32)
            OC[u] = tick(OC[u], 64)

        def o_(u, lo_, hi_):
            b, br = b0 + u // 2, u % 2
            if lo_ == 0:
                n = sq - 128
                top = jnp.concatenate([OT[u, 0], OT[u, 1]], axis=0).T
                bot = jnp.where(lax.broadcasted_iota(jnp.int32, (n, 128), 1) < 64, OC[u][0:n], OC[u][n:2 * n])
                lo = lax.broadcasted_iota(jnp.int32, (sq, 128), 1) < 64
                mid = jnp.concatenate([top, bot], axis=0) * jnp.where(lo, rinv(u, 0), rinv(u, 1))
                tiles = (O[u, 0], mid, O[u, 1])
                get = _make_lhs(lambda x: tiles[x % 3][(x // 3) * hq:(x // 3 + 1) * hq], O_LHS_PROG)
                LH[u] = {p[0]: get(p[0]).astype(bf16) for p in O_PRODS}
            _bilinear_run(OA.setdefault(u, {}), O_PRODS, oord[lo_:hi_], lambda r: LH[u][O_PRODS[r][0]],
                          weights(2 + br, O_PRODS), tick)
            fin = _bilinear_finish(OA[u], O_OUT_PROG) if hi_ == NPROD else {}
            for n in (range(5) if fin else ()):
                for i in range(2):
                    s, a = fin[i * 5 + n]
                    rows = slice(i * hq, (i + 1) * hq)
                    cols = slice(br * d + n * 128, br * d + (n + 1) * 128)
                    if first_hp:
                        new = a if s > 0 else -a
                    else:
                        new = acc[b, rows, cols] + a if s > 0 else acc[b, rows, cols] - a
                    if last_hp:
                        obuf[b, rows, cols] = new.astype(obuf.dtype)
                    if not last_hp:
                        acc[b, rows, cols] = new
            if br == 1 and lo_ > 0 and last_hp:
                pltpu.make_async_copy(obuf.at[b], o_hbm.at[b], o_sem).start()

        fns = {"qa": lambda u: q_(u, 0, QSPLIT), "qb": lambda u: q_(u, QSPLIT, NPROD),
               "oa": lambda u: o_(u, 0, OSPLIT), "ob": lambda u: o_(u, OSPLIT, NPROD),
               "s00": lambda u: s_(u, 0, 0), "s01": lambda u: s_(u, 0, 1),
               "s10": lambda u: s_(u, 1, 0), "s11": lambda u: s_(u, 1, 1),
               "m0": lambda u: m_(u, 0), "m1": lambda u: m_(u, 1),
               "t0": lambda u: t_(u, 0), "t1": lambda u: t_(u, 1), "c": c_}
        sched = _schedule(2 * nbat, pat)
        first, dmas, preps = extra
        for f in first:
            f()
        total = 2 * nbat * 1992
        lastq = max(i for i, it in enumerate(sched) if it[0][0] == "q")
        wpre, xpre = preps
        for k, f in enumerate(wpre):
            lo_, hi_ = (PLO, total - PHI) if nbat > 1 else (SWLO, SWHI)
            later("w", lo_ + k * (hi_ - lo_) // len(wpre), f)
        for i, item in enumerate(sched):
            fns[item[0]](item[1])
            if i == lastq:
                for k, f in enumerate(xpre):
                    later("x", SXLO + k * (total - SXHI - clock[0] - SXLO) // len(xpre), f)
        flush("w")
        flush("x")
        assert not pending

    for k in range(4):
        w_start(0, k)
    x_start(0)
    kv_start(0)
    x_start(1)
    for g in range(1, C0):
        kv_start(g)
        x_start(g + 1)
    for m in range(4):
        w_wait(m)
        prep_w(0, m, m, 0, 8)
    x_wait(0)
    for br in range(2):
        prep_x(0, br)

    def issued(g):
        return jnp.minimum(jnp.minimum(RATE * (g + 1) + C0, g + LA), G1 + BB)

    def small(b0, carry):
        half = nb // 2
        m = (b0 - half) >> 1

        @pl.when(b0 + 1 < nb)
        def _():
            x_wait(b0 + 1)

        @pl.when(jnp.logical_and(b0 >= half, (b0 & 1) == 0))
        def _():
            w_wait(m)

        kv_wait(b0)

        hi = issued(b0)
        prev = jnp.where(b0 == 0, C0, issued(b0 - 1))

        def pf_x(k, w):
            @pl.when(jnp.logical_and(prev + k < hi, prev + k + 1 < nb))
            def _():
                x_start(prev + k + 1, (w,))

        def pf_kv(k):
            @pl.when(prev + k < hi)
            def _():
                kv_start(prev + k)

        def pf_w():
            w_start_dyn(jnp.where(b0 == W2AT, 2, 1), jnp.where(b0 == W2AT, 0, (b0 >> 1) - 1),
                        jnp.logical_or(b0 == W2AT, jnp.logical_and(b0 <= half, (b0 & 1) == 0)))

        first = [pf_w] + [functools.partial(pf_x, k, w) for k in range(RATE) for w in range(2)]
        first += [functools.partial(pf_kv, k) for k in range(RATE)]
        zero = b0 >> 20
        preps = ([functools.partial(prep_w, 1, jnp.where(b0 >= half, m, 3), jnp.maximum(m, 0), (b0 & 1) * 4, 4,
                                    (part, SWPARTS), zero) for part in range(SWPARTS)],
                 [functools.partial(prep_x, jnp.minimum(b0 + 1, nb - 1), br, part, zero)
                  for br in range(2) for part in range(XPARTS)])
        body(b0, 1, (first, [], preps), (SPAT, SQORD, SOORD), 0, first_hp=True)
        return carry

    def big(par, last, hp, i, carry):
        b0 = i * BB
        g0 = hp * nb + b0

        if not last:
            w_wait(i)

        kvg_wait(i)

        def pf_kv():
            @pl.when(g0 + BB < ng)
            def _():
                kvg_start(g0 + BB)

        if last:
            extra = ([pf_kv], [], ([], []))
        else:
            hn = jnp.where(i == 3, hp + 2, hp + 1)
            extra = ([lambda: w_start_dyn(hn, (i + 1) & 3, hn < nhp)] +
                     [functools.partial(kvg_start, g0 + BB)], [],
                     ([functools.partial(prep_w, 1 - par, i, i, 0, 8, (part, PPARTS), i >> 20)
                       for part in range(PPARTS)], []))
        body(g0, BB, extra, (LPAT, LQORD, LOORD) if last else (PAT, QORD, OORD), par, last_hp=last)
        return carry

    spb = nb // BB
    assert spb == 4 and G1 == nb
    if SKIP_SMALL in (0, 2):
        lax.fori_loop(0, nb, small, 0)
    if SKIP_SMALL == 2:
        prep_x(0, 0)
        acc[0, 0:128, 0:128] = wc[1][0:128, 0:128].astype(f32)
        pltpu.make_async_copy(obuf, o_hbm, o_sem).start()
        pltpu.make_async_copy(obuf, o_hbm, o_sem).wait()
        return

    def pair(t, carry):
        lax.fori_loop(jnp.where(t > 0, 0, spb), spb, functools.partial(big, 0, False, 2 * t), 0)
        lax.fori_loop(0, jnp.where(2 * t + 1 < nhp - 1, spb, 0), functools.partial(big, 1, False, 2 * t + 1), 0)
        return carry

    if SKIP_SMALL != 3:
        lax.fori_loop(0, nhp // 2, pair, 0)
    else:
        prep_w(1, 0, 0, 0, 8)
    if SKIP_SMALL in (0, 3):
        lax.fori_loop(0, spb, functools.partial(big, 1, True, nhp - 1), 0)
    pltpu.make_async_copy(obuf, o_hbm, o_sem).wait()


@jax.jit
def pallas_concat_heads__gqa_block_cached__mha_block_cached__near_ridge_kernel(
    A_x, A_k_cache, A_v_cache, A_wq, A_wo, B_x, B_k_cache, B_v_cache, B_wq, B_wo):
    B, Sq, D = A_x.shape
    _, H, Sk, Dh = A_k_cache.shape
    nhp = H // 2
    assert B == 16 and G1 % B == 0 and 2 * BB <= B and C0 >= 1
    n_iss = C0
    for g0 in range(G1):
        assert n_iss >= min(g0 + 2, G1 + BB), (g0, n_iss)
        hi = min(RATE * (g0 + 1) + C0, g0 + LA, G1 + BB)
        assert 0 <= hi - n_iss <= RATE
        n_iss = hi
    assert n_iss == G1 + BB, n_iss
    assert 10 <= W2AT <= 15 and 5 <= LA <= B

    def tr(c):
        return jnp.swapaxes(c, 2, 3).reshape(B, nhp, 2 * Dh, Sk)

    any_spec = pl.BlockSpec(memory_space=pl.ANY)
    return pl.pallas_call(
        functools.partial(_kernel, scale=Dh ** -0.5 * LOG2E, nhp=nhp, nb=B),
        in_specs=[any_spec] * 10,
        out_specs=any_spec,
        out_shape=jax.ShapeDtypeStruct((B, Sq, 2 * D), A_x.dtype),
        scratch_shapes=[pltpu.VMEM((B, ACCR, 2 * D), f32),
                        pltpu.VMEM((B, 2, D // 128, Sq // 2, 128), u32),
                        pltpu.VMEM((4 * 15 * 64, 128), u32),
                        pltpu.VMEM((B, 4, 2 * Dh, Sk), bf16),
                        pltpu.VMEM((B, Sq, 2 * D), bf16),
                        pltpu.VMEM((2 * BB * Sq, Sk), u32),
                        pltpu.VMEM((2 * BB * Sq // 4, 6 * 128), u32),
                        pltpu.VMEM((B * 2 * Sq // 4, XCW * 128), u32),
                        pltpu.VMEM((4 * 64, WCW * 128), u32),
                        pltpu.VMEM((4 * 64, WCW * 128), u32),
                        pltpu.SemaphoreType.DMA((B + 4,)),
                        pltpu.SemaphoreType.DMA((B,)),
                        pltpu.SemaphoreType.DMA((4,)),
                        pltpu.SemaphoreType.DMA(())],
        compiler_params=pltpu.CompilerParams(
            disable_bounds_checks=True,
            vmem_limit_bytes=110 * 1024 * 1024),
    )(A_x, tr(A_k_cache), tr(A_v_cache), A_wq, A_wo, B_x, tr(B_k_cache), tr(B_v_cache), B_wq, B_wo)
```

```python
import functools
import jax
import jax.numpy as jnp
from jax import lax
import jax.experimental.pallas as pl
import jax.experimental.pallas.tpu as pltpu

BB = 4
G1 = 16
C0 = 2
RATE = 2
PFPOS = 1
PFSTEP = 3
PSKIP = 2
OBUF = 1
SKIP_SMALL = 0
KVTOP = 8
QSPLIT = 13
OSPLIT = 13
PPARTS = 25
PEND = 10
XCW = 32
WCW = 40
ACCR = 160
WQT = 3
WOT = 5
MERGE = 0
TOK = 1
W2AT = 11
LA = 6
XPARTS = 25
SWPARTS = 12
QCH = 80
QD = 9999
QS = 60
PCH = 160
SD = 9999
SS = 40
PLO = 300
PHI = 600
SWLO = 100
SWHI = 1000
SXLO = 1800
SXHI = 100
VNOCSE = 1
NOCSE = 1
PAT = "s00:0,s01:0,m0:-1,t0:-1,qb:2,qa:3,s10:0,s11:0,m1:-1,t1:-1,oa:-2,ob:-2"
SPAT = "qa@0,qb@0,qa@1,qb@1,s00@0,s10@0,s11@0,s00@1,s10@1,s01@0,t1@0,m1@0,s11@1,m0@0,t0@0,c@0,m1@1,s01@1,oa@0,t1@1,c@1,t0@1,m0@1,ob@0,oa@1,ob@1"
LOG2E = 1.4426950408889634
bf16 = jnp.bfloat16
f32 = jnp.float32
u32 = jnp.uint32
NT = (((1,), (1,)), ((), ()))

O_LHS_PROG = [(100, 4, 5, 1), (101, 0, 1, -1), (102, 3, 101, 1), (103, 2, 100, 1), (104, 0, 3, 1), (105, 2, 3, -1), (106, 0, 2, 1), (107, 2, 101, -1), (108, 3, 5, 1), (109, 1, 103, 1), (110, 2, 5, 1), (111, 3, 100, -1), (112, 5, 101, 1), (113, 4, 102, -1), (114, 0, 100, 1)]
O_OUT_PROG = [(100, 5, 8, -1), (101, 3, 100, 1), (102, 2, 7, -1), (103, 0, 102, 1)]
O_PRODS = [((101, 1), [(2, 1), (5, 1), (10, -1), (12, 1)], [(102, 1)]), ((104, 1), [(3, 1)], [(100, -1)]), ((111, 1), [(0, 1), (3, 1)], [(5, 1)]), ((5, 1), [(5, 1), (10, -1)], [(5, -1), (103, 1)]), ((112, 1), [(5, 1), (10, -1), (12, 1)], [(103, -1)]), ((114, 1), [(0, 1), (3, 1), (5, 1)], [(101, 1)]), ((0, 1), [(0, 1), (5, 1)], [(0, 1), (101, -1)]), ((107, -1), [(10, 1), (12, -1)], [(0, -1)]), ((110, 1), [(12, 1)], [(0, 1), (2, 1)]), ((1, 1), [(2, 1), (7, 1)], [(2, 1), (4, -1)]), ((104, 1), [(1, 1), (2, 1), (4, 1), (7, 1), (9, 1)], [(4, 1)]), ((106, 1), [(1, 1)], [(1, 1), (4, -1)]), ((1, 1), [(6, 1)], [(1, 1), (3, -1)]), ((109, 1), [(6, 1), (8, 1)], [(3, 1)]), ((2, 1), [(1, 1), (11, -1)], [(1, -1), (6, 1)]), ((103, 1), [(6, 1), (8, 1), (13, -1)], [(3, -1), (6, 1)]), ((100, 1), [(0, 1), (3, 1), (5, 1), (13, 1)], [(3, -1), (8, 1)]), ((4, 1), [(8, 1), (13, -1)], [(6, -1), (8, 1)]), ((110, 1), [(6, 1), (8, 1), (11, -1), (13, -1), (14, -1)], [(6, -1)]), ((105, 1), [(1, 1), (14, 1)], [(4, 1), (6, -1)]), ((108, 1), [(14, 1)], [(6, -1), (9, 1)]), ((3, 1), [(4, 1), (14, -1)], [(4, -1), (9, 1)]), ((4, 1), [(9, 1)], [(7, -1), (9, 1)]), ((102, 1), [(2, 1), (7, 1), (9, 1)], [(4, -1), (7, 1)]), ((113, -1), [(7, 1), (9, 1)], [(7, -1)])]
Q_LHS_PROG = [(100, 3, 8, -1), (101, 0, 2, 1), (102, 7, 101, -1), (103, 5, 100, 1), (104, 4, 6, -1), (105, 4, 9, -1), (106, 7, 9, -1), (107, 0, 103, -1), (108, 6, 8, -1), (109, 5, 102, 1), (110, 1, 4, -1), (111, 5, 8, -1), (112, 6, 9, -1), (113, 4, 7, -1), (114, 2, 4, -1), (115, 1, 6, -1), (116, 2, 7, -1), (117, 1, 3, -1), (118, 3, 6, -1)]
Q_OUT_PROG = [(100, 0, 3, 1), (101, 4, 5, 1), (102, 0, 1, -1), (103, 2, 101, 1), (104, 2, 5, 1), (105, 1, 100, -1)]
Q_PRODS = [((6, -1), [(6, 1), (8, 1), (11, -1), (13, -1), (14, -1)], [(104, 1)]), ((101, 1), [(12, 1)], [(104, 1)]), ((4, 1), [(1, 1), (2, 1), (4, 1), (7, 1), (9, 1)], [(100, 1)]), ((111, -1), [(3, 1)], [(100, 1)]), ((118, -1), [(6, 1), (8, 1), (13, -1)], [(103, 1)]), ((3, 1), [(6, 1), (8, 1)], [(1, 1), (103, 1)]), ((114, 1), [(2, 1), (7, 1)], [(1, 1)]), ((117, 1), [(6, 1)], [(1, 1)]), ((115, -1), [(1, 1), (11, -1)], [(2, 1)]), ((0, -1), [(10, 1), (12, -1)], [(2, -1), (102, 1)]), ((116, 1), [(2, 1), (5, 1), (10, -1), (12, 1)], [(102, 1)]), ((102, 1), [(5, 1), (10, -1), (12, 1)], [(5, 1), (102, 1)]), ((109, -1), [(5, 1), (10, -1)], [(5, 1)]), ((112, -1), [(14, 1)], [(3, 1), (5, 1)]), ((104, 1), [(1, 1), (14, 1)], [(2, 1), (3, -1)]), ((105, -1), [(4, 1), (14, -1)], [(3, 1)]), ((5, 1), [(0, 1), (3, 1)], [(3, 1), (101, -1)]), ((100, -1), [(0, 1), (3, 1), (5, 1), (13, 1)], [(101, 1)]), ((103, 1), [(0, 1), (3, 1), (5, 1)], [(0, 1), (101, 1)]), ((110, 1), [(1, 1)], [(0, 1), (2, 1)]), ((107, 1), [(0, 1), (5, 1)], [(0, 1)]), ((113, -1), [(2, 1), (7, 1), (9, 1)], [(105, -1)]), ((7, -1), [(7, 1), (9, 1)], [(4, -1), (105, -1)]), ((106, -1), [(9, 1)], [(4, 1)]), ((108, -1), [(8, 1), (13, -1)], [(4, 1)])]
NPROD = len(O_PRODS)


def _normalize(prods):
    out = []
    for (var, sgn), w, g in prods:
        sgn *= w[0][1]
        out.append((var, [(y, c * w[0][1]) for y, c in w], [(z, c * sgn) for z, c in g]))
    return out


OORD = "1.0.3.2.5.6.8.9.4.24.11.12.10.14.13.15.16.17.18.19.20.21.22.23.7"
QORD = "14.15.16.17.18.19.20.21.22.24.23.0.1.6.2.7.3.4.5.8.9.10.11.12.13"
SOORD = "7.23.22.21.20.19.18.16.17.15.13.12.10.11.14.9.8.24.6.5.2.3.4.0.1"
SQORD = "14.15.16.17.18.10.20.21.22.24.1.23.6.2.7.0.3.8.4.5.9.19.11.12.13"
LOORD = OORD
LQORD = QORD
LPAT = PAT
O_PRODS = _normalize(O_PRODS)
Q_PRODS = _normalize(Q_PRODS)
W_FORMS = [p[1] for p in O_PRODS]


def _positive_outputs(prods, prog):
    for flips in range(1 << 6):
        sg = [(-1 if (flips >> (r % 6)) & 1 else 1) for r in range(len(prods))]
        pos = {}
        for r, p in enumerate(prods):
            for z, c in p[2]:
                pos[z] = max(pos.get(z, -1), c * sg[r])
        for t, a, b, s in reversed(prog):
            st = pos.pop(t)
            pos[a] = max(pos.get(a, -1), st)
            pos[b] = max(pos.get(b, -1), st * s)
        if min(pos.values()) > 0:
            return sg
    raise AssertionError


Q_SIGN = _positive_outputs(Q_PRODS, Q_OUT_PROG)
Q_PRODS = [(v, w, [(z, c * s) for z, c in g]) for (v, w, g), s in zip(Q_PRODS, Q_SIGN)]


def _make_lhs(block, prog):
    vals = {}

    def get(v):
        if v not in vals:
            vals[v] = block(v)
        return vals[v]

    for t, a, b, s in prog:
        vals[t] = get(a) + get(b) if s > 0 else get(a) - get(b)
    return get


def _acc_add(accs, z, sgn, m):
    if z not in accs:
        accs[z] = (sgn, m)
    else:
        s0, a = accs[z]
        accs[z] = (s0, a + m) if s0 == sgn else ((1, a - m) if s0 > 0 else (1, m - a))


def _bilinear_run(accs, prods, which, lhs_of, w_of, tick):
    for r in which:
        m = tick(jnp.dot(lhs_of(r), w_of(r), preferred_element_type=f32), 20)
        for z, c in prods[r][2]:
            _acc_add(accs, z, c, m)


def _bilinear_finish(accs, prog):
    for t, a, b, s in reversed(prog):
        st, v = accs.pop(t)
        _acc_add(accs, a, st, v)
        _acc_add(accs, b, st * s, v)
    return accs


def _mul(i, n):
    return i * n if isinstance(i, int) else pl.multiple_of(i * n, 16)


def _as_bf16(packed):
    return pltpu.bitcast(packed, bf16)


def _as_f32(packed):
    return pltpu.bitcast(packed, bf16).astype(f32)


def _q_operands(c):
    assert all(s > 0 for row in c for s, _ in row)
    (t0, t1, t2), (b0, b1, b2) = [[a for _, a in row] for row in c]
    lo = lax.broadcasted_iota(jnp.int32, t0.shape, 1) < 64
    return [[jnp.where(lo, t0, b0), jnp.where(lo, t1, t0 - b0), jnp.where(lo, b0 - t0, pltpu.roll(b1, 64, 1))],
            [jnp.where(lo, t2, b2), jnp.where(lo, pltpu.roll(t1, 64, 1), t2 - b2), jnp.where(lo, b2 - t2, b1)]]


def _scores_half(qh, kt, h, j, tick):
    k0, k1, k2 = (0, 64, 128) if h == 0 else (256, 320, 192)
    out = []
    for c in (2 * j, 2 * j + 1):
        cs = slice(c * 128, (c + 1) * 128)
        w = [kt[k0:k0 + 128, cs],
             jnp.concatenate([kt[k2:k2 + 64, cs], kt[k1:k1 + 64, cs]], axis=0),
             jnp.concatenate([kt[k0:k0 + 64, cs], kt[k2:k2 + 64, cs]], axis=0)]
        m = [tick(jnp.dot(qh[i], w[i], preferred_element_type=f32), 20) for i in range(3)]
        out.append(jnp.concatenate([m[0] + m[1], m[0] + m[2]], axis=0))
    return out


def _softmax(s):
    m = jnp.max(s, axis=1, keepdims=True)
    p = jnp.exp2(s - m)
    p0, p1, p2, p3 = (p[:, i * 128:(i + 1) * 128] for i in range(4))
    s01, s23 = p0 + p1, p2 + p3
    t = s01 + s23
    l = jnp.sum(t, axis=1, keepdims=True)
    r = pl.reciprocal(l, approx=True)
    r = r * (2.0 - l * r)
    return jnp.concatenate([s01, jnp.minimum(s23, t), p0, p2, p1, p3], axis=1).astype(bf16), r


def _pv_weights(vt, h, i):
    d0, d1, d2 = (0, 64, 128) if h == 0 else (256, 320, 192)

    def v(d, c):
        return vt[d:d + 64, c * 128:(c + 1) * 128]

    def f(d, c):
        return v(d, c).astype(f32)

    if i == 0:
        return jnp.concatenate([jnp.concatenate([v(d0, c), v(d1, c + 1)], axis=0) for c in (0, 2)], axis=1)
    if i == 1:
        w = [jnp.concatenate([f(d2, c), f(d1, c) - f(d1, c + 1)], axis=0) for c in (0, 2)]
    else:
        w = [jnp.concatenate([f(d0, c + 1) - f(d0, c), f(d2, c + 1)], axis=0) for c in (0, 2)]
    return jnp.concatenate(w, axis=1).astype(bf16)


def _schedule(nu, pat):
    if "@" in pat:
        return [(a.split("@")[0], int(a.split("@")[1])) for a in pat.split(",")]
    pat = [(a.split(":")[0], int(a.split(":")[1])) for a in pat.split(",")]
    order = []
    for t in range(-6, nu + 6):
        for name, lag in pat:
            u = t + lag
            if 0 <= u < nu:
                order.append((name, u))
    return order


def _kernel(ax, ak, av, awq, awo, bx, bk, bv, bwq, bwo, o_hbm,
            acc, x32, w32, kvbuf, obuf, pbuf, qbuf, xc32, wc0, wc1,
            kv_sem, x_sem, w_sem, o_sem, *, scale, nhp, nb):
    xbuf, wbuf = (r.bitcast(bf16) for r in (x32, w32))
    pbuf, qbuf, xc = (r.bitcast(bf16) for r in (pbuf, qbuf, xc32))
    wc = [r.bitcast(bf16) for r in (wc0, wc1)]
    sq = xbuf.shape[3]
    hq = sq // 2
    d = awq.shape[0]
    hw = kvbuf.shape[2]
    wrows = wbuf.shape[0] // 4
    ng = nhp * nb
    lg = nb.bit_length() - 1
    assert nb == 1 << lg

    def kv_start(g, which=(0, 1, 2, 3)):
        hp, b = (g >> lg) & (nhp - 1), g & (nb - 1)
        for i, src in enumerate((ak, av, bk, bv)):
            if i in which:
                sem = kv_sem.at[jnp.where(g < nb, b, nb + (b >> 2))]
                pltpu.make_async_copy(src.at[b, hp], kvbuf.at[b, i], sem).start()

    def kv_wait(b):
        pltpu.make_async_copy(kvbuf.at[b], kvbuf.at[b], kv_sem.at[b]).wait()

    def kvg_start(g):
        hp, i4 = g >> lg, (g >> 2) & 3
        b = pl.multiple_of(i4 * BB, BB)
        for i, src in enumerate((ak, av, bk, bv)):
            pltpu.make_async_copy(src.at[pl.ds(b, BB), hp], kvbuf.at[pl.ds(b, BB), i], kv_sem.at[nb + i4]).start()

    def kvg_wait(i4):
        v = kvbuf.at[pl.ds(i4 * BB, BB)]
        pltpu.make_async_copy(v, v, kv_sem.at[nb + i4]).wait()

    def x_start(b, which=(0, 1)):
        for i, src in enumerate((ax, bx)):
            if i in which:
                for c in range(xbuf.shape[2]):
                    pltpu.make_async_copy(src.at[b, :, pl.ds(c * 128, 128)], xbuf.at[b, i, c], x_sem.at[b]).start()

    def x_wait(b):
        pltpu.make_async_copy(xbuf.at[b], xbuf.at[b], x_sem.at[b]).wait()

    def w_start(h, m):
        off = h * hw if isinstance(h, int) else pl.multiple_of(h * hw, 128)
        if m < 2:
            for c in range(hw // 128):
                pltpu.make_async_copy((awq, bwq)[m].at[:, pl.ds(off + c * 128, 128)],
                                      wbuf.at[pl.ds(m * wrows + c * d, d)], w_sem.at[m]).start()
        else:
            for c in range(d // 128):
                pltpu.make_async_copy((awo, bwo)[m - 2].at[pl.ds(off, hw), pl.ds(c * 128, 128)],
                                      wbuf.at[pl.ds(m * wrows + c * hw, hw)], w_sem.at[m]).start()

    def w_start_dyn(h, m, valid):
        for k in range(4):
            @pl.when(jnp.logical_and(m == k, valid))
            def _():
                w_start(h, k)

    def w_wait(m):
        v = wbuf.at[pl.ds(_mul(m, wrows), wrows)]
        pltpu.make_async_copy(v, v, w_sem.at[m]).wait()

    def prep_w(dst, msrc, mdst, row, nrows, part=None, zero=None):
        if isinstance(msrc, int):
            sa, sc = (5, 1) if msrc < 2 else (1, 3)
            off = [(msrc * 15 + (y // 5) * sa + (y % 5) * sc) * 64 + row * 8 for y in range(15)]
        else:
            sa, sc = jnp.where(msrc < 2, 5, 1), jnp.where(msrc < 2, 1, 3)
            off = [pl.multiple_of((msrc * 15 + (y // 5) * sa + (y % 5) * sc) * 64 + row * 8, 64 if isinstance(row, int) and row == 0 else 32)
                   for y in range(15)]
        r16 = _mul(mdst * 8 + row, 16)
        if not isinstance(r16, int):
            r16 = pl.multiple_of(r16, 128 if isinstance(row, int) and row == 0 else 64)
        for r, form in enumerate(W_FORMS):
            if part is not None and r % part[1] != part[0]:
                continue
            if len(form) == 1:
                val = _as_bf16(w32[pl.ds(off[form[0][0]], nrows * 8), :])
            else:
                val = None
                for y, c in form:
                    t = _as_f32(w32[pl.ds(off[y], nrows * 8), :])
                    val = t if val is None else (val + t if c > 0 else val - t)
                val = val.astype(bf16)
            wc[dst][pl.ds(r16, nrows * 16), r * 128:(r + 1) * 128] = val
        if zero is not None:
            c0 = part[0] * 128
            return lambda: wc[dst][pl.ds(pl.multiple_of(r16 + zero * 16, 16), 16), c0:c0 + 128].astype(f32)[0:8]

    def prep_x(b, br, part=None, zero=None):
        get = _make_lhs(
            lambda z: _as_f32(x32[b, br, z % 5, (z // 5) * (hq // 2):(z // 5 + 1) * (hq // 2), :]) * scale,
            Q_LHS_PROG)
        for r, p in enumerate(Q_PRODS):
            if part is not None and r * XPARTS // NPROD != part:
                continue
            c0 = r * 128
            xc[pl.ds(_mul(b * 2 + br, hq), hq), r * 128:(r + 1) * 128] = (get(p[0]) * Q_SIGN[r]).astype(bf16)
        if zero is not None:
            return lambda: xc[pl.ds(_mul(b * 2 + br + zero, hq), 16), c0:c0 + 128].astype(f32)[0:8]

    def body(g0, nbat, extra, pat, cs, first_hp=False, last_hp=False):
        hp = g0 >> lg
        b0 = g0 & (nb - 1)
        R, O, OT, OC = {}, {}, {}, {}

        def prow(u, h):
            return (2 * u + h) * sq

        def weights(m, prods):
            def w_of(r):
                s = W_FORMS.index(prods[r][1])
                return wc[cs][m * 128:(m + 1) * 128, s * 128:(s + 1) * 128]
            return w_of

        QA, OA, SC, LH = {}, {}, {}, {}
        pending = []
        clock = [0]
        zero16 = pl.multiple_of((g0 >> 20) * 16, 16)

        def later(key, delay, emit):
            pending.append((clock[0] + delay, key, emit))
            pending.sort(key=lambda e: e[0])

        def flush(key):
            for e in [e for e in pending if e[1] == key]:
                pending.remove(e)
                e[2]()

        def tick(o, cycles):
            t0 = clock[0]
            clock[0] += cycles
            groups = o.shape[0] // 8
            rows = None
            while pending and pending[0][0] <= clock[0]:
                due, _, emit = pending.pop(0)
                tok = emit()
                if tok is None or not TOK:
                    continue
                g = min(max((due - t0) * groups // cycles, 0), groups - 1)
                rows = rows or [o[8 * i:8 * i + 8] for i in range(groups)]
                rows[g] = jnp.minimum(rows[g], jnp.maximum(rows[g], tok()))
            return o if rows is None else jnp.concatenate(rows, axis=0)

        pat, qord, oord = pat
        qord = [int(i) for i in qord.split(".")]
        oord = [int(i) for i in oord.split(".")]

        def q_(u, lo_, hi_):
            b, br = b0 + u // 2, u % 2

            def lhs_of(r):
                return xc[pl.ds(_mul(b * 2 + br, hq), hq), r * 128:(r + 1) * 128]

            _bilinear_run(QA.setdefault(u, {}), Q_PRODS, qord[lo_:hi_], lhs_of, weights(br, Q_PRODS), tick)
            if hi_ == len(Q_PRODS):
                fin = _bilinear_finish(QA[u], Q_OUT_PROG)
                c = [[fin[i * 3 + n] for n in range(3)] for i in range(2)]
                nch = hq // QCH

                def chunk(k):
                    ck = [[(s, a[k * QCH:(k + 1) * QCH]) for s, a in row] for row in c]
                    r0 = u * hq + k * QCH
                    for h, ops in enumerate(_q_operands(ck)):
                        for i, a in enumerate(ops):
                            qbuf[r0:r0 + QCH, (3 * h + i) * 128:(3 * h + i + 1) * 128] = a.astype(bf16)
                    return lambda: qbuf[pl.ds(r0 + zero16, 16), 0:128].astype(f32)[0:8]

                for k in range(nch):
                    later(("q", u), QD + k * QS, functools.partial(chunk, k))

        def s_(u, h, j):
            b, br = b0 + u // 2, u % 2
            flush(("q", u))
            qh = [qbuf[u * hq:(u + 1) * hq, (3 * h + i) * 128:(3 * h + i + 1) * 128] for i in range(3)]
            SC[u, h, j] = _scores_half(qh, kvbuf.at[b, 2 * br], h, j, tick)
            if j == 1:
                s = jnp.concatenate(SC[u, h, 0] + SC[u, h, 1], axis=1)
                R[u, h] = []

                def chunk(k):
                    p, r = _softmax(s[k * PCH:(k + 1) * PCH])
                    R[u, h].append(r)
                    r0 = prow(u, h) + k * PCH
                    pbuf[r0:r0 + PCH, :] = p
                    return lambda: pbuf[pl.ds(r0 + zero16, 16), 0:128].astype(f32)[0:8]

                for k in range(sq // PCH):
                    later(("p", u, h), SD + k * SS, functools.partial(chunk, k))

        def rinv(u, h):
            return jnp.concatenate(R[u, h], axis=0)

        def m_(u, h, half):
            flush(("p", u, h))
            vt = kvbuf.at[b0 + u // 2 + (g0 >> 20) * half * VNOCSE, 2 * (u % 2) + 1]
            r0 = prow(u, h) + half * hq
            res = [tick(lax.dot_general(pbuf[r0:r0 + hq, i * 256:(i + 1) * 256], _pv_weights(vt, h, i), NT,
                                        preferred_element_type=f32), 40) for i in range(3)]
            lo = lax.broadcasted_iota(jnp.int32, (hq, 128), 1) < 64
            r = rinv(u, h)[half * hq:(half + 1) * hq]
            O[u, h, half] = (res[0] + jnp.where(lo, res[2], res[1])) * r
            OT[u, h, half] = jnp.where(lo, res[1], res[2]) * r

        def o_(u, lo_, hi_):
            b, br = b0 + u // 2, u % 2
            if lo_ == 0:
                lo = lax.broadcasted_iota(jnp.int32, (hq, 128), 1) < 64
                mid = [jnp.where(lo, OT[u, 0, i], OT[u, 1, i]) +
                       pltpu.roll(jnp.where(lo, OT[u, 1, i], OT[u, 0, i]), 64, 1) for i in range(2)]
                tiles = [[O[u, 0, i], mid[i], O[u, 1, i]] for i in range(2)]
                get = _make_lhs(lambda x: tiles[x // 3][x % 3], O_LHS_PROG)
                LH[u] = {p[0]: get(p[0]).astype(bf16) for p in O_PRODS}
            _bilinear_run(OA.setdefault(u, {}), O_PRODS, oord[lo_:hi_], lambda r: LH[u][O_PRODS[r][0]],
                          weights(2 + br, O_PRODS), tick)
            fin = _bilinear_finish(OA[u], O_OUT_PROG) if hi_ == NPROD else {}
            for n in (range(5) if fin else ()):
                for i in range(2):
                    s, a = fin[i * 5 + n]
                    rows = slice(i * hq, (i + 1) * hq)
                    cols = slice(br * d + n * 128, br * d + (n + 1) * 128)
                    if first_hp:
                        new = a if s > 0 else -a
                    else:
                        new = acc[b, rows, cols] + a if s > 0 else acc[b, rows, cols] - a
                    if last_hp:
                        obuf[b, rows, cols] = new.astype(obuf.dtype)
                    if not last_hp:
                        acc[b, rows, cols] = new
            if br == 1 and lo_ > 0 and last_hp:
                pltpu.make_async_copy(obuf.at[b], o_hbm.at[b], o_sem).start()

        fns = {"qa": lambda u: q_(u, 0, QSPLIT), "qb": lambda u: q_(u, QSPLIT, NPROD),
               "oa": lambda u: o_(u, 0, OSPLIT), "ob": lambda u: o_(u, OSPLIT, NPROD),
               "s00": lambda u: s_(u, 0, 0), "s01": lambda u: s_(u, 0, 1),
               "s10": lambda u: s_(u, 1, 0), "s11": lambda u: s_(u, 1, 1),
               "m0": lambda u: m_(u, 0, 0), "m1": lambda u: m_(u, 1, 0),
               "t0": lambda u: m_(u, 0, 1), "t1": lambda u: m_(u, 1, 1), "c": lambda u: None}
        sched = _schedule(2 * nbat, pat)
        first, dmas, preps = extra
        for f in first:
            f()
        total = 2 * nbat * 1960
        lastq = max(i for i, it in enumerate(sched) if it[0][0] == "q")
        wpre, xpre = preps
        for k, f in enumerate(wpre):
            lo_, hi_ = (PLO, total - PHI) if nbat > 1 else (SWLO, SWHI)
            later("w", lo_ + k * (hi_ - lo_) // len(wpre), f)
        for i, item in enumerate(sched):
            fns[item[0]](item[1])
            if i == lastq:
                for k, f in enumerate(xpre):
                    later("x", SXLO + k * (total - SXHI - clock[0] - SXLO) // len(xpre), f)
        flush("w")
        flush("x")
        assert not pending

    for k in range(4):
        w_start(0, k)
    x_start(0)
    kv_start(0)
    x_start(1)
    for g in range(1, C0):
        kv_start(g)
        x_start(g + 1)
    for m in range(4):
        w_wait(m)
        prep_w(0, m, m, 0, 8)
    x_wait(0)
    for br in range(2):
        prep_x(0, br)

    def issued(g):
        return jnp.minimum(jnp.minimum(RATE * (g + 1) + C0, g + LA), G1 + BB)

    def small(b0, carry):
        half = nb // 2
        m = (b0 - half) >> 1

        @pl.when(b0 + 1 < nb)
        def _():
            x_wait(b0 + 1)

        @pl.when(jnp.logical_and(b0 >= half, (b0 & 1) == 0))
        def _():
            w_wait(m)

        kv_wait(b0)

        hi = issued(b0)
        prev = jnp.where(b0 == 0, C0, issued(b0 - 1))

        def pf_x(k, w):
            @pl.when(jnp.logical_and(prev + k < hi, prev + k + 1 < nb))
            def _():
                x_start(prev + k + 1, (w,))

        def pf_kv(k):
            @pl.when(prev + k < hi)
            def _():
                kv_start(prev + k)

        def pf_w():
            w_start_dyn(jnp.where(b0 == W2AT, 2, 1), jnp.where(b0 == W2AT, 0, (b0 >> 1) - 1),
                        jnp.logical_or(b0 == W2AT, jnp.logical_and(b0 <= half, (b0 & 1) == 0)))

        first = [pf_w] + [functools.partial(pf_x, k, w) for k in range(RATE) for w in range(2)]
        first += [functools.partial(pf_kv, k) for k in range(RATE)]
        zero = b0 >> 20
        preps = ([functools.partial(prep_w, 1, jnp.where(b0 >= half, m, 3), jnp.maximum(m, 0), (b0 & 1) * 4, 4,
                                    (part, SWPARTS), zero) for part in range(SWPARTS)],
                 [functools.partial(prep_x, jnp.minimum(b0 + 1, nb - 1), br, part, zero)
                  for br in range(2) for part in range(XPARTS)])
        body(b0, 1, (first, [], preps), (SPAT, SQORD, SOORD), 0, first_hp=True)
        return carry

    def big(par, last, hp, i, carry):
        b0 = i * BB
        g0 = hp * nb + b0

        if not last:
            w_wait(i)

        kvg_wait(i)

        def pf_kv():
            @pl.when(g0 + BB < ng)
            def _():
                kvg_start(g0 + BB)

        if last:
            extra = ([pf_kv], [], ([], []))
        else:
            hn = jnp.where(i == 3, hp + 2, hp + 1)
            extra = ([lambda: w_start_dyn(hn, (i + 1) & 3, hn < nhp)] +
                     [functools.partial(kvg_start, g0 + BB)], [],
                     ([functools.partial(prep_w, 1 - par, i, i, 0, 8, (part, PPARTS), i >> 20)
                       for part in range(PPARTS)], []))
        body(g0, BB, extra, (LPAT, LQORD, LOORD) if last else (PAT, QORD, OORD), par, last_hp=last)
        return carry

    spb = nb // BB
    assert spb == 4 and G1 == nb
    if SKIP_SMALL in (0, 2):
        lax.fori_loop(0, nb, small, 0)
    if SKIP_SMALL == 2:
        prep_x(0, 0)
        acc[0, 0:128, 0:128] = wc[1][0:128, 0:128].astype(f32)
        pltpu.make_async_copy(obuf, o_hbm, o_sem).start()
        pltpu.make_async_copy(obuf, o_hbm, o_sem).wait()
        return

    def pair(t, carry):
        lax.fori_loop(jnp.where(t > 0, 0, spb), spb, functools.partial(big, 0, False, 2 * t), 0)
        lax.fori_loop(0, jnp.where(2 * t + 1 < nhp - 1, spb, 0), functools.partial(big, 1, False, 2 * t + 1), 0)
        return carry

    if SKIP_SMALL != 3:
        lax.fori_loop(0, nhp // 2, pair, 0)
    else:
        prep_w(1, 0, 0, 0, 8)
    if SKIP_SMALL in (0, 3):
        lax.fori_loop(0, spb, functools.partial(big, 1, True, nhp - 1), 0)
    pltpu.make_async_copy(obuf, o_hbm, o_sem).wait()


@jax.jit
def pallas_concat_heads__gqa_block_cached__mha_block_cached__near_ridge_kernel(
    A_x, A_k_cache, A_v_cache, A_wq, A_wo, B_x, B_k_cache, B_v_cache, B_wq, B_wo):
    B, Sq, D = A_x.shape
    _, H, Sk, Dh = A_k_cache.shape
    nhp = H // 2
    assert B == 16 and G1 % B == 0 and 2 * BB <= B and C0 >= 1
    n_iss = C0
    for g0 in range(G1):
        assert n_iss >= min(g0 + 2, G1 + BB), (g0, n_iss)
        hi = min(RATE * (g0 + 1) + C0, g0 + LA, G1 + BB)
        assert 0 <= hi - n_iss <= RATE
        n_iss = hi
    assert n_iss == G1 + BB, n_iss
    assert 10 <= W2AT <= 15 and 5 <= LA <= B

    def tr(c):
        return jnp.swapaxes(c, 2, 3).reshape(B, nhp, 2 * Dh, Sk)

    any_spec = pl.BlockSpec(memory_space=pl.ANY)
    return pl.pallas_call(
        functools.partial(_kernel, scale=Dh ** -0.5 * LOG2E, nhp=nhp, nb=B),
        in_specs=[any_spec] * 10,
        out_specs=any_spec,
        out_shape=jax.ShapeDtypeStruct((B, Sq, 2 * D), A_x.dtype),
        scratch_shapes=[pltpu.VMEM((B, ACCR, 2 * D), f32),
                        pltpu.VMEM((B, 2, D // 128, Sq // 2, 128), u32),
                        pltpu.VMEM((4 * 15 * 64, 128), u32),
                        pltpu.VMEM((B, 4, 2 * Dh, Sk), bf16),
                        pltpu.VMEM((B, Sq, 2 * D), bf16),
                        pltpu.VMEM((2 * BB * Sq, 6 * 128), u32),
                        pltpu.VMEM((2 * BB * Sq // 4, 6 * 128), u32),
                        pltpu.VMEM((B * 2 * Sq // 4, XCW * 128), u32),
                        pltpu.VMEM((4 * 64, WCW * 128), u32),
                        pltpu.VMEM((4 * 64, WCW * 128), u32),
                        pltpu.SemaphoreType.DMA((B + 4,)),
                        pltpu.SemaphoreType.DMA((B,)),
                        pltpu.SemaphoreType.DMA((4,)),
                        pltpu.SemaphoreType.DMA(())],
        compiler_params=pltpu.CompilerParams(
            disable_bounds_checks=True,
            vmem_limit_bytes=110 * 1024 * 1024),
    )(A_x, tr(A_k_cache), tr(A_v_cache), A_wq, A_wo, B_x, tr(B_k_cache), tr(B_v_cache), B_wq, B_wo)
```

```python
import functools
import jax
import jax.numpy as jnp
from jax import lax
import jax.experimental.pallas as pl
import jax.experimental.pallas.tpu as pltpu

BB = 4
G1 = 16
C0 = 2
RATE = 2
PFPOS = 1
PFSTEP = 3
PSKIP = 2
OBUF = 1
SKIP_SMALL = 0
KVTOP = 8
QSPLIT = 11
OSPLIT = 10
PPARTS = 25
PEND = 10
XCW = 32
WCW = 40
ACCR = 160
WQT = 3
WOT = 5
MERGE = 0
TOK = 1
W2AT = 11
LA = 6
XPARTS = 25
SWPARTS = 12
QCH = 80
QD = 9999
QS = 60
PCH = 160
SD = 9999
SS = 40
PLO = 300
PHI = 400
SWLO = 100
SWHI = 1000
SXLO = 1800
SXHI = 100
VNOCSE = 1
SQSPLIT = 13
SOSPLIT = 13
LQSPLIT = 11
LOSPLIT = 10
NOCSE = 1
PAT = "s00:0,qa:2,s01:0,m1:-1,t1:-1,s10:0,oa:-2,qb:2,s11:0,m0:0,t0:0,ob:-2"
SPAT = "qa@0,qb@0,qa@1,qb@1,s00@0,s10@0,s11@0,s00@1,s10@1,s01@0,t1@0,m1@0,s11@1,m0@0,t0@0,m1@1,s01@1,oa@0,t1@1,t0@1,m0@1,ob@0,oa@1,ob@1"
LOG2E = 1.4426950408889634
bf16 = jnp.bfloat16
f32 = jnp.float32
u32 = jnp.uint32
NT = (((1,), (1,)), ((), ()))

O_LHS_PROG = [(100, 4, 5, 1), (101, 0, 1, -1), (102, 3, 101, 1), (103, 2, 100, 1), (104, 0, 3, 1), (105, 2, 3, -1), (106, 0, 2, 1), (107, 2, 101, -1), (108, 3, 5, 1), (109, 1, 103, 1), (110, 2, 5, 1), (111, 3, 100, -1), (112, 5, 101, 1), (113, 4, 102, -1), (114, 0, 100, 1)]
O_OUT_PROG = [(100, 5, 8, -1), (101, 3, 100, 1), (102, 2, 7, -1), (103, 0, 102, 1)]
O_PRODS = [((101, 1), [(2, 1), (5, 1), (10, -1), (12, 1)], [(102, 1)]), ((104, 1), [(3, 1)], [(100, -1)]), ((111, 1), [(0, 1), (3, 1)], [(5, 1)]), ((5, 1), [(5, 1), (10, -1)], [(5, -1), (103, 1)]), ((112, 1), [(5, 1), (10, -1), (12, 1)], [(103, -1)]), ((114, 1), [(0, 1), (3, 1), (5, 1)], [(101, 1)]), ((0, 1), [(0, 1), (5, 1)], [(0, 1), (101, -1)]), ((107, -1), [(10, 1), (12, -1)], [(0, -1)]), ((110, 1), [(12, 1)], [(0, 1), (2, 1)]), ((1, 1), [(2, 1), (7, 1)], [(2, 1), (4, -1)]), ((104, 1), [(1, 1), (2, 1), (4, 1), (7, 1), (9, 1)], [(4, 1)]), ((106, 1), [(1, 1)], [(1, 1), (4, -1)]), ((1, 1), [(6, 1)], [(1, 1), (3, -1)]), ((109, 1), [(6, 1), (8, 1)], [(3, 1)]), ((2, 1), [(1, 1), (11, -1)], [(1, -1), (6, 1)]), ((103, 1), [(6, 1), (8, 1), (13, -1)], [(3, -1), (6, 1)]), ((100, 1), [(0, 1), (3, 1), (5, 1), (13, 1)], [(3, -1), (8, 1)]), ((4, 1), [(8, 1), (13, -1)], [(6, -1), (8, 1)]), ((110, 1), [(6, 1), (8, 1), (11, -1), (13, -1), (14, -1)], [(6, -1)]), ((105, 1), [(1, 1), (14, 1)], [(4, 1), (6, -1)]), ((108, 1), [(14, 1)], [(6, -1), (9, 1)]), ((3, 1), [(4, 1), (14, -1)], [(4, -1), (9, 1)]), ((4, 1), [(9, 1)], [(7, -1), (9, 1)]), ((102, 1), [(2, 1), (7, 1), (9, 1)], [(4, -1), (7, 1)]), ((113, -1), [(7, 1), (9, 1)], [(7, -1)])]
Q_LHS_PROG = [(100, 3, 8, -1), (101, 0, 2, 1), (102, 7, 101, -1), (103, 5, 100, 1), (104, 4, 6, -1), (105, 4, 9, -1), (106, 7, 9, -1), (107, 0, 103, -1), (108, 6, 8, -1), (109, 5, 102, 1), (110, 1, 4, -1), (111, 5, 8, -1), (112, 6, 9, -1), (113, 4, 7, -1), (114, 2, 4, -1), (115, 1, 6, -1), (116, 2, 7, -1), (117, 1, 3, -1), (118, 3, 6, -1)]
Q_OUT_PROG = [(100, 0, 3, 1), (101, 4, 5, 1), (102, 0, 1, -1), (103, 2, 101, 1), (104, 2, 5, 1), (105, 1, 100, -1)]
Q_PRODS = [((6, -1), [(6, 1), (8, 1), (11, -1), (13, -1), (14, -1)], [(104, 1)]), ((101, 1), [(12, 1)], [(104, 1)]), ((4, 1), [(1, 1), (2, 1), (4, 1), (7, 1), (9, 1)], [(100, 1)]), ((111, -1), [(3, 1)], [(100, 1)]), ((118, -1), [(6, 1), (8, 1), (13, -1)], [(103, 1)]), ((3, 1), [(6, 1), (8, 1)], [(1, 1), (103, 1)]), ((114, 1), [(2, 1), (7, 1)], [(1, 1)]), ((117, 1), [(6, 1)], [(1, 1)]), ((115, -1), [(1, 1), (11, -1)], [(2, 1)]), ((0, -1), [(10, 1), (12, -1)], [(2, -1), (102, 1)]), ((116, 1), [(2, 1), (5, 1), (10, -1), (12, 1)], [(102, 1)]), ((102, 1), [(5, 1), (10, -1), (12, 1)], [(5, 1), (102, 1)]), ((109, -1), [(5, 1), (10, -1)], [(5, 1)]), ((112, -1), [(14, 1)], [(3, 1), (5, 1)]), ((104, 1), [(1, 1), (14, 1)], [(2, 1), (3, -1)]), ((105, -1), [(4, 1), (14, -1)], [(3, 1)]), ((5, 1), [(0, 1), (3, 1)], [(3, 1), (101, -1)]), ((100, -1), [(0, 1), (3, 1), (5, 1), (13, 1)], [(101, 1)]), ((103, 1), [(0, 1), (3, 1), (5, 1)], [(0, 1), (101, 1)]), ((110, 1), [(1, 1)], [(0, 1), (2, 1)]), ((107, 1), [(0, 1), (5, 1)], [(0, 1)]), ((113, -1), [(2, 1), (7, 1), (9, 1)], [(105, -1)]), ((7, -1), [(7, 1), (9, 1)], [(4, -1), (105, -1)]), ((106, -1), [(9, 1)], [(4, 1)]), ((108, -1), [(8, 1), (13, -1)], [(4, 1)])]
NPROD = len(O_PRODS)


def _normalize(prods):
    out = []
    for (var, sgn), w, g in prods:
        sgn *= w[0][1]
        out.append((var, [(y, c * w[0][1]) for y, c in w], [(z, c * sgn) for z, c in g]))
    return out


OORD = "0.6.1.5.3.2.8.9.4.24.11.12.14.10.16.19.13.15.17.18.20.22.21.23.7"
QORD = "9.15.16.24.19.20.21.1.18.22.17.23.2.0.3.7.4.5.8.6.14.12.10.11.13"
SOORD = "7.23.22.21.20.19.18.16.17.15.13.12.10.11.14.9.8.24.6.5.2.3.4.0.1"
SQORD = "14.15.16.17.18.10.20.21.22.24.1.23.6.2.7.0.3.8.4.5.9.19.11.12.13"
LOORD = OORD
LQORD = QORD
LPAT = PAT
O_PRODS = _normalize(O_PRODS)
Q_PRODS = _normalize(Q_PRODS)
W_FORMS = [p[1] for p in O_PRODS]


def _positive_outputs(prods, prog):
    for flips in range(1 << 6):
        sg = [(-1 if (flips >> (r % 6)) & 1 else 1) for r in range(len(prods))]
        pos = {}
        for r, p in enumerate(prods):
            for z, c in p[2]:
                pos[z] = max(pos.get(z, -1), c * sg[r])
        for t, a, b, s in reversed(prog):
            st = pos.pop(t)
            pos[a] = max(pos.get(a, -1), st)
            pos[b] = max(pos.get(b, -1), st * s)
        if min(pos.values()) > 0:
            return sg
    raise AssertionError


Q_SIGN = _positive_outputs(Q_PRODS, Q_OUT_PROG)
Q_PRODS = [(v, w, [(z, c * s) for z, c in g]) for (v, w, g), s in zip(Q_PRODS, Q_SIGN)]


def _make_lhs(block, prog):
    vals = {}

    def get(v):
        if v not in vals:
            vals[v] = block(v)
        return vals[v]

    for t, a, b, s in prog:
        vals[t] = get(a) + get(b) if s > 0 else get(a) - get(b)
    return get


def _acc_add(accs, z, sgn, m):
    if z not in accs:
        accs[z] = (sgn, m)
    else:
        s0, a = accs[z]
        accs[z] = (s0, a + m) if s0 == sgn else ((1, a - m) if s0 > 0 else (1, m - a))


def _bilinear_run(accs, prods, which, lhs_of, w_of, tick):
    for r in which:
        m = tick(jnp.dot(lhs_of(r), w_of(r), preferred_element_type=f32), 20)
        for z, c in prods[r][2]:
            _acc_add(accs, z, c, m)


def _bilinear_finish(accs, prog):
    for t, a, b, s in reversed(prog):
        st, v = accs.pop(t)
        _acc_add(accs, a, st, v)
        _acc_add(accs, b, st * s, v)
    return accs


def _mul(i, n):
    return i * n if isinstance(i, int) else pl.multiple_of(i * n, 16)


def _as_bf16(packed):
    return pltpu.bitcast(packed, bf16)


def _as_f32(packed):
    return pltpu.bitcast(packed, bf16).astype(f32)


def _q_operands(c):
    assert all(s > 0 for row in c for s, _ in row)
    (t0, t1, t2), (b0, b1, b2) = [[a for _, a in row] for row in c]
    lo = lax.broadcasted_iota(jnp.int32, t0.shape, 1) < 64
    return [[jnp.where(lo, t0, b0), jnp.where(lo, t1, t0 - b0), jnp.where(lo, b0 - t0, pltpu.roll(b1, 64, 1))],
            [jnp.where(lo, t2, b2), jnp.where(lo, pltpu.roll(t1, 64, 1), t2 - b2), jnp.where(lo, b2 - t2, b1)]]


def _scores_half(qh, kt, h, j, tick):
    k0, k1, k2 = (0, 64, 128) if h == 0 else (256, 320, 192)
    out = []
    for c in (2 * j, 2 * j + 1):
        cs = slice(c * 128, (c + 1) * 128)
        w = [kt[k0:k0 + 128, cs],
             jnp.concatenate([kt[k2:k2 + 64, cs], kt[k1:k1 + 64, cs]], axis=0),
             jnp.concatenate([kt[k0:k0 + 64, cs], kt[k2:k2 + 64, cs]], axis=0)]
        m = [tick(jnp.dot(qh[i], w[i], preferred_element_type=f32), 20) for i in range(3)]
        out.append(jnp.concatenate([m[0] + m[1], m[0] + m[2]], axis=0))
    return out


def _softmax(s):
    m = jnp.max(s, axis=1, keepdims=True)
    p = jnp.exp2(s - m)
    p0, p1, p2, p3 = (p[:, i * 128:(i + 1) * 128] for i in range(4))
    s01, s23 = p0 + p1, p2 + p3
    t = s01 + s23
    l = jnp.sum(t, axis=1, keepdims=True)
    r = pl.reciprocal(l, approx=True)
    r = r * (2.0 - l * r)
    return jnp.concatenate([s01, jnp.minimum(s23, t), p0, p2, p1, p3], axis=1).astype(bf16), r


def _pv_weights(vt, h, i):
    d0, d1, d2 = (0, 64, 128) if h == 0 else (256, 320, 192)

    def v(d, c):
        return vt[d:d + 64, c * 128:(c + 1) * 128]

    def f(d, c):
        return v(d, c).astype(f32)

    if i == 0:
        return jnp.concatenate([jnp.concatenate([v(d0, c), v(d1, c + 1)], axis=0) for c in (0, 2)], axis=1)
    if i == 1:
        w = [jnp.concatenate([f(d2, c), f(d1, c) - f(d1, c + 1)], axis=0) for c in (0, 2)]
    else:
        w = [jnp.concatenate([f(d0, c + 1) - f(d0, c), f(d2, c + 1)], axis=0) for c in (0, 2)]
    return jnp.concatenate(w, axis=1).astype(bf16)


def _schedule(nu, pat):
    if "@" in pat:
        return [(a.split("@")[0], int(a.split("@")[1])) for a in pat.split(",")]
    pat = [(a.split(":")[0], int(a.split(":")[1])) for a in pat.split(",")]
    order = []
    for t in range(-6, nu + 6):
        for name, lag in pat:
            u = t + lag
            if 0 <= u < nu:
                order.append((name, u))
    return order


def _kernel(ax, ak, av, awq, awo, bx, bk, bv, bwq, bwo, o_hbm,
            acc, x32, w32, kvbuf, obuf, pbuf, qbuf, xc32, wc0, wc1,
            kv_sem, x_sem, w_sem, o_sem, *, scale, nhp, nb):
    xbuf, wbuf = (r.bitcast(bf16) for r in (x32, w32))
    pbuf, qbuf, xc = (r.bitcast(bf16) for r in (pbuf, qbuf, xc32))
    wc = [r.bitcast(bf16) for r in (wc0, wc1)]
    sq = xbuf.shape[3]
    hq = sq // 2
    d = awq.shape[0]
    hw = kvbuf.shape[2]
    wrows = wbuf.shape[0] // 4
    ng = nhp * nb
    lg = nb.bit_length() - 1
    assert nb == 1 << lg

    def kv_start(g, which=(0, 1, 2, 3)):
        hp, b = (g >> lg) & (nhp - 1), g & (nb - 1)
        for i, src in enumerate((ak, av, bk, bv)):
            if i in which:
                sem = kv_sem.at[jnp.where(g < nb, b, nb + (b >> 2))]
                pltpu.make_async_copy(src.at[b, hp], kvbuf.at[b, i], sem).start()

    def kv_wait(b):
        pltpu.make_async_copy(kvbuf.at[b], kvbuf.at[b], kv_sem.at[b]).wait()

    def kvg_start(g):
        hp, i4 = g >> lg, (g >> 2) & 3
        b = pl.multiple_of(i4 * BB, BB)
        for i, src in enumerate((ak, av, bk, bv)):
            pltpu.make_async_copy(src.at[pl.ds(b, BB), hp], kvbuf.at[pl.ds(b, BB), i], kv_sem.at[nb + i4]).start()

    def kvg_wait(i4):
        v = kvbuf.at[pl.ds(i4 * BB, BB)]
        pltpu.make_async_copy(v, v, kv_sem.at[nb + i4]).wait()

    def x_start(b, which=(0, 1)):
        for i, src in enumerate((ax, bx)):
            if i in which:
                for c in range(xbuf.shape[2]):
                    pltpu.make_async_copy(src.at[b, :, pl.ds(c * 128, 128)], xbuf.at[b, i, c], x_sem.at[b]).start()

    def x_wait(b):
        pltpu.make_async_copy(xbuf.at[b], xbuf.at[b], x_sem.at[b]).wait()

    def w_start(h, m):
        off = h * hw if isinstance(h, int) else pl.multiple_of(h * hw, 128)
        if m < 2:
            for c in range(hw // 128):
                pltpu.make_async_copy((awq, bwq)[m].at[:, pl.ds(off + c * 128, 128)],
                                      wbuf.at[pl.ds(m * wrows + c * d, d)], w_sem.at[m]).start()
        else:
            for c in range(d // 128):
                pltpu.make_async_copy((awo, bwo)[m - 2].at[pl.ds(off, hw), pl.ds(c * 128, 128)],
                                      wbuf.at[pl.ds(m * wrows + c * hw, hw)], w_sem.at[m]).start()

    def w_start_dyn(h, m, valid):
        for k in range(4):
            @pl.when(jnp.logical_and(m == k, valid))
            def _():
                w_start(h, k)

    def w_wait(m):
        v = wbuf.at[pl.ds(_mul(m, wrows), wrows)]
        pltpu.make_async_copy(v, v, w_sem.at[m]).wait()

    def prep_w(dst, msrc, mdst, row, nrows, part=None, zero=None):
        if isinstance(msrc, int):
            sa, sc = (5, 1) if msrc < 2 else (1, 3)
            off = [(msrc * 15 + (y // 5) * sa + (y % 5) * sc) * 64 + row * 8 for y in range(15)]
        else:
            sa, sc = jnp.where(msrc < 2, 5, 1), jnp.where(msrc < 2, 1, 3)
            off = [pl.multiple_of((msrc * 15 + (y // 5) * sa + (y % 5) * sc) * 64 + row * 8, 64 if isinstance(row, int) and row == 0 else 32)
                   for y in range(15)]
        r16 = _mul(mdst * 8 + row, 16)
        if not isinstance(r16, int):
            r16 = pl.multiple_of(r16, 128 if isinstance(row, int) and row == 0 else 64)
        for r, form in enumerate(W_FORMS):
            if part is not None and r % part[1] != part[0]:
                continue
            if len(form) == 1:
                val = _as_bf16(w32[pl.ds(off[form[0][0]], nrows * 8), :])
            else:
                val = None
                for y, c in form:
                    t = _as_f32(w32[pl.ds(off[y], nrows * 8), :])
                    val = t if val is None else (val + t if c > 0 else val - t)
                val = val.astype(bf16)
            wc[dst][pl.ds(r16, nrows * 16), r * 128:(r + 1) * 128] = val
        if zero is not None:
            c0 = part[0] * 128
            return lambda: wc[dst][pl.ds(pl.multiple_of(r16 + zero * 16, 16), 16), c0:c0 + 128].astype(f32)[0:8]

    def prep_x(b, br, part=None, zero=None):
        get = _make_lhs(
            lambda z: _as_f32(x32[b, br, z % 5, (z // 5) * (hq // 2):(z // 5 + 1) * (hq // 2), :]) * scale,
            Q_LHS_PROG)
        for r, p in enumerate(Q_PRODS):
            if part is not None and r * XPARTS // NPROD != part:
                continue
            c0 = r * 128
            xc[pl.ds(_mul(b * 2 + br, hq), hq), r * 128:(r + 1) * 128] = (get(p[0]) * Q_SIGN[r]).astype(bf16)
        if zero is not None:
            return lambda: xc[pl.ds(_mul(b * 2 + br + zero, hq), 16), c0:c0 + 128].astype(f32)[0:8]

    def body(g0, nbat, extra, pat, cs, first_hp=False, last_hp=False):
        hp = g0 >> lg
        b0 = g0 & (nb - 1)
        R, O, OT, OC = {}, {}, {}, {}

        def prow(u, h):
            return (2 * u + h) * sq

        def weights(m, prods):
            def w_of(r):
                s = W_FORMS.index(prods[r][1])
                return wc[cs][m * 128:(m + 1) * 128, s * 128:(s + 1) * 128]
            return w_of

        QA, OA, SC, LH = {}, {}, {}, {}
        pending = []
        clock = [0]
        zero16 = pl.multiple_of((g0 >> 20) * 16, 16)

        def later(key, delay, emit):
            pending.append((clock[0] + delay, key, emit))
            pending.sort(key=lambda e: e[0])

        def flush(key):
            for e in [e for e in pending if e[1] == key]:
                pending.remove(e)
                e[2]()

        def tick(o, cycles):
            t0 = clock[0]
            clock[0] += cycles
            groups = o.shape[0] // 8
            rows = None
            while pending and pending[0][0] <= clock[0]:
                due, _, emit = pending.pop(0)
                tok = emit()
                if tok is None or not TOK:
                    continue
                g = min(max((due - t0) * groups // cycles, 0), groups - 1)
                rows = rows or [o[8 * i:8 * i + 8] for i in range(groups)]
                rows[g] = jnp.minimum(rows[g], jnp.maximum(rows[g], tok()))
            return o if rows is None else jnp.concatenate(rows, axis=0)

        pat, qord, oord, qsp, osp = pat
        qord = [int(i) for i in qord.split(".")]
        oord = [int(i) for i in oord.split(".")]

        def q_(u, lo_, hi_):
            b, br = b0 + u // 2, u % 2

            def lhs_of(r):
                return xc[pl.ds(_mul(b * 2 + br, hq), hq), r * 128:(r + 1) * 128]

            _bilinear_run(QA.setdefault(u, {}), Q_PRODS, qord[lo_:hi_], lhs_of, weights(br, Q_PRODS), tick)
            if hi_ == len(Q_PRODS):
                fin = _bilinear_finish(QA[u], Q_OUT_PROG)
                c = [[fin[i * 3 + n] for n in range(3)] for i in range(2)]
                nch = hq // QCH

                def chunk(k):
                    ck = [[(s, a[k * QCH:(k + 1) * QCH]) for s, a in row] for row in c]
                    r0 = u * hq + k * QCH
                    for h, ops in enumerate(_q_operands(ck)):
                        for i, a in enumerate(ops):
                            qbuf[r0:r0 + QCH, (3 * h + i) * 128:(3 * h + i + 1) * 128] = a.astype(bf16)
                    return lambda: qbuf[pl.ds(r0 + zero16, 16), 0:128].astype(f32)[0:8]

                for k in range(nch):
                    later(("q", u), QD + k * QS, functools.partial(chunk, k))

        def s_(u, h, j):
            b, br = b0 + u // 2, u % 2
            flush(("q", u))
            qh = [qbuf[u * hq:(u + 1) * hq, (3 * h + i) * 128:(3 * h + i + 1) * 128] for i in range(3)]
            SC[u, h, j] = _scores_half(qh, kvbuf.at[b, 2 * br], h, j, tick)
            if j == 1:
                s = jnp.concatenate(SC[u, h, 0] + SC[u, h, 1], axis=1)
                R[u, h] = []

                def chunk(k):
                    p, r = _softmax(s[k * PCH:(k + 1) * PCH])
                    R[u, h].append(r)
                    r0 = prow(u, h) + k * PCH
                    pbuf[r0:r0 + PCH, :] = p
                    return lambda: pbuf[pl.ds(r0 + zero16, 16), 0:128].astype(f32)[0:8]

                for k in range(sq // PCH):
                    later(("p", u, h), SD + k * SS, functools.partial(chunk, k))

        def rinv(u, h):
            return jnp.concatenate(R[u, h], axis=0)

        def m_(u, h, half):
            flush(("p", u, h))
            vt = kvbuf.at[b0 + u // 2 + (g0 >> 20) * half * VNOCSE, 2 * (u % 2) + 1]
            r0 = prow(u, h) + half * hq
            res = [tick(lax.dot_general(pbuf[r0:r0 + hq, i * 256:(i + 1) * 256], _pv_weights(vt, h, i), NT,
                                        preferred_element_type=f32), 40) for i in range(3)]
            lo = lax.broadcasted_iota(jnp.int32, (hq, 128), 1) < 64
            r = rinv(u, h)[half * hq:(half + 1) * hq]
            O[u, h, half] = (res[0] + jnp.where(lo, res[2], res[1])) * r
            OT[u, h, half] = jnp.where(lo, res[1], res[2]) * r

        def o_(u, lo_, hi_):
            b, br = b0 + u // 2, u % 2
            if lo_ == 0:
                lo = lax.broadcasted_iota(jnp.int32, (hq, 128), 1) < 64
                mid = [jnp.where(lo, OT[u, 0, i], OT[u, 1, i]) +
                       pltpu.roll(jnp.where(lo, OT[u, 1, i], OT[u, 0, i]), 64, 1) for i in range(2)]
                tiles = [[O[u, 0, i], mid[i], O[u, 1, i]] for i in range(2)]
                get = _make_lhs(lambda x: tiles[x // 3][x % 3], O_LHS_PROG)
                LH[u] = {p[0]: get(p[0]).astype(bf16) for p in O_PRODS}
            _bilinear_run(OA.setdefault(u, {}), O_PRODS, oord[lo_:hi_], lambda r: LH[u][O_PRODS[r][0]],
                          weights(2 + br, O_PRODS), tick)
            fin = _bilinear_finish(OA[u], O_OUT_PROG) if hi_ == NPROD else {}
            for n in (range(5) if fin else ()):
                for i in range(2):
                    s, a = fin[i * 5 + n]
                    rows = slice(i * hq, (i + 1) * hq)
                    cols = slice(br * d + n * 128, br * d + (n + 1) * 128)
                    if first_hp:
                        new = a if s > 0 else -a
                    else:
                        new = acc[b, rows, cols] + a if s > 0 else acc[b, rows, cols] - a
                    if last_hp:
                        obuf[b, rows, cols] = new.astype(obuf.dtype)
                    if not last_hp:
                        acc[b, rows, cols] = new
            if br == 1 and lo_ > 0 and last_hp:
                pltpu.make_async_copy(obuf.at[b], o_hbm.at[b], o_sem).start()

        fns = {"qa": lambda u: q_(u, 0, qsp), "qb": lambda u: q_(u, qsp, NPROD),
               "oa": lambda u: o_(u, 0, osp), "ob": lambda u: o_(u, osp, NPROD),
               "s00": lambda u: s_(u, 0, 0), "s01": lambda u: s_(u, 0, 1),
               "s10": lambda u: s_(u, 1, 0), "s11": lambda u: s_(u, 1, 1),
               "m0": lambda u: m_(u, 0, 0), "m1": lambda u: m_(u, 1, 0),
               "t0": lambda u: m_(u, 0, 1), "t1": lambda u: m_(u, 1, 1), "c": lambda u: None}
        sched = _schedule(2 * nbat, pat)
        first, dmas, preps = extra
        for f in first:
            f()
        total = 2 * nbat * 1960
        lastq = max(i for i, it in enumerate(sched) if it[0][0] == "q")
        wpre, xpre = preps
        for k, f in enumerate(wpre):
            lo_, hi_ = (PLO, total - PHI) if nbat > 1 else (SWLO, SWHI)
            later("w", lo_ + k * (hi_ - lo_) // len(wpre), f)
        for i, item in enumerate(sched):
            fns[item[0]](item[1])
            if i == lastq:
                for k, f in enumerate(xpre):
                    later("x", SXLO + k * (total - SXHI - clock[0] - SXLO) // len(xpre), f)
        flush("w")
        flush("x")
        assert not pending

    for k in range(4):
        w_start(0, k)
    x_start(0)
    kv_start(0)
    x_start(1)
    for g in range(1, C0):
        kv_start(g)
        x_start(g + 1)
    for m in range(4):
        w_wait(m)
        prep_w(0, m, m, 0, 8)
    x_wait(0)
    for br in range(2):
        prep_x(0, br)

    def issued(g):
        return jnp.minimum(jnp.minimum(RATE * (g + 1) + C0, g + LA), G1 + BB)

    def small(b0, carry):
        half = nb // 2
        m = (b0 - half) >> 1

        @pl.when(b0 + 1 < nb)
        def _():
            x_wait(b0 + 1)

        @pl.when(jnp.logical_and(b0 >= half, (b0 & 1) == 0))
        def _():
            w_wait(m)

        kv_wait(b0)

        hi = issued(b0)
        prev = jnp.where(b0 == 0, C0, issued(b0 - 1))

        def pf_x(k, w):
            @pl.when(jnp.logical_and(prev + k < hi, prev + k + 1 < nb))
            def _():
                x_start(prev + k + 1, (w,))

        def pf_kv(k):
            @pl.when(prev + k < hi)
            def _():
                kv_start(prev + k)

        def pf_w():
            w_start_dyn(jnp.where(b0 == W2AT, 2, 1), jnp.where(b0 == W2AT, 0, (b0 >> 1) - 1),
                        jnp.logical_or(b0 == W2AT, jnp.logical_and(b0 <= half, (b0 & 1) == 0)))

        first = [pf_w] + [functools.partial(pf_x, k, w) for k in range(RATE) for w in range(2)]
        first += [functools.partial(pf_kv, k) for k in range(RATE)]
        zero = b0 >> 20
        preps = ([functools.partial(prep_w, 1, jnp.where(b0 >= half, m, 3), jnp.maximum(m, 0), (b0 & 1) * 4, 4,
                                    (part, SWPARTS), zero) for part in range(SWPARTS)],
                 [functools.partial(prep_x, jnp.minimum(b0 + 1, nb - 1), br, part, zero)
                  for br in range(2) for part in range(XPARTS)])
        body(b0, 1, (first, [], preps), (SPAT, SQORD, SOORD, SQSPLIT, SOSPLIT), 0, first_hp=True)
        return carry

    def big(par, last, hp, i, carry):
        b0 = i * BB
        g0 = hp * nb + b0

        if not last:
            w_wait(i)

        kvg_wait(i)

        def pf_kv():
            @pl.when(g0 + BB < ng)
            def _():
                kvg_start(g0 + BB)

        if last:
            extra = ([pf_kv], [], ([], []))
        else:
            hn = jnp.where(i == 3, hp + 2, hp + 1)
            extra = ([lambda: w_start_dyn(hn, (i + 1) & 3, hn < nhp)] +
                     [functools.partial(kvg_start, g0 + BB)], [],
                     ([functools.partial(prep_w, 1 - par, i, i, 0, 8, (part, PPARTS), i >> 20)
                       for part in range(PPARTS)], []))
        body(g0, BB, extra, (LPAT, LQORD, LOORD, LQSPLIT, LOSPLIT) if last else (PAT, QORD, OORD, QSPLIT, OSPLIT), par, last_hp=last)
        return carry

    spb = nb // BB
    assert spb == 4 and G1 == nb
    if SKIP_SMALL in (0, 2):
        lax.fori_loop(0, nb, small, 0)
    if SKIP_SMALL == 2:
        prep_x(0, 0)
        acc[0, 0:128, 0:128] = wc[1][0:128, 0:128].astype(f32)
        pltpu.make_async_copy(obuf, o_hbm, o_sem).start()
        pltpu.make_async_copy(obuf, o_hbm, o_sem).wait()
        return

    def pair(t, carry):
        lax.fori_loop(jnp.where(t > 0, 0, spb), spb, functools.partial(big, 0, False, 2 * t), 0)
        lax.fori_loop(0, jnp.where(2 * t + 1 < nhp - 1, spb, 0), functools.partial(big, 1, False, 2 * t + 1), 0)
        return carry

    if SKIP_SMALL != 3:
        lax.fori_loop(0, nhp // 2, pair, 0)
    else:
        prep_w(1, 0, 0, 0, 8)
    if SKIP_SMALL in (0, 3):
        lax.fori_loop(0, spb, functools.partial(big, 1, True, nhp - 1), 0)
    pltpu.make_async_copy(obuf, o_hbm, o_sem).wait()


@jax.jit
def pallas_concat_heads__gqa_block_cached__mha_block_cached__near_ridge_kernel(
    A_x, A_k_cache, A_v_cache, A_wq, A_wo, B_x, B_k_cache, B_v_cache, B_wq, B_wo):
    B, Sq, D = A_x.shape
    _, H, Sk, Dh = A_k_cache.shape
    nhp = H // 2
    assert B == 16 and G1 % B == 0 and 2 * BB <= B and C0 >= 1
    n_iss = C0
    for g0 in range(G1):
        assert n_iss >= min(g0 + 2, G1 + BB), (g0, n_iss)
        hi = min(RATE * (g0 + 1) + C0, g0 + LA, G1 + BB)
        assert 0 <= hi - n_iss <= RATE
        n_iss = hi
    assert n_iss == G1 + BB, n_iss
    assert 10 <= W2AT <= 15 and 5 <= LA <= B

    def tr(c):
        return jnp.swapaxes(c, 2, 3).reshape(B, nhp, 2 * Dh, Sk)

    any_spec = pl.BlockSpec(memory_space=pl.ANY)
    return pl.pallas_call(
        functools.partial(_kernel, scale=Dh ** -0.5 * LOG2E, nhp=nhp, nb=B),
        in_specs=[any_spec] * 10,
        out_specs=any_spec,
        out_shape=jax.ShapeDtypeStruct((B, Sq, 2 * D), A_x.dtype),
        scratch_shapes=[pltpu.VMEM((B, ACCR, 2 * D), f32),
                        pltpu.VMEM((B, 2, D // 128, Sq // 2, 128), u32),
                        pltpu.VMEM((4 * 15 * 64, 128), u32),
                        pltpu.VMEM((B, 4, 2 * Dh, Sk), bf16),
                        pltpu.VMEM((B, Sq, 2 * D), bf16),
                        pltpu.VMEM((2 * BB * Sq, 6 * 128), u32),
                        pltpu.VMEM((2 * BB * Sq // 4, 6 * 128), u32),
                        pltpu.VMEM((B * 2 * Sq // 4, XCW * 128), u32),
                        pltpu.VMEM((4 * 64, WCW * 128), u32),
                        pltpu.VMEM((4 * 64, WCW * 128), u32),
                        pltpu.SemaphoreType.DMA((B + 4,)),
                        pltpu.SemaphoreType.DMA((B,)),
                        pltpu.SemaphoreType.DMA((4,)),
                        pltpu.SemaphoreType.DMA(())],
        compiler_params=pltpu.CompilerParams(
            disable_bounds_checks=True,
            vmem_limit_bytes=110 * 1024 * 1024),
    )(A_x, tr(A_k_cache), tr(A_v_cache), A_wq, A_wo, B_x, tr(B_k_cache), tr(B_v_cache), B_wq, B_wo)
```

```python
import functools
import jax
import jax.numpy as jnp
from jax import lax
import jax.experimental.pallas as pl
import jax.experimental.pallas.tpu as pltpu

BB = 4
G1 = 16
C0 = 2
RATE = 2
PFPOS = 1
PFSTEP = 3
PSKIP = 2
OBUF = 1
SKIP_SMALL = 0
KVTOP = 8
QSPLIT = 11
OSPLIT = 10
PPARTS = 25
PEND = 10
XCW = 32
WCW = 40
ACCR = 160
WQT = 3
WOT = 5
MERGE = 0
TOK = 1
W2AT = 11
LA = 6
XPARTS = 25
SWPARTS = 12
QCH = 80
QD = 9999
QS = 60
PCH = 160
SD = 9999
SS = 40
PLO = 300
PHI = 400
SWLO = 60
SWHI = 1080
SXLO = 1700
SXHI = 120
DIST = 2
LB = 2
LC = 6
VNOCSE = 1
SQSPLIT = 13
SOSPLIT = 13
LQSPLIT = 11
LOSPLIT = 10
NOCSE = 1
PAT = "s00:0,qa:2,s01:0,m1:-1,t1:-1,s10:0,oa:-2,qb:2,s11:0,m0:0,t0:0,ob:-2"
SPAT = "qa@0,qb@0,qa@1,s00@0,s10@0,s11@0,s01@0,qb@1,m1@0,m0@0,t0@0,s00@1,s01@1,t1@0,s10@1,s11@1,oa@0,m0@1,m1@1,t0@1,t1@1,ob@0,oa@1,ob@1"
LOG2E = 1.4426950408889634
bf16 = jnp.bfloat16
f32 = jnp.float32
u32 = jnp.uint32
NT = (((1,), (1,)), ((), ()))

O_LHS_PROG = [(100, 4, 5, 1), (101, 0, 1, -1), (102, 3, 101, 1), (103, 2, 100, 1), (104, 0, 3, 1), (105, 2, 3, -1), (106, 0, 2, 1), (107, 2, 101, -1), (108, 3, 5, 1), (109, 1, 103, 1), (110, 2, 5, 1), (111, 3, 100, -1), (112, 5, 101, 1), (113, 4, 102, -1), (114, 0, 100, 1)]
O_OUT_PROG = [(100, 5, 8, -1), (101, 3, 100, 1), (102, 2, 7, -1), (103, 0, 102, 1)]
O_PRODS = [((101, 1), [(2, 1), (5, 1), (10, -1), (12, 1)], [(102, 1)]), ((104, 1), [(3, 1)], [(100, -1)]), ((111, 1), [(0, 1), (3, 1)], [(5, 1)]), ((5, 1), [(5, 1), (10, -1)], [(5, -1), (103, 1)]), ((112, 1), [(5, 1), (10, -1), (12, 1)], [(103, -1)]), ((114, 1), [(0, 1), (3, 1), (5, 1)], [(101, 1)]), ((0, 1), [(0, 1), (5, 1)], [(0, 1), (101, -1)]), ((107, -1), [(10, 1), (12, -1)], [(0, -1)]), ((110, 1), [(12, 1)], [(0, 1), (2, 1)]), ((1, 1), [(2, 1), (7, 1)], [(2, 1), (4, -1)]), ((104, 1), [(1, 1), (2, 1), (4, 1), (7, 1), (9, 1)], [(4, 1)]), ((106, 1), [(1, 1)], [(1, 1), (4, -1)]), ((1, 1), [(6, 1)], [(1, 1), (3, -1)]), ((109, 1), [(6, 1), (8, 1)], [(3, 1)]), ((2, 1), [(1, 1), (11, -1)], [(1, -1), (6, 1)]), ((103, 1), [(6, 1), (8, 1), (13, -1)], [(3, -1), (6, 1)]), ((100, 1), [(0, 1), (3, 1), (5, 1), (13, 1)], [(3, -1), (8, 1)]), ((4, 1), [(8, 1), (13, -1)], [(6, -1), (8, 1)]), ((110, 1), [(6, 1), (8, 1), (11, -1), (13, -1), (14, -1)], [(6, -1)]), ((105, 1), [(1, 1), (14, 1)], [(4, 1), (6, -1)]), ((108, 1), [(14, 1)], [(6, -1), (9, 1)]), ((3, 1), [(4, 1), (14, -1)], [(4, -1), (9, 1)]), ((4, 1), [(9, 1)], [(7, -1), (9, 1)]), ((102, 1), [(2, 1), (7, 1), (9, 1)], [(4, -1), (7, 1)]), ((113, -1), [(7, 1), (9, 1)], [(7, -1)])]
Q_LHS_PROG = [(100, 3, 8, -1), (101, 0, 2, 1), (102, 7, 101, -1), (103, 5, 100, 1), (104, 4, 6, -1), (105, 4, 9, -1), (106, 7, 9, -1), (107, 0, 103, -1), (108, 6, 8, -1), (109, 5, 102, 1), (110, 1, 4, -1), (111, 5, 8, -1), (112, 6, 9, -1), (113, 4, 7, -1), (114, 2, 4, -1), (115, 1, 6, -1), (116, 2, 7, -1), (117, 1, 3, -1), (118, 3, 6, -1)]
Q_OUT_PROG = [(100, 0, 3, 1), (101, 4, 5, 1), (102, 0, 1, -1), (103, 2, 101, 1), (104, 2, 5, 1), (105, 1, 100, -1)]
Q_PRODS = [((6, -1), [(6, 1), (8, 1), (11, -1), (13, -1), (14, -1)], [(104, 1)]), ((101, 1), [(12, 1)], [(104, 1)]), ((4, 1), [(1, 1), (2, 1), (4, 1), (7, 1), (9, 1)], [(100, 1)]), ((111, -1), [(3, 1)], [(100, 1)]), ((118, -1), [(6, 1), (8, 1), (13, -1)], [(103, 1)]), ((3, 1), [(6, 1), (8, 1)], [(1, 1), (103, 1)]), ((114, 1), [(2, 1), (7, 1)], [(1, 1)]), ((117, 1), [(6, 1)], [(1, 1)]), ((115, -1), [(1, 1), (11, -1)], [(2, 1)]), ((0, -1), [(10, 1), (12, -1)], [(2, -1), (102, 1)]), ((116, 1), [(2, 1), (5, 1), (10, -1), (12, 1)], [(102, 1)]), ((102, 1), [(5, 1), (10, -1), (12, 1)], [(5, 1), (102, 1)]), ((109, -1), [(5, 1), (10, -1)], [(5, 1)]), ((112, -1), [(14, 1)], [(3, 1), (5, 1)]), ((104, 1), [(1, 1), (14, 1)], [(2, 1), (3, -1)]), ((105, -1), [(4, 1), (14, -1)], [(3, 1)]), ((5, 1), [(0, 1), (3, 1)], [(3, 1), (101, -1)]), ((100, -1), [(0, 1), (3, 1), (5, 1), (13, 1)], [(101, 1)]), ((103, 1), [(0, 1), (3, 1), (5, 1)], [(0, 1), (101, 1)]), ((110, 1), [(1, 1)], [(0, 1), (2, 1)]), ((107, 1), [(0, 1), (5, 1)], [(0, 1)]), ((113, -1), [(2, 1), (7, 1), (9, 1)], [(105, -1)]), ((7, -1), [(7, 1), (9, 1)], [(4, -1), (105, -1)]), ((106, -1), [(9, 1)], [(4, 1)]), ((108, -1), [(8, 1), (13, -1)], [(4, 1)])]
NPROD = len(O_PRODS)


def _normalize(prods):
    out = []
    for (var, sgn), w, g in prods:
        sgn *= w[0][1]
        out.append((var, [(y, c * w[0][1]) for y, c in w], [(z, c * sgn) for z, c in g]))
    return out


OORD = "0.6.1.5.3.2.8.9.4.24.11.12.14.10.16.19.13.15.17.18.20.22.21.23.7"
QORD = "9.15.16.24.19.20.21.1.18.22.17.23.2.0.3.7.4.5.8.6.14.12.10.11.13"
SOORD = "7.22.23.20.19.18.16.17.21.15.13.12.10.11.14.9.8.24.6.5.2.3.4.0.1"
SQORD = "3.16.17.15.18.10.20.21.24.7.22.1.23.6.2.0.14.8.4.5.9.19.11.12.13"
LOORD = OORD
LQORD = QORD
LPAT = PAT
O_PRODS = _normalize(O_PRODS)
Q_PRODS = _normalize(Q_PRODS)
W_FORMS = [p[1] for p in O_PRODS]


def _positive_outputs(prods, prog):
    for flips in range(1 << 6):
        sg = [(-1 if (flips >> (r % 6)) & 1 else 1) for r in range(len(prods))]
        pos = {}
        for r, p in enumerate(prods):
            for z, c in p[2]:
                pos[z] = max(pos.get(z, -1), c * sg[r])
        for t, a, b, s in reversed(prog):
            st = pos.pop(t)
            pos[a] = max(pos.get(a, -1), st)
            pos[b] = max(pos.get(b, -1), st * s)
        if min(pos.values()) > 0:
            return sg
    raise AssertionError


Q_SIGN = _positive_outputs(Q_PRODS, Q_OUT_PROG)
Q_PRODS = [(v, w, [(z, c * s) for z, c in g]) for (v, w, g), s in zip(Q_PRODS, Q_SIGN)]


def _make_lhs(block, prog):
    vals = {}

    def get(v):
        if v not in vals:
            vals[v] = block(v)
        return vals[v]

    for t, a, b, s in prog:
        vals[t] = get(a) + get(b) if s > 0 else get(a) - get(b)
    return get


def _acc_add(accs, z, sgn, m):
    if z not in accs:
        accs[z] = (sgn, m)
    else:
        s0, a = accs[z]
        accs[z] = (s0, a + m) if s0 == sgn else ((1, a - m) if s0 > 0 else (1, m - a))


def _bilinear_run(accs, prods, which, lhs_of, w_of, tick):
    for r in which:
        m = tick(jnp.dot(lhs_of(r), w_of(r), preferred_element_type=f32), 20)
        for z, c in prods[r][2]:
            _acc_add(accs, z, c, m)


def _bilinear_finish(accs, prog):
    for t, a, b, s in reversed(prog):
        st, v = accs.pop(t)
        _acc_add(accs, a, st, v)
        _acc_add(accs, b, st * s, v)
    return accs


def _mul(i, n):
    return i * n if isinstance(i, int) else pl.multiple_of(i * n, 16)


def _as_bf16(packed):
    return pltpu.bitcast(packed, bf16)


def _as_f32(packed):
    return pltpu.bitcast(packed, bf16).astype(f32)


def _q_operands(c):
    assert all(s > 0 for row in c for s, _ in row)
    (t0, t1, t2), (b0, b1, b2) = [[a for _, a in row] for row in c]
    lo = lax.broadcasted_iota(jnp.int32, t0.shape, 1) < 64
    return [[jnp.where(lo, t0, b0), jnp.where(lo, t1, t0 - b0), jnp.where(lo, b0 - t0, pltpu.roll(b1, 64, 1))],
            [jnp.where(lo, t2, b2), jnp.where(lo, pltpu.roll(t1, 64, 1), t2 - b2), jnp.where(lo, b2 - t2, b1)]]


def _scores_half(qh, kt, h, j, tick):
    k0, k1, k2 = (0, 64, 128) if h == 0 else (256, 320, 192)
    out = []
    for c in (2 * j, 2 * j + 1):
        cs = slice(c * 128, (c + 1) * 128)
        w = [kt[k0:k0 + 128, cs],
             jnp.concatenate([kt[k2:k2 + 64, cs], kt[k1:k1 + 64, cs]], axis=0),
             jnp.concatenate([kt[k0:k0 + 64, cs], kt[k2:k2 + 64, cs]], axis=0)]
        m = [tick(jnp.dot(qh[i], w[i], preferred_element_type=f32), 20) for i in range(3)]
        out.append(jnp.concatenate([m[0] + m[1], m[0] + m[2]], axis=0))
    return out


def _softmax(s):
    m = jnp.max(s, axis=1, keepdims=True)
    p = jnp.exp2(s - m)
    p0, p1, p2, p3 = (p[:, i * 128:(i + 1) * 128] for i in range(4))
    s01, s23 = p0 + p1, p2 + p3
    t = s01 + s23
    l = jnp.sum(t, axis=1, keepdims=True)
    r = pl.reciprocal(l, approx=True)
    r = r * (2.0 - l * r)
    return jnp.concatenate([s01, jnp.minimum(s23, t), p0, p2, p1, p3], axis=1).astype(bf16), r


def _pv_weights(vt, h, i):
    d0, d1, d2 = (0, 64, 128) if h == 0 else (256, 320, 192)

    def v(d, c):
        return vt[d:d + 64, c * 128:(c + 1) * 128]

    def f(d, c):
        return v(d, c).astype(f32)

    if i == 0:
        return jnp.concatenate([jnp.concatenate([v(d0, c), v(d1, c + 1)], axis=0) for c in (0, 2)], axis=1)
    if i == 1:
        w = [jnp.concatenate([f(d2, c), f(d1, c) - f(d1, c + 1)], axis=0) for c in (0, 2)]
    else:
        w = [jnp.concatenate([f(d0, c + 1) - f(d0, c), f(d2, c + 1)], axis=0) for c in (0, 2)]
    return jnp.concatenate(w, axis=1).astype(bf16)


def _schedule(nu, pat):
    if "@" in pat:
        return [(a.split("@")[0], int(a.split("@")[1])) for a in pat.split(",")]
    pat = [(a.split(":")[0], int(a.split(":")[1])) for a in pat.split(",")]
    order = []
    for t in range(-6, nu + 6):
        for name, lag in pat:
            u = t + lag
            if 0 <= u < nu:
                order.append((name, u))
    return order


def _kernel(ax, ak, av, awq, awo, bx, bk, bv, bwq, bwo, o_hbm,
            acc, x32, w32, kvbuf, obuf, pbuf, qbuf, xc32, wc0, wc1,
            kv_sem, x_sem, w_sem, o_sem, *, scale, nhp, nb):
    xbuf, wbuf = (r.bitcast(bf16) for r in (x32, w32))
    pbuf, qbuf, xc = (r.bitcast(bf16) for r in (pbuf, qbuf, xc32))
    wc = [r.bitcast(bf16) for r in (wc0, wc1)]
    sq = xbuf.shape[3]
    hq = sq // 2
    d = awq.shape[0]
    hw = kvbuf.shape[2]
    wrows = wbuf.shape[0] // 4
    ng = nhp * nb
    lg = nb.bit_length() - 1
    assert nb == 1 << lg

    def kv_start(g, which=(0, 1, 2, 3)):
        hp, b = (g >> lg) & (nhp - 1), g & (nb - 1)
        for i, src in enumerate((ak, av, bk, bv)):
            if i in which:
                sem = kv_sem.at[jnp.where(g < nb, b, nb + (b >> 2))]
                pltpu.make_async_copy(src.at[b, hp], kvbuf.at[b, i], sem).start()

    def kv_wait(b):
        pltpu.make_async_copy(kvbuf.at[b], kvbuf.at[b], kv_sem.at[b]).wait()

    def kvg_start(g):
        hp, i4 = g >> lg, (g >> 2) & 3
        b = pl.multiple_of(i4 * BB, BB)
        for i, src in enumerate((ak, av, bk, bv)):
            pltpu.make_async_copy(src.at[pl.ds(b, BB), hp], kvbuf.at[pl.ds(b, BB), i], kv_sem.at[nb + i4]).start()

    def kvg_wait(i4):
        v = kvbuf.at[pl.ds(i4 * BB, BB)]
        pltpu.make_async_copy(v, v, kv_sem.at[nb + i4]).wait()

    def x_start(b, which=(0, 1)):
        for i, src in enumerate((ax, bx)):
            if i in which:
                for c in range(xbuf.shape[2]):
                    pltpu.make_async_copy(src.at[b, :, pl.ds(c * 128, 128)], xbuf.at[b, i, c], x_sem.at[b]).start()

    def x_wait(b):
        pltpu.make_async_copy(xbuf.at[b], xbuf.at[b], x_sem.at[b]).wait()

    def w_start(h, m):
        off = h * hw if isinstance(h, int) else pl.multiple_of(h * hw, 128)
        if m < 2:
            for c in range(hw // 128):
                pltpu.make_async_copy((awq, bwq)[m].at[:, pl.ds(off + c * 128, 128)],
                                      wbuf.at[pl.ds(m * wrows + c * d, d)], w_sem.at[m]).start()
        else:
            for c in range(d // 128):
                pltpu.make_async_copy((awo, bwo)[m - 2].at[pl.ds(off, hw), pl.ds(c * 128, 128)],
                                      wbuf.at[pl.ds(m * wrows + c * hw, hw)], w_sem.at[m]).start()

    def w_start_dyn(h, m, valid):
        for k in range(4):
            @pl.when(jnp.logical_and(m == k, valid))
            def _():
                w_start(h, k)

    def w_wait(m):
        v = wbuf.at[pl.ds(_mul(m, wrows), wrows)]
        pltpu.make_async_copy(v, v, w_sem.at[m]).wait()

    def prep_w(dst, msrc, mdst, row, nrows, part=None, zero=None):
        if isinstance(msrc, int):
            sa, sc = (5, 1) if msrc < 2 else (1, 3)
            off = [(msrc * 15 + (y // 5) * sa + (y % 5) * sc) * 64 + row * 8 for y in range(15)]
        else:
            sa, sc = jnp.where(msrc < 2, 5, 1), jnp.where(msrc < 2, 1, 3)
            off = [pl.multiple_of((msrc * 15 + (y // 5) * sa + (y % 5) * sc) * 64 + row * 8, 64 if isinstance(row, int) and row == 0 else 32)
                   for y in range(15)]
        r16 = _mul(mdst * 8 + row, 16)
        if not isinstance(r16, int):
            r16 = pl.multiple_of(r16, 128 if isinstance(row, int) and row == 0 else 64)
        for r, form in enumerate(W_FORMS):
            if part is not None and r % part[1] != part[0]:
                continue
            if len(form) == 1:
                val = _as_bf16(w32[pl.ds(off[form[0][0]], nrows * 8), :])
            else:
                val = None
                for y, c in form:
                    t = _as_f32(w32[pl.ds(off[y], nrows * 8), :])
                    val = t if val is None else (val + t if c > 0 else val - t)
                val = val.astype(bf16)
            wc[dst][pl.ds(r16, nrows * 16), r * 128:(r + 1) * 128] = val
        if zero is not None:
            c0 = part[0] * 128
            return lambda: wc[dst][pl.ds(pl.multiple_of(r16 + zero * 16, 16), 16), c0:c0 + 128].astype(f32)[0:8]

    def prep_x(b, br, part=None, zero=None):
        get = _make_lhs(
            lambda z: _as_f32(x32[b, br, z % 5, (z // 5) * (hq // 2):(z // 5 + 1) * (hq // 2), :]) * scale,
            Q_LHS_PROG)
        for r, p in enumerate(Q_PRODS):
            if part is not None and r * XPARTS // NPROD != part:
                continue
            c0 = r * 128
            xc[pl.ds(_mul(b * 2 + br, hq), hq), r * 128:(r + 1) * 128] = (get(p[0]) * Q_SIGN[r]).astype(bf16)
        if zero is not None:
            return lambda: xc[pl.ds(_mul(b * 2 + br + zero, hq), 16), c0:c0 + 128].astype(f32)[0:8]

    def body(g0, nbat, extra, pat, cs, first_hp=False, last_hp=False):
        hp = g0 >> lg
        b0 = g0 & (nb - 1)
        R, O, OT, OC = {}, {}, {}, {}

        def prow(u, h):
            return (2 * u + h) * sq

        def weights(m, prods):
            def w_of(r):
                s = W_FORMS.index(prods[r][1])
                return wc[cs][m * 128:(m + 1) * 128, s * 128:(s + 1) * 128]
            return w_of

        QA, OA, SC, LH = {}, {}, {}, {}
        pending = []
        clock = [0]
        zero16 = pl.multiple_of((g0 >> 20) * 16, 16)

        def later(key, delay, emit):
            pending.append((clock[0] + delay, key, emit))
            pending.sort(key=lambda e: e[0])

        def flush(key):
            for e in [e for e in pending if e[1] == key]:
                pending.remove(e)
                e[2]()

        def tick(o, cycles):
            t0 = clock[0]
            clock[0] += cycles
            groups = o.shape[0] // 8
            rows = None
            while pending and pending[0][0] <= clock[0]:
                due, _, emit = pending.pop(0)
                tok = emit()
                if tok is None or not TOK:
                    continue
                g = min(max((due - t0) * groups // cycles, 0), groups - 1)
                rows = rows or [o[8 * i:8 * i + 8] for i in range(groups)]
                rows[g] = jnp.minimum(rows[g], jnp.maximum(rows[g], tok()))
            return o if rows is None else jnp.concatenate(rows, axis=0)

        pat, qord, oord, qsp, osp = pat
        qord = [int(i) for i in qord.split(".")]
        oord = [int(i) for i in oord.split(".")]

        def q_(u, lo_, hi_):
            b, br = b0 + u // 2, u % 2

            def lhs_of(r):
                return xc[pl.ds(_mul(b * 2 + br, hq), hq), r * 128:(r + 1) * 128]

            _bilinear_run(QA.setdefault(u, {}), Q_PRODS, qord[lo_:hi_], lhs_of, weights(br, Q_PRODS), tick)
            if hi_ == len(Q_PRODS):
                fin = _bilinear_finish(QA[u], Q_OUT_PROG)
                c = [[fin[i * 3 + n] for n in range(3)] for i in range(2)]
                nch = hq // QCH

                def chunk(k):
                    ck = [[(s, a[k * QCH:(k + 1) * QCH]) for s, a in row] for row in c]
                    r0 = u * hq + k * QCH
                    for h, ops in enumerate(_q_operands(ck)):
                        for i, a in enumerate(ops):
                            qbuf[r0:r0 + QCH, (3 * h + i) * 128:(3 * h + i + 1) * 128] = a.astype(bf16)
                    return lambda: qbuf[pl.ds(r0 + zero16, 16), 0:128].astype(f32)[0:8]

                for k in range(nch):
                    later(("q", u), QD + k * QS, functools.partial(chunk, k))

        def s_(u, h, j):
            b, br = b0 + u // 2, u % 2
            flush(("q", u))
            qh = [qbuf[u * hq:(u + 1) * hq, (3 * h + i) * 128:(3 * h + i + 1) * 128] for i in range(3)]
            SC[u, h, j] = _scores_half(qh, kvbuf.at[b, 2 * br], h, j, tick)
            if j == 1:
                s = jnp.concatenate(SC[u, h, 0] + SC[u, h, 1], axis=1)
                R[u, h] = []

                def chunk(k):
                    p, r = _softmax(s[k * PCH:(k + 1) * PCH])
                    R[u, h].append(r)
                    r0 = prow(u, h) + k * PCH
                    pbuf[r0:r0 + PCH, :] = p
                    return lambda: pbuf[pl.ds(r0 + zero16, 16), 0:128].astype(f32)[0:8]

                for k in range(sq // PCH):
                    later(("p", u, h), SD + k * SS, functools.partial(chunk, k))

        def rinv(u, h):
            return jnp.concatenate(R[u, h], axis=0)

        def m_(u, h, half):
            flush(("p", u, h))
            vt = kvbuf.at[b0 + u // 2 + (g0 >> 20) * half * VNOCSE, 2 * (u % 2) + 1]
            r0 = prow(u, h) + half * hq
            res = [tick(lax.dot_general(pbuf[r0:r0 + hq, i * 256:(i + 1) * 256], _pv_weights(vt, h, i), NT,
                                        preferred_element_type=f32), 40) for i in range(3)]
            lo = lax.broadcasted_iota(jnp.int32, (hq, 128), 1) < 64
            r = rinv(u, h)[half * hq:(half + 1) * hq]
            O[u, h, half] = (res[0] + jnp.where(lo, res[2], res[1])) * r
            OT[u, h, half] = jnp.where(lo, res[1], res[2]) * r

        def o_(u, lo_, hi_):
            b, br = b0 + u // 2, u % 2
            if lo_ == 0:
                lo = lax.broadcasted_iota(jnp.int32, (hq, 128), 1) < 64
                mid = [jnp.where(lo, OT[u, 0, i], OT[u, 1, i]) +
                       pltpu.roll(jnp.where(lo, OT[u, 1, i], OT[u, 0, i]), 64, 1) for i in range(2)]
                tiles = [[O[u, 0, i], mid[i], O[u, 1, i]] for i in range(2)]
                get = _make_lhs(lambda x: tiles[x // 3][x % 3], O_LHS_PROG)
                LH[u] = {p[0]: get(p[0]).astype(bf16) for p in O_PRODS}
            _bilinear_run(OA.setdefault(u, {}), O_PRODS, oord[lo_:hi_], lambda r: LH[u][O_PRODS[r][0]],
                          weights(2 + br, O_PRODS), tick)
            fin = _bilinear_finish(OA[u], O_OUT_PROG) if hi_ == NPROD else {}
            for n in (range(5) if fin else ()):
                for i in range(2):
                    s, a = fin[i * 5 + n]
                    rows = slice(i * hq, (i + 1) * hq)
                    cols = slice(br * d + n * 128, br * d + (n + 1) * 128)
                    if first_hp:
                        new = a if s > 0 else -a
                    else:
                        new = acc[b, rows, cols] + a if s > 0 else acc[b, rows, cols] - a
                    if last_hp:
                        obuf[b, rows, cols] = new.astype(obuf.dtype)
                    if not last_hp:
                        acc[b, rows, cols] = new
            if br == 1 and lo_ > 0 and last_hp:
                pltpu.make_async_copy(obuf.at[b], o_hbm.at[b], o_sem).start()

        fns = {"qa": lambda u: q_(u, 0, qsp), "qb": lambda u: q_(u, qsp, NPROD),
               "oa": lambda u: o_(u, 0, osp), "ob": lambda u: o_(u, osp, NPROD),
               "s00": lambda u: s_(u, 0, 0), "s01": lambda u: s_(u, 0, 1),
               "s10": lambda u: s_(u, 1, 0), "s11": lambda u: s_(u, 1, 1),
               "m0": lambda u: m_(u, 0, 0), "m1": lambda u: m_(u, 1, 0),
               "t0": lambda u: m_(u, 0, 1), "t1": lambda u: m_(u, 1, 1), "c": lambda u: None}
        sched = _schedule(2 * nbat, pat)
        first, dmas, preps = extra
        for f in first:
            f()
        total = 2 * nbat * 1960
        lastq = max(i for i, it in enumerate(sched) if it[0][0] == "q")
        wpre, xpre = preps
        for k, f in enumerate(wpre):
            lo_, hi_ = (PLO, total - PHI) if nbat > 1 else (SWLO, SWHI)
            later("w", lo_ + k * (hi_ - lo_) // len(wpre), f)
        for i, item in enumerate(sched):
            fns[item[0]](item[1])
            if i == lastq:
                for k, f in enumerate(xpre):
                    later("x", SXLO + k * (total - SXHI - clock[0] - SXLO) // len(xpre), f)
        flush("w")
        flush("x")
        assert not pending

    for k in range(4):
        w_start(0, k)
    x_start(0)
    kv_start(0)
    x_start(1)
    for g in range(1, C0):
        kv_start(g)
        x_start(g + 1)
    for m in range(4):
        w_wait(m)
        prep_w(0, m, m, 0, 8)
    x_wait(0)
    for br in range(2):
        prep_x(0, br)

    def issued(g):
        return jnp.minimum(jnp.minimum(RATE * (g + 1) + C0, jnp.maximum(g + LA, LB * g - LC)), G1 + DIST * BB)

    def small(b0, carry):
        half = nb // 2
        m = (b0 - half) >> 1

        @pl.when(b0 + 1 < nb)
        def _():
            x_wait(b0 + 1)

        @pl.when(jnp.logical_and(b0 >= half, (b0 & 1) == 0))
        def _():
            w_wait(m)

        kv_wait(b0)

        hi = issued(b0)
        prev = jnp.where(b0 == 0, C0, issued(b0 - 1))

        def pf_x(k, w):
            @pl.when(jnp.logical_and(prev + k < hi, prev + k + 1 < nb))
            def _():
                x_start(prev + k + 1, (w,))

        def pf_kv(k):
            @pl.when(prev + k < hi)
            def _():
                kv_start(prev + k)

        def pf_w():
            w_start_dyn(jnp.where(b0 == W2AT, 2, 1), jnp.where(b0 == W2AT, 0, (b0 >> 1) - 1),
                        jnp.logical_or(b0 == W2AT, jnp.logical_and(b0 <= half, (b0 & 1) == 0)))

        first = [pf_w] + [functools.partial(pf_x, k, w) for k in range(RATE) for w in range(2)]
        first += [functools.partial(pf_kv, k) for k in range(RATE)]
        zero = b0 >> 20
        preps = ([functools.partial(prep_w, 1, jnp.where(b0 >= half, m, 3), jnp.maximum(m, 0), (b0 & 1) * 4, 4,
                                    (part, SWPARTS), zero) for part in range(SWPARTS)],
                 [functools.partial(prep_x, jnp.minimum(b0 + 1, nb - 1), br, part, zero)
                  for br in range(2) for part in range(XPARTS)])
        body(b0, 1, (first, [], preps), (SPAT, SQORD, SOORD, SQSPLIT, SOSPLIT), 0, first_hp=True)
        return carry

    def big(par, last, hp, i, carry):
        b0 = i * BB
        g0 = hp * nb + b0

        if not last:
            w_wait(i)

        kvg_wait(i)

        def pf_kv():
            @pl.when(g0 + DIST * BB < ng)
            def _():
                kvg_start(g0 + DIST * BB)

        if last:
            extra = ([pf_kv], [], ([], []))
        else:
            hn = jnp.where(i == 3, hp + 2, hp + 1)
            extra = ([lambda: w_start_dyn(hn, (i + 1) & 3, hn < nhp)] +
                     [functools.partial(kvg_start, g0 + DIST * BB)], [],
                     ([functools.partial(prep_w, 1 - par, i, i, 0, 8, (part, PPARTS), i >> 20)
                       for part in range(PPARTS)], []))
        body(g0, BB, extra, (LPAT, LQORD, LOORD, LQSPLIT, LOSPLIT) if last else (PAT, QORD, OORD, QSPLIT, OSPLIT), par, last_hp=last)
        return carry

    spb = nb // BB
    assert spb == 4 and G1 == nb
    if SKIP_SMALL in (0, 2):
        lax.fori_loop(0, nb, small, 0)
    if SKIP_SMALL == 2:
        prep_x(0, 0)
        acc[0, 0:128, 0:128] = wc[1][0:128, 0:128].astype(f32)
        pltpu.make_async_copy(obuf, o_hbm, o_sem).start()
        pltpu.make_async_copy(obuf, o_hbm, o_sem).wait()
        return

    def pair(t, carry):
        lax.fori_loop(jnp.where(t > 0, 0, spb), spb, functools.partial(big, 0, False, 2 * t), 0)
        lax.fori_loop(0, jnp.where(2 * t + 1 < nhp - 1, spb, 0), functools.partial(big, 1, False, 2 * t + 1), 0)
        return carry

    if SKIP_SMALL != 3:
        lax.fori_loop(0, nhp // 2, pair, 0)
    else:
        prep_w(1, 0, 0, 0, 8)
    if SKIP_SMALL in (0, 3):
        lax.fori_loop(0, spb, functools.partial(big, 1, True, nhp - 1), 0)
    pltpu.make_async_copy(obuf, o_hbm, o_sem).wait()


@jax.jit
def pallas_concat_heads__gqa_block_cached__mha_block_cached__near_ridge_kernel(
    A_x, A_k_cache, A_v_cache, A_wq, A_wo, B_x, B_k_cache, B_v_cache, B_wq, B_wo):
    B, Sq, D = A_x.shape
    _, H, Sk, Dh = A_k_cache.shape
    nhp = H // 2
    assert B == 16 and G1 % B == 0 and 2 * BB <= B and C0 >= 1
    n_iss = C0
    for g0 in range(G1):
        assert n_iss >= g0 + 2, (g0, n_iss)
        hi = min(RATE * (g0 + 1) + C0, max(g0 + LA, LB * g0 - LC), G1 + DIST * BB)
        assert hi <= g0 + B
        assert 0 <= hi - n_iss <= RATE
        n_iss = hi
    assert n_iss == G1 + DIST * BB, n_iss
    assert 10 <= W2AT <= 15 and 5 <= LA <= B

    def tr(c):
        return jnp.swapaxes(c, 2, 3).reshape(B, nhp, 2 * Dh, Sk)

    any_spec = pl.BlockSpec(memory_space=pl.ANY)
    return pl.pallas_call(
        functools.partial(_kernel, scale=Dh ** -0.5 * LOG2E, nhp=nhp, nb=B),
        in_specs=[any_spec] * 10,
        out_specs=any_spec,
        out_shape=jax.ShapeDtypeStruct((B, Sq, 2 * D), A_x.dtype),
        scratch_shapes=[pltpu.VMEM((B, ACCR, 2 * D), f32),
                        pltpu.VMEM((B, 2, D // 128, Sq // 2, 128), u32),
                        pltpu.VMEM((4 * 15 * 64, 128), u32),
                        pltpu.VMEM((B, 4, 2 * Dh, Sk), bf16),
                        pltpu.VMEM((B, Sq, 2 * D), bf16),
                        pltpu.VMEM((2 * BB * Sq, 6 * 128), u32),
                        pltpu.VMEM((2 * BB * Sq // 4, 6 * 128), u32),
                        pltpu.VMEM((B * 2 * Sq // 4, XCW * 128), u32),
                        pltpu.VMEM((4 * 64, WCW * 128), u32),
                        pltpu.VMEM((4 * 64, WCW * 128), u32),
                        pltpu.SemaphoreType.DMA((B + 4,)),
                        pltpu.SemaphoreType.DMA((B,)),
                        pltpu.SemaphoreType.DMA((4,)),
                        pltpu.SemaphoreType.DMA(())],
        compiler_params=pltpu.CompilerParams(
            disable_bounds_checks=True,
            vmem_limit_bytes=110 * 1024 * 1024),
    )(A_x, tr(A_k_cache), tr(A_v_cache), A_wq, A_wo, B_x, tr(B_k_cache), tr(B_v_cache), B_wq, B_wo)
```

```python
import functools
import jax
import jax.numpy as jnp
from jax import lax
import jax.experimental.pallas as pl
import jax.experimental.pallas.tpu as pltpu

BB = 4
G1 = 16
C0 = 2
RATE = 2
PFPOS = 1
PFSTEP = 3
PSKIP = 2
OBUF = 1
SKIP_SMALL = 0
KVTOP = 8
QSPLIT = 11
OSPLIT = 10
PPARTS = 25
PEND = 10
XCW = 32
WCW = 40
ACCR = 160
WQT = 3
WOT = 5
MERGE = 0
TOK = 1
W2AT = 11
LA = 6
XPARTS = 25
SWPARTS = 12
QCH = 80
QD = 9999
QS = 60
PCH = 160
SD = 9999
SS = 40
PLO = 300
PHI = 400
SWLO = 60
SWHI = 1080
SXLO = 1700
SXHI = 120
DIST = 2
LB = 2
LC = 6
VNOCSE = 1
SQSPLIT = 13
SOSPLIT = 13
LQSPLIT = 11
LOSPLIT = 10
NOCSE = 1
PAT = "qa@0,qb@0,qa@1,qb@1,qa@2,s00@0,s01@0,s10@0,qb@2,s11@0,m0@0,t0@0,s00@1,qa@3,s01@1,t1@0,s10@1,qb@3,m1@0,s11@1,m0@1,t0@1,s00@2,qa@4,s01@2,m1@1,t1@1,s10@2,oa@0,qb@4,s11@2,m0@2,t0@2,ob@0,s00@3,qa@5,s01@3,t1@2,m1@2,s10@3,oa@1,qb@5,s11@3,m0@3,t0@3,ob@1,s00@4,oa@2,qa@6,s01@4,m1@3,t1@3,s10@4,s11@4,m0@4,t0@4,ob@2,s00@5,qb@6,qa@7,s01@5,m1@4,t1@4,s10@5,oa@3,qb@7,s11@5,m0@5,t0@5,ob@3,s00@6,s01@6,m1@5,t1@5,s10@6,oa@4,s11@6,m0@6,t0@6,ob@4,s00@7,s01@7,m1@6,t1@6,s10@7,oa@5,s11@7,m0@7,t0@7,ob@5,m1@7,t1@7,oa@6,ob@6,oa@7,ob@7"
SPAT = "qa@0,qb@0,qa@1,s00@0,s10@0,s11@0,s01@0,qb@1,m1@0,m0@0,t0@0,s00@1,s01@1,t1@0,s10@1,s11@1,oa@0,m0@1,m1@1,t0@1,t1@1,ob@0,oa@1,ob@1"
LOG2E = 1.4426950408889634
bf16 = jnp.bfloat16
f32 = jnp.float32
u32 = jnp.uint32
NT = (((1,), (1,)), ((), ()))

O_LHS_PROG = [(100, 4, 5, 1), (101, 0, 1, -1), (102, 3, 101, 1), (103, 2, 100, 1), (104, 0, 3, 1), (105, 2, 3, -1), (106, 0, 2, 1), (107, 2, 101, -1), (108, 3, 5, 1), (109, 1, 103, 1), (110, 2, 5, 1), (111, 3, 100, -1), (112, 5, 101, 1), (113, 4, 102, -1), (114, 0, 100, 1)]
O_OUT_PROG = [(100, 5, 8, -1), (101, 3, 100, 1), (102, 2, 7, -1), (103, 0, 102, 1)]
O_PRODS = [((101, 1), [(2, 1), (5, 1), (10, -1), (12, 1)], [(102, 1)]), ((104, 1), [(3, 1)], [(100, -1)]), ((111, 1), [(0, 1), (3, 1)], [(5, 1)]), ((5, 1), [(5, 1), (10, -1)], [(5, -1), (103, 1)]), ((112, 1), [(5, 1), (10, -1), (12, 1)], [(103, -1)]), ((114, 1), [(0, 1), (3, 1), (5, 1)], [(101, 1)]), ((0, 1), [(0, 1), (5, 1)], [(0, 1), (101, -1)]), ((107, -1), [(10, 1), (12, -1)], [(0, -1)]), ((110, 1), [(12, 1)], [(0, 1), (2, 1)]), ((1, 1), [(2, 1), (7, 1)], [(2, 1), (4, -1)]), ((104, 1), [(1, 1), (2, 1), (4, 1), (7, 1), (9, 1)], [(4, 1)]), ((106, 1), [(1, 1)], [(1, 1), (4, -1)]), ((1, 1), [(6, 1)], [(1, 1), (3, -1)]), ((109, 1), [(6, 1), (8, 1)], [(3, 1)]), ((2, 1), [(1, 1), (11, -1)], [(1, -1), (6, 1)]), ((103, 1), [(6, 1), (8, 1), (13, -1)], [(3, -1), (6, 1)]), ((100, 1), [(0, 1), (3, 1), (5, 1), (13, 1)], [(3, -1), (8, 1)]), ((4, 1), [(8, 1), (13, -1)], [(6, -1), (8, 1)]), ((110, 1), [(6, 1), (8, 1), (11, -1), (13, -1), (14, -1)], [(6, -1)]), ((105, 1), [(1, 1), (14, 1)], [(4, 1), (6, -1)]), ((108, 1), [(14, 1)], [(6, -1), (9, 1)]), ((3, 1), [(4, 1), (14, -1)], [(4, -1), (9, 1)]), ((4, 1), [(9, 1)], [(7, -1), (9, 1)]), ((102, 1), [(2, 1), (7, 1), (9, 1)], [(4, -1), (7, 1)]), ((113, -1), [(7, 1), (9, 1)], [(7, -1)])]
Q_LHS_PROG = [(100, 3, 8, -1), (101, 0, 2, 1), (102, 7, 101, -1), (103, 5, 100, 1), (104, 4, 6, -1), (105, 4, 9, -1), (106, 7, 9, -1), (107, 0, 103, -1), (108, 6, 8, -1), (109, 5, 102, 1), (110, 1, 4, -1), (111, 5, 8, -1), (112, 6, 9, -1), (113, 4, 7, -1), (114, 2, 4, -1), (115, 1, 6, -1), (116, 2, 7, -1), (117, 1, 3, -1), (118, 3, 6, -1)]
Q_OUT_PROG = [(100, 0, 3, 1), (101, 4, 5, 1), (102, 0, 1, -1), (103, 2, 101, 1), (104, 2, 5, 1), (105, 1, 100, -1)]
Q_PRODS = [((6, -1), [(6, 1), (8, 1), (11, -1), (13, -1), (14, -1)], [(104, 1)]), ((101, 1), [(12, 1)], [(104, 1)]), ((4, 1), [(1, 1), (2, 1), (4, 1), (7, 1), (9, 1)], [(100, 1)]), ((111, -1), [(3, 1)], [(100, 1)]), ((118, -1), [(6, 1), (8, 1), (13, -1)], [(103, 1)]), ((3, 1), [(6, 1), (8, 1)], [(1, 1), (103, 1)]), ((114, 1), [(2, 1), (7, 1)], [(1, 1)]), ((117, 1), [(6, 1)], [(1, 1)]), ((115, -1), [(1, 1), (11, -1)], [(2, 1)]), ((0, -1), [(10, 1), (12, -1)], [(2, -1), (102, 1)]), ((116, 1), [(2, 1), (5, 1), (10, -1), (12, 1)], [(102, 1)]), ((102, 1), [(5, 1), (10, -1), (12, 1)], [(5, 1), (102, 1)]), ((109, -1), [(5, 1), (10, -1)], [(5, 1)]), ((112, -1), [(14, 1)], [(3, 1), (5, 1)]), ((104, 1), [(1, 1), (14, 1)], [(2, 1), (3, -1)]), ((105, -1), [(4, 1), (14, -1)], [(3, 1)]), ((5, 1), [(0, 1), (3, 1)], [(3, 1), (101, -1)]), ((100, -1), [(0, 1), (3, 1), (5, 1), (13, 1)], [(101, 1)]), ((103, 1), [(0, 1), (3, 1), (5, 1)], [(0, 1), (101, 1)]), ((110, 1), [(1, 1)], [(0, 1), (2, 1)]), ((107, 1), [(0, 1), (5, 1)], [(0, 1)]), ((113, -1), [(2, 1), (7, 1), (9, 1)], [(105, -1)]), ((7, -1), [(7, 1), (9, 1)], [(4, -1), (105, -1)]), ((106, -1), [(9, 1)], [(4, 1)]), ((108, -1), [(8, 1), (13, -1)], [(4, 1)])]
NPROD = len(O_PRODS)


def _normalize(prods):
    out = []
    for (var, sgn), w, g in prods:
        sgn *= w[0][1]
        out.append((var, [(y, c * w[0][1]) for y, c in w], [(z, c * sgn) for z, c in g]))
    return out


OORD = "0.6.1.5.3.2.8.9.4.24.11.12.14.10.16.19.13.15.17.18.20.22.21.23.7"
QORD = "9.15.16.24.19.20.21.1.18.22.17.23.2.0.3.7.4.5.8.6.14.12.10.11.13"
SOORD = "7.22.23.20.18.16.17.19.21.15.13.12.10.11.14.9.2.8.24.6.5.1.3.4.0"
SQORD = "3.16.24.15.18.10.20.21.17.7.22.1.23.6.2.0.14.8.4.5.9.19.11.12.13"
LOORD = OORD
LQORD = QORD
LPAT = PAT
O_PRODS = _normalize(O_PRODS)
Q_PRODS = _normalize(Q_PRODS)
W_FORMS = [p[1] for p in O_PRODS]


def _positive_outputs(prods, prog):
    for flips in range(1 << 6):
        sg = [(-1 if (flips >> (r % 6)) & 1 else 1) for r in range(len(prods))]
        pos = {}
        for r, p in enumerate(prods):
            for z, c in p[2]:
                pos[z] = max(pos.get(z, -1), c * sg[r])
        for t, a, b, s in reversed(prog):
            st = pos.pop(t)
            pos[a] = max(pos.get(a, -1), st)
            pos[b] = max(pos.get(b, -1), st * s)
        if min(pos.values()) > 0:
            return sg
    raise AssertionError


Q_SIGN = _positive_outputs(Q_PRODS, Q_OUT_PROG)
Q_PRODS = [(v, w, [(z, c * s) for z, c in g]) for (v, w, g), s in zip(Q_PRODS, Q_SIGN)]


def _make_lhs(block, prog):
    vals = {}

    def get(v):
        if v not in vals:
            vals[v] = block(v)
        return vals[v]

    for t, a, b, s in prog:
        vals[t] = get(a) + get(b) if s > 0 else get(a) - get(b)
    return get


def _acc_add(accs, z, sgn, m):
    if z not in accs:
        accs[z] = (sgn, m)
    else:
        s0, a = accs[z]
        accs[z] = (s0, a + m) if s0 == sgn else ((1, a - m) if s0 > 0 else (1, m - a))


def _bilinear_run(accs, prods, which, lhs_of, w_of, tick):
    for r in which:
        m = tick(jnp.dot(lhs_of(r), w_of(r), preferred_element_type=f32), 20)
        for z, c in prods[r][2]:
            _acc_add(accs, z, c, m)


def _bilinear_finish(accs, prog):
    for t, a, b, s in reversed(prog):
        st, v = accs.pop(t)
        _acc_add(accs, a, st, v)
        _acc_add(accs, b, st * s, v)
    return accs


def _mul(i, n):
    return i * n if isinstance(i, int) else pl.multiple_of(i * n, 16)


def _as_bf16(packed):
    return pltpu.bitcast(packed, bf16)


def _as_f32(packed):
    return pltpu.bitcast(packed, bf16).astype(f32)


def _q_operands(c):
    assert all(s > 0 for row in c for s, _ in row)
    (t0, t1, t2), (b0, b1, b2) = [[a for _, a in row] for row in c]
    lo = lax.broadcasted_iota(jnp.int32, t0.shape, 1) < 64
    return [[jnp.where(lo, t0, b0), jnp.where(lo, t1, t0 - b0), jnp.where(lo, b0 - t0, pltpu.roll(b1, 64, 1))],
            [jnp.where(lo, t2, b2), jnp.where(lo, pltpu.roll(t1, 64, 1), t2 - b2), jnp.where(lo, b2 - t2, b1)]]


def _scores_half(qh, kt, h, j, tick):
    k0, k1, k2 = (0, 64, 128) if h == 0 else (256, 320, 192)
    out = []
    for c in (2 * j, 2 * j + 1):
        cs = slice(c * 128, (c + 1) * 128)
        w = [kt[k0:k0 + 128, cs],
             jnp.concatenate([kt[k2:k2 + 64, cs], kt[k1:k1 + 64, cs]], axis=0),
             jnp.concatenate([kt[k0:k0 + 64, cs], kt[k2:k2 + 64, cs]], axis=0)]
        m = [tick(jnp.dot(qh[i], w[i], preferred_element_type=f32), 20) for i in range(3)]
        out.append(jnp.concatenate([m[0] + m[1], m[0] + m[2]], axis=0))
    return out


def _softmax(s):
    m = jnp.max(s, axis=1, keepdims=True)
    p = jnp.exp2(s - m)
    p0, p1, p2, p3 = (p[:, i * 128:(i + 1) * 128] for i in range(4))
    s01, s23 = p0 + p1, p2 + p3
    t = s01 + s23
    l = jnp.sum(t, axis=1, keepdims=True)
    r = pl.reciprocal(l, approx=True)
    r = r * (2.0 - l * r)
    return jnp.concatenate([s01, jnp.minimum(s23, t), p0, p2, p1, p3], axis=1).astype(bf16), r


def _pv_weights(vt, h, i):
    d0, d1, d2 = (0, 64, 128) if h == 0 else (256, 320, 192)

    def v(d, c):
        return vt[d:d + 64, c * 128:(c + 1) * 128]

    def f(d, c):
        return v(d, c).astype(f32)

    if i == 0:
        return jnp.concatenate([jnp.concatenate([v(d0, c), v(d1, c + 1)], axis=0) for c in (0, 2)], axis=1)
    if i == 1:
        w = [jnp.concatenate([f(d2, c), f(d1, c) - f(d1, c + 1)], axis=0) for c in (0, 2)]
    else:
        w = [jnp.concatenate([f(d0, c + 1) - f(d0, c), f(d2, c + 1)], axis=0) for c in (0, 2)]
    return jnp.concatenate(w, axis=1).astype(bf16)


def _schedule(nu, pat):
    if "@" in pat:
        return [(a.split("@")[0], int(a.split("@")[1])) for a in pat.split(",")]
    pat = [(a.split(":")[0], int(a.split(":")[1])) for a in pat.split(",")]
    order = []
    for t in range(-6, nu + 6):
        for name, lag in pat:
            u = t + lag
            if 0 <= u < nu:
                order.append((name, u))
    return order


def _kernel(ax, ak, av, awq, awo, bx, bk, bv, bwq, bwo, o_hbm,
            acc, x32, w32, kvbuf, obuf, pbuf, qbuf, xc32, wc0, wc1,
            kv_sem, x_sem, w_sem, o_sem, *, scale, nhp, nb):
    xbuf, wbuf = (r.bitcast(bf16) for r in (x32, w32))
    pbuf, qbuf, xc = (r.bitcast(bf16) for r in (pbuf, qbuf, xc32))
    wc = [r.bitcast(bf16) for r in (wc0, wc1)]
    sq = xbuf.shape[3]
    hq = sq // 2
    d = awq.shape[0]
    hw = kvbuf.shape[2]
    wrows = wbuf.shape[0] // 4
    ng = nhp * nb
    lg = nb.bit_length() - 1
    assert nb == 1 << lg

    def kv_start(g, which=(0, 1, 2, 3)):
        hp, b = (g >> lg) & (nhp - 1), g & (nb - 1)
        for i, src in enumerate((ak, av, bk, bv)):
            if i in which:
                sem = kv_sem.at[jnp.where(g < nb, b, nb + (b >> 2))]
                pltpu.make_async_copy(src.at[b, hp], kvbuf.at[b, i], sem).start()

    def kv_wait(b):
        pltpu.make_async_copy(kvbuf.at[b], kvbuf.at[b], kv_sem.at[b]).wait()

    def kvg_start(g):
        hp, i4 = g >> lg, (g >> 2) & 3
        b = pl.multiple_of(i4 * BB, BB)
        for i, src in enumerate((ak, av, bk, bv)):
            pltpu.make_async_copy(src.at[pl.ds(b, BB), hp], kvbuf.at[pl.ds(b, BB), i], kv_sem.at[nb + i4]).start()

    def kvg_wait(i4):
        v = kvbuf.at[pl.ds(i4 * BB, BB)]
        pltpu.make_async_copy(v, v, kv_sem.at[nb + i4]).wait()

    def x_start(b, which=(0, 1)):
        for i, src in enumerate((ax, bx)):
            if i in which:
                for c in range(xbuf.shape[2]):
                    pltpu.make_async_copy(src.at[b, :, pl.ds(c * 128, 128)], xbuf.at[b, i, c], x_sem.at[b]).start()

    def x_wait(b):
        pltpu.make_async_copy(xbuf.at[b], xbuf.at[b], x_sem.at[b]).wait()

    def w_start(h, m):
        off = h * hw if isinstance(h, int) else pl.multiple_of(h * hw, 128)
        if m < 2:
            for c in range(hw // 128):
                pltpu.make_async_copy((awq, bwq)[m].at[:, pl.ds(off + c * 128, 128)],
                                      wbuf.at[pl.ds(m * wrows + c * d, d)], w_sem.at[m]).start()
        else:
            for c in range(d // 128):
                pltpu.make_async_copy((awo, bwo)[m - 2].at[pl.ds(off, hw), pl.ds(c * 128, 128)],
                                      wbuf.at[pl.ds(m * wrows + c * hw, hw)], w_sem.at[m]).start()

    def w_start_dyn(h, m, valid):
        for k in range(4):
            @pl.when(jnp.logical_and(m == k, valid))
            def _():
                w_start(h, k)

    def w_wait(m):
        v = wbuf.at[pl.ds(_mul(m, wrows), wrows)]
        pltpu.make_async_copy(v, v, w_sem.at[m]).wait()

    def prep_w(dst, msrc, mdst, row, nrows, part=None, zero=None):
        if isinstance(msrc, int):
            sa, sc = (5, 1) if msrc < 2 else (1, 3)
            off = [(msrc * 15 + (y // 5) * sa + (y % 5) * sc) * 64 + row * 8 for y in range(15)]
        else:
            sa, sc = jnp.where(msrc < 2, 5, 1), jnp.where(msrc < 2, 1, 3)
            off = [pl.multiple_of((msrc * 15 + (y // 5) * sa + (y % 5) * sc) * 64 + row * 8, 64 if isinstance(row, int) and row == 0 else 32)
                   for y in range(15)]
        r16 = _mul(mdst * 8 + row, 16)
        if not isinstance(r16, int):
            r16 = pl.multiple_of(r16, 128 if isinstance(row, int) and row == 0 else 64)
        for r, form in enumerate(W_FORMS):
            if part is not None and r % part[1] != part[0]:
                continue
            if len(form) == 1:
                val = _as_bf16(w32[pl.ds(off[form[0][0]], nrows * 8), :])
            else:
                val = None
                for y, c in form:
                    t = _as_f32(w32[pl.ds(off[y], nrows * 8), :])
                    val = t if val is None else (val + t if c > 0 else val - t)
                val = val.astype(bf16)
            wc[dst][pl.ds(r16, nrows * 16), r * 128:(r + 1) * 128] = val
        if zero is not None:
            c0 = part[0] * 128
            return lambda: wc[dst][pl.ds(pl.multiple_of(r16 + zero * 16, 16), 16), c0:c0 + 128].astype(f32)[0:8]

    def prep_x(b, br, part=None, zero=None):
        get = _make_lhs(
            lambda z: _as_f32(x32[b, br, z % 5, (z // 5) * (hq // 2):(z // 5 + 1) * (hq // 2), :]) * scale,
            Q_LHS_PROG)
        for r, p in enumerate(Q_PRODS):
            if part is not None and r * XPARTS // NPROD != part:
                continue
            c0 = r * 128
            xc[pl.ds(_mul(b * 2 + br, hq), hq), r * 128:(r + 1) * 128] = (get(p[0]) * Q_SIGN[r]).astype(bf16)
        if zero is not None:
            return lambda: xc[pl.ds(_mul(b * 2 + br + zero, hq), 16), c0:c0 + 128].astype(f32)[0:8]

    def body(g0, nbat, extra, pat, cs, first_hp=False, last_hp=False):
        hp = g0 >> lg
        b0 = g0 & (nb - 1)
        R, O, OT, OC = {}, {}, {}, {}

        def prow(u, h):
            return (2 * u + h) * sq

        def weights(m, prods):
            def w_of(r):
                s = W_FORMS.index(prods[r][1])
                return wc[cs][m * 128:(m + 1) * 128, s * 128:(s + 1) * 128]
            return w_of

        QA, OA, SC, LH = {}, {}, {}, {}
        pending = []
        clock = [0]
        zero16 = pl.multiple_of((g0 >> 20) * 16, 16)

        def later(key, delay, emit):
            pending.append((clock[0] + delay, key, emit))
            pending.sort(key=lambda e: e[0])

        def flush(key):
            for e in [e for e in pending if e[1] == key]:
                pending.remove(e)
                e[2]()

        def tick(o, cycles):
            t0 = clock[0]
            clock[0] += cycles
            groups = o.shape[0] // 8
            rows = None
            while pending and pending[0][0] <= clock[0]:
                due, _, emit = pending.pop(0)
                tok = emit()
                if tok is None or not TOK:
                    continue
                g = min(max((due - t0) * groups // cycles, 0), groups - 1)
                rows = rows or [o[8 * i:8 * i + 8] for i in range(groups)]
                rows[g] = jnp.minimum(rows[g], jnp.maximum(rows[g], tok()))
            return o if rows is None else jnp.concatenate(rows, axis=0)

        pat, qord, oord, qsp, osp = pat
        qord = [int(i) for i in qord.split(".")]
        oord = [int(i) for i in oord.split(".")]

        def q_(u, lo_, hi_):
            b, br = b0 + u // 2, u % 2

            def lhs_of(r):
                return xc[pl.ds(_mul(b * 2 + br, hq), hq), r * 128:(r + 1) * 128]

            _bilinear_run(QA.setdefault(u, {}), Q_PRODS, qord[lo_:hi_], lhs_of, weights(br, Q_PRODS), tick)
            if hi_ == len(Q_PRODS):
                fin = _bilinear_finish(QA[u], Q_OUT_PROG)
                c = [[fin[i * 3 + n] for n in range(3)] for i in range(2)]
                nch = hq // QCH

                def chunk(k):
                    ck = [[(s, a[k * QCH:(k + 1) * QCH]) for s, a in row] for row in c]
                    r0 = u * hq + k * QCH
                    for h, ops in enumerate(_q_operands(ck)):
                        for i, a in enumerate(ops):
                            qbuf[r0:r0 + QCH, (3 * h + i) * 128:(3 * h + i + 1) * 128] = a.astype(bf16)
                    return lambda: qbuf[pl.ds(r0 + zero16, 16), 0:128].astype(f32)[0:8]

                for k in range(nch):
                    later(("q", u), QD + k * QS, functools.partial(chunk, k))

        def s_(u, h, j):
            b, br = b0 + u // 2, u % 2
            flush(("q", u))
            qh = [qbuf[u * hq:(u + 1) * hq, (3 * h + i) * 128:(3 * h + i + 1) * 128] for i in range(3)]
            SC[u, h, j] = _scores_half(qh, kvbuf.at[b, 2 * br], h, j, tick)
            if j == 1:
                s = jnp.concatenate(SC[u, h, 0] + SC[u, h, 1], axis=1)
                R[u, h] = []

                def chunk(k):
                    p, r = _softmax(s[k * PCH:(k + 1) * PCH])
                    R[u, h].append(r)
                    r0 = prow(u, h) + k * PCH
                    pbuf[r0:r0 + PCH, :] = p
                    return lambda: pbuf[pl.ds(r0 + zero16, 16), 0:128].astype(f32)[0:8]

                for k in range(sq // PCH):
                    later(("p", u, h), SD + k * SS, functools.partial(chunk, k))

        def rinv(u, h):
            return jnp.concatenate(R[u, h], axis=0)

        def m_(u, h, half):
            flush(("p", u, h))
            vt = kvbuf.at[b0 + u // 2 + (g0 >> 20) * half * VNOCSE, 2 * (u % 2) + 1]
            r0 = prow(u, h) + half * hq
            res = [tick(lax.dot_general(pbuf[r0:r0 + hq, i * 256:(i + 1) * 256], _pv_weights(vt, h, i), NT,
                                        preferred_element_type=f32), 40) for i in range(3)]
            lo = lax.broadcasted_iota(jnp.int32, (hq, 128), 1) < 64
            r = rinv(u, h)[half * hq:(half + 1) * hq]
            O[u, h, half] = (res[0] + jnp.where(lo, res[2], res[1])) * r
            OT[u, h, half] = jnp.where(lo, res[1], res[2]) * r

        def o_(u, lo_, hi_):
            b, br = b0 + u // 2, u % 2
            if lo_ == 0:
                lo = lax.broadcasted_iota(jnp.int32, (hq, 128), 1) < 64
                mid = [jnp.where(lo, OT[u, 0, i], OT[u, 1, i]) +
                       pltpu.roll(jnp.where(lo, OT[u, 1, i], OT[u, 0, i]), 64, 1) for i in range(2)]
                tiles = [[O[u, 0, i], mid[i], O[u, 1, i]] for i in range(2)]
                get = _make_lhs(lambda x: tiles[x // 3][x % 3], O_LHS_PROG)
                LH[u] = {p[0]: get(p[0]).astype(bf16) for p in O_PRODS}
            _bilinear_run(OA.setdefault(u, {}), O_PRODS, oord[lo_:hi_], lambda r: LH[u][O_PRODS[r][0]],
                          weights(2 + br, O_PRODS), tick)
            fin = _bilinear_finish(OA[u], O_OUT_PROG) if hi_ == NPROD else {}
            for n in (range(5) if fin else ()):
                for i in range(2):
                    s, a = fin[i * 5 + n]
                    rows = slice(i * hq, (i + 1) * hq)
                    cols = slice(br * d + n * 128, br * d + (n + 1) * 128)
                    if first_hp:
                        new = a if s > 0 else -a
                    else:
                        new = acc[b, rows, cols] + a if s > 0 else acc[b, rows, cols] - a
                    if last_hp:
                        obuf[b, rows, cols] = new.astype(obuf.dtype)
                    if not last_hp:
                        acc[b, rows, cols] = new
            if br == 1 and lo_ > 0 and last_hp:
                pltpu.make_async_copy(obuf.at[b], o_hbm.at[b], o_sem).start()

        fns = {"qa": lambda u: q_(u, 0, qsp), "qb": lambda u: q_(u, qsp, NPROD),
               "oa": lambda u: o_(u, 0, osp), "ob": lambda u: o_(u, osp, NPROD),
               "s00": lambda u: s_(u, 0, 0), "s01": lambda u: s_(u, 0, 1),
               "s10": lambda u: s_(u, 1, 0), "s11": lambda u: s_(u, 1, 1),
               "m0": lambda u: m_(u, 0, 0), "m1": lambda u: m_(u, 1, 0),
               "t0": lambda u: m_(u, 0, 1), "t1": lambda u: m_(u, 1, 1), "c": lambda u: None}
        sched = _schedule(2 * nbat, pat)
        first, dmas, preps = extra
        for f in first:
            f()
        total = 2 * nbat * 1960
        lastq = max(i for i, it in enumerate(sched) if it[0][0] == "q")
        wpre, xpre = preps
        for k, f in enumerate(wpre):
            lo_, hi_ = (PLO, total - PHI) if nbat > 1 else (SWLO, SWHI)
            later("w", lo_ + k * (hi_ - lo_) // len(wpre), f)
        for i, item in enumerate(sched):
            fns[item[0]](item[1])
            if i == lastq:
                for k, f in enumerate(xpre):
                    later("x", SXLO + k * (total - SXHI - clock[0] - SXLO) // len(xpre), f)
        flush("w")
        flush("x")
        assert not pending

    for k in range(4):
        w_start(0, k)
    x_start(0)
    kv_start(0)
    x_start(1)
    for g in range(1, C0):
        kv_start(g)
        x_start(g + 1)
    for m in range(4):
        w_wait(m)
        prep_w(0, m, m, 0, 8)
    x_wait(0)
    for br in range(2):
        prep_x(0, br)

    def issued(g):
        return jnp.minimum(jnp.minimum(RATE * (g + 1) + C0, jnp.maximum(g + LA, LB * g - LC)), G1 + DIST * BB)

    def small(b0, carry):
        half = nb // 2
        m = (b0 - half) >> 1

        @pl.when(b0 + 1 < nb)
        def _():
            x_wait(b0 + 1)

        @pl.when(jnp.logical_and(b0 >= half, (b0 & 1) == 0))
        def _():
            w_wait(m)

        kv_wait(b0)

        hi = issued(b0)
        prev = jnp.where(b0 == 0, C0, issued(b0 - 1))

        def pf_x(k, w):
            @pl.when(jnp.logical_and(prev + k < hi, prev + k + 1 < nb))
            def _():
                x_start(prev + k + 1, (w,))

        def pf_kv(k):
            @pl.when(prev + k < hi)
            def _():
                kv_start(prev + k)

        def pf_w():
            w_start_dyn(jnp.where(b0 == W2AT, 2, 1), jnp.where(b0 == W2AT, 0, (b0 >> 1) - 1),
                        jnp.logical_or(b0 == W2AT, jnp.logical_and(b0 <= half, (b0 & 1) == 0)))

        first = [pf_w] + [functools.partial(pf_x, k, w) for k in range(RATE) for w in range(2)]
        first += [functools.partial(pf_kv, k) for k in range(RATE)]
        zero = b0 >> 20
        preps = ([functools.partial(prep_w, 1, jnp.where(b0 >= half, m, 3), jnp.maximum(m, 0), (b0 & 1) * 4, 4,
                                    (part, SWPARTS), zero) for part in range(SWPARTS)],
                 [functools.partial(prep_x, jnp.minimum(b0 + 1, nb - 1), br, part, zero)
                  for br in range(2) for part in range(XPARTS)])
        body(b0, 1, (first, [], preps), (SPAT, SQORD, SOORD, SQSPLIT, SOSPLIT), 0, first_hp=True)
        return carry

    def big(par, last, hp, i, carry):
        b0 = i * BB
        g0 = hp * nb + b0

        if not last:
            w_wait(i)

        kvg_wait(i)

        def pf_kv():
            @pl.when(g0 + DIST * BB < ng)
            def _():
                kvg_start(g0 + DIST * BB)

        if last:
            extra = ([pf_kv], [], ([], []))
        else:
            hn = jnp.where(i == 3, hp + 2, hp + 1)
            extra = ([lambda: w_start_dyn(hn, (i + 1) & 3, hn < nhp)] +
                     [functools.partial(kvg_start, g0 + DIST * BB)], [],
                     ([functools.partial(prep_w, 1 - par, i, i, 0, 8, (part, PPARTS), i >> 20)
                       for part in range(PPARTS)], []))
        body(g0, BB, extra, (LPAT, LQORD, LOORD, LQSPLIT, LOSPLIT) if last else (PAT, QORD, OORD, QSPLIT, OSPLIT), par, last_hp=last)
        return carry

    spb = nb // BB
    assert spb == 4 and G1 == nb
    if SKIP_SMALL in (0, 2):
        lax.fori_loop(0, nb, small, 0)
    if SKIP_SMALL == 2:
        prep_x(0, 0)
        def _rd(i, c):
            v = wc[1][pl.ds(pl.multiple_of(i * 16, 16), 16), :].astype(f32)
            acc[0, 0:16, :] += v[:, 0:1280] + v[:, 1280:2560] + v[:, 2560:3840]
            return c
        lax.fori_loop(0, 32, _rd, 0)
        obuf[0] = acc[0, 0:160].astype(bf16)
        pltpu.make_async_copy(obuf, o_hbm, o_sem).start()
        pltpu.make_async_copy(obuf, o_hbm, o_sem).wait()
        return

    def pair(t, carry):
        lax.fori_loop(jnp.where(t > 0, 0, spb), spb, functools.partial(big, 0, False, 2 * t), 0)
        lax.fori_loop(0, jnp.where(2 * t + 1 < nhp - 1, spb, 0), functools.partial(big, 1, False, 2 * t + 1), 0)
        return carry

    if SKIP_SMALL != 3:
        lax.fori_loop(0, nhp // 2, pair, 0)
    else:
        prep_w(1, 0, 0, 0, 8)
    if SKIP_SMALL in (0, 3):
        lax.fori_loop(0, spb, functools.partial(big, 1, True, nhp - 1), 0)
    pltpu.make_async_copy(obuf, o_hbm, o_sem).wait()


@jax.jit
def pallas_concat_heads__gqa_block_cached__mha_block_cached__near_ridge_kernel(
    A_x, A_k_cache, A_v_cache, A_wq, A_wo, B_x, B_k_cache, B_v_cache, B_wq, B_wo):
    B, Sq, D = A_x.shape
    _, H, Sk, Dh = A_k_cache.shape
    nhp = H // 2
    assert B == 16 and G1 % B == 0 and 2 * BB <= B and C0 >= 1
    n_iss = C0
    for g0 in range(G1):
        assert n_iss >= g0 + 2, (g0, n_iss)
        hi = min(RATE * (g0 + 1) + C0, max(g0 + LA, LB * g0 - LC), G1 + DIST * BB)
        assert hi <= g0 + B
        assert 0 <= hi - n_iss <= RATE
        n_iss = hi
    assert n_iss == G1 + DIST * BB, n_iss
    assert 10 <= W2AT <= 15 and 5 <= LA <= B

    def tr(c):
        return jnp.swapaxes(c, 2, 3).reshape(B, nhp, 2 * Dh, Sk)

    any_spec = pl.BlockSpec(memory_space=pl.ANY)
    return pl.pallas_call(
        functools.partial(_kernel, scale=Dh ** -0.5 * LOG2E, nhp=nhp, nb=B),
        in_specs=[any_spec] * 10,
        out_specs=any_spec,
        out_shape=jax.ShapeDtypeStruct((B, Sq, 2 * D), A_x.dtype),
        scratch_shapes=[pltpu.VMEM((B, ACCR, 2 * D), f32),
                        pltpu.VMEM((B, 2, D // 128, Sq // 2, 128), u32),
                        pltpu.VMEM((4 * 15 * 64, 128), u32),
                        pltpu.VMEM((B, 4, 2 * Dh, Sk), bf16),
                        pltpu.VMEM((B, Sq, 2 * D), bf16),
                        pltpu.VMEM((2 * BB * Sq, 6 * 128), u32),
                        pltpu.VMEM((2 * BB * Sq // 4, 6 * 128), u32),
                        pltpu.VMEM((B * 2 * Sq // 4, XCW * 128), u32),
                        pltpu.VMEM((4 * 64, WCW * 128), u32),
                        pltpu.VMEM((4 * 64, WCW * 128), u32),
                        pltpu.SemaphoreType.DMA((B + 4,)),
                        pltpu.SemaphoreType.DMA((B,)),
                        pltpu.SemaphoreType.DMA((4,)),
                        pltpu.SemaphoreType.DMA(())],
        compiler_params=pltpu.CompilerParams(
            disable_bounds_checks=True,
            vmem_limit_bytes=110 * 1024 * 1024),
    )(A_x, tr(A_k_cache), tr(A_v_cache), A_wq, A_wo, B_x, tr(B_k_cache), tr(B_v_cache), B_wq, B_wo)
```

```python
import functools

import jax
import jax.numpy as jnp
from jax import lax
import jax.experimental.pallas as pl
import jax.experimental.pallas.tpu as pltpu

bf16 = jnp.bfloat16
f32 = jnp.float32
u32 = jnp.uint32
NT = (((1,), (1,)), ((), ()))
LOG2E = 1.4426950408889634

BB = 4
DIST = 2
C0, RATE, LA, LB, LC = 2, 2, 6, 2, 6
W2AT = 11
XCW, WCW = 32, 40

PAT = (
    "qa@0,qb@0,qa@1,qb@1,qa@2,s00@0,s01@0,s10@0,qb@2,s11@0,m0@0,t0@0,s00@1,qa@3,s01@1,t1@0,s10@1,qb@3,m1@0,"
    "s11@1,m0@1,t0@1,s00@2,qa@4,s01@2,m1@1,t1@1,s10@2,oa@0,qb@4,s11@2,m0@2,t0@2,ob@0,s00@3,qa@5,s01@3,t1@2,"
    "m1@2,s10@3,oa@1,qb@5,s11@3,m0@3,t0@3,ob@1,s00@4,oa@2,qa@6,s01@4,m1@3,t1@3,s10@4,s11@4,m0@4,t0@4,ob@2,"
    "s00@5,qb@6,qa@7,s01@5,m1@4,t1@4,s10@5,oa@3,qb@7,s11@5,m0@5,t0@5,ob@3,s00@6,s01@6,m1@5,t1@5,s10@6,oa@4,"
    "s11@6,m0@6,t0@6,ob@4,s00@7,s01@7,m1@6,t1@6,s10@7,oa@5,s11@7,m0@7,t0@7,ob@5,m1@7,t1@7,oa@6,ob@6,oa@7,"
    "ob@7")
SPAT = (
    "qa@0,qb@0,qa@1,s00@0,s10@0,s11@0,s01@0,qb@1,m1@0,m0@0,t0@0,s00@1,s01@1,t1@0,s10@1,s11@1,oa@0,m0@1,m1@1,"
    "t0@1,t1@1,ob@0,oa@1,ob@1")
LPAT = PAT
QORD = "9.16.24.21.19.1.15.20.18.22.17.23.2.0.3.7.4.5.6.8.14.12.10.11.13"
OORD = "0.6.1.5.3.2.8.9.4.24.12.11.14.10.16.19.13.15.17.18.20.22.21.23.7"
SQORD = "3.16.24.15.18.10.20.21.17.7.22.1.23.6.2.0.14.8.4.5.9.19.11.12.13"
SOORD = "7.22.23.20.18.16.17.19.21.15.13.12.10.11.14.9.2.8.24.6.5.1.3.4.0"
LQORD = QORD
LOORD = OORD
STEADY = (PAT, QORD, OORD, 11, 10)
RAMP = (SPAT, SQORD, SOORD, 13, 13)
LAST = (LPAT, LQORD, LOORD, 11, 10)
PLO, PHI, SWLO, SWHI, SXLO, SXHI, SWPARTS, XPARTS = 300, 400, 60, 1080, 1700, 120, 12, 25

O_LHS_PROG = [
    (100, 4, 5, 1), (101, 0, 1, -1), (102, 3, 101, 1), (103, 2, 100, 1), (104, 0, 3, 1),
    (105, 2, 3, -1), (106, 0, 2, 1), (107, 2, 101, -1), (108, 3, 5, 1), (109, 1, 103, 1),
    (110, 2, 5, 1), (111, 3, 100, -1), (112, 5, 101, 1), (113, 4, 102, -1), (114, 0, 100, 1),
]
O_OUT_PROG = [
    (100, 5, 8, -1), (101, 3, 100, 1), (102, 2, 7, -1), (103, 0, 102, 1),
]
O_PRODS = [
    ((101, 1), [(2, 1), (5, 1), (10, -1), (12, 1)], [(102, 1)]),
    ((104, 1), [(3, 1)], [(100, -1)]),
    ((111, 1), [(0, 1), (3, 1)], [(5, 1)]),
    ((5, 1), [(5, 1), (10, -1)], [(5, -1), (103, 1)]),
    ((112, 1), [(5, 1), (10, -1), (12, 1)], [(103, -1)]),
    ((114, 1), [(0, 1), (3, 1), (5, 1)], [(101, 1)]),
    ((0, 1), [(0, 1), (5, 1)], [(0, 1), (101, -1)]),
    ((107, -1), [(10, 1), (12, -1)], [(0, -1)]),
    ((110, 1), [(12, 1)], [(0, 1), (2, 1)]),
    ((1, 1), [(2, 1), (7, 1)], [(2, 1), (4, -1)]),
    ((104, 1), [(1, 1), (2, 1), (4, 1), (7, 1), (9, 1)], [(4, 1)]),
    ((106, 1), [(1, 1)], [(1, 1), (4, -1)]),
    ((1, 1), [(6, 1)], [(1, 1), (3, -1)]),
    ((109, 1), [(6, 1), (8, 1)], [(3, 1)]),
    ((2, 1), [(1, 1), (11, -1)], [(1, -1), (6, 1)]),
    ((103, 1), [(6, 1), (8, 1), (13, -1)], [(3, -1), (6, 1)]),
    ((100, 1), [(0, 1), (3, 1), (5, 1), (13, 1)], [(3, -1), (8, 1)]),
    ((4, 1), [(8, 1), (13, -1)], [(6, -1), (8, 1)]),
    ((110, 1), [(6, 1), (8, 1), (11, -1), (13, -1), (14, -1)], [(6, -1)]),
    ((105, 1), [(1, 1), (14, 1)], [(4, 1), (6, -1)]),
    ((108, 1), [(14, 1)], [(6, -1), (9, 1)]),
    ((3, 1), [(4, 1), (14, -1)], [(4, -1), (9, 1)]),
    ((4, 1), [(9, 1)], [(7, -1), (9, 1)]),
    ((102, 1), [(2, 1), (7, 1), (9, 1)], [(4, -1), (7, 1)]),
    ((113, -1), [(7, 1), (9, 1)], [(7, -1)]),
]
Q_LHS_PROG = [
    (100, 3, 8, -1), (101, 0, 2, 1), (102, 7, 101, -1), (103, 5, 100, 1), (104, 4, 6, -1),
    (105, 4, 9, -1), (106, 7, 9, -1), (107, 0, 103, -1), (108, 6, 8, -1), (109, 5, 102, 1),
    (110, 1, 4, -1), (111, 5, 8, -1), (112, 6, 9, -1), (113, 4, 7, -1), (114, 2, 4, -1),
    (115, 1, 6, -1), (116, 2, 7, -1), (117, 1, 3, -1), (118, 3, 6, -1),
]
Q_OUT_PROG = [
    (100, 0, 3, 1), (101, 4, 5, 1), (102, 0, 1, -1), (103, 2, 101, 1), (104, 2, 5, 1),
    (105, 1, 100, -1),
]
Q_PRODS = [
    ((6, -1), [(6, 1), (8, 1), (11, -1), (13, -1), (14, -1)], [(104, 1)]),
    ((101, 1), [(12, 1)], [(104, 1)]),
    ((4, 1), [(1, 1), (2, 1), (4, 1), (7, 1), (9, 1)], [(100, 1)]),
    ((111, -1), [(3, 1)], [(100, 1)]),
    ((118, -1), [(6, 1), (8, 1), (13, -1)], [(103, 1)]),
    ((3, 1), [(6, 1), (8, 1)], [(1, 1), (103, 1)]),
    ((114, 1), [(2, 1), (7, 1)], [(1, 1)]),
    ((117, 1), [(6, 1)], [(1, 1)]),
    ((115, -1), [(1, 1), (11, -1)], [(2, 1)]),
    ((0, -1), [(10, 1), (12, -1)], [(2, -1), (102, 1)]),
    ((116, 1), [(2, 1), (5, 1), (10, -1), (12, 1)], [(102, 1)]),
    ((102, 1), [(5, 1), (10, -1), (12, 1)], [(5, 1), (102, 1)]),
    ((109, -1), [(5, 1), (10, -1)], [(5, 1)]),
    ((112, -1), [(14, 1)], [(3, 1), (5, 1)]),
    ((104, 1), [(1, 1), (14, 1)], [(2, 1), (3, -1)]),
    ((105, -1), [(4, 1), (14, -1)], [(3, 1)]),
    ((5, 1), [(0, 1), (3, 1)], [(3, 1), (101, -1)]),
    ((100, -1), [(0, 1), (3, 1), (5, 1), (13, 1)], [(101, 1)]),
    ((103, 1), [(0, 1), (3, 1), (5, 1)], [(0, 1), (101, 1)]),
    ((110, 1), [(1, 1)], [(0, 1), (2, 1)]),
    ((107, 1), [(0, 1), (5, 1)], [(0, 1)]),
    ((113, -1), [(2, 1), (7, 1), (9, 1)], [(105, -1)]),
    ((7, -1), [(7, 1), (9, 1)], [(4, -1), (105, -1)]),
    ((106, -1), [(9, 1)], [(4, 1)]),
    ((108, -1), [(8, 1), (13, -1)], [(4, 1)]),
]
NPROD = len(O_PRODS)


def _normalize(prods):
    out = []
    for (var, sgn), w, g in prods:
        sgn *= w[0][1]
        out.append((var, [(y, c * w[0][1]) for y, c in w], [(z, c * sgn) for z, c in g]))
    return out


def _positive_outputs(prods, prog):
    for flips in range(1 << 6):
        sg = [(-1 if (flips >> (r % 6)) & 1 else 1) for r in range(len(prods))]
        pos = {}
        for r, p in enumerate(prods):
            for z, c in p[2]:
                pos[z] = max(pos.get(z, -1), c * sg[r])
        for t, a, b, s in reversed(prog):
            st = pos.pop(t)
            pos[a] = max(pos.get(a, -1), st)
            pos[b] = max(pos.get(b, -1), st * s)
        if min(pos.values()) > 0:
            return sg
    raise AssertionError


O_PRODS = _normalize(O_PRODS)
Q_PRODS = _normalize(Q_PRODS)
W_FORMS = [p[1] for p in O_PRODS]
Q_SIGN = _positive_outputs(Q_PRODS, Q_OUT_PROG)
Q_PRODS = [(v, w, [(z, c * s) for z, c in g]) for (v, w, g), s in zip(Q_PRODS, Q_SIGN)]


def _make_lhs(block, prog):
    vals = {}

    def get(v):
        if v not in vals:
            vals[v] = block(v)
        return vals[v]

    for t, a, b, s in prog:
        vals[t] = get(a) + get(b) if s > 0 else get(a) - get(b)
    return get


def _acc_add(accs, z, sgn, m):
    if z not in accs:
        accs[z] = (sgn, m)
    else:
        s0, a = accs[z]
        accs[z] = (s0, a + m) if s0 == sgn else ((1, a - m) if s0 > 0 else (1, m - a))


def _bilinear_run(accs, prods, which, lhs_of, w_of, tick):
    for r in which:
        m = tick(jnp.dot(lhs_of(r), w_of(r), preferred_element_type=f32), 20)
        for z, c in prods[r][2]:
            _acc_add(accs, z, c, m)


def _bilinear_finish(accs, prog):
    for t, a, b, s in reversed(prog):
        st, v = accs.pop(t)
        _acc_add(accs, a, st, v)
        _acc_add(accs, b, st * s, v)
    return accs


def _mul(i, n):
    return i * n if isinstance(i, int) else pl.multiple_of(i * n, 16)


def _as_bf16(packed):
    return pltpu.bitcast(packed, bf16)


def _as_f32(packed):
    return pltpu.bitcast(packed, bf16).astype(f32)


def _q_operands(c):
    assert all(s > 0 for row in c for s, _ in row)
    (t0, t1, t2), (b0, b1, b2) = [[a for _, a in row] for row in c]
    lo = lax.broadcasted_iota(jnp.int32, t0.shape, 1) < 64
    return [[jnp.where(lo, t0, b0), jnp.where(lo, t1, t0 - b0), jnp.where(lo, b0 - t0, pltpu.roll(b1, 64, 1))],
            [jnp.where(lo, t2, b2), jnp.where(lo, pltpu.roll(t1, 64, 1), t2 - b2), jnp.where(lo, b2 - t2, b1)]]


def _scores_half(qh, kt, h, j, tick):
    k0, k1, k2 = (0, 64, 128) if h == 0 else (256, 320, 192)
    out = []
    for c in (2 * j, 2 * j + 1):
        cs = slice(c * 128, (c + 1) * 128)
        w = [kt[k0:k0 + 128, cs],
             jnp.concatenate([kt[k2:k2 + 64, cs], kt[k1:k1 + 64, cs]], axis=0),
             jnp.concatenate([kt[k0:k0 + 64, cs], kt[k2:k2 + 64, cs]], axis=0)]
        m = [tick(jnp.dot(qh[i], w[i], preferred_element_type=f32), 20) for i in range(3)]
        out.append(jnp.concatenate([m[0] + m[1], m[0] + m[2]], axis=0))
    return out


def _softmax(s):
    m = jnp.max(s, axis=1, keepdims=True)
    p = jnp.exp2(s - m)
    p0, p1, p2, p3 = (p[:, i * 128:(i + 1) * 128] for i in range(4))
    s01, s23 = p0 + p1, p2 + p3
    t = s01 + s23
    l = jnp.sum(t, axis=1, keepdims=True)
    r = pl.reciprocal(l, approx=True)
    r = r * (2.0 - l * r)
    return jnp.concatenate([s01, jnp.minimum(s23, t), p0, p2, p1, p3], axis=1).astype(bf16), r


def _pv_weights(vt, h, i):
    d0, d1, d2 = (0, 64, 128) if h == 0 else (256, 320, 192)

    def v(d, c):
        return vt[d:d + 64, c * 128:(c + 1) * 128]

    def f(d, c):
        return v(d, c).astype(f32)

    if i == 0:
        return jnp.concatenate([jnp.concatenate([v(d0, c), v(d1, c + 1)], axis=0) for c in (0, 2)], axis=1)
    if i == 1:
        w = [jnp.concatenate([f(d2, c), f(d1, c) - f(d1, c + 1)], axis=0) for c in (0, 2)]
    else:
        w = [jnp.concatenate([f(d0, c + 1) - f(d0, c), f(d2, c + 1)], axis=0) for c in (0, 2)]
    return jnp.concatenate(w, axis=1).astype(bf16)


def _kernel(ax, ak, av, awq, awo, bx, bk, bv, bwq, bwo, o_hbm,
            acc, x32, w32, kvbuf, obuf, pbuf, qbuf, xc32, wc0, wc1,
            kv_sem, x_sem, w_sem, o_sem, *, scale, nhp, nb):
    xbuf, wbuf = (r.bitcast(bf16) for r in (x32, w32))
    pbuf, qbuf, xc = (r.bitcast(bf16) for r in (pbuf, qbuf, xc32))
    wc = [r.bitcast(bf16) for r in (wc0, wc1)]
    sq = xbuf.shape[3]
    hq = sq // 2
    d = awq.shape[0]
    hw = kvbuf.shape[2]
    wrows = wbuf.shape[0] // 4
    ng = nhp * nb
    lg = nb.bit_length() - 1
    spb = nb // BB

    def kv_start(g):
        hp, b = (g >> lg) & (nhp - 1), g & (nb - 1)
        for i, src in enumerate((ak, av, bk, bv)):
            sem = kv_sem.at[jnp.where(g < nb, b, nb + (b >> 2))]
            pltpu.make_async_copy(src.at[b, hp], kvbuf.at[b, i], sem).start()

    def kv_wait(b):
        pltpu.make_async_copy(kvbuf.at[b], kvbuf.at[b], kv_sem.at[b]).wait()

    def kvg_start(g):
        hp, i4 = g >> lg, (g >> 2) & 3
        b = pl.multiple_of(i4 * BB, BB)
        for i, src in enumerate((ak, av, bk, bv)):
            pltpu.make_async_copy(src.at[pl.ds(b, BB), hp], kvbuf.at[pl.ds(b, BB), i], kv_sem.at[nb + i4]).start()

    def kvg_wait(i4):
        v = kvbuf.at[pl.ds(i4 * BB, BB)]
        pltpu.make_async_copy(v, v, kv_sem.at[nb + i4]).wait()

    def x_start(b, which=(0, 1)):
        for i, src in enumerate((ax, bx)):
            if i in which:
                for c in range(xbuf.shape[2]):
                    pltpu.make_async_copy(src.at[b, :, pl.ds(c * 128, 128)], xbuf.at[b, i, c], x_sem.at[b]).start()

    def x_wait(b):
        pltpu.make_async_copy(xbuf.at[b], xbuf.at[b], x_sem.at[b]).wait()

    def w_start(h, m):
        off = h * hw if isinstance(h, int) else pl.multiple_of(h * hw, 128)
        if m < 2:
            for c in range(hw // 128):
                pltpu.make_async_copy((awq, bwq)[m].at[:, pl.ds(off + c * 128, 128)],
                                      wbuf.at[pl.ds(m * wrows + c * d, d)], w_sem.at[m]).start()
        else:
            for c in range(d // 128):
                pltpu.make_async_copy((awo, bwo)[m - 2].at[pl.ds(off, hw), pl.ds(c * 128, 128)],
                                      wbuf.at[pl.ds(m * wrows + c * hw, hw)], w_sem.at[m]).start()

    def w_start_dyn(h, m, valid):
        for k in range(4):
            @pl.when(jnp.logical_and(m == k, valid))
            def _():
                w_start(h, k)

    def w_wait(m):
        v = wbuf.at[pl.ds(_mul(m, wrows), wrows)]
        pltpu.make_async_copy(v, v, w_sem.at[m]).wait()

    def prep_w(dst, msrc, mdst, row, nrows, part=None, zero=None):
        whole = isinstance(row, int) and row == 0
        if isinstance(msrc, int):
            sa, sc = (5, 1) if msrc < 2 else (1, 3)
            off = [(msrc * 15 + (y // 5) * sa + (y % 5) * sc) * 64 + row * 8 for y in range(15)]
        else:
            sa, sc = jnp.where(msrc < 2, 5, 1), jnp.where(msrc < 2, 1, 3)
            off = [pl.multiple_of((msrc * 15 + (y // 5) * sa + (y % 5) * sc) * 64 + row * 8, 64 if whole else 32)
                   for y in range(15)]
        r16 = _mul(mdst * 8 + row, 16)
        if not isinstance(r16, int):
            r16 = pl.multiple_of(r16, 128 if whole else 64)
        for r, form in enumerate(W_FORMS):
            if part is not None and r % part[1] != part[0]:
                continue
            if len(form) == 1:
                val = _as_bf16(w32[pl.ds(off[form[0][0]], nrows * 8), :])
            else:
                val = None
                for y, c in form:
                    t = _as_f32(w32[pl.ds(off[y], nrows * 8), :])
                    val = t if val is None else (val + t if c > 0 else val - t)
                val = val.astype(bf16)
            wc[dst][pl.ds(r16, nrows * 16), r * 128:(r + 1) * 128] = val
        if zero is not None:
            c0 = part[0] * 128
            return lambda: wc[dst][pl.ds(pl.multiple_of(r16 + zero * 16, 16), 16), c0:c0 + 128].astype(f32)[0:8]

    def prep_x(b, br, part=None, zero=None):
        get = _make_lhs(
            lambda z: _as_f32(x32[b, br, z % 5, (z // 5) * (hq // 2):(z // 5 + 1) * (hq // 2), :]) * scale,
            Q_LHS_PROG)
        for r, p in enumerate(Q_PRODS):
            if part is not None and r * XPARTS // NPROD != part:
                continue
            c0 = r * 128
            xc[pl.ds(_mul(b * 2 + br, hq), hq), r * 128:(r + 1) * 128] = (get(p[0]) * Q_SIGN[r]).astype(bf16)
        if zero is not None:
            return lambda: xc[pl.ds(_mul(b * 2 + br + zero, hq), 16), c0:c0 + 128].astype(f32)[0:8]

    def body(g0, nbat, first, wpre, xpre, plan, cs, first_hp=False, last_hp=False):
        b0 = g0 & (nb - 1)
        pat, qord, oord, qsp, osp = plan
        sched = [(a.split("@")[0], int(a.split("@")[1])) for a in pat.split(",")]
        qord = [int(i) for i in qord.split(".")]
        oord = [int(i) for i in oord.split(".")]
        assert all(sched.index(("ob", u)) < sched.index(("ob", u + 1)) for u in range(0, 2 * nbat, 2))
        R, O, OT, QA, OA, SC, LH = {}, {}, {}, {}, {}, {}, {}
        lazy = {}
        pending = []
        clock = [0]

        def tick(o, cycles):
            t0 = clock[0]
            clock[0] += cycles
            groups = o.shape[0] // 8
            rows = None
            while pending and pending[0][0] <= clock[0]:
                due, emit = pending.pop(0)
                tok = emit()
                g = min(max((due - t0) * groups // cycles, 0), groups - 1)
                rows = rows or [o[8 * i:8 * i + 8] for i in range(groups)]
                rows[g] = jnp.minimum(rows[g], jnp.maximum(rows[g], tok()))
            return o if rows is None else jnp.concatenate(rows, axis=0)

        def later(delay, emit):
            pending.append((clock[0] + delay, emit))
            pending.sort(key=lambda e: e[0])

        def prow(u, h):
            return (2 * u + h) * sq

        def weights(m, prods):
            def w_of(r):
                s = W_FORMS.index(prods[r][1])
                return wc[cs][m * 128:(m + 1) * 128, s * 128:(s + 1) * 128]
            return w_of

        def q_(u, lo_, hi_):
            b, br = b0 + u // 2, u % 2

            def lhs_of(r):
                return xc[pl.ds(_mul(b * 2 + br, hq), hq), r * 128:(r + 1) * 128]

            _bilinear_run(QA.setdefault(u, {}), Q_PRODS, qord[lo_:hi_], lhs_of, weights(br, Q_PRODS), tick)
            if hi_ == NPROD:
                fin = _bilinear_finish(QA[u], Q_OUT_PROG)

                def store_q():
                    c = [[fin[i * 3 + n] for n in range(3)] for i in range(2)]
                    for h, ops in enumerate(_q_operands(c)):
                        for i, a in enumerate(ops):
                            qbuf[u * hq:(u + 1) * hq, (3 * h + i) * 128:(3 * h + i + 1) * 128] = a.astype(bf16)

                lazy["q", u] = store_q

        def s_(u, h, j):
            b, br = b0 + u // 2, u % 2
            lazy.pop(("q", u), lambda: None)()
            qh = [qbuf[u * hq:(u + 1) * hq, (3 * h + i) * 128:(3 * h + i + 1) * 128] for i in range(3)]
            SC[u, h, j] = _scores_half(qh, kvbuf.at[b, 2 * br], h, j, tick)
            if j == 1:
                s = jnp.concatenate(SC[u, h, 0] + SC[u, h, 1], axis=1)

                def store_p():
                    p, R[u, h] = _softmax(s)
                    pbuf[prow(u, h):prow(u, h) + sq, :] = p

                lazy["p", u, h] = store_p

        def m_(u, h, half):
            lazy.pop(("p", u, h), lambda: None)()
            vt = kvbuf.at[b0 + u // 2 + (g0 >> 20) * half, 2 * (u % 2) + 1]
            r0 = prow(u, h) + half * hq
            res = [tick(lax.dot_general(pbuf[r0:r0 + hq, i * 256:(i + 1) * 256], _pv_weights(vt, h, i), NT,
                                        preferred_element_type=f32), 40) for i in range(3)]
            lo = lax.broadcasted_iota(jnp.int32, (hq, 128), 1) < 64
            r = R[u, h][half * hq:(half + 1) * hq]
            O[u, h, half] = (res[0] + jnp.where(lo, res[2], res[1])) * r
            OT[u, h, half] = jnp.where(lo, res[1], res[2]) * r

        def o_(u, lo_, hi_):
            b, br = b0 + u // 2, u % 2
            if lo_ == 0:
                lo = lax.broadcasted_iota(jnp.int32, (hq, 128), 1) < 64
                mid = [jnp.where(lo, OT[u, 0, i], OT[u, 1, i]) +
                       pltpu.roll(jnp.where(lo, OT[u, 1, i], OT[u, 0, i]), 64, 1) for i in range(2)]
                tiles = [[O[u, 0, i], mid[i], O[u, 1, i]] for i in range(2)]
                get = _make_lhs(lambda x: tiles[x // 3][x % 3], O_LHS_PROG)
                LH[u] = {p[0]: get(p[0]).astype(bf16) for p in O_PRODS}
            _bilinear_run(OA.setdefault(u, {}), O_PRODS, oord[lo_:hi_], lambda r: LH[u][O_PRODS[r][0]],
                          weights(2 + br, O_PRODS), tick)
            if hi_ < NPROD:
                return
            fin = _bilinear_finish(OA[u], O_OUT_PROG)
            for n in range(5):
                for i in range(2):
                    s, a = fin[i * 5 + n]
                    rows = slice(i * hq, (i + 1) * hq)
                    cols = slice(br * d + n * 128, br * d + (n + 1) * 128)
                    if first_hp:
                        new = a if s > 0 else -a
                    else:
                        new = acc[b, rows, cols] + a if s > 0 else acc[b, rows, cols] - a
                    if last_hp:
                        obuf[b, rows, cols] = new.astype(obuf.dtype)
                    else:
                        acc[b, rows, cols] = new
            if br == 1 and last_hp:
                pltpu.make_async_copy(obuf.at[b], o_hbm.at[b], o_sem).start()

        fns = {"qa": lambda u: q_(u, 0, qsp), "qb": lambda u: q_(u, qsp, NPROD),
               "oa": lambda u: o_(u, 0, osp), "ob": lambda u: o_(u, osp, NPROD),
               "s00": lambda u: s_(u, 0, 0), "s01": lambda u: s_(u, 0, 1),
               "s10": lambda u: s_(u, 1, 0), "s11": lambda u: s_(u, 1, 1),
               "m0": lambda u: m_(u, 0, 0), "m1": lambda u: m_(u, 1, 0),
               "t0": lambda u: m_(u, 0, 1), "t1": lambda u: m_(u, 1, 1)}
        for f in first:
            f()
        total = 2 * nbat * 1960
        lastq = max(i for i, it in enumerate(sched) if it[0][0] == "q")
        for k, f in enumerate(wpre):
            lo_, hi_ = (PLO, total - PHI) if nbat > 1 else (SWLO, SWHI)
            later(lo_ + k * (hi_ - lo_) // len(wpre), f)
        for i, item in enumerate(sched):
            fns[item[0]](item[1])
            if i == lastq:
                for k, f in enumerate(xpre):
                    later(SXLO + k * (total - SXHI - clock[0] - SXLO) // len(xpre), f)
        assert not pending and not lazy

    for k in range(4):
        w_start(0, k)
    x_start(0)
    kv_start(0)
    x_start(1)
    for g in range(1, C0):
        kv_start(g)
        x_start(g + 1)
    for m in range(4):
        w_wait(m)
        prep_w(0, m, m, 0, 8)
    x_wait(0)
    for br in range(2):
        prep_x(0, br)

    def issued(g):
        return jnp.minimum(jnp.minimum(RATE * (g + 1) + C0, jnp.maximum(g + LA, LB * g - LC)), nb + DIST * BB)

    def ramp(b0, carry):
        half = nb // 2
        m = (b0 - half) >> 1

        @pl.when(b0 + 1 < nb)
        def _():
            x_wait(b0 + 1)

        @pl.when(jnp.logical_and(b0 >= half, (b0 & 1) == 0))
        def _():
            w_wait(m)

        kv_wait(b0)

        hi = issued(b0)
        prev = jnp.where(b0 == 0, C0, issued(b0 - 1))

        def pf_x(k, w):
            @pl.when(jnp.logical_and(prev + k < hi, prev + k + 1 < nb))
            def _():
                x_start(prev + k + 1, (w,))

        def pf_kv(k):
            @pl.when(prev + k < hi)
            def _():
                kv_start(prev + k)

        def pf_w():
            w_start_dyn(jnp.where(b0 == W2AT, 2, 1), jnp.where(b0 == W2AT, 0, (b0 >> 1) - 1),
                        jnp.logical_or(b0 == W2AT, jnp.logical_and(b0 <= half, (b0 & 1) == 0)))

        first = [pf_w] + [functools.partial(pf_x, k, w) for k in range(RATE) for w in range(2)]
        first += [functools.partial(pf_kv, k) for k in range(RATE)]
        zero = b0 >> 20
        wpre = [functools.partial(prep_w, 1, jnp.where(b0 >= half, m, 3), jnp.maximum(m, 0), (b0 & 1) * 4, 4,
                                  (part, SWPARTS), zero) for part in range(SWPARTS)]
        xpre = [functools.partial(prep_x, jnp.minimum(b0 + 1, nb - 1), br, part, zero)
                for br in range(2) for part in range(XPARTS)]
        body(b0, 1, first, wpre, xpre, RAMP, 0, first_hp=True)
        return carry

    def step(par, last, hp, i, carry):
        g0 = hp * nb + i * BB

        if not last:
            w_wait(i)

        kvg_wait(i)

        if last:
            def pf_kv():
                @pl.when(g0 + DIST * BB < ng)
                def _():
                    kvg_start(g0 + DIST * BB)

            body(g0, BB, [pf_kv], [], [], LAST, par, last_hp=True)
        else:
            hn = jnp.where(i == 3, hp + 2, hp + 1)
            first = [lambda: w_start_dyn(hn, (i + 1) & 3, hn < nhp), functools.partial(kvg_start, g0 + DIST * BB)]
            wpre = [functools.partial(prep_w, 1 - par, i, i, 0, 8, (part, NPROD), i >> 20) for part in range(NPROD)]
            body(g0, BB, first, wpre, [], STEADY, par)
        return carry

    def pair(t, carry):
        lax.fori_loop(jnp.where(t > 0, 0, spb), spb, functools.partial(step, 0, False, 2 * t), 0)
        lax.fori_loop(0, jnp.where(2 * t + 1 < nhp - 1, spb, 0), functools.partial(step, 1, False, 2 * t + 1), 0)
        return carry

    lax.fori_loop(0, nb, ramp, 0)
    lax.fori_loop(0, nhp // 2, pair, 0)
    lax.fori_loop(0, spb, functools.partial(step, 1, True, nhp - 1), 0)
    pltpu.make_async_copy(obuf, o_hbm, o_sem).wait()


@jax.jit
def pallas_concat_heads__gqa_block_cached__mha_block_cached__near_ridge_kernel(
    A_x: jax.Array,
    A_k_cache: jax.Array,
    A_v_cache: jax.Array,
    A_wq: jax.Array,
    A_wo: jax.Array,
    B_x: jax.Array,
    B_k_cache: jax.Array,
    B_v_cache: jax.Array,
    B_wq: jax.Array,
    B_wo: jax.Array,
):
    B, Sq, D = A_x.shape
    _, H, Sk, Dh = A_k_cache.shape
    nhp = H // 2
    assert (B, Sq, D, Sk, Dh) == (16, 160, 640, 512, 192) and A_wq.shape[1] == H * Dh
    assert nhp >= 4 and nhp & (nhp - 1) == 0 and B_k_cache.shape == A_k_cache.shape
    n_iss = C0
    for g0 in range(B):
        assert n_iss >= g0 + 2
        hi = min(RATE * (g0 + 1) + C0, max(g0 + LA, LB * g0 - LC), B + DIST * BB)
        assert hi <= g0 + B and 0 <= hi - n_iss <= RATE
        n_iss = hi
    assert n_iss == B + DIST * BB and 10 <= W2AT <= 15

    def tr(c):
        return jnp.swapaxes(c, 2, 3).reshape(B, nhp, 2 * Dh, Sk)

    any_spec = pl.BlockSpec(memory_space=pl.ANY)
    return pl.pallas_call(
        functools.partial(_kernel, scale=Dh ** -0.5 * LOG2E, nhp=nhp, nb=B),
        in_specs=[any_spec] * 10,
        out_specs=any_spec,
        out_shape=jax.ShapeDtypeStruct((B, Sq, 2 * D), A_x.dtype),
        scratch_shapes=[pltpu.VMEM((B, Sq, 2 * D), f32),
                        pltpu.VMEM((B, 2, D // 128, Sq // 2, 128), u32),
                        pltpu.VMEM((4 * 15 * 64, 128), u32),
                        pltpu.VMEM((B, 4, 2 * Dh, Sk), bf16),
                        pltpu.VMEM((B, Sq, 2 * D), bf16),
                        pltpu.VMEM((2 * BB * Sq, 6 * 128), u32),
                        pltpu.VMEM((2 * BB * Sq // 4, 6 * 128), u32),
                        pltpu.VMEM((B * 2 * Sq // 4, XCW * 128), u32),
                        pltpu.VMEM((4 * 64, WCW * 128), u32),
                        pltpu.VMEM((4 * 64, WCW * 128), u32),
                        pltpu.SemaphoreType.DMA((B + 4,)),
                        pltpu.SemaphoreType.DMA((B,)),
                        pltpu.SemaphoreType.DMA((4,)),
                        pltpu.SemaphoreType.DMA(())],
        compiler_params=pltpu.CompilerParams(
            disable_bounds_checks=True,
            vmem_limit_bytes=110 * 1024 * 1024),
    )(A_x, tr(A_k_cache), tr(A_v_cache), A_wq, A_wo, B_x, tr(B_k_cache), tr(B_v_cache), B_wq, B_wo)
```

```python
import functools

import jax
import jax.numpy as jnp
from jax import lax
import jax.experimental.pallas as pl
import jax.experimental.pallas.tpu as pltpu

bf16 = jnp.bfloat16
f32 = jnp.float32
u32 = jnp.uint32
NT = (((1,), (1,)), ((), ()))
LOG2E = 1.4426950408889634

BB = 4
DIST = 2
C0, RATE, LA, LB, LC = 2, 2, 6, 2, 6
W2AT = 11
XCW, WCW = 32, 40

PAT = (
    "qa@0,qb@0,qa@1,qb@1,qa@2,s00@0,s01@0,s10@0,qb@2,s11@0,m0@0,t0@0,s00@1,qa@3,s01@1,t1@0,s10@1,qb@3,m1@0,"
    "s11@1,m0@1,t0@1,s00@2,qa@4,s01@2,m1@1,t1@1,s10@2,oa@0,s11@2,m0@2,t0@2,ob@0,s00@3,qa@5,qb@4,s01@3,t1@2,"
    "m1@2,s10@3,oa@1,qb@5,s11@3,m0@3,t0@3,ob@1,s00@4,oa@2,qa@6,s01@4,m1@3,t1@3,s10@4,s11@4,m0@4,t0@4,s00@5,"
    "ob@2,qb@6,qa@7,s01@5,m1@4,t1@4,s10@5,oa@3,qb@7,s11@5,m0@5,t0@5,ob@3,s00@6,oa@4,s01@6,s10@6,m1@5,t1@5,"
    "s11@6,m0@6,t0@6,ob@4,s00@7,s01@7,m1@6,t1@6,s10@7,oa@5,s11@7,m0@7,t0@7,ob@5,m1@7,t1@7,oa@6,ob@6,oa@7,"
    "ob@7")
SPAT = (
    "qa@0,qb@0,qa@1,s00@0,s10@0,s11@0,s01@0,qb@1,m1@0,m0@0,t0@0,s00@1,s01@1,t1@0,s10@1,s11@1,oa@0,m0@1,m1@1,"
    "t0@1,t1@1,ob@0,oa@1,ob@1")
LPAT = PAT
QORD = "9.16.24.21.19.1.15.20.18.22.17.23.12.3.2.4.5.7.6.8.14.0.10.11.13"
OORD = "0.6.1.5.3.2.8.9.4.24.12.11.14.10.16.19.13.15.17.18.20.22.21.23.7"
SQORD = "3.16.24.15.18.10.20.21.9.7.22.1.23.6.12.0.2.14.8.17.13.11.4.5.19"
SOORD = "4.0.3.1.5.6.8.2.9.14.24.10.12.13.15.21.11.19.17.16.18.20.23.22.7"
LQORD = QORD
LOORD = OORD
STEADY = (PAT, QORD, OORD, 11, 10)
RAMP = (SPAT, SQORD, SOORD, 13, 13)
LAST = (LPAT, LQORD, LOORD, 11, 10)
PLO, PHI, SWLO, SWHI, SXLO, SXHI = 300, 520, 140, 920, 1580, 100

O_LHS_PROG = [
    (100, 4, 5, 1), (101, 0, 1, -1), (102, 3, 101, 1), (103, 2, 100, 1), (104, 0, 3, 1),
    (105, 2, 3, -1), (106, 0, 2, 1), (107, 2, 101, -1), (108, 3, 5, 1), (109, 1, 103, 1),
    (110, 2, 5, 1), (111, 3, 100, -1), (112, 5, 101, 1), (113, 4, 102, -1), (114, 0, 100, 1),
]
O_OUT_PROG = [
    (100, 5, 8, -1), (101, 3, 100, 1), (102, 2, 7, -1), (103, 0, 102, 1),
]
O_PRODS = [
    ((101, 1), [(2, 1), (5, 1), (10, -1), (12, 1)], [(102, 1)]),
    ((104, 1), [(3, 1)], [(100, -1)]),
    ((111, 1), [(0, 1), (3, 1)], [(5, 1)]),
    ((5, 1), [(5, 1), (10, -1)], [(5, -1), (103, 1)]),
    ((112, 1), [(5, 1), (10, -1), (12, 1)], [(103, -1)]),
    ((114, 1), [(0, 1), (3, 1), (5, 1)], [(101, 1)]),
    ((0, 1), [(0, 1), (5, 1)], [(0, 1), (101, -1)]),
    ((107, -1), [(10, 1), (12, -1)], [(0, -1)]),
    ((110, 1), [(12, 1)], [(0, 1), (2, 1)]),
    ((1, 1), [(2, 1), (7, 1)], [(2, 1), (4, -1)]),
    ((104, 1), [(1, 1), (2, 1), (4, 1), (7, 1), (9, 1)], [(4, 1)]),
    ((106, 1), [(1, 1)], [(1, 1), (4, -1)]),
    ((1, 1), [(6, 1)], [(1, 1), (3, -1)]),
    ((109, 1), [(6, 1), (8, 1)], [(3, 1)]),
    ((2, 1), [(1, 1), (11, -1)], [(1, -1), (6, 1)]),
    ((103, 1), [(6, 1), (8, 1), (13, -1)], [(3, -1), (6, 1)]),
    ((100, 1), [(0, 1), (3, 1), (5, 1), (13, 1)], [(3, -1), (8, 1)]),
    ((4, 1), [(8, 1), (13, -1)], [(6, -1), (8, 1)]),
    ((110, 1), [(6, 1), (8, 1), (11, -1), (13, -1), (14, -1)], [(6, -1)]),
    ((105, 1), [(1, 1), (14, 1)], [(4, 1), (6, -1)]),
    ((108, 1), [(14, 1)], [(6, -1), (9, 1)]),
    ((3, 1), [(4, 1), (14, -1)], [(4, -1), (9, 1)]),
    ((4, 1), [(9, 1)], [(7, -1), (9, 1)]),
    ((102, 1), [(2, 1), (7, 1), (9, 1)], [(4, -1), (7, 1)]),
    ((113, -1), [(7, 1), (9, 1)], [(7, -1)]),
]
Q_LHS_PROG = [
    (100, 3, 8, -1), (101, 0, 2, 1), (102, 7, 101, -1), (103, 5, 100, 1), (104, 4, 6, -1),
    (105, 4, 9, -1), (106, 7, 9, -1), (107, 0, 103, -1), (108, 6, 8, -1), (109, 5, 102, 1),
    (110, 1, 4, -1), (111, 5, 8, -1), (112, 6, 9, -1), (113, 4, 7, -1), (114, 2, 4, -1),
    (115, 1, 6, -1), (116, 2, 7, -1), (117, 1, 3, -1), (118, 3, 6, -1),
]
Q_OUT_PROG = [
    (100, 0, 3, 1), (101, 4, 5, 1), (102, 0, 1, -1), (103, 2, 101, 1), (104, 2, 5, 1),
    (105, 1, 100, -1),
]
Q_PRODS = [
    ((6, -1), [(6, 1), (8, 1), (11, -1), (13, -1), (14, -1)], [(104, 1)]),
    ((101, 1), [(12, 1)], [(104, 1)]),
    ((4, 1), [(1, 1), (2, 1), (4, 1), (7, 1), (9, 1)], [(100, 1)]),
    ((111, -1), [(3, 1)], [(100, 1)]),
    ((118, -1), [(6, 1), (8, 1), (13, -1)], [(103, 1)]),
    ((3, 1), [(6, 1), (8, 1)], [(1, 1), (103, 1)]),
    ((114, 1), [(2, 1), (7, 1)], [(1, 1)]),
    ((117, 1), [(6, 1)], [(1, 1)]),
    ((115, -1), [(1, 1), (11, -1)], [(2, 1)]),
    ((0, -1), [(10, 1), (12, -1)], [(2, -1), (102, 1)]),
    ((116, 1), [(2, 1), (5, 1), (10, -1), (12, 1)], [(102, 1)]),
    ((102, 1), [(5, 1), (10, -1), (12, 1)], [(5, 1), (102, 1)]),
    ((109, -1), [(5, 1), (10, -1)], [(5, 1)]),
    ((112, -1), [(14, 1)], [(3, 1), (5, 1)]),
    ((104, 1), [(1, 1), (14, 1)], [(2, 1), (3, -1)]),
    ((105, -1), [(4, 1), (14, -1)], [(3, 1)]),
    ((5, 1), [(0, 1), (3, 1)], [(3, 1), (101, -1)]),
    ((100, -1), [(0, 1), (3, 1), (5, 1), (13, 1)], [(101, 1)]),
    ((103, 1), [(0, 1), (3, 1), (5, 1)], [(0, 1), (101, 1)]),
    ((110, 1), [(1, 1)], [(0, 1), (2, 1)]),
    ((107, 1), [(0, 1), (5, 1)], [(0, 1)]),
    ((113, -1), [(2, 1), (7, 1), (9, 1)], [(105, -1)]),
    ((7, -1), [(7, 1), (9, 1)], [(4, -1), (105, -1)]),
    ((106, -1), [(9, 1)], [(4, 1)]),
    ((108, -1), [(8, 1), (13, -1)], [(4, 1)]),
]
NPROD = len(O_PRODS)


def _normalize(prods):
    out = []
    for (var, sgn), w, g in prods:
        sgn *= w[0][1]
        out.append((var, [(y, c * w[0][1]) for y, c in w], [(z, c * sgn) for z, c in g]))
    return out


def _positive_outputs(prods, prog):
    for flips in range(1 << 6):
        sg = [(-1 if (flips >> (r % 6)) & 1 else 1) for r in range(len(prods))]
        pos = {}
        for r, p in enumerate(prods):
            for z, c in p[2]:
                pos[z] = max(pos.get(z, -1), c * sg[r])
        for t, a, b, s in reversed(prog):
            st = pos.pop(t)
            pos[a] = max(pos.get(a, -1), st)
            pos[b] = max(pos.get(b, -1), st * s)
        if min(pos.values()) > 0:
            return sg
    raise AssertionError


O_PRODS = _normalize(O_PRODS)
Q_PRODS = _normalize(Q_PRODS)
W_FORMS = [p[1] for p in O_PRODS]
Q_SIGN = _positive_outputs(Q_PRODS, Q_OUT_PROG)
Q_PRODS = [(v, w, [(z, c * s) for z, c in g]) for (v, w, g), s in zip(Q_PRODS, Q_SIGN)]


def _make_lhs(block, prog):
    vals = {}

    def get(v):
        if v not in vals:
            vals[v] = block(v)
        return vals[v]

    for t, a, b, s in prog:
        vals[t] = get(a) + get(b) if s > 0 else get(a) - get(b)
    return get


def _acc_add(accs, z, sgn, m):
    if z not in accs:
        accs[z] = (sgn, m)
    else:
        s0, a = accs[z]
        accs[z] = (s0, a + m) if s0 == sgn else ((1, a - m) if s0 > 0 else (1, m - a))


def _bilinear_run(accs, prods, which, lhs_of, w_of, tick):
    for r in which:
        m = tick(jnp.dot(lhs_of(r), w_of(r), preferred_element_type=f32), 20)
        for z, c in prods[r][2]:
            _acc_add(accs, z, c, m)


def _bilinear_finish(accs, prog):
    for t, a, b, s in reversed(prog):
        st, v = accs.pop(t)
        _acc_add(accs, a, st, v)
        _acc_add(accs, b, st * s, v)
    return accs


def _mul(i, n):
    return i * n if isinstance(i, int) else pl.multiple_of(i * n, 16)


def _as_bf16(packed):
    return pltpu.bitcast(packed, bf16)


def _as_f32(packed):
    return pltpu.bitcast(packed, bf16).astype(f32)


def _q_operands(c):
    assert all(s > 0 for row in c for s, _ in row)
    (t0, t1, t2), (b0, b1, b2) = [[a for _, a in row] for row in c]
    lo = lax.broadcasted_iota(jnp.int32, t0.shape, 1) < 64
    return [[jnp.where(lo, t0, b0), jnp.where(lo, t1, t0 - b0), jnp.where(lo, b0 - t0, pltpu.roll(b1, 64, 1))],
            [jnp.where(lo, t2, b2), jnp.where(lo, pltpu.roll(t1, 64, 1), t2 - b2), jnp.where(lo, b2 - t2, b1)]]


def _scores_half(qh, kt, h, j, tick):
    k0, k1, k2 = (0, 64, 128) if h == 0 else (256, 320, 192)
    out = []
    for c in (2 * j, 2 * j + 1):
        cs = slice(c * 128, (c + 1) * 128)
        w = [kt[k0:k0 + 128, cs],
             jnp.concatenate([kt[k2:k2 + 64, cs], kt[k1:k1 + 64, cs]], axis=0),
             jnp.concatenate([kt[k0:k0 + 64, cs], kt[k2:k2 + 64, cs]], axis=0)]
        m = [tick(jnp.dot(qh[i], w[i], preferred_element_type=f32), 20) for i in range(3)]
        out.append(jnp.concatenate([m[0] + m[1], m[0] + m[2]], axis=0))
    return out


def _softmax(s):
    m = jnp.max(s, axis=1, keepdims=True)
    p = jnp.exp2(s - m)
    p0, p1, p2, p3 = (p[:, i * 128:(i + 1) * 128] for i in range(4))
    s01, s23 = p0 + p1, p2 + p3
    t = s01 + s23
    l = jnp.sum(t, axis=1, keepdims=True)
    r = pl.reciprocal(l, approx=True)
    r = r * (2.0 - l * r)
    return jnp.concatenate([s01, jnp.minimum(s23, t), p0, p2, p1, p3], axis=1).astype(bf16), r


def _pv_weights(vt, h, i):
    d0, d1, d2 = (0, 64, 128) if h == 0 else (256, 320, 192)

    def v(d, c):
        return vt[d:d + 64, c * 128:(c + 1) * 128]

    def f(d, c):
        return v(d, c).astype(f32)

    if i == 0:
        return jnp.concatenate([jnp.concatenate([v(d0, c), v(d1, c + 1)], axis=0) for c in (0, 2)], axis=1)
    if i == 1:
        w = [jnp.concatenate([f(d2, c), f(d1, c) - f(d1, c + 1)], axis=0) for c in (0, 2)]
    else:
        w = [jnp.concatenate([f(d0, c + 1) - f(d0, c), f(d2, c + 1)], axis=0) for c in (0, 2)]
    return jnp.concatenate(w, axis=1).astype(bf16)


def _kernel(ax, ak, av, awq, awo, bx, bk, bv, bwq, bwo, o_hbm,
            acc, x32, w32, kvbuf, obuf, pbuf, qbuf, xc32, wc0, wc1,
            kv_sem, x_sem, w_sem, o_sem, *, scale, nhp, nb):
    xbuf, wbuf = (r.bitcast(bf16) for r in (x32, w32))
    pbuf, qbuf, xc = (r.bitcast(bf16) for r in (pbuf, qbuf, xc32))
    wc = [r.bitcast(bf16) for r in (wc0, wc1)]
    sq = xbuf.shape[3]
    hq = sq // 2
    d = awq.shape[0]
    hw = kvbuf.shape[2]
    wrows = wbuf.shape[0] // 4
    ng = nhp * nb
    lg = nb.bit_length() - 1
    spb = nb // BB

    def kv_start(g):
        hp, b = (g >> lg) & (nhp - 1), g & (nb - 1)
        for i, src in enumerate((ak, av, bk, bv)):
            sem = kv_sem.at[jnp.where(g < nb, b, nb + (b >> 2))]
            pltpu.make_async_copy(src.at[b, hp], kvbuf.at[b, i], sem).start()

    def kv_wait(b):
        pltpu.make_async_copy(kvbuf.at[b], kvbuf.at[b], kv_sem.at[b]).wait()

    def kvg_start(g):
        hp, i4 = g >> lg, (g >> 2) & 3
        b = pl.multiple_of(i4 * BB, BB)
        for i, src in enumerate((ak, av, bk, bv)):
            pltpu.make_async_copy(src.at[pl.ds(b, BB), hp], kvbuf.at[pl.ds(b, BB), i], kv_sem.at[nb + i4]).start()

    def kvg_wait(i4):
        v = kvbuf.at[pl.ds(i4 * BB, BB)]
        pltpu.make_async_copy(v, v, kv_sem.at[nb + i4]).wait()

    def x_start(b, which=(0, 1)):
        for i, src in enumerate((ax, bx)):
            if i in which:
                for c in range(xbuf.shape[2]):
                    pltpu.make_async_copy(src.at[b, :, pl.ds(c * 128, 128)], xbuf.at[b, i, c], x_sem.at[b]).start()

    def x_wait(b):
        pltpu.make_async_copy(xbuf.at[b], xbuf.at[b], x_sem.at[b]).wait()

    def w_start(h, m):
        off = h * hw if isinstance(h, int) else pl.multiple_of(h * hw, 128)
        if m < 2:
            for c in range(hw // 128):
                pltpu.make_async_copy((awq, bwq)[m].at[:, pl.ds(off + c * 128, 128)],
                                      wbuf.at[pl.ds(m * wrows + c * d, d)], w_sem.at[m]).start()
        else:
            for c in range(d // 128):
                pltpu.make_async_copy((awo, bwo)[m - 2].at[pl.ds(off, hw), pl.ds(c * 128, 128)],
                                      wbuf.at[pl.ds(m * wrows + c * hw, hw)], w_sem.at[m]).start()

    def w_start_dyn(h, m, valid):
        for k in range(4):
            @pl.when(jnp.logical_and(m == k, valid))
            def _():
                w_start(h, k)

    def w_wait(m):
        v = wbuf.at[pl.ds(_mul(m, wrows), wrows)]
        pltpu.make_async_copy(v, v, w_sem.at[m]).wait()

    def prep_w(dst, msrc, mdst, row, nrows, zero=None, sub=0):
        whole = isinstance(row, int) and row == 0
        if isinstance(msrc, int):
            sa, sc = (5, 1) if msrc < 2 else (1, 3)
            off = [(msrc * 15 + (y // 5) * sa + (y % 5) * sc) * 64 + row * 8 for y in range(15)]
        else:
            sa, sc = jnp.where(msrc < 2, 5, 1), jnp.where(msrc < 2, 1, 3)
            off = [pl.multiple_of((msrc * 15 + (y // 5) * sa + (y % 5) * sc) * 64 + row * 8, 64 if whole else 32)
                   for y in range(15)]
        r16 = _mul(mdst * 8 + row, 16)
        if not isinstance(r16, int):
            r16 = pl.multiple_of(r16, 128 if whole else 64)
        for r, form in enumerate(W_FORMS):
            if len(form) == 1:
                val = _as_bf16(w32[pl.ds(off[form[0][0]] + sub * 8, nrows * 8), :])
            else:
                val = None
                for y, c in form:
                    t = _as_f32(w32[pl.ds(off[y] + sub * 8, nrows * 8), :])
                    val = t if val is None else (val + t if c > 0 else val - t)
                val = val.astype(bf16)
            wc[dst][pl.ds(r16 + sub * 16, nrows * 16), r * 128:(r + 1) * 128] = val
        if zero is not None:
            return lambda: wc[dst][pl.ds(pl.multiple_of(r16 + zero * 16 + sub * 16, 16), 16), 0:128].astype(f32)[0:8]

    def prep_x(b, br, k0=0, k1=5, zero=None):
        get = _make_lhs(
            lambda z: _as_f32(x32[b, br, z % 5, (z // 5) * (hq // 2) + k0 * 8:(z // 5) * (hq // 2) + k1 * 8, :])
            * scale, Q_LHS_PROG)
        for r, p in enumerate(Q_PRODS):
            xc[pl.ds(_mul(b * 2 + br, hq) + k0 * 16, (k1 - k0) * 16), r * 128:(r + 1) * 128] = (
                get(p[0]) * Q_SIGN[r]).astype(bf16)
        if zero is not None:
            c0 = (NPROD - 1) * 128
            return lambda: xc[pl.ds(_mul(b * 2 + br + zero, hq) + k0 * 16, 16), c0:c0 + 128].astype(f32)[0:8]

    def body(g0, nbat, first, wpre, xpre, plan, cs, first_hp=False, last_hp=False):
        b0 = g0 & (nb - 1)
        pat, qord, oord, qsp, osp = plan
        sched = [(a.split("@")[0], int(a.split("@")[1])) for a in pat.split(",")]
        qord = [int(i) for i in qord.split(".")]
        oord = [int(i) for i in oord.split(".")]
        assert all(sched.index(("ob", u)) < sched.index(("ob", u + 1)) for u in range(0, 2 * nbat, 2))
        R, O, OT, QA, OA, SC, LH = {}, {}, {}, {}, {}, {}, {}
        lazy = {}
        pending = []
        clock = [0]

        def tick(o, cycles):
            t0 = clock[0]
            clock[0] += cycles
            groups = o.shape[0] // 8
            rows = None
            while pending and pending[0][0] <= clock[0]:
                due, emit = pending.pop(0)
                tok = emit()
                g = min(max((due - t0) * groups // cycles, 0), groups - 1)
                rows = rows or [o[8 * i:8 * i + 8] for i in range(groups)]
                rows[g] = jnp.minimum(rows[g], jnp.maximum(rows[g], tok()))
            return o if rows is None else jnp.concatenate(rows, axis=0)

        def later(delay, emit):
            pending.append((clock[0] + delay, emit))
            pending.sort(key=lambda e: e[0])

        def prow(u, h):
            return (2 * u + h) * sq

        def weights(m, prods):
            def w_of(r):
                s = W_FORMS.index(prods[r][1])
                return wc[cs][m * 128:(m + 1) * 128, s * 128:(s + 1) * 128]
            return w_of

        def q_(u, lo_, hi_):
            b, br = b0 + u // 2, u % 2

            def lhs_of(r):
                return xc[pl.ds(_mul(b * 2 + br, hq), hq), r * 128:(r + 1) * 128]

            _bilinear_run(QA.setdefault(u, {}), Q_PRODS, qord[lo_:hi_], lhs_of, weights(br, Q_PRODS), tick)
            if hi_ == NPROD:
                fin = _bilinear_finish(QA[u], Q_OUT_PROG)

                def store_q():
                    c = [[fin[i * 3 + n] for n in range(3)] for i in range(2)]
                    for h, ops in enumerate(_q_operands(c)):
                        for i, a in enumerate(ops):
                            qbuf[u * hq:(u + 1) * hq, (3 * h + i) * 128:(3 * h + i + 1) * 128] = a.astype(bf16)

                lazy["q", u] = store_q

        def s_(u, h, j):
            b, br = b0 + u // 2, u % 2
            lazy.pop(("q", u), lambda: None)()
            qh = [qbuf[u * hq:(u + 1) * hq, (3 * h + i) * 128:(3 * h + i + 1) * 128] for i in range(3)]
            SC[u, h, j] = _scores_half(qh, kvbuf.at[b, 2 * br], h, j, tick)
            if j == 1:
                s = jnp.concatenate(SC[u, h, 0] + SC[u, h, 1], axis=1)

                def store_p():
                    p, R[u, h] = _softmax(s)
                    pbuf[prow(u, h):prow(u, h) + sq, :] = p

                lazy["p", u, h] = store_p

        def m_(u, h, half):
            lazy.pop(("p", u, h), lambda: None)()
            vt = kvbuf.at[b0 + u // 2 + (g0 >> 20) * half, 2 * (u % 2) + 1]
            r0 = prow(u, h) + half * hq
            res = [tick(lax.dot_general(pbuf[r0:r0 + hq, i * 256:(i + 1) * 256], _pv_weights(vt, h, i), NT,
                                        preferred_element_type=f32), 40) for i in range(3)]
            lo = lax.broadcasted_iota(jnp.int32, (hq, 128), 1) < 64
            r = R[u, h][half * hq:(half + 1) * hq]
            O[u, h, half] = (res[0] + jnp.where(lo, res[2], res[1])) * r
            OT[u, h, half] = jnp.where(lo, res[1], res[2]) * r

        def o_(u, lo_, hi_):
            b, br = b0 + u // 2, u % 2
            if lo_ == 0:
                lo = lax.broadcasted_iota(jnp.int32, (hq, 128), 1) < 64
                mid = [jnp.where(lo, OT[u, 0, i], OT[u, 1, i]) +
                       pltpu.roll(jnp.where(lo, OT[u, 1, i], OT[u, 0, i]), 64, 1) for i in range(2)]
                tiles = [[O[u, 0, i], mid[i], O[u, 1, i]] for i in range(2)]
                get = _make_lhs(lambda x: tiles[x // 3][x % 3], O_LHS_PROG)
                LH[u] = {p[0]: get(p[0]).astype(bf16) for p in O_PRODS}
            _bilinear_run(OA.setdefault(u, {}), O_PRODS, oord[lo_:hi_], lambda r: LH[u][O_PRODS[r][0]],
                          weights(2 + br, O_PRODS), tick)
            if hi_ < NPROD:
                return
            fin = _bilinear_finish(OA[u], O_OUT_PROG)
            for n in range(5):
                for i in range(2):
                    s, a = fin[i * 5 + n]
                    rows = slice(i * hq, (i + 1) * hq)
                    cols = slice(br * d + n * 128, br * d + (n + 1) * 128)
                    if first_hp:
                        new = a if s > 0 else -a
                    else:
                        new = acc[b, rows, cols] + a if s > 0 else acc[b, rows, cols] - a
                    if last_hp:
                        obuf[b, rows, cols] = new.astype(obuf.dtype)
                    else:
                        acc[b, rows, cols] = new
            if br == 1 and last_hp:
                pltpu.make_async_copy(obuf.at[b], o_hbm.at[b], o_sem).start()

        fns = {"qa": lambda u: q_(u, 0, qsp), "qb": lambda u: q_(u, qsp, NPROD),
               "oa": lambda u: o_(u, 0, osp), "ob": lambda u: o_(u, osp, NPROD),
               "s00": lambda u: s_(u, 0, 0), "s01": lambda u: s_(u, 0, 1),
               "s10": lambda u: s_(u, 1, 0), "s11": lambda u: s_(u, 1, 1),
               "m0": lambda u: m_(u, 0, 0), "m1": lambda u: m_(u, 1, 0),
               "t0": lambda u: m_(u, 0, 1), "t1": lambda u: m_(u, 1, 1)}
        for f in first:
            f()
        total = 2 * nbat * 1960
        lastq = max(i for i, it in enumerate(sched) if it[0][0] == "q")
        for k, f in enumerate(wpre):
            lo_, hi_ = (PLO, total - PHI) if nbat > 1 else (SWLO, SWHI)
            later(lo_ + k * (hi_ - lo_) // len(wpre), f)
        for i, item in enumerate(sched):
            fns[item[0]](item[1])
            if i == lastq:
                for k, f in enumerate(xpre):
                    later(SXLO + k * (total - SXHI - clock[0] - SXLO) // len(xpre), f)
        assert not pending and not lazy

    for k in range(4):
        w_start(0, k)
    x_start(0)
    kv_start(0)
    x_start(1)
    for g in range(1, C0):
        kv_start(g)
        x_start(g + 1)
    for m in range(4):
        w_wait(m)
        prep_w(0, m, m, 0, 8)
    x_wait(0)
    for br in range(2):
        prep_x(0, br)

    def issued(g):
        return jnp.minimum(jnp.minimum(RATE * (g + 1) + C0, jnp.maximum(g + LA, LB * g - LC)), nb + DIST * BB)

    def ramp(b0, carry):
        half = nb // 2
        m = (b0 - half) >> 1

        @pl.when(b0 + 1 < nb)
        def _():
            x_wait(b0 + 1)

        @pl.when(jnp.logical_and(b0 >= half, (b0 & 1) == 0))
        def _():
            w_wait(m)

        kv_wait(b0)

        hi = issued(b0)
        prev = jnp.where(b0 == 0, C0, issued(b0 - 1))

        def pf_x(k, w):
            @pl.when(jnp.logical_and(prev + k < hi, prev + k + 1 < nb))
            def _():
                x_start(prev + k + 1, (w,))

        def pf_kv(k):
            @pl.when(prev + k < hi)
            def _():
                kv_start(prev + k)

        def pf_w():
            w_start_dyn(jnp.where(b0 == W2AT, 2, 1), jnp.where(b0 == W2AT, 0, (b0 >> 1) - 1),
                        jnp.logical_or(b0 == W2AT, jnp.logical_and(b0 <= half, (b0 & 1) == 0)))

        first = [pf_w] + [functools.partial(pf_x, k, w) for k in range(RATE) for w in range(2)]
        first += [functools.partial(pf_kv, k) for k in range(RATE)]
        zero = b0 >> 20
        wpre = [functools.partial(prep_w, 1, jnp.where(b0 >= half, m, 3), jnp.maximum(m, 0), (b0 & 1) * 4, 1,
                                  zero, k) for k in range(4)]
        xpre = [functools.partial(prep_x, jnp.minimum(b0 + 1, nb - 1), br, k, k + 1, zero)
                for br in range(2) for k in range(5)]
        body(b0, 1, first, wpre, xpre, RAMP, 0, first_hp=True)
        return carry

    def step(par, last, hp, i, carry):
        g0 = hp * nb + i * BB

        if not last:
            w_wait(i)

        kvg_wait(i)

        if last:
            def pf_kv():
                @pl.when(g0 + DIST * BB < ng)
                def _():
                    kvg_start(g0 + DIST * BB)

            body(g0, BB, [pf_kv], [], [], LAST, par, last_hp=True)
        else:
            hn = jnp.where(i == 3, hp + 2, hp + 1)
            first = [lambda: w_start_dyn(hn, (i + 1) & 3, hn < nhp), functools.partial(kvg_start, g0 + DIST * BB)]
            wpre = [functools.partial(prep_w, 1 - par, i, i, 0, 1, i >> 20, k) for k in range(8)]
            body(g0, BB, first, wpre, [], STEADY, par)
        return carry

    def pair(t, carry):
        lax.fori_loop(jnp.where(t > 0, 0, spb), spb, functools.partial(step, 0, False, 2 * t), 0)
        lax.fori_loop(0, jnp.where(2 * t + 1 < nhp - 1, spb, 0), functools.partial(step, 1, False, 2 * t + 1), 0)
        return carry

    lax.fori_loop(0, nb, ramp, 0)
    lax.fori_loop(0, nhp // 2, pair, 0)
    lax.fori_loop(0, spb, functools.partial(step, 1, True, nhp - 1), 0)
    pltpu.make_async_copy(obuf, o_hbm, o_sem).wait()


@jax.jit
def pallas_concat_heads__gqa_block_cached__mha_block_cached__near_ridge_kernel(
    A_x: jax.Array,
    A_k_cache: jax.Array,
    A_v_cache: jax.Array,
    A_wq: jax.Array,
    A_wo: jax.Array,
    B_x: jax.Array,
    B_k_cache: jax.Array,
    B_v_cache: jax.Array,
    B_wq: jax.Array,
    B_wo: jax.Array,
):
    B, Sq, D = A_x.shape
    _, H, Sk, Dh = A_k_cache.shape
    nhp = H // 2
    assert (B, Sq, D, Sk, Dh) == (16, 160, 640, 512, 192) and A_wq.shape[1] == H * Dh
    assert nhp >= 4 and nhp & (nhp - 1) == 0 and B_k_cache.shape == A_k_cache.shape
    n_iss = C0
    for g0 in range(B):
        assert n_iss >= g0 + 2
        hi = min(RATE * (g0 + 1) + C0, max(g0 + LA, LB * g0 - LC), B + DIST * BB)
        assert hi <= g0 + B and 0 <= hi - n_iss <= RATE
        n_iss = hi
    assert n_iss == B + DIST * BB and 10 <= W2AT <= 15

    def tr(c):
        return jnp.swapaxes(c, 2, 3).reshape(B, nhp, 2 * Dh, Sk)

    any_spec = pl.BlockSpec(memory_space=pl.ANY)
    return pl.pallas_call(
        functools.partial(_kernel, scale=Dh ** -0.5 * LOG2E, nhp=nhp, nb=B),
        in_specs=[any_spec] * 10,
        out_specs=any_spec,
        out_shape=jax.ShapeDtypeStruct((B, Sq, 2 * D), A_x.dtype),
        scratch_shapes=[pltpu.VMEM((B, Sq, 2 * D), f32),
                        pltpu.VMEM((B, 2, D // 128, Sq // 2, 128), u32),
                        pltpu.VMEM((4 * 15 * 64, 128), u32),
                        pltpu.VMEM((B, 4, 2 * Dh, Sk), bf16),
                        pltpu.VMEM((B, Sq, 2 * D), bf16),
                        pltpu.VMEM((2 * BB * Sq, 6 * 128), u32),
                        pltpu.VMEM((2 * BB * Sq // 4, 6 * 128), u32),
                        pltpu.VMEM((B * 2 * Sq // 4, XCW * 128), u32),
                        pltpu.VMEM((4 * 64, WCW * 128), u32),
                        pltpu.VMEM((4 * 64, WCW * 128), u32),
                        pltpu.SemaphoreType.DMA((B + 4,)),
                        pltpu.SemaphoreType.DMA((B,)),
                        pltpu.SemaphoreType.DMA((4,)),
                        pltpu.SemaphoreType.DMA(())],
        compiler_params=pltpu.CompilerParams(
            disable_bounds_checks=True,
            vmem_limit_bytes=110 * 1024 * 1024),
    )(A_x, tr(A_k_cache), tr(A_v_cache), A_wq, A_wo, B_x, tr(B_k_cache), tr(B_v_cache), B_wq, B_wo)
```

```python
import functools

import jax
import jax.numpy as jnp
from jax import lax
import jax.experimental.pallas as pl
import jax.experimental.pallas.tpu as pltpu

bf16 = jnp.bfloat16
f32 = jnp.float32
u32 = jnp.uint32
NT = (((1,), (1,)), ((), ()))
LOG2E = 1.4426950408889634

BB = 4
DIST = 2
C0, RATE, LA, LB, LC = 2, 2, 6, 2, 6
W2AT = 11
XCW, WCW = 32, 40

PAT = (
    "qa@0,qb@0,qa@1,qb@1,qa@2,s00@0,s01@0,s10@0,qb@2,s11@0,m0@0,t0@0,s00@1,qa@3,s01@1,t1@0,s10@1,qb@3,m1@0,"
    "s11@1,m0@1,t0@1,s00@2,qa@4,s01@2,m1@1,t1@1,s10@2,oa@0,s11@2,m0@2,t0@2,ob@0,s00@3,qa@5,qb@4,s01@3,t1@2,"
    "m1@2,s10@3,oa@1,qb@5,s11@3,m0@3,t0@3,ob@1,s00@4,oa@2,qa@6,s01@4,m1@3,t1@3,s10@4,s11@4,m0@4,t0@4,s00@5,"
    "ob@2,qb@6,qa@7,s01@5,m1@4,t1@4,s10@5,oa@3,qb@7,s11@5,m0@5,t0@5,ob@3,s00@6,oa@4,s01@6,s10@6,m1@5,t1@5,"
    "s11@6,m0@6,t0@6,ob@4,s00@7,s01@7,m1@6,t1@6,s10@7,oa@5,s11@7,m0@7,t0@7,ob@5,m1@7,t1@7,oa@6,ob@6,oa@7,"
    "ob@7")
SPAT = (
    "qa@0,qb@0,qa@1,s00@0,s10@0,s11@0,s01@0,qb@1,m1@0,m0@0,t0@0,s00@1,s01@1,t1@0,s10@1,s11@1,oa@0,m0@1,m1@1,"
    "t0@1,t1@1,ob@0,oa@1,ob@1")
LPAT = (
    "qa@0,qb@0,qa@1,qb@1,qa@2,s00@0,s01@0,s10@0,qb@2,s11@0,m0@0,s10@1,t0@0,s00@1,qa@3,s01@1,t1@0,qb@3,m1@0,"
    "s11@1,m0@1,t0@1,s00@2,qa@4,s01@2,m1@1,t1@1,s10@2,oa@0,s11@2,m0@2,ob@0,t0@2,s00@3,qa@5,qb@4,s01@3,t1@2,"
    "m1@2,s10@3,oa@1,qb@5,s11@3,m0@3,t0@3,ob@1,s00@4,qa@6,oa@2,s01@4,m1@3,t1@3,s10@4,s11@4,m0@4,t0@4,s00@5,"
    "ob@2,qb@6,qa@7,s01@5,m1@4,t1@4,s10@5,oa@3,qb@7,s11@5,m0@5,t0@5,ob@3,s00@6,oa@4,s01@6,s10@6,m1@5,t1@5,"
    "s11@6,m0@6,t0@6,ob@4,s00@7,s01@7,m1@6,t1@6,s10@7,oa@5,s11@7,m0@7,t0@7,ob@5,m1@7,t1@7,oa@6,ob@6,oa@7,"
    "ob@7")
QORD = "9.16.24.21.19.1.15.20.18.22.17.23.12.3.2.4.5.7.6.8.14.0.10.11.13"
OORD = "0.6.1.5.3.2.8.9.4.24.12.11.14.10.16.19.13.15.17.18.20.22.21.23.7"
SQORD = "3.16.24.15.18.10.20.21.9.7.22.1.23.6.12.0.2.14.8.17.13.11.4.5.19"
SOORD = "4.0.3.1.5.6.8.2.9.14.24.10.12.13.15.21.11.19.17.16.18.20.23.22.7"
LQORD = "9.16.24.21.19.1.15.20.18.22.17.23.12.3.2.4.7.6.8.5.14.0.10.11.13"
LOORD = "0.6.1.5.3.2.8.9.4.24.12.11.14.10.16.19.13.15.17.18.20.22.21.23.7"
STEADY = (PAT, QORD, OORD, 11, 10)
RAMP = (SPAT, SQORD, SOORD, 13, 13)
LAST = (LPAT, LQORD, LOORD, 11, 10)
PLO, PHI, SWLO, SWHI, SXLO, SXHI = 300, 520, 140, 920, 1580, 100

O_LHS_PROG = [
    (100, 4, 5, 1), (101, 0, 1, -1), (102, 3, 101, 1), (103, 2, 100, 1), (104, 0, 3, 1),
    (105, 2, 3, -1), (106, 0, 2, 1), (107, 2, 101, -1), (108, 3, 5, 1), (109, 1, 103, 1),
    (110, 2, 5, 1), (111, 3, 100, -1), (112, 5, 101, 1), (113, 4, 102, -1), (114, 0, 100, 1),
]
O_OUT_PROG = [
    (100, 5, 8, -1), (101, 3, 100, 1), (102, 2, 7, -1), (103, 0, 102, 1),
]
O_PRODS = [
    ((101, 1), [(2, 1), (5, 1), (10, -1), (12, 1)], [(102, 1)]),
    ((104, 1), [(3, 1)], [(100, -1)]),
    ((111, 1), [(0, 1), (3, 1)], [(5, 1)]),
    ((5, 1), [(5, 1), (10, -1)], [(5, -1), (103, 1)]),
    ((112, 1), [(5, 1), (10, -1), (12, 1)], [(103, -1)]),
    ((114, 1), [(0, 1), (3, 1), (5, 1)], [(101, 1)]),
    ((0, 1), [(0, 1), (5, 1)], [(0, 1), (101, -1)]),
    ((107, -1), [(10, 1), (12, -1)], [(0, -1)]),
    ((110, 1), [(12, 1)], [(0, 1), (2, 1)]),
    ((1, 1), [(2, 1), (7, 1)], [(2, 1), (4, -1)]),
    ((104, 1), [(1, 1), (2, 1), (4, 1), (7, 1), (9, 1)], [(4, 1)]),
    ((106, 1), [(1, 1)], [(1, 1), (4, -1)]),
    ((1, 1), [(6, 1)], [(1, 1), (3, -1)]),
    ((109, 1), [(6, 1), (8, 1)], [(3, 1)]),
    ((2, 1), [(1, 1), (11, -1)], [(1, -1), (6, 1)]),
    ((103, 1), [(6, 1), (8, 1), (13, -1)], [(3, -1), (6, 1)]),
    ((100, 1), [(0, 1), (3, 1), (5, 1), (13, 1)], [(3, -1), (8, 1)]),
    ((4, 1), [(8, 1), (13, -1)], [(6, -1), (8, 1)]),
    ((110, 1), [(6, 1), (8, 1), (11, -1), (13, -1), (14, -1)], [(6, -1)]),
    ((105, 1), [(1, 1), (14, 1)], [(4, 1), (6, -1)]),
    ((108, 1), [(14, 1)], [(6, -1), (9, 1)]),
    ((3, 1), [(4, 1), (14, -1)], [(4, -1), (9, 1)]),
    ((4, 1), [(9, 1)], [(7, -1), (9, 1)]),
    ((102, 1), [(2, 1), (7, 1), (9, 1)], [(4, -1), (7, 1)]),
    ((113, -1), [(7, 1), (9, 1)], [(7, -1)]),
]
Q_LHS_PROG = [
    (100, 3, 8, -1), (101, 0, 2, 1), (102, 7, 101, -1), (103, 5, 100, 1), (104, 4, 6, -1),
    (105, 4, 9, -1), (106, 7, 9, -1), (107, 0, 103, -1), (108, 6, 8, -1), (109, 5, 102, 1),
    (110, 1, 4, -1), (111, 5, 8, -1), (112, 6, 9, -1), (113, 4, 7, -1), (114, 2, 4, -1),
    (115, 1, 6, -1), (116, 2, 7, -1), (117, 1, 3, -1), (118, 3, 6, -1),
]
Q_OUT_PROG = [
    (100, 0, 3, 1), (101, 4, 5, 1), (102, 0, 1, -1), (103, 2, 101, 1), (104, 2, 5, 1),
    (105, 1, 100, -1),
]
Q_PRODS = [
    ((6, -1), [(6, 1), (8, 1), (11, -1), (13, -1), (14, -1)], [(104, 1)]),
    ((101, 1), [(12, 1)], [(104, 1)]),
    ((4, 1), [(1, 1), (2, 1), (4, 1), (7, 1), (9, 1)], [(100, 1)]),
    ((111, -1), [(3, 1)], [(100, 1)]),
    ((118, -1), [(6, 1), (8, 1), (13, -1)], [(103, 1)]),
    ((3, 1), [(6, 1), (8, 1)], [(1, 1), (103, 1)]),
    ((114, 1), [(2, 1), (7, 1)], [(1, 1)]),
    ((117, 1), [(6, 1)], [(1, 1)]),
    ((115, -1), [(1, 1), (11, -1)], [(2, 1)]),
    ((0, -1), [(10, 1), (12, -1)], [(2, -1), (102, 1)]),
    ((116, 1), [(2, 1), (5, 1), (10, -1), (12, 1)], [(102, 1)]),
    ((102, 1), [(5, 1), (10, -1), (12, 1)], [(5, 1), (102, 1)]),
    ((109, -1), [(5, 1), (10, -1)], [(5, 1)]),
    ((112, -1), [(14, 1)], [(3, 1), (5, 1)]),
    ((104, 1), [(1, 1), (14, 1)], [(2, 1), (3, -1)]),
    ((105, -1), [(4, 1), (14, -1)], [(3, 1)]),
    ((5, 1), [(0, 1), (3, 1)], [(3, 1), (101, -1)]),
    ((100, -1), [(0, 1), (3, 1), (5, 1), (13, 1)], [(101, 1)]),
    ((103, 1), [(0, 1), (3, 1), (5, 1)], [(0, 1), (101, 1)]),
    ((110, 1), [(1, 1)], [(0, 1), (2, 1)]),
    ((107, 1), [(0, 1), (5, 1)], [(0, 1)]),
    ((113, -1), [(2, 1), (7, 1), (9, 1)], [(105, -1)]),
    ((7, -1), [(7, 1), (9, 1)], [(4, -1), (105, -1)]),
    ((106, -1), [(9, 1)], [(4, 1)]),
    ((108, -1), [(8, 1), (13, -1)], [(4, 1)]),
]
NPROD = len(O_PRODS)


def _normalize(prods):
    out = []
    for (var, sgn), w, g in prods:
        sgn *= w[0][1]
        out.append((var, [(y, c * w[0][1]) for y, c in w], [(z, c * sgn) for z, c in g]))
    return out


def _positive_outputs(prods, prog):
    for flips in range(1 << 6):
        sg = [(-1 if (flips >> (r % 6)) & 1 else 1) for r in range(len(prods))]
        pos = {}
        for r, p in enumerate(prods):
            for z, c in p[2]:
                pos[z] = max(pos.get(z, -1), c * sg[r])
        for t, a, b, s in reversed(prog):
            st = pos.pop(t)
            pos[a] = max(pos.get(a, -1), st)
            pos[b] = max(pos.get(b, -1), st * s)
        if min(pos.values()) > 0:
            return sg
    raise AssertionError


O_PRODS = _normalize(O_PRODS)
Q_PRODS = _normalize(Q_PRODS)
W_FORMS = [p[1] for p in O_PRODS]
Q_SIGN = _positive_outputs(Q_PRODS, Q_OUT_PROG)
Q_PRODS = [(v, w, [(z, c * s) for z, c in g]) for (v, w, g), s in zip(Q_PRODS, Q_SIGN)]


def _make_lhs(block, prog):
    vals = {}

    def get(v):
        if v not in vals:
            vals[v] = block(v)
        return vals[v]

    for t, a, b, s in prog:
        vals[t] = get(a) + get(b) if s > 0 else get(a) - get(b)
    return get


def _acc_add(accs, z, sgn, m):
    if z not in accs:
        accs[z] = (sgn, m)
    else:
        s0, a = accs[z]
        accs[z] = (s0, a + m) if s0 == sgn else ((1, a - m) if s0 > 0 else (1, m - a))


def _bilinear_run(accs, prods, which, lhs_of, w_of, tick):
    for r in which:
        m = tick(jnp.dot(lhs_of(r), w_of(r), preferred_element_type=f32), 20)
        for z, c in prods[r][2]:
            _acc_add(accs, z, c, m)


def _bilinear_finish(accs, prog):
    for t, a, b, s in reversed(prog):
        st, v = accs.pop(t)
        _acc_add(accs, a, st, v)
        _acc_add(accs, b, st * s, v)
    return accs


def _mul(i, n):
    return i * n if isinstance(i, int) else pl.multiple_of(i * n, 16)


def _as_bf16(packed):
    return pltpu.bitcast(packed, bf16)


def _as_f32(packed):
    return pltpu.bitcast(packed, bf16).astype(f32)


def _q_operands(c):
    assert all(s > 0 for row in c for s, _ in row)
    (t0, t1, t2), (b0, b1, b2) = [[a for _, a in row] for row in c]
    lo = lax.broadcasted_iota(jnp.int32, t0.shape, 1) < 64
    return [[jnp.where(lo, t0, b0), jnp.where(lo, t1, t0 - b0), jnp.where(lo, b0 - t0, pltpu.roll(b1, 64, 1))],
            [jnp.where(lo, t2, b2), jnp.where(lo, pltpu.roll(t1, 64, 1), t2 - b2), jnp.where(lo, b2 - t2, b1)]]


def _scores_half(qh, kt, h, j, tick):
    k0, k1, k2 = (0, 64, 128) if h == 0 else (256, 320, 192)
    out = []
    for c in (2 * j, 2 * j + 1):
        cs = slice(c * 128, (c + 1) * 128)
        w = [kt[k0:k0 + 128, cs],
             jnp.concatenate([kt[k2:k2 + 64, cs], kt[k1:k1 + 64, cs]], axis=0),
             jnp.concatenate([kt[k0:k0 + 64, cs], kt[k2:k2 + 64, cs]], axis=0)]
        m = [tick(jnp.dot(qh[i], w[i], preferred_element_type=f32), 20) for i in range(3)]
        out.append(jnp.concatenate([m[0] + m[1], m[0] + m[2]], axis=0))
    return out


def _softmax(s):
    m = jnp.max(s, axis=1, keepdims=True)
    p = jnp.exp2(s - m)
    p0, p1, p2, p3 = (p[:, i * 128:(i + 1) * 128] for i in range(4))
    s01, s23 = p0 + p1, p2 + p3
    t = s01 + s23
    l = jnp.sum(t, axis=1, keepdims=True)
    r = pl.reciprocal(l, approx=True)
    r = r * (2.0 - l * r)
    return jnp.concatenate([s01, jnp.minimum(s23, t), p0, p2, p1, p3], axis=1).astype(bf16), r


def _pv_weights(vt, h, i):
    d0, d1, d2 = (0, 64, 128) if h == 0 else (256, 320, 192)

    def v(d, c):
        return vt[d:d + 64, c * 128:(c + 1) * 128]

    def f(d, c):
        return v(d, c).astype(f32)

    if i == 0:
        return jnp.concatenate([jnp.concatenate([v(d0, c), v(d1, c + 1)], axis=0) for c in (0, 2)], axis=1)
    if i == 1:
        w = [jnp.concatenate([f(d2, c), f(d1, c) - f(d1, c + 1)], axis=0) for c in (0, 2)]
    else:
        w = [jnp.concatenate([f(d0, c + 1) - f(d0, c), f(d2, c + 1)], axis=0) for c in (0, 2)]
    return jnp.concatenate(w, axis=1).astype(bf16)


def _kernel(ax, ak, av, awq, awo, bx, bk, bv, bwq, bwo, o_hbm,
            acc, x32, w32, kvbuf, obuf, pbuf, qbuf, xc32, wc0, wc1,
            kv_sem, x_sem, w_sem, o_sem, *, scale, nhp, nb):
    xbuf, wbuf = (r.bitcast(bf16) for r in (x32, w32))
    pbuf, qbuf, xc = (r.bitcast(bf16) for r in (pbuf, qbuf, xc32))
    wc = [r.bitcast(bf16) for r in (wc0, wc1)]
    sq = xbuf.shape[3]
    hq = sq // 2
    d = awq.shape[0]
    hw = kvbuf.shape[2]
    wrows = wbuf.shape[0] // 4
    ng = nhp * nb
    lg = nb.bit_length() - 1
    spb = nb // BB

    def kv_start(g):
        hp, b = (g >> lg) & (nhp - 1), g & (nb - 1)
        for i, src in enumerate((ak, av, bk, bv)):
            sem = kv_sem.at[jnp.where(g < nb, b, nb + (b >> 2))]
            pltpu.make_async_copy(src.at[b, hp], kvbuf.at[b, i], sem).start()

    def kv_wait(b):
        pltpu.make_async_copy(kvbuf.at[b], kvbuf.at[b], kv_sem.at[b]).wait()

    def kvg_start(g):
        hp, i4 = g >> lg, (g >> 2) & 3
        b = pl.multiple_of(i4 * BB, BB)
        for i, src in enumerate((ak, av, bk, bv)):
            pltpu.make_async_copy(src.at[pl.ds(b, BB), hp], kvbuf.at[pl.ds(b, BB), i], kv_sem.at[nb + i4]).start()

    def kvg_wait(i4):
        v = kvbuf.at[pl.ds(i4 * BB, BB)]
        pltpu.make_async_copy(v, v, kv_sem.at[nb + i4]).wait()

    def x_start(b, which=(0, 1)):
        for i, src in enumerate((ax, bx)):
            if i in which:
                for c in range(xbuf.shape[2]):
                    pltpu.make_async_copy(src.at[b, :, pl.ds(c * 128, 128)], xbuf.at[b, i, c], x_sem.at[b]).start()

    def x_wait(b):
        pltpu.make_async_copy(xbuf.at[b], xbuf.at[b], x_sem.at[b]).wait()

    def w_start(h, m):
        off = h * hw if isinstance(h, int) else pl.multiple_of(h * hw, 128)
        if m < 2:
            for c in range(hw // 128):
                pltpu.make_async_copy((awq, bwq)[m].at[:, pl.ds(off + c * 128, 128)],
                                      wbuf.at[pl.ds(m * wrows + c * d, d)], w_sem.at[m]).start()
        else:
            for c in range(d // 128):
                pltpu.make_async_copy((awo, bwo)[m - 2].at[pl.ds(off, hw), pl.ds(c * 128, 128)],
                                      wbuf.at[pl.ds(m * wrows + c * hw, hw)], w_sem.at[m]).start()

    def w_start_dyn(h, m, valid):
        for k in range(4):
            @pl.when(jnp.logical_and(m == k, valid))
            def _():
                w_start(h, k)

    def w_wait(m):
        v = wbuf.at[pl.ds(_mul(m, wrows), wrows)]
        pltpu.make_async_copy(v, v, w_sem.at[m]).wait()

    def prep_w(dst, msrc, mdst, row, nrows, zero=None, sub=0):
        whole = isinstance(row, int) and row == 0
        if isinstance(msrc, int):
            sa, sc = (5, 1) if msrc < 2 else (1, 3)
            off = [(msrc * 15 + (y // 5) * sa + (y % 5) * sc) * 64 + row * 8 for y in range(15)]
        else:
            sa, sc = jnp.where(msrc < 2, 5, 1), jnp.where(msrc < 2, 1, 3)
            off = [pl.multiple_of((msrc * 15 + (y // 5) * sa + (y % 5) * sc) * 64 + row * 8, 64 if whole else 32)
                   for y in range(15)]
        r16 = _mul(mdst * 8 + row, 16)
        if not isinstance(r16, int):
            r16 = pl.multiple_of(r16, 128 if whole else 64)
        for r, form in enumerate(W_FORMS):
            if len(form) == 1:
                val = _as_bf16(w32[pl.ds(off[form[0][0]] + sub * 8, nrows * 8), :])
            else:
                val = None
                for y, c in form:
                    t = _as_f32(w32[pl.ds(off[y] + sub * 8, nrows * 8), :])
                    val = t if val is None else (val + t if c > 0 else val - t)
                val = val.astype(bf16)
            wc[dst][pl.ds(r16 + sub * 16, nrows * 16), r * 128:(r + 1) * 128] = val
        if zero is not None:
            return lambda: wc[dst][pl.ds(pl.multiple_of(r16 + zero * 16 + sub * 16, 16), 16), 0:128].astype(f32)[0:8]

    def prep_x(b, br, k0=0, k1=5, zero=None):
        get = _make_lhs(
            lambda z: _as_f32(x32[b, br, z % 5, (z // 5) * (hq // 2) + k0 * 8:(z // 5) * (hq // 2) + k1 * 8, :])
            * scale, Q_LHS_PROG)
        for r, p in enumerate(Q_PRODS):
            xc[pl.ds(_mul(b * 2 + br, hq) + k0 * 16, (k1 - k0) * 16), r * 128:(r + 1) * 128] = (
                get(p[0]) * Q_SIGN[r]).astype(bf16)
        if zero is not None:
            c0 = (NPROD - 1) * 128
            return lambda: xc[pl.ds(_mul(b * 2 + br + zero, hq) + k0 * 16, 16), c0:c0 + 128].astype(f32)[0:8]

    def body(g0, nbat, first, wpre, xpre, plan, cs, first_hp=False, last_hp=False):
        b0 = g0 & (nb - 1)
        pat, qord, oord, qsp, osp = plan
        sched = [(a.split("@")[0], int(a.split("@")[1])) for a in pat.split(",")]
        qord = [int(i) for i in qord.split(".")]
        oord = [int(i) for i in oord.split(".")]
        assert all(sched.index(("ob", u)) < sched.index(("ob", u + 1)) for u in range(0, 2 * nbat, 2))
        R, O, OT, QA, OA, SC, LH = {}, {}, {}, {}, {}, {}, {}
        lazy = {}
        pending = []
        clock = [0]

        def tick(o, cycles):
            t0 = clock[0]
            clock[0] += cycles
            groups = o.shape[0] // 8
            rows = None
            while pending and pending[0][0] <= clock[0]:
                due, emit = pending.pop(0)
                tok = emit()
                g = min(max((due - t0) * groups // cycles, 0), groups - 1)
                rows = rows or [o[8 * i:8 * i + 8] for i in range(groups)]
                rows[g] = jnp.minimum(rows[g], jnp.maximum(rows[g], tok()))
            return o if rows is None else jnp.concatenate(rows, axis=0)

        def later(delay, emit):
            pending.append((clock[0] + delay, emit))
            pending.sort(key=lambda e: e[0])

        def prow(u, h):
            return (2 * u + h) * sq

        def weights(m, prods):
            def w_of(r):
                s = W_FORMS.index(prods[r][1])
                return wc[cs][m * 128:(m + 1) * 128, s * 128:(s + 1) * 128]
            return w_of

        def q_(u, lo_, hi_):
            b, br = b0 + u // 2, u % 2

            def lhs_of(r):
                return xc[pl.ds(_mul(b * 2 + br, hq), hq), r * 128:(r + 1) * 128]

            _bilinear_run(QA.setdefault(u, {}), Q_PRODS, qord[lo_:hi_], lhs_of, weights(br, Q_PRODS), tick)
            if hi_ == NPROD:
                fin = _bilinear_finish(QA[u], Q_OUT_PROG)

                def store_q():
                    c = [[fin[i * 3 + n] for n in range(3)] for i in range(2)]
                    for h, ops in enumerate(_q_operands(c)):
                        for i, a in enumerate(ops):
                            qbuf[u * hq:(u + 1) * hq, (3 * h + i) * 128:(3 * h + i + 1) * 128] = a.astype(bf16)

                lazy["q", u] = store_q

        def s_(u, h, j):
            b, br = b0 + u // 2, u % 2
            lazy.pop(("q", u), lambda: None)()
            qh = [qbuf[u * hq:(u + 1) * hq, (3 * h + i) * 128:(3 * h + i + 1) * 128] for i in range(3)]
            SC[u, h, j] = _scores_half(qh, kvbuf.at[b, 2 * br], h, j, tick)
            if j == 1:
                s = jnp.concatenate(SC[u, h, 0] + SC[u, h, 1], axis=1)

                def store_p():
                    p, R[u, h] = _softmax(s)
                    pbuf[prow(u, h):prow(u, h) + sq, :] = p

                lazy["p", u, h] = store_p

        def m_(u, h, half):
            lazy.pop(("p", u, h), lambda: None)()
            vt = kvbuf.at[b0 + u // 2 + (g0 >> 20) * half, 2 * (u % 2) + 1]
            r0 = prow(u, h) + half * hq
            res = [tick(lax.dot_general(pbuf[r0:r0 + hq, i * 256:(i + 1) * 256], _pv_weights(vt, h, i), NT,
                                        preferred_element_type=f32), 40) for i in range(3)]
            lo = lax.broadcasted_iota(jnp.int32, (hq, 128), 1) < 64
            r = R[u, h][half * hq:(half + 1) * hq]
            O[u, h, half] = (res[0] + jnp.where(lo, res[2], res[1])) * r
            OT[u, h, half] = jnp.where(lo, res[1], res[2]) * r

        def o_(u, lo_, hi_):
            b, br = b0 + u // 2, u % 2
            if lo_ == 0:
                lo = lax.broadcasted_iota(jnp.int32, (hq, 128), 1) < 64
                mid = [jnp.where(lo, OT[u, 0, i], OT[u, 1, i]) +
                       pltpu.roll(jnp.where(lo, OT[u, 1, i], OT[u, 0, i]), 64, 1) for i in range(2)]
                tiles = [[O[u, 0, i], mid[i], O[u, 1, i]] for i in range(2)]
                get = _make_lhs(lambda x: tiles[x // 3][x % 3], O_LHS_PROG)
                LH[u] = {p[0]: get(p[0]).astype(bf16) for p in O_PRODS}
            _bilinear_run(OA.setdefault(u, {}), O_PRODS, oord[lo_:hi_], lambda r: LH[u][O_PRODS[r][0]],
                          weights(2 + br, O_PRODS), tick)
            if hi_ < NPROD:
                return
            fin = _bilinear_finish(OA[u], O_OUT_PROG)
            for n in range(5):
                for i in range(2):
                    s, a = fin[i * 5 + n]
                    rows = slice(i * hq, (i + 1) * hq)
                    cols = slice(br * d + n * 128, br * d + (n + 1) * 128)
                    if first_hp:
                        new = a if s > 0 else -a
                    else:
                        new = acc[b, rows, cols] + a if s > 0 else acc[b, rows, cols] - a
                    if last_hp:
                        obuf[b, rows, cols] = new.astype(obuf.dtype)
                    else:
                        acc[b, rows, cols] = new
            if br == 1 and last_hp:
                pltpu.make_async_copy(obuf.at[b], o_hbm.at[b], o_sem).start()

        fns = {"qa": lambda u: q_(u, 0, qsp), "qb": lambda u: q_(u, qsp, NPROD),
               "oa": lambda u: o_(u, 0, osp), "ob": lambda u: o_(u, osp, NPROD),
               "s00": lambda u: s_(u, 0, 0), "s01": lambda u: s_(u, 0, 1),
               "s10": lambda u: s_(u, 1, 0), "s11": lambda u: s_(u, 1, 1),
               "m0": lambda u: m_(u, 0, 0), "m1": lambda u: m_(u, 1, 0),
               "t0": lambda u: m_(u, 0, 1), "t1": lambda u: m_(u, 1, 1)}
        for f in first:
            f()
        total = 2 * nbat * 1960
        lastq = max(i for i, it in enumerate(sched) if it[0][0] == "q")
        for k, f in enumerate(wpre):
            lo_, hi_ = (PLO, total - PHI) if nbat > 1 else (SWLO, SWHI)
            later(lo_ + k * (hi_ - lo_) // len(wpre), f)
        for i, item in enumerate(sched):
            fns[item[0]](item[1])
            if i == lastq:
                for k, f in enumerate(xpre):
                    later(SXLO + k * (total - SXHI - clock[0] - SXLO) // len(xpre), f)
        assert not pending and not lazy

    for k in range(4):
        w_start(0, k)
    x_start(0)
    kv_start(0)
    x_start(1)
    for g in range(1, C0):
        kv_start(g)
        x_start(g + 1)
    for m in range(4):
        w_wait(m)
        prep_w(0, m, m, 0, 8)
    x_wait(0)
    for br in range(2):
        prep_x(0, br)

    def issued(g):
        return jnp.minimum(jnp.minimum(RATE * (g + 1) + C0, jnp.maximum(g + LA, LB * g - LC)), nb + DIST * BB)

    def ramp(b0, carry):
        half = nb // 2
        m = (b0 - half) >> 1

        @pl.when(b0 + 1 < nb)
        def _():
            x_wait(b0 + 1)

        @pl.when(jnp.logical_and(b0 >= half, (b0 & 1) == 0))
        def _():
            w_wait(m)

        kv_wait(b0)

        hi = issued(b0)
        prev = jnp.where(b0 == 0, C0, issued(b0 - 1))

        def pf_x(k, w):
            @pl.when(jnp.logical_and(prev + k < hi, prev + k + 1 < nb))
            def _():
                x_start(prev + k + 1, (w,))

        def pf_kv(k):
            @pl.when(prev + k < hi)
            def _():
                kv_start(prev + k)

        def pf_w():
            w_start_dyn(jnp.where(b0 == W2AT, 2, 1), jnp.where(b0 == W2AT, 0, (b0 >> 1) - 1),
                        jnp.logical_or(b0 == W2AT, jnp.logical_and(b0 <= half, (b0 & 1) == 0)))

        first = [pf_w] + [functools.partial(pf_x, k, w) for k in range(RATE) for w in range(2)]
        first += [functools.partial(pf_kv, k) for k in range(RATE)]
        zero = b0 >> 20
        wpre = [functools.partial(prep_w, 1, jnp.where(b0 >= half, m, 3), jnp.maximum(m, 0), (b0 & 1) * 4, 1,
                                  zero, k) for k in range(4)]
        xpre = [functools.partial(prep_x, jnp.minimum(b0 + 1, nb - 1), br, k, k + 1, zero)
                for br in range(2) for k in range(5)]
        body(b0, 1, first, wpre, xpre, RAMP, 0, first_hp=True)
        return carry

    def step(par, last, hp, i, carry):
        g0 = hp * nb + i * BB

        if not last:
            w_wait(i)

        kvg_wait(i)

        if last:
            def pf_kv():
                @pl.when(g0 + DIST * BB < ng)
                def _():
                    kvg_start(g0 + DIST * BB)

            body(g0, BB, [pf_kv], [], [], LAST, par, last_hp=True)
        else:
            hn = jnp.where(i == 3, hp + 2, hp + 1)
            first = [lambda: w_start_dyn(hn, (i + 1) & 3, hn < nhp), functools.partial(kvg_start, g0 + DIST * BB)]
            wpre = [functools.partial(prep_w, 1 - par, i, i, 0, 1, i >> 20, k) for k in range(8)]
            body(g0, BB, first, wpre, [], STEADY, par)
        return carry

    def pair(t, carry):
        lax.fori_loop(jnp.where(t > 0, 0, spb), spb, functools.partial(step, 0, False, 2 * t), 0)
        lax.fori_loop(0, jnp.where(2 * t + 1 < nhp - 1, spb, 0), functools.partial(step, 1, False, 2 * t + 1), 0)
        return carry

    lax.fori_loop(0, nb, ramp, 0)
    lax.fori_loop(0, nhp // 2, pair, 0)
    lax.fori_loop(0, spb, functools.partial(step, 1, True, nhp - 1), 0)
    pltpu.make_async_copy(obuf, o_hbm, o_sem).wait()


@jax.jit
def pallas_concat_heads__gqa_block_cached__mha_block_cached__near_ridge_kernel(
    A_x: jax.Array,
    A_k_cache: jax.Array,
    A_v_cache: jax.Array,
    A_wq: jax.Array,
    A_wo: jax.Array,
    B_x: jax.Array,
    B_k_cache: jax.Array,
    B_v_cache: jax.Array,
    B_wq: jax.Array,
    B_wo: jax.Array,
):
    B, Sq, D = A_x.shape
    _, H, Sk, Dh = A_k_cache.shape
    nhp = H // 2
    assert (B, Sq, D, Sk, Dh) == (16, 160, 640, 512, 192) and A_wq.shape[1] == H * Dh
    assert nhp >= 4 and nhp & (nhp - 1) == 0 and B_k_cache.shape == A_k_cache.shape
    n_iss = C0
    for g0 in range(B):
        assert n_iss >= g0 + 2
        hi = min(RATE * (g0 + 1) + C0, max(g0 + LA, LB * g0 - LC), B + DIST * BB)
        assert hi <= g0 + B and 0 <= hi - n_iss <= RATE
        n_iss = hi
    assert n_iss == B + DIST * BB and 10 <= W2AT <= 15

    def tr(c):
        return jnp.swapaxes(c, 2, 3).reshape(B, nhp, 2 * Dh, Sk)

    any_spec = pl.BlockSpec(memory_space=pl.ANY)
    return pl.pallas_call(
        functools.partial(_kernel, scale=Dh ** -0.5 * LOG2E, nhp=nhp, nb=B),
        in_specs=[any_spec] * 10,
        out_specs=any_spec,
        out_shape=jax.ShapeDtypeStruct((B, Sq, 2 * D), A_x.dtype),
        scratch_shapes=[pltpu.VMEM((B, Sq, 2 * D), f32),
                        pltpu.VMEM((B, 2, D // 128, Sq // 2, 128), u32),
                        pltpu.VMEM((4 * 15 * 64, 128), u32),
                        pltpu.VMEM((B, 4, 2 * Dh, Sk), bf16),
                        pltpu.VMEM((B, Sq, 2 * D), bf16),
                        pltpu.VMEM((2 * BB * Sq, 6 * 128), u32),
                        pltpu.VMEM((2 * BB * Sq // 4, 6 * 128), u32),
                        pltpu.VMEM((B * 2 * Sq // 4, XCW * 128), u32),
                        pltpu.VMEM((4 * 64, WCW * 128), u32),
                        pltpu.VMEM((4 * 64, WCW * 128), u32),
                        pltpu.SemaphoreType.DMA((B + 4,)),
                        pltpu.SemaphoreType.DMA((B,)),
                        pltpu.SemaphoreType.DMA((4,)),
                        pltpu.SemaphoreType.DMA(())],
        compiler_params=pltpu.CompilerParams(
            disable_bounds_checks=True,
            vmem_limit_bytes=110 * 1024 * 1024),
    )(A_x, tr(A_k_cache), tr(A_v_cache), A_wq, A_wo, B_x, tr(B_k_cache), tr(B_v_cache), B_wq, B_wo)
```

```python
import functools

import jax
import jax.numpy as jnp
from jax import lax
import jax.experimental.pallas as pl
import jax.experimental.pallas.tpu as pltpu

bf16 = jnp.bfloat16
f32 = jnp.float32
u32 = jnp.uint32
NT = (((1,), (1,)), ((), ()))
LOG2E = 1.4426950408889634

BB = 4
DIST = 2
C0, RATE, LA, LB, LC = 2, 2, 6, 2, 6
W2AT = 11
XCW, WCW = 32, 40

PAT = (
    "qa@0,qb@0,qa@1,qb@1,qa@2,s00@0,s01@0,s10@0,qb@2,s11@0,m0@0,t0@0,s00@1,qa@3,s01@1,t1@0,s10@1,qb@3,m1@0,"
    "s11@1,m0@1,t0@1,s00@2,qa@4,s01@2,m1@1,t1@1,s10@2,oa@0,s11@2,m0@2,ob@0,t0@2,s00@3,qa@5,qb@4,s01@3,t1@2,"
    "m1@2,s10@3,oa@1,qb@5,s11@3,m0@3,t0@3,ob@1,s00@4,oa@2,qa@6,s01@4,m1@3,t1@3,s10@4,s11@4,m0@4,t0@4,s00@5,"
    "ob@2,qb@6,qa@7,s01@5,m1@4,t1@4,s10@5,oa@3,qb@7,s11@5,m0@5,t0@5,ob@3,s00@6,oa@4,s01@6,s10@6,m1@5,t1@5,"
    "s11@6,m0@6,t0@6,ob@4,s00@7,s01@7,m1@6,t1@6,s10@7,oa@5,s11@7,m0@7,t0@7,ob@5,m1@7,t1@7,oa@6,ob@6,oa@7,"
    "ob@7")
SPAT = (
    "qa@0,qb@0,qa@1,s00@0,s10@0,s11@0,s01@0,qb@1,m1@0,m0@0,t0@0,s00@1,t1@0,s10@1,s01@1,s11@1,oa@0,m0@1,m1@1,"
    "t0@1,t1@1,ob@0,oa@1,ob@1")
LPAT = (
    "qa@0,qb@0,qa@1,qb@1,qa@2,s00@0,s01@0,s10@0,qb@2,s11@0,m0@0,s10@1,t0@0,s00@1,qa@3,s01@1,t1@0,qb@3,m1@0,"
    "s11@1,m0@1,t0@1,s00@2,qa@4,s01@2,m1@1,t1@1,s10@2,oa@0,s11@2,m0@2,ob@0,t0@2,s00@3,qa@5,qb@4,s01@3,t1@2,"
    "m1@2,s10@3,oa@1,qb@5,s11@3,m0@3,t0@3,ob@1,s00@4,qa@6,oa@2,s01@4,m1@3,t1@3,s10@4,s11@4,m0@4,t0@4,s00@5,"
    "ob@2,qb@6,qa@7,s01@5,m1@4,t1@4,s10@5,oa@3,qb@7,s11@5,m0@5,t0@5,ob@3,s00@6,oa@4,s01@6,s10@6,m1@5,t1@5,"
    "s11@6,m0@6,t0@6,ob@4,s00@7,s01@7,m1@6,t1@6,s10@7,oa@5,s11@7,m0@7,t0@7,ob@5,m1@7,t1@7,oa@6,ob@6,oa@7,"
    "ob@7")
QORD = "9.16.24.21.19.1.15.18.22.17.20.12.3.2.4.5.23.7.6.8.14.0.10.11.13"
OORD = "0.6.1.5.3.2.8.9.4.24.12.11.14.10.16.19.13.15.17.18.20.22.21.23.7"
SQORD = "3.16.24.15.18.7.20.21.9.10.22.1.23.6.12.0.2.14.8.17.13.11.4.5.19"
SOORD = "4.0.3.1.5.6.8.2.9.14.24.10.12.13.15.21.11.19.17.16.18.20.23.22.7"
LQORD = "9.16.24.21.19.1.15.20.18.22.17.23.12.3.2.4.7.6.8.5.14.0.10.11.13"
LOORD = "0.6.1.5.3.2.8.9.4.24.12.11.14.10.16.19.13.15.17.18.20.22.21.23.7"
STEADY = (PAT, QORD, OORD, 11, 10)
RAMP = (SPAT, SQORD, SOORD, 13, 13)
LAST = (LPAT, LQORD, LOORD, 11, 10)
PLO, PHI, SWLO, SWHI, SXLO, SXHI = 300, 520, 140, 920, 1500, 160

O_LHS_PROG = [
    (100, 4, 5, 1), (101, 0, 1, -1), (102, 3, 101, 1), (103, 2, 100, 1), (104, 0, 3, 1),
    (105, 2, 3, -1), (106, 0, 2, 1), (107, 2, 101, -1), (108, 3, 5, 1), (109, 1, 103, 1),
    (110, 2, 5, 1), (111, 3, 100, -1), (112, 5, 101, 1), (113, 4, 102, -1), (114, 0, 100, 1),
]
O_OUT_PROG = [
    (100, 5, 8, -1), (101, 3, 100, 1), (102, 2, 7, -1), (103, 0, 102, 1),
]
O_PRODS = [
    ((101, 1), [(2, 1), (5, 1), (10, -1), (12, 1)], [(102, 1)]),
    ((104, 1), [(3, 1)], [(100, -1)]),
    ((111, 1), [(0, 1), (3, 1)], [(5, 1)]),
    ((5, 1), [(5, 1), (10, -1)], [(5, -1), (103, 1)]),
    ((112, 1), [(5, 1), (10, -1), (12, 1)], [(103, -1)]),
    ((114, 1), [(0, 1), (3, 1), (5, 1)], [(101, 1)]),
    ((0, 1), [(0, 1), (5, 1)], [(0, 1), (101, -1)]),
    ((107, -1), [(10, 1), (12, -1)], [(0, -1)]),
    ((110, 1), [(12, 1)], [(0, 1), (2, 1)]),
    ((1, 1), [(2, 1), (7, 1)], [(2, 1), (4, -1)]),
    ((104, 1), [(1, 1), (2, 1), (4, 1), (7, 1), (9, 1)], [(4, 1)]),
    ((106, 1), [(1, 1)], [(1, 1), (4, -1)]),
    ((1, 1), [(6, 1)], [(1, 1), (3, -1)]),
    ((109, 1), [(6, 1), (8, 1)], [(3, 1)]),
    ((2, 1), [(1, 1), (11, -1)], [(1, -1), (6, 1)]),
    ((103, 1), [(6, 1), (8, 1), (13, -1)], [(3, -1), (6, 1)]),
    ((100, 1), [(0, 1), (3, 1), (5, 1), (13, 1)], [(3, -1), (8, 1)]),
    ((4, 1), [(8, 1), (13, -1)], [(6, -1), (8, 1)]),
    ((110, 1), [(6, 1), (8, 1), (11, -1), (13, -1), (14, -1)], [(6, -1)]),
    ((105, 1), [(1, 1), (14, 1)], [(4, 1), (6, -1)]),
    ((108, 1), [(14, 1)], [(6, -1), (9, 1)]),
    ((3, 1), [(4, 1), (14, -1)], [(4, -1), (9, 1)]),
    ((4, 1), [(9, 1)], [(7, -1), (9, 1)]),
    ((102, 1), [(2, 1), (7, 1), (9, 1)], [(4, -1), (7, 1)]),
    ((113, -1), [(7, 1), (9, 1)], [(7, -1)]),
]
Q_LHS_PROG = [
    (100, 3, 8, -1), (101, 0, 2, 1), (102, 7, 101, -1), (103, 5, 100, 1), (104, 4, 6, -1),
    (105, 4, 9, -1), (106, 7, 9, -1), (107, 0, 103, -1), (108, 6, 8, -1), (109, 5, 102, 1),
    (110, 1, 4, -1), (111, 5, 8, -1), (112, 6, 9, -1), (113, 4, 7, -1), (114, 2, 4, -1),
    (115, 1, 6, -1), (116, 2, 7, -1), (117, 1, 3, -1), (118, 3, 6, -1),
]
Q_OUT_PROG = [
    (100, 0, 3, 1), (101, 4, 5, 1), (102, 0, 1, -1), (103, 2, 101, 1), (104, 2, 5, 1),
    (105, 1, 100, -1),
]
Q_PRODS = [
    ((6, -1), [(6, 1), (8, 1), (11, -1), (13, -1), (14, -1)], [(104, 1)]),
    ((101, 1), [(12, 1)], [(104, 1)]),
    ((4, 1), [(1, 1), (2, 1), (4, 1), (7, 1), (9, 1)], [(100, 1)]),
    ((111, -1), [(3, 1)], [(100, 1)]),
    ((118, -1), [(6, 1), (8, 1), (13, -1)], [(103, 1)]),
    ((3, 1), [(6, 1), (8, 1)], [(1, 1), (103, 1)]),
    ((114, 1), [(2, 1), (7, 1)], [(1, 1)]),
    ((117, 1), [(6, 1)], [(1, 1)]),
    ((115, -1), [(1, 1), (11, -1)], [(2, 1)]),
    ((0, -1), [(10, 1), (12, -1)], [(2, -1), (102, 1)]),
    ((116, 1), [(2, 1), (5, 1), (10, -1), (12, 1)], [(102, 1)]),
    ((102, 1), [(5, 1), (10, -1), (12, 1)], [(5, 1), (102, 1)]),
    ((109, -1), [(5, 1), (10, -1)], [(5, 1)]),
    ((112, -1), [(14, 1)], [(3, 1), (5, 1)]),
    ((104, 1), [(1, 1), (14, 1)], [(2, 1), (3, -1)]),
    ((105, -1), [(4, 1), (14, -1)], [(3, 1)]),
    ((5, 1), [(0, 1), (3, 1)], [(3, 1), (101, -1)]),
    ((100, -1), [(0, 1), (3, 1), (5, 1), (13, 1)], [(101, 1)]),
    ((103, 1), [(0, 1), (3, 1), (5, 1)], [(0, 1), (101, 1)]),
    ((110, 1), [(1, 1)], [(0, 1), (2, 1)]),
    ((107, 1), [(0, 1), (5, 1)], [(0, 1)]),
    ((113, -1), [(2, 1), (7, 1), (9, 1)], [(105, -1)]),
    ((7, -1), [(7, 1), (9, 1)], [(4, -1), (105, -1)]),
    ((106, -1), [(9, 1)], [(4, 1)]),
    ((108, -1), [(8, 1), (13, -1)], [(4, 1)]),
]
NPROD = len(O_PRODS)


def _normalize(prods):
    out = []
    for (var, sgn), w, g in prods:
        sgn *= w[0][1]
        out.append((var, [(y, c * w[0][1]) for y, c in w], [(z, c * sgn) for z, c in g]))
    return out


def _positive_outputs(prods, prog):
    for flips in range(1 << 6):
        sg = [(-1 if (flips >> (r % 6)) & 1 else 1) for r in range(len(prods))]
        pos = {}
        for r, p in enumerate(prods):
            for z, c in p[2]:
                pos[z] = max(pos.get(z, -1), c * sg[r])
        for t, a, b, s in reversed(prog):
            st = pos.pop(t)
            pos[a] = max(pos.get(a, -1), st)
            pos[b] = max(pos.get(b, -1), st * s)
        if min(pos.values()) > 0:
            return sg
    raise AssertionError


O_PRODS = _normalize(O_PRODS)
Q_PRODS = _normalize(Q_PRODS)
W_FORMS = [p[1] for p in O_PRODS]
Q_SIGN = _positive_outputs(Q_PRODS, Q_OUT_PROG)
Q_PRODS = [(v, w, [(z, c * s) for z, c in g]) for (v, w, g), s in zip(Q_PRODS, Q_SIGN)]


def _make_lhs(block, prog):
    vals = {}

    def get(v):
        if v not in vals:
            vals[v] = block(v)
        return vals[v]

    for t, a, b, s in prog:
        vals[t] = get(a) + get(b) if s > 0 else get(a) - get(b)
    return get


def _acc_add(accs, z, sgn, m):
    if z not in accs:
        accs[z] = (sgn, m)
    else:
        s0, a = accs[z]
        accs[z] = (s0, a + m) if s0 == sgn else ((1, a - m) if s0 > 0 else (1, m - a))


def _bilinear_run(accs, prods, which, lhs_of, w_of, tick):
    for r in which:
        m = tick(jnp.dot(lhs_of(r), w_of(r), preferred_element_type=f32), 20)
        for z, c in prods[r][2]:
            _acc_add(accs, z, c, m)


def _bilinear_finish(accs, prog):
    for t, a, b, s in reversed(prog):
        st, v = accs.pop(t)
        _acc_add(accs, a, st, v)
        _acc_add(accs, b, st * s, v)
    return accs


def _mul(i, n):
    return i * n if isinstance(i, int) else pl.multiple_of(i * n, 16)


def _q_operands(c):
    assert all(s > 0 for row in c for s, _ in row)
    (t0, t1, t2), (b0, b1, b2) = [[a for _, a in row] for row in c]
    lo = lax.broadcasted_iota(jnp.int32, t0.shape, 1) < 64
    return [[jnp.where(lo, t0, b0), jnp.where(lo, t1, t0 - b0), jnp.where(lo, b0 - t0, pltpu.roll(b1, 64, 1))],
            [jnp.where(lo, t2, b2), jnp.where(lo, pltpu.roll(t1, 64, 1), t2 - b2), jnp.where(lo, b2 - t2, b1)]]


def _scores_half(qh, kt, h, j, tick):
    k0, k1, k2 = (0, 64, 128) if h == 0 else (256, 320, 192)
    out = []
    for c in (2 * j, 2 * j + 1):
        cs = slice(c * 128, (c + 1) * 128)
        w = [kt[k0:k0 + 128, cs],
             jnp.concatenate([kt[k2:k2 + 64, cs], kt[k1:k1 + 64, cs]], axis=0),
             jnp.concatenate([kt[k0:k0 + 64, cs], kt[k2:k2 + 64, cs]], axis=0)]
        m = [tick(jnp.dot(qh[i], w[i], preferred_element_type=f32), 20) for i in range(3)]
        out.append(jnp.concatenate([m[0] + m[1], m[0] + m[2]], axis=0))
    return out


def _softmax(s):
    m = jnp.max(s, axis=1, keepdims=True)
    p = jnp.exp2(s - m)
    p0, p1, p2, p3 = (p[:, i * 128:(i + 1) * 128] for i in range(4))
    s01, s23 = p0 + p1, p2 + p3
    t = s01 + s23
    l = jnp.sum(t, axis=1, keepdims=True)
    r = pl.reciprocal(l, approx=True)
    r = r * (2.0 - l * r)
    return jnp.concatenate([s01, jnp.minimum(s23, t), p0, p2, p1, p3], axis=1).astype(bf16), r


def _pv_weights(vt, h, i):
    d0, d1, d2 = (0, 64, 128) if h == 0 else (256, 320, 192)

    def v(d, c):
        return vt[d:d + 64, c * 128:(c + 1) * 128]

    def f(d, c):
        return v(d, c).astype(f32)

    if i == 0:
        return jnp.concatenate([jnp.concatenate([v(d0, c), v(d1, c + 1)], axis=0) for c in (0, 2)], axis=1)
    if i == 1:
        w = [jnp.concatenate([f(d2, c), f(d1, c) - f(d1, c + 1)], axis=0) for c in (0, 2)]
    else:
        w = [jnp.concatenate([f(d0, c + 1) - f(d0, c), f(d2, c + 1)], axis=0) for c in (0, 2)]
    return jnp.concatenate(w, axis=1).astype(bf16)


def _kernel(ax, ak, av, awq, awo, bx, bk, bv, bwq, bwo, o_hbm,
            acc, xbuf, wbuf, kvbuf, obuf, pbuf, qbuf, xc32, wc0, wc1,
            kv_sem, x_sem, w_sem, o_sem, *, scale, nhp, nb):
    pbuf, qbuf, xc = (r.bitcast(bf16) for r in (pbuf, qbuf, xc32))
    wc = [r.bitcast(bf16) for r in (wc0, wc1)]
    sq = xbuf.shape[2]
    hq = sq // 2
    d = awq.shape[0]
    hw = kvbuf.shape[2]
    wrows = wbuf.shape[0] // 4
    ng = nhp * nb
    lg = nb.bit_length() - 1
    spb = nb // BB

    def kv_start(g):
        hp, b = (g >> lg) & (nhp - 1), g & (nb - 1)
        for i, src in enumerate((ak, av, bk, bv)):
            sem = kv_sem.at[jnp.where(g < nb, b, nb + (b >> 2))]
            pltpu.make_async_copy(src.at[b, hp], kvbuf.at[b, i], sem).start()

    def kv_wait(b):
        pltpu.make_async_copy(kvbuf.at[b], kvbuf.at[b], kv_sem.at[b]).wait()

    def kvg_start(g):
        hp, i4 = g >> lg, (g >> 2) & 3
        b = pl.multiple_of(i4 * BB, BB)
        for i, src in enumerate((ak, av, bk, bv)):
            pltpu.make_async_copy(src.at[pl.ds(b, BB), hp], kvbuf.at[pl.ds(b, BB), i], kv_sem.at[nb + i4]).start()

    def kvg_wait(i4):
        v = kvbuf.at[pl.ds(i4 * BB, BB)]
        pltpu.make_async_copy(v, v, kv_sem.at[nb + i4]).wait()

    def x_start(b, which=(0, 1)):
        for i, src in enumerate((ax, bx)):
            if i in which:
                pltpu.make_async_copy(src.at[b], xbuf.at[b, i], x_sem.at[b]).start()

    def x_wait(b):
        pltpu.make_async_copy(xbuf.at[b], xbuf.at[b], x_sem.at[b]).wait()

    def w_start(h, m):
        off = h * hw if isinstance(h, int) else pl.multiple_of(h * hw, 128)
        if m < 2:
            for c in range(hw // 128):
                pltpu.make_async_copy((awq, bwq)[m].at[:, pl.ds(off + c * 128, 128)],
                                      wbuf.at[pl.ds(m * wrows + c * d, d)], w_sem.at[m]).start()
        else:
            for c in range(d // 128):
                pltpu.make_async_copy((awo, bwo)[m - 2].at[pl.ds(off, hw), pl.ds(c * 128, 128)],
                                      wbuf.at[pl.ds(m * wrows + c * hw, hw)], w_sem.at[m]).start()

    def w_start_dyn(h, m, valid):
        for k in range(4):
            @pl.when(jnp.logical_and(m == k, valid))
            def _():
                w_start(h, k)

    def w_wait(m):
        v = wbuf.at[pl.ds(_mul(m, wrows), wrows)]
        pltpu.make_async_copy(v, v, w_sem.at[m]).wait()

    def prep_w(dst, msrc, mdst, row, nrows, zero=None, sub=0):
        whole = isinstance(row, int) and row == 0
        if isinstance(msrc, int):
            sa, sc = (5, 1) if msrc < 2 else (1, 3)
            off = [(msrc * 15 + (y // 5) * sa + (y % 5) * sc) * 128 + row * 16 for y in range(15)]
        else:
            sa, sc = jnp.where(msrc < 2, 5, 1), jnp.where(msrc < 2, 1, 3)
            off = [pl.multiple_of((msrc * 15 + (y // 5) * sa + (y % 5) * sc) * 128 + row * 16, 128 if whole else 64)
                   for y in range(15)]
        r16 = _mul(mdst * 8 + row, 16)
        if not isinstance(r16, int):
            r16 = pl.multiple_of(r16, 128 if whole else 64)
        for r, form in enumerate(W_FORMS):
            if len(form) == 1:
                val = wbuf[pl.ds(off[form[0][0]] + sub * 16, nrows * 16), :]
            else:
                val = None
                for y, c in form:
                    t = wbuf[pl.ds(off[y] + sub * 16, nrows * 16), :].astype(f32)
                    val = t if val is None else (val + t if c > 0 else val - t)
                val = val.astype(bf16)
            wc[dst][pl.ds(r16 + sub * 16, nrows * 16), r * 128:(r + 1) * 128] = val
        if zero is not None:
            return lambda: wc[dst][pl.ds(pl.multiple_of(r16 + zero * 16 + sub * 16, 16), 16), 0:128].astype(f32)[0:8]

    def prep_x(b, br, k0=0, k1=5, zero=None):
        get = _make_lhs(
            lambda z: xbuf[b, br, (z // 5) * hq + k0 * 16:(z // 5) * hq + k1 * 16,
                           (z % 5) * 128:(z % 5 + 1) * 128].astype(f32) * scale, Q_LHS_PROG)
        for r, p in enumerate(Q_PRODS):
            xc[pl.ds(_mul(b * 2 + br, hq) + k0 * 16, (k1 - k0) * 16), r * 128:(r + 1) * 128] = (
                get(p[0]) * Q_SIGN[r]).astype(bf16)
        if zero is not None:
            c0 = (NPROD - 1) * 128
            return lambda: xc[pl.ds(_mul(b * 2 + br + zero, hq) + k0 * 16, 16), c0:c0 + 128].astype(f32)[0:8]

    def body(g0, nbat, first, wpre, xpre, plan, cs, first_hp=False, last_hp=False):
        b0 = g0 & (nb - 1)
        pat, qord, oord, qsp, osp = plan
        sched = [(a.split("@")[0], int(a.split("@")[1])) for a in pat.split(",")]
        qord = [int(i) for i in qord.split(".")]
        oord = [int(i) for i in oord.split(".")]
        assert all(sched.index(("ob", u)) < sched.index(("ob", u + 1)) for u in range(0, 2 * nbat, 2))
        R, O, OT, QA, OA, SC, LH = {}, {}, {}, {}, {}, {}, {}
        lazy = {}
        pending = []
        clock = [0]

        def tick(o, cycles):
            t0 = clock[0]
            clock[0] += cycles
            groups = o.shape[0] // 8
            rows = None
            while pending and pending[0][0] <= clock[0]:
                due, emit = pending.pop(0)
                tok = emit()
                g = min(max((due - t0) * groups // cycles, 0), groups - 1)
                rows = rows or [o[8 * i:8 * i + 8] for i in range(groups)]
                rows[g] = jnp.minimum(rows[g], jnp.maximum(rows[g], tok()))
            return o if rows is None else jnp.concatenate(rows, axis=0)

        def later(delay, emit):
            pending.append((clock[0] + delay, emit))
            pending.sort(key=lambda e: e[0])

        def prow(u, h):
            return (2 * u + h) * sq

        def weights(m, prods):
            def w_of(r):
                s = W_FORMS.index(prods[r][1])
                return wc[cs][m * 128:(m + 1) * 128, s * 128:(s + 1) * 128]
            return w_of

        def q_(u, lo_, hi_):
            b, br = b0 + u // 2, u % 2

            def lhs_of(r):
                return xc[pl.ds(_mul(b * 2 + br, hq), hq), r * 128:(r + 1) * 128]

            _bilinear_run(QA.setdefault(u, {}), Q_PRODS, qord[lo_:hi_], lhs_of, weights(br, Q_PRODS), tick)
            if hi_ == NPROD:
                fin = _bilinear_finish(QA[u], Q_OUT_PROG)

                def store_q():
                    c = [[fin[i * 3 + n] for n in range(3)] for i in range(2)]
                    for h, ops in enumerate(_q_operands(c)):
                        for i, a in enumerate(ops):
                            qbuf[u * hq:(u + 1) * hq, (3 * h + i) * 128:(3 * h + i + 1) * 128] = a.astype(bf16)

                lazy["q", u] = store_q

        def s_(u, h, j):
            b, br = b0 + u // 2, u % 2
            lazy.pop(("q", u), lambda: None)()
            qh = [qbuf[u * hq:(u + 1) * hq, (3 * h + i) * 128:(3 * h + i + 1) * 128] for i in range(3)]
            SC[u, h, j] = _scores_half(qh, kvbuf.at[b, 2 * br], h, j, tick)
            if j == 1:
                s = jnp.concatenate(SC[u, h, 0] + SC[u, h, 1], axis=1)

                def store_p():
                    p, R[u, h] = _softmax(s)
                    pbuf[prow(u, h):prow(u, h) + sq, :] = p

                lazy["p", u, h] = store_p

        def m_(u, h, half):
            lazy.pop(("p", u, h), lambda: None)()
            vt = kvbuf.at[b0 + u // 2 + (g0 >> 20) * half, 2 * (u % 2) + 1]
            r0 = prow(u, h) + half * hq
            res = [tick(lax.dot_general(pbuf[r0:r0 + hq, i * 256:(i + 1) * 256], _pv_weights(vt, h, i), NT,
                                        preferred_element_type=f32), 40) for i in range(3)]
            lo = lax.broadcasted_iota(jnp.int32, (hq, 128), 1) < 64
            r = R[u, h][half * hq:(half + 1) * hq]
            O[u, h, half] = (res[0] + jnp.where(lo, res[2], res[1])) * r
            OT[u, h, half] = jnp.where(lo, res[1], res[2]) * r

        def o_(u, lo_, hi_):
            b, br = b0 + u // 2, u % 2
            if lo_ == 0:
                lo = lax.broadcasted_iota(jnp.int32, (hq, 128), 1) < 64
                mid = [jnp.where(lo, OT[u, 0, i], OT[u, 1, i]) +
                       pltpu.roll(jnp.where(lo, OT[u, 1, i], OT[u, 0, i]), 64, 1) for i in range(2)]
                tiles = [[O[u, 0, i], mid[i], O[u, 1, i]] for i in range(2)]
                get = _make_lhs(lambda x: tiles[x // 3][x % 3], O_LHS_PROG)
                LH[u] = {p[0]: get(p[0]).astype(bf16) for p in O_PRODS}
            _bilinear_run(OA.setdefault(u, {}), O_PRODS, oord[lo_:hi_], lambda r: LH[u][O_PRODS[r][0]],
                          weights(2 + br, O_PRODS), tick)
            if hi_ < NPROD:
                return
            fin = _bilinear_finish(OA[u], O_OUT_PROG)
            for n in range(5):
                for i in range(2):
                    s, a = fin[i * 5 + n]
                    rows = slice(i * hq, (i + 1) * hq)
                    cols = slice(br * d + n * 128, br * d + (n + 1) * 128)
                    if first_hp:
                        new = a if s > 0 else -a
                    else:
                        new = acc[b, rows, cols] + a if s > 0 else acc[b, rows, cols] - a
                    if last_hp:
                        obuf[b, rows, cols] = new.astype(obuf.dtype)
                    else:
                        acc[b, rows, cols] = new
            if br == 1 and last_hp:
                pltpu.make_async_copy(obuf.at[b], o_hbm.at[b], o_sem).start()

        fns = {"qa": lambda u: q_(u, 0, qsp), "qb": lambda u: q_(u, qsp, NPROD),
               "oa": lambda u: o_(u, 0, osp), "ob": lambda u: o_(u, osp, NPROD),
               "s00": lambda u: s_(u, 0, 0), "s01": lambda u: s_(u, 0, 1),
               "s10": lambda u: s_(u, 1, 0), "s11": lambda u: s_(u, 1, 1),
               "m0": lambda u: m_(u, 0, 0), "m1": lambda u: m_(u, 1, 0),
               "t0": lambda u: m_(u, 0, 1), "t1": lambda u: m_(u, 1, 1)}
        for f in first:
            f()
        total = 2 * nbat * 1960
        lastq = max(i for i, it in enumerate(sched) if it[0][0] == "q")
        for k, f in enumerate(wpre):
            lo_, hi_ = (PLO, total - PHI) if nbat > 1 else (SWLO, SWHI)
            later(lo_ + k * (hi_ - lo_) // len(wpre), f)
        for i, item in enumerate(sched):
            fns[item[0]](item[1])
            if i == lastq:
                for k, f in enumerate(xpre):
                    later(SXLO + k * (total - SXHI - clock[0] - SXLO) // len(xpre), f)
        assert not pending and not lazy

    for k in range(4):
        w_start(0, k)
    x_start(0)
    kv_start(0)
    x_start(1)
    for g in range(1, C0):
        kv_start(g)
        x_start(g + 1)
    for m in range(4):
        w_wait(m)
        prep_w(0, m, m, 0, 8)
    x_wait(0)
    for br in range(2):
        prep_x(0, br)

    def issued(g):
        return jnp.minimum(jnp.minimum(RATE * (g + 1) + C0, jnp.maximum(g + LA, LB * g - LC)), nb + DIST * BB)

    def ramp(b0, carry):
        half = nb // 2
        m = (b0 - half) >> 1

        @pl.when(b0 + 1 < nb)
        def _():
            x_wait(b0 + 1)

        @pl.when(jnp.logical_and(b0 >= half, (b0 & 1) == 0))
        def _():
            w_wait(m)

        kv_wait(b0)

        hi = issued(b0)
        prev = jnp.where(b0 == 0, C0, issued(b0 - 1))

        def pf_x(k, w):
            @pl.when(jnp.logical_and(prev + k < hi, prev + k + 1 < nb))
            def _():
                x_start(prev + k + 1, (w,))

        def pf_kv(k):
            @pl.when(prev + k < hi)
            def _():
                kv_start(prev + k)

        def pf_w():
            w_start_dyn(jnp.where(b0 == W2AT, 2, 1), jnp.where(b0 == W2AT, 0, (b0 >> 1) - 1),
                        jnp.logical_or(b0 == W2AT, jnp.logical_and(b0 <= half, (b0 & 1) == 0)))

        first = [pf_w] + [functools.partial(pf_x, k, w) for k in range(RATE) for w in range(2)]
        first += [functools.partial(pf_kv, k) for k in range(RATE)]
        zero = b0 >> 20
        wpre = [functools.partial(prep_w, 1, jnp.where(b0 >= half, m, 3), jnp.maximum(m, 0), (b0 & 1) * 4, 1,
                                  zero, k) for k in range(4)]
        xpre = [functools.partial(prep_x, jnp.minimum(b0 + 1, nb - 1), br, k, k + 1, zero)
                for br in range(2) for k in range(5)]
        body(b0, 1, first, wpre, xpre, RAMP, 0, first_hp=True)
        return carry

    def step(par, last, hp, i, carry):
        g0 = hp * nb + i * BB

        if not last:
            w_wait(i)

        kvg_wait(i)

        if last:
            def pf_kv():
                @pl.when(g0 + DIST * BB < ng)
                def _():
                    kvg_start(g0 + DIST * BB)

            body(g0, BB, [pf_kv], [], [], LAST, par, last_hp=True)
        else:
            hn = jnp.where(i == 3, hp + 2, hp + 1)
            first = [lambda: w_start_dyn(hn, (i + 1) & 3, hn < nhp), functools.partial(kvg_start, g0 + DIST * BB)]
            wpre = [functools.partial(prep_w, 1 - par, i, i, 0, 1, i >> 20, k) for k in range(8)]
            body(g0, BB, first, wpre, [], STEADY, par)
        return carry

    def pair(t, carry):
        lax.fori_loop(jnp.where(t > 0, 0, spb), spb, functools.partial(step, 0, False, 2 * t), 0)
        lax.fori_loop(0, jnp.where(2 * t + 1 < nhp - 1, spb, 0), functools.partial(step, 1, False, 2 * t + 1), 0)
        return carry

    lax.fori_loop(0, nb, ramp, 0)
    lax.fori_loop(0, nhp // 2, pair, 0)
    lax.fori_loop(0, spb, functools.partial(step, 1, True, nhp - 1), 0)
    pltpu.make_async_copy(obuf, o_hbm, o_sem).wait()


@jax.jit
def pallas_concat_heads__gqa_block_cached__mha_block_cached__near_ridge_kernel(
    A_x: jax.Array,
    A_k_cache: jax.Array,
    A_v_cache: jax.Array,
    A_wq: jax.Array,
    A_wo: jax.Array,
    B_x: jax.Array,
    B_k_cache: jax.Array,
    B_v_cache: jax.Array,
    B_wq: jax.Array,
    B_wo: jax.Array,
):
    B, Sq, D = A_x.shape
    _, H, Sk, Dh = A_k_cache.shape
    nhp = H // 2
    assert (B, Sq, D, Sk, Dh) == (16, 160, 640, 512, 192) and A_wq.shape[1] == H * Dh
    assert nhp >= 4 and nhp & (nhp - 1) == 0 and B_k_cache.shape == A_k_cache.shape
    n_iss = C0
    for g0 in range(B):
        assert n_iss >= g0 + 2
        hi = min(RATE * (g0 + 1) + C0, max(g0 + LA, LB * g0 - LC), B + DIST * BB)
        assert hi <= g0 + B and 0 <= hi - n_iss <= RATE
        n_iss = hi
    assert n_iss == B + DIST * BB and 10 <= W2AT <= 15

    def tr(c):
        return jnp.swapaxes(c, 2, 3).reshape(B, nhp, 2 * Dh, Sk)

    any_spec = pl.BlockSpec(memory_space=pl.ANY)
    return pl.pallas_call(
        functools.partial(_kernel, scale=Dh ** -0.5 * LOG2E, nhp=nhp, nb=B),
        in_specs=[any_spec] * 10,
        out_specs=any_spec,
        out_shape=jax.ShapeDtypeStruct((B, Sq, 2 * D), A_x.dtype),
        scratch_shapes=[pltpu.VMEM((B, Sq, 2 * D), f32),
                        pltpu.VMEM((B, 2, Sq, D), bf16),
                        pltpu.VMEM((4 * 15 * 128, 128), bf16),
                        pltpu.VMEM((B, 4, 2 * Dh, Sk), bf16),
                        pltpu.VMEM((B, Sq, 2 * D), bf16),
                        pltpu.VMEM((2 * BB * Sq, 6 * 128), u32),
                        pltpu.VMEM((2 * BB * Sq // 4, 6 * 128), u32),
                        pltpu.VMEM((B * 2 * Sq // 4, XCW * 128), u32),
                        pltpu.VMEM((4 * 64, WCW * 128), u32),
                        pltpu.VMEM((4 * 64, WCW * 128), u32),
                        pltpu.SemaphoreType.DMA((B + 4,)),
                        pltpu.SemaphoreType.DMA((B,)),
                        pltpu.SemaphoreType.DMA((4,)),
                        pltpu.SemaphoreType.DMA(())],
        compiler_params=pltpu.CompilerParams(
            disable_bounds_checks=True,
            vmem_limit_bytes=110 * 1024 * 1024),
    )(A_x, tr(A_k_cache), tr(A_v_cache), A_wq, A_wo, B_x, tr(B_k_cache), tr(B_v_cache), B_wq, B_wo)
```

```python
import functools

import jax
import jax.numpy as jnp
from jax import lax
import jax.experimental.pallas as pl
import jax.experimental.pallas.tpu as pltpu

bf16 = jnp.bfloat16
f32 = jnp.float32
u32 = jnp.uint32
NT = (((1,), (1,)), ((), ()))
LOG2E = 1.4426950408889634

BB = 4
DIST = 2
C0, RATE, LA, LB, LC = 2, 2, 6, 2, 6
W2AT = 11
XCW, WCW = 32, 40

PAT = (
    "qa@0,qb@0,qa@1,qb@1,qa@2,s00@0,s01@0,s10@0,qb@2,s11@0,m0@0,t0@0,s00@1,qa@3,s01@1,t1@0,s10@1,qb@3,m1@0,"
    "s11@1,m0@1,t0@1,s00@2,qa@4,s01@2,m1@1,t1@1,s10@2,oa@0,s11@2,m0@2,ob@0,t0@2,s00@3,qa@5,qb@4,s01@3,t1@2,"
    "m1@2,s10@3,oa@1,qb@5,s11@3,m0@3,t0@3,ob@1,s00@4,oa@2,qa@6,s01@4,m1@3,t1@3,s10@4,s11@4,m0@4,t0@4,s00@5,"
    "ob@2,qb@6,qa@7,s01@5,m1@4,t1@4,s10@5,oa@3,qb@7,s11@5,m0@5,t0@5,ob@3,s00@6,oa@4,s01@6,s10@6,m1@5,t1@5,"
    "s11@6,m0@6,t0@6,ob@4,s00@7,s01@7,m1@6,t1@6,s10@7,oa@5,s11@7,m0@7,t0@7,ob@5,m1@7,t1@7,oa@6,ob@6,oa@7,"
    "ob@7")
SPAT = (
    "qa@0,qb@0,qa@1,s00@0,s10@0,s11@0,s01@0,qb@1,m1@0,m0@0,t0@0,s00@1,t1@0,s10@1,s01@1,s11@1,oa@0,m0@1,m1@1,"
    "t0@1,t1@1,ob@0,oa@1,ob@1")
LPAT = (
    "qa@0,qb@0,qa@1,qb@1,qa@2,s00@0,s01@0,s10@0,qb@2,s11@0,m0@0,s10@1,t0@0,s00@1,qa@3,s01@1,t1@0,qb@3,m1@0,"
    "s11@1,m0@1,t0@1,s00@2,qa@4,s01@2,m1@1,t1@1,s10@2,oa@0,s11@2,m0@2,ob@0,t0@2,s00@3,qa@5,qb@4,s01@3,t1@2,"
    "m1@2,s10@3,oa@1,qb@5,s11@3,m0@3,t0@3,ob@1,s00@4,qa@6,oa@2,s01@4,m1@3,t1@3,s10@4,s11@4,m0@4,t0@4,s00@5,"
    "ob@2,qb@6,qa@7,s01@5,m1@4,t1@4,s10@5,oa@3,qb@7,s11@5,m0@5,t0@5,ob@3,s00@6,oa@4,s01@6,s10@6,m1@5,t1@5,"
    "s11@6,m0@6,t0@6,ob@4,s00@7,s01@7,m1@6,t1@6,s10@7,oa@5,s11@7,m0@7,t0@7,ob@5,m1@7,t1@7,oa@6,ob@6,oa@7,"
    "ob@7")
QORD = "9.16.24.21.19.1.15.18.22.17.20.12.3.2.4.5.23.7.6.8.14.0.10.11.13"
OORD = "0.6.1.5.3.2.8.9.4.24.12.11.14.10.16.19.13.15.17.18.20.22.21.23.7"
SQORD = "3.16.24.15.18.7.20.21.9.10.22.1.23.6.12.0.2.14.8.17.13.11.4.5.19"
SOORD = "4.0.3.1.5.6.8.2.9.14.24.10.12.13.15.21.11.19.17.16.18.20.23.22.7"
LQORD = "9.16.24.21.19.1.15.20.18.22.17.23.12.3.2.4.7.6.8.5.14.0.10.11.13"
LOORD = "0.6.1.5.3.2.8.9.4.24.12.11.14.10.16.19.13.15.17.18.20.22.21.23.7"
STEADY = (PAT, QORD, OORD, 11, 10)
RAMP = (SPAT, SQORD, SOORD, 13, 13)
LAST = (LPAT, LQORD, LOORD, 11, 10)
PLO, PHI, SWLO, SWHI, SXLO, SXHI = 300, 520, 140, 920, 1500, 160

O_LHS_PROG = [
    (100, 4, 5, 1), (101, 0, 1, -1), (102, 3, 101, 1), (103, 2, 100, 1), (104, 0, 3, 1),
    (105, 2, 3, -1), (106, 0, 2, 1), (107, 2, 101, -1), (108, 3, 5, 1), (109, 1, 103, 1),
    (110, 2, 5, 1), (111, 3, 100, -1), (112, 5, 101, 1), (113, 4, 102, -1), (114, 0, 100, 1),
]
O_OUT_PROG = [
    (100, 5, 8, -1), (101, 3, 100, 1), (102, 2, 7, -1), (103, 0, 102, 1),
]
O_PRODS = [
    ((101, 1), [(2, 1), (5, 1), (10, -1), (12, 1)], [(102, 1)]),
    ((104, 1), [(3, 1)], [(100, -1)]),
    ((111, 1), [(0, 1), (3, 1)], [(5, 1)]),
    ((5, 1), [(5, 1), (10, -1)], [(5, -1), (103, 1)]),
    ((112, 1), [(5, 1), (10, -1), (12, 1)], [(103, -1)]),
    ((114, 1), [(0, 1), (3, 1), (5, 1)], [(101, 1)]),
    ((0, 1), [(0, 1), (5, 1)], [(0, 1), (101, -1)]),
    ((107, -1), [(10, 1), (12, -1)], [(0, -1)]),
    ((110, 1), [(12, 1)], [(0, 1), (2, 1)]),
    ((1, 1), [(2, 1), (7, 1)], [(2, 1), (4, -1)]),
    ((104, 1), [(1, 1), (2, 1), (4, 1), (7, 1), (9, 1)], [(4, 1)]),
    ((106, 1), [(1, 1)], [(1, 1), (4, -1)]),
    ((1, 1), [(6, 1)], [(1, 1), (3, -1)]),
    ((109, 1), [(6, 1), (8, 1)], [(3, 1)]),
    ((2, 1), [(1, 1), (11, -1)], [(1, -1), (6, 1)]),
    ((103, 1), [(6, 1), (8, 1), (13, -1)], [(3, -1), (6, 1)]),
    ((100, 1), [(0, 1), (3, 1), (5, 1), (13, 1)], [(3, -1), (8, 1)]),
    ((4, 1), [(8, 1), (13, -1)], [(6, -1), (8, 1)]),
    ((110, 1), [(6, 1), (8, 1), (11, -1), (13, -1), (14, -1)], [(6, -1)]),
    ((105, 1), [(1, 1), (14, 1)], [(4, 1), (6, -1)]),
    ((108, 1), [(14, 1)], [(6, -1), (9, 1)]),
    ((3, 1), [(4, 1), (14, -1)], [(4, -1), (9, 1)]),
    ((4, 1), [(9, 1)], [(7, -1), (9, 1)]),
    ((102, 1), [(2, 1), (7, 1), (9, 1)], [(4, -1), (7, 1)]),
    ((113, -1), [(7, 1), (9, 1)], [(7, -1)]),
]
Q_LHS_PROG = [
    (100, 3, 8, -1), (101, 0, 2, 1), (102, 7, 101, -1), (103, 5, 100, 1), (104, 4, 6, -1),
    (105, 4, 9, -1), (106, 7, 9, -1), (107, 0, 103, -1), (108, 6, 8, -1), (109, 5, 102, 1),
    (110, 1, 4, -1), (111, 5, 8, -1), (112, 6, 9, -1), (113, 4, 7, -1), (114, 2, 4, -1),
    (115, 1, 6, -1), (116, 2, 7, -1), (117, 1, 3, -1), (118, 3, 6, -1),
]
Q_OUT_PROG = [
    (100, 0, 3, 1), (101, 4, 5, 1), (102, 0, 1, -1), (103, 2, 101, 1), (104, 2, 5, 1),
    (105, 1, 100, -1),
]
Q_PRODS = [
    ((6, -1), [(6, 1), (8, 1), (11, -1), (13, -1), (14, -1)], [(104, 1)]),
    ((101, 1), [(12, 1)], [(104, 1)]),
    ((4, 1), [(1, 1), (2, 1), (4, 1), (7, 1), (9, 1)], [(100, 1)]),
    ((111, -1), [(3, 1)], [(100, 1)]),
    ((118, -1), [(6, 1), (8, 1), (13, -1)], [(103, 1)]),
    ((3, 1), [(6, 1), (8, 1)], [(1, 1), (103, 1)]),
    ((114, 1), [(2, 1), (7, 1)], [(1, 1)]),
    ((117, 1), [(6, 1)], [(1, 1)]),
    ((115, -1), [(1, 1), (11, -1)], [(2, 1)]),
    ((0, -1), [(10, 1), (12, -1)], [(2, -1), (102, 1)]),
    ((116, 1), [(2, 1), (5, 1), (10, -1), (12, 1)], [(102, 1)]),
    ((102, 1), [(5, 1), (10, -1), (12, 1)], [(5, 1), (102, 1)]),
    ((109, -1), [(5, 1), (10, -1)], [(5, 1)]),
    ((112, -1), [(14, 1)], [(3, 1), (5, 1)]),
    ((104, 1), [(1, 1), (14, 1)], [(2, 1), (3, -1)]),
    ((105, -1), [(4, 1), (14, -1)], [(3, 1)]),
    ((5, 1), [(0, 1), (3, 1)], [(3, 1), (101, -1)]),
    ((100, -1), [(0, 1), (3, 1), (5, 1), (13, 1)], [(101, 1)]),
    ((103, 1), [(0, 1), (3, 1), (5, 1)], [(0, 1), (101, 1)]),
    ((110, 1), [(1, 1)], [(0, 1), (2, 1)]),
    ((107, 1), [(0, 1), (5, 1)], [(0, 1)]),
    ((113, -1), [(2, 1), (7, 1), (9, 1)], [(105, -1)]),
    ((7, -1), [(7, 1), (9, 1)], [(4, -1), (105, -1)]),
    ((106, -1), [(9, 1)], [(4, 1)]),
    ((108, -1), [(8, 1), (13, -1)], [(4, 1)]),
]
NPROD = len(O_PRODS)


def _normalize(prods):
    out = []
    for (var, sgn), w, g in prods:
        sgn *= w[0][1]
        out.append((var, [(y, c * w[0][1]) for y, c in w], [(z, c * sgn) for z, c in g]))
    return out


def _positive_outputs(prods, prog):
    for flips in range(1 << 6):
        sg = [(-1 if (flips >> (r % 6)) & 1 else 1) for r in range(len(prods))]
        pos = {}
        for r, p in enumerate(prods):
            for z, c in p[2]:
                pos[z] = max(pos.get(z, -1), c * sg[r])
        for t, a, b, s in reversed(prog):
            st = pos.pop(t)
            pos[a] = max(pos.get(a, -1), st)
            pos[b] = max(pos.get(b, -1), st * s)
        if min(pos.values()) > 0:
            return sg
    raise AssertionError


O_PRODS = _normalize(O_PRODS)
Q_PRODS = _normalize(Q_PRODS)
W_FORMS = [p[1] for p in O_PRODS]
Q_SIGN = _positive_outputs(Q_PRODS, Q_OUT_PROG)
Q_PRODS = [(v, w, [(z, c * s) for z, c in g]) for (v, w, g), s in zip(Q_PRODS, Q_SIGN)]


def _make_lhs(block, prog):
    vals = {}

    def get(v):
        if v not in vals:
            vals[v] = block(v)
        return vals[v]

    for t, a, b, s in prog:
        vals[t] = get(a) + get(b) if s > 0 else get(a) - get(b)
    return get


def _acc_add(accs, z, sgn, m):
    if z not in accs:
        accs[z] = (sgn, m)
    else:
        s0, a = accs[z]
        accs[z] = (s0, a + m) if s0 == sgn else ((1, a - m) if s0 > 0 else (1, m - a))


def _bilinear_run(accs, prods, which, lhs_of, w_of, tick):
    for r in which:
        m = tick(jnp.dot(lhs_of(r), w_of(r), preferred_element_type=f32), 20)
        for z, c in prods[r][2]:
            _acc_add(accs, z, c, m)


def _bilinear_finish(accs, prog):
    for t, a, b, s in reversed(prog):
        st, v = accs.pop(t)
        _acc_add(accs, a, st, v)
        _acc_add(accs, b, st * s, v)
    return accs


def _mul(i, n):
    return i * n if isinstance(i, int) else pl.multiple_of(i * n, 16)


class _Packed:
    def __init__(self, ref):
        self.ref = ref

    @staticmethod
    def _rows(r):
        if isinstance(r, slice):
            return slice(r.start // 2, r.stop // 2)
        start, n = r
        if isinstance(start, int):
            return slice(start // 2, (start + n) // 2)
        return pl.ds(pl.multiple_of(lax.shift_right_logical(start, 1), 8), n // 2)

    def __getitem__(self, idx):
        return pltpu.bitcast(self.ref[self._rows(idx[0]), idx[1]], bf16)

    def __setitem__(self, idx, val):
        self.ref[self._rows(idx[0]), idx[1]] = pltpu.bitcast(val, u32)


def _q_operands(c):
    assert all(s > 0 for row in c for s, _ in row)
    (t0, t1, t2), (b0, b1, b2) = [[a for _, a in row] for row in c]
    lo = lax.broadcasted_iota(jnp.int32, t0.shape, 1) < 64
    return [[jnp.where(lo, t0, b0), jnp.where(lo, t1, t0 - b0), jnp.where(lo, b0 - t0, pltpu.roll(b1, 64, 1))],
            [jnp.where(lo, t2, b2), jnp.where(lo, pltpu.roll(t1, 64, 1), t2 - b2), jnp.where(lo, b2 - t2, b1)]]


def _scores_half(qh, kt, h, j, tick):
    k0, k1, k2 = (0, 64, 128) if h == 0 else (256, 320, 192)
    out = []
    for c in (2 * j, 2 * j + 1):
        cs = slice(c * 128, (c + 1) * 128)
        w = [kt[k0:k0 + 128, cs],
             jnp.concatenate([kt[k2:k2 + 64, cs], kt[k1:k1 + 64, cs]], axis=0),
             jnp.concatenate([kt[k0:k0 + 64, cs], kt[k2:k2 + 64, cs]], axis=0)]
        m = [tick(jnp.dot(qh[i], w[i], preferred_element_type=f32), 20) for i in range(3)]
        out.append(jnp.concatenate([m[0] + m[1], m[0] + m[2]], axis=0))
    return out


def _softmax(s):
    m = jnp.max(s, axis=1, keepdims=True)
    p = jnp.exp2(s - m)
    p0, p1, p2, p3 = (p[:, i * 128:(i + 1) * 128] for i in range(4))
    s01, s23 = p0 + p1, p2 + p3
    t = s01 + s23
    l = jnp.sum(t, axis=1, keepdims=True)
    r = pl.reciprocal(l, approx=True)
    r = r * (2.0 - l * r)
    return jnp.concatenate([s01, jnp.minimum(s23, t), p0, p2, p1, p3], axis=1).astype(bf16), r


def _pv_weights(vt, h, i):
    d0, d1, d2 = (0, 64, 128) if h == 0 else (256, 320, 192)

    def v(d, c):
        return vt[d:d + 64, c * 128:(c + 1) * 128]

    def f(d, c):
        return v(d, c).astype(f32)

    if i == 0:
        return jnp.concatenate([jnp.concatenate([v(d0, c), v(d1, c + 1)], axis=0) for c in (0, 2)], axis=1)
    if i == 1:
        w = [jnp.concatenate([f(d2, c), f(d1, c) - f(d1, c + 1)], axis=0) for c in (0, 2)]
    else:
        w = [jnp.concatenate([f(d0, c + 1) - f(d0, c), f(d2, c + 1)], axis=0) for c in (0, 2)]
    return jnp.concatenate(w, axis=1).astype(bf16)


def _kernel(ax, ak, av, awq, awo, bx, bk, bv, bwq, bwo, o_hbm,
            acc, xbuf, wbuf, kvbuf, obuf, pbuf, qbuf, xc32, wc0, wc1,
            kv_sem, x_sem, w_sem, o_sem, *, scale, nhp, nb):
    pbuf, qbuf, xc = (_Packed(r) for r in (pbuf, qbuf, xc32))
    wc = [_Packed(r) for r in (wc0, wc1)]
    sq = xbuf.shape[2]
    hq = sq // 2
    d = awq.shape[0]
    hw = kvbuf.shape[2]
    wrows = wbuf.shape[0] // 4
    ng = nhp * nb
    lg = nb.bit_length() - 1
    spb = nb // BB

    def kv_start(g):
        hp, b = (g >> lg) & (nhp - 1), g & (nb - 1)
        for i, src in enumerate((ak, av, bk, bv)):
            sem = kv_sem.at[jnp.where(g < nb, b, nb + (b >> 2))]
            pltpu.make_async_copy(src.at[b, hp], kvbuf.at[b, i], sem).start()

    def kv_wait(b):
        pltpu.make_async_copy(kvbuf.at[b], kvbuf.at[b], kv_sem.at[b]).wait()

    def kvg_start(g):
        hp, i4 = g >> lg, (g >> 2) & 3
        b = pl.multiple_of(i4 * BB, BB)
        for i, src in enumerate((ak, av, bk, bv)):
            pltpu.make_async_copy(src.at[pl.ds(b, BB), hp], kvbuf.at[pl.ds(b, BB), i], kv_sem.at[nb + i4]).start()

    def kvg_wait(i4):
        v = kvbuf.at[pl.ds(i4 * BB, BB)]
        pltpu.make_async_copy(v, v, kv_sem.at[nb + i4]).wait()

    def x_start(b, which=(0, 1)):
        for i, src in enumerate((ax, bx)):
            if i in which:
                pltpu.make_async_copy(src.at[b], xbuf.at[b, i], x_sem.at[b]).start()

    def x_wait(b):
        pltpu.make_async_copy(xbuf.at[b], xbuf.at[b], x_sem.at[b]).wait()

    def w_start(h, m):
        off = h * hw if isinstance(h, int) else pl.multiple_of(h * hw, 128)
        if m < 2:
            for c in range(hw // 128):
                pltpu.make_async_copy((awq, bwq)[m].at[:, pl.ds(off + c * 128, 128)],
                                      wbuf.at[pl.ds(m * wrows + c * d, d)], w_sem.at[m]).start()
        else:
            for c in range(d // 128):
                pltpu.make_async_copy((awo, bwo)[m - 2].at[pl.ds(off, hw), pl.ds(c * 128, 128)],
                                      wbuf.at[pl.ds(m * wrows + c * hw, hw)], w_sem.at[m]).start()

    def w_start_dyn(h, m, valid):
        for k in range(4):
            @pl.when(jnp.logical_and(m == k, valid))
            def _():
                w_start(h, k)

    def w_wait(m):
        v = wbuf.at[pl.ds(_mul(m, wrows), wrows)]
        pltpu.make_async_copy(v, v, w_sem.at[m]).wait()

    def prep_w(dst, msrc, mdst, row, nrows, zero=None, sub=0):
        whole = isinstance(row, int) and row == 0
        if isinstance(msrc, int):
            sa, sc = (5, 1) if msrc < 2 else (1, 3)
            off = [(msrc * 15 + (y // 5) * sa + (y % 5) * sc) * 128 + row * 16 for y in range(15)]
        else:
            sa, sc = jnp.where(msrc < 2, 5, 1), jnp.where(msrc < 2, 1, 3)
            off = [pl.multiple_of((msrc * 15 + (y // 5) * sa + (y % 5) * sc) * 128 + row * 16, 128 if whole else 64)
                   for y in range(15)]
        r16 = _mul(mdst * 8 + row, 16)
        if not isinstance(r16, int):
            r16 = pl.multiple_of(r16, 128 if whole else 64)
        for r, form in enumerate(W_FORMS):
            if len(form) == 1:
                val = wbuf[pl.ds(off[form[0][0]] + sub * 16, nrows * 16), :]
            else:
                val = None
                for y, c in form:
                    t = wbuf[pl.ds(off[y] + sub * 16, nrows * 16), :].astype(f32)
                    val = t if val is None else (val + t if c > 0 else val - t)
                val = val.astype(bf16)
            wc[dst][(r16 + sub * 16, nrows * 16), r * 128:(r + 1) * 128] = val
        if zero is not None:
            return lambda: wc[dst][(pl.multiple_of(r16 + zero * 16 + sub * 16, 16), 16), 0:128].astype(f32)[0:8]

    def prep_x(b, br, k0=0, k1=5, zero=None):
        get = _make_lhs(
            lambda z: xbuf[b, br, (z // 5) * hq + k0 * 16:(z // 5) * hq + k1 * 16,
                           (z % 5) * 128:(z % 5 + 1) * 128].astype(f32) * scale, Q_LHS_PROG)
        for r, p in enumerate(Q_PRODS):
            xc[(_mul(b * 2 + br, hq) + k0 * 16, (k1 - k0) * 16), r * 128:(r + 1) * 128] = (
                get(p[0]) * Q_SIGN[r]).astype(bf16)
        if zero is not None:
            c0 = (NPROD - 1) * 128
            return lambda: xc[(_mul(b * 2 + br + zero, hq) + k0 * 16, 16), c0:c0 + 128].astype(f32)[0:8]

    def body(g0, nbat, first, wpre, xpre, plan, cs, first_hp=False, last_hp=False):
        b0 = g0 & (nb - 1)
        pat, qord, oord, qsp, osp = plan
        sched = [(a.split("@")[0], int(a.split("@")[1])) for a in pat.split(",")]
        qord = [int(i) for i in qord.split(".")]
        oord = [int(i) for i in oord.split(".")]
        assert all(sched.index(("ob", u)) < sched.index(("ob", u + 1)) for u in range(0, 2 * nbat, 2))
        R, O, OT, QA, OA, SC, LH = {}, {}, {}, {}, {}, {}, {}
        lazy = {}
        pending = []
        clock = [0]

        def tick(o, cycles):
            t0 = clock[0]
            clock[0] += cycles
            groups = o.shape[0] // 8
            rows = None
            while pending and pending[0][0] <= clock[0]:
                due, emit = pending.pop(0)
                tok = emit()
                g = min(max((due - t0) * groups // cycles, 0), groups - 1)
                rows = rows or [o[8 * i:8 * i + 8] for i in range(groups)]
                rows[g] = jnp.minimum(rows[g], jnp.maximum(rows[g], tok()))
            return o if rows is None else jnp.concatenate(rows, axis=0)

        def later(delay, emit):
            pending.append((clock[0] + delay, emit))
            pending.sort(key=lambda e: e[0])

        def prow(u, h):
            return (2 * u + h) * sq

        def weights(m, prods):
            def w_of(r):
                s = W_FORMS.index(prods[r][1])
                return wc[cs][m * 128:(m + 1) * 128, s * 128:(s + 1) * 128]
            return w_of

        def q_(u, lo_, hi_):
            b, br = b0 + u // 2, u % 2

            def lhs_of(r):
                return xc[(_mul(b * 2 + br, hq), hq), r * 128:(r + 1) * 128]

            _bilinear_run(QA.setdefault(u, {}), Q_PRODS, qord[lo_:hi_], lhs_of, weights(br, Q_PRODS), tick)
            if hi_ == NPROD:
                fin = _bilinear_finish(QA[u], Q_OUT_PROG)

                def store_q():
                    c = [[fin[i * 3 + n] for n in range(3)] for i in range(2)]
                    for h, ops in enumerate(_q_operands(c)):
                        for i, a in enumerate(ops):
                            qbuf[u * hq:(u + 1) * hq, (3 * h + i) * 128:(3 * h + i + 1) * 128] = a.astype(bf16)

                lazy["q", u] = store_q

        def s_(u, h, j):
            b, br = b0 + u // 2, u % 2
            lazy.pop(("q", u), lambda: None)()
            qh = [qbuf[u * hq:(u + 1) * hq, (3 * h + i) * 128:(3 * h + i + 1) * 128] for i in range(3)]
            SC[u, h, j] = _scores_half(qh, kvbuf.at[b, 2 * br], h, j, tick)
            if j == 1:
                s = jnp.concatenate(SC[u, h, 0] + SC[u, h, 1], axis=1)

                def store_p():
                    p, R[u, h] = _softmax(s)
                    pbuf[prow(u, h):prow(u, h) + sq, :] = p

                lazy["p", u, h] = store_p

        def m_(u, h, half):
            lazy.pop(("p", u, h), lambda: None)()
            vt = kvbuf.at[b0 + u // 2 + (g0 >> 20) * half, 2 * (u % 2) + 1]
            r0 = prow(u, h) + half * hq
            res = [tick(lax.dot_general(pbuf[r0:r0 + hq, i * 256:(i + 1) * 256], _pv_weights(vt, h, i), NT,
                                        preferred_element_type=f32), 40) for i in range(3)]
            lo = lax.broadcasted_iota(jnp.int32, (hq, 128), 1) < 64
            r = R[u, h][half * hq:(half + 1) * hq]
            O[u, h, half] = (res[0] + jnp.where(lo, res[2], res[1])) * r
            OT[u, h, half] = jnp.where(lo, res[1], res[2]) * r

        def o_(u, lo_, hi_):
            b, br = b0 + u // 2, u % 2
            if lo_ == 0:
                lo = lax.broadcasted_iota(jnp.int32, (hq, 128), 1) < 64
                mid = [jnp.where(lo, OT[u, 0, i], OT[u, 1, i]) +
                       pltpu.roll(jnp.where(lo, OT[u, 1, i], OT[u, 0, i]), 64, 1) for i in range(2)]
                tiles = [[O[u, 0, i], mid[i], O[u, 1, i]] for i in range(2)]
                get = _make_lhs(lambda x: tiles[x // 3][x % 3], O_LHS_PROG)
                LH[u] = {p[0]: get(p[0]).astype(bf16) for p in O_PRODS}
            _bilinear_run(OA.setdefault(u, {}), O_PRODS, oord[lo_:hi_], lambda r: LH[u][O_PRODS[r][0]],
                          weights(2 + br, O_PRODS), tick)
            if hi_ < NPROD:
                return
            fin = _bilinear_finish(OA[u], O_OUT_PROG)
            for n in range(5):
                for i in range(2):
                    s, a = fin[i * 5 + n]
                    rows = slice(i * hq, (i + 1) * hq)
                    cols = slice(br * d + n * 128, br * d + (n + 1) * 128)
                    if first_hp:
                        new = a if s > 0 else -a
                    else:
                        new = acc[b, rows, cols] + a if s > 0 else acc[b, rows, cols] - a
                    if last_hp:
                        obuf[b, rows, cols] = new.astype(obuf.dtype)
                    else:
                        acc[b, rows, cols] = new
            if br == 1 and last_hp:
                pltpu.make_async_copy(obuf.at[b], o_hbm.at[b], o_sem).start()

        fns = {"qa": lambda u: q_(u, 0, qsp), "qb": lambda u: q_(u, qsp, NPROD),
               "oa": lambda u: o_(u, 0, osp), "ob": lambda u: o_(u, osp, NPROD),
               "s00": lambda u: s_(u, 0, 0), "s01": lambda u: s_(u, 0, 1),
               "s10": lambda u: s_(u, 1, 0), "s11": lambda u: s_(u, 1, 1),
               "m0": lambda u: m_(u, 0, 0), "m1": lambda u: m_(u, 1, 0),
               "t0": lambda u: m_(u, 0, 1), "t1": lambda u: m_(u, 1, 1)}
        for f in first:
            f()
        total = 2 * nbat * 1960
        lastq = max(i for i, it in enumerate(sched) if it[0][0] == "q")
        for k, f in enumerate(wpre):
            lo_, hi_ = (PLO, total - PHI) if nbat > 1 else (SWLO, SWHI)
            later(lo_ + k * (hi_ - lo_) // len(wpre), f)
        for i, item in enumerate(sched):
            fns[item[0]](item[1])
            if i == lastq:
                for k, f in enumerate(xpre):
                    later(SXLO + k * (total - SXHI - clock[0] - SXLO) // len(xpre), f)
        assert not pending and not lazy

    for k in range(4):
        w_start(0, k)
    x_start(0)
    kv_start(0)
    x_start(1)
    for g in range(1, C0):
        kv_start(g)
        x_start(g + 1)
    for m in range(4):
        w_wait(m)
        prep_w(0, m, m, 0, 8)
    x_wait(0)
    for br in range(2):
        prep_x(0, br)

    def issued(g):
        return jnp.minimum(jnp.minimum(RATE * (g + 1) + C0, jnp.maximum(g + LA, LB * g - LC)), nb + DIST * BB)

    def ramp(b0, carry):
        half = nb // 2
        m = (b0 - half) >> 1

        @pl.when(b0 + 1 < nb)
        def _():
            x_wait(b0 + 1)

        @pl.when(jnp.logical_and(b0 >= half, (b0 & 1) == 0))
        def _():
            w_wait(m)

        kv_wait(b0)

        hi = issued(b0)
        prev = jnp.where(b0 == 0, C0, issued(b0 - 1))

        def pf_x(k, w):
            @pl.when(jnp.logical_and(prev + k < hi, prev + k + 1 < nb))
            def _():
                x_start(prev + k + 1, (w,))

        def pf_kv(k):
            @pl.when(prev + k < hi)
            def _():
                kv_start(prev + k)

        def pf_w():
            w_start_dyn(jnp.where(b0 == W2AT, 2, 1), jnp.where(b0 == W2AT, 0, (b0 >> 1) - 1),
                        jnp.logical_or(b0 == W2AT, jnp.logical_and(b0 <= half, (b0 & 1) == 0)))

        first = [pf_w] + [functools.partial(pf_x, k, w) for k in range(RATE) for w in range(2)]
        first += [functools.partial(pf_kv, k) for k in range(RATE)]
        zero = b0 >> 20
        wpre = [functools.partial(prep_w, 1, jnp.where(b0 >= half, m, 3), jnp.maximum(m, 0), (b0 & 1) * 4, 1,
                                  zero, k) for k in range(4)]
        xpre = [functools.partial(prep_x, jnp.minimum(b0 + 1, nb - 1), br, k, k + 1, zero)
                for br in range(2) for k in range(5)]
        body(b0, 1, first, wpre, xpre, RAMP, 0, first_hp=True)
        return carry

    def step(par, last, hp, i, carry):
        g0 = hp * nb + i * BB

        if not last:
            w_wait(i)

        kvg_wait(i)

        if last:
            def pf_kv():
                @pl.when(g0 + DIST * BB < ng)
                def _():
                    kvg_start(g0 + DIST * BB)

            body(g0, BB, [pf_kv], [], [], LAST, par, last_hp=True)
        else:
            hn = jnp.where(i == 3, hp + 2, hp + 1)
            first = [lambda: w_start_dyn(hn, (i + 1) & 3, hn < nhp), functools.partial(kvg_start, g0 + DIST * BB)]
            wpre = [functools.partial(prep_w, 1 - par, i, i, 0, 1, i >> 20, k) for k in range(8)]
            body(g0, BB, first, wpre, [], STEADY, par)
        return carry

    def pair(t, carry):
        lax.fori_loop(jnp.where(t > 0, 0, spb), spb, functools.partial(step, 0, False, 2 * t), 0)
        lax.fori_loop(0, jnp.where(2 * t + 1 < nhp - 1, spb, 0), functools.partial(step, 1, False, 2 * t + 1), 0)
        return carry

    lax.fori_loop(0, nb, ramp, 0)
    lax.fori_loop(0, nhp // 2, pair, 0)
    lax.fori_loop(0, spb, functools.partial(step, 1, True, nhp - 1), 0)
    pltpu.make_async_copy(obuf, o_hbm, o_sem).wait()


@jax.jit
def pallas_concat_heads__gqa_block_cached__mha_block_cached__near_ridge_kernel(
    A_x: jax.Array,
    A_k_cache: jax.Array,
    A_v_cache: jax.Array,
    A_wq: jax.Array,
    A_wo: jax.Array,
    B_x: jax.Array,
    B_k_cache: jax.Array,
    B_v_cache: jax.Array,
    B_wq: jax.Array,
    B_wo: jax.Array,
):
    B, Sq, D = A_x.shape
    _, H, Sk, Dh = A_k_cache.shape
    nhp = H // 2
    assert (B, Sq, D, Sk, Dh) == (16, 160, 640, 512, 192) and A_wq.shape[1] == H * Dh
    assert nhp >= 4 and nhp & (nhp - 1) == 0 and B_k_cache.shape == A_k_cache.shape
    n_iss = C0
    for g0 in range(B):
        assert n_iss >= g0 + 2
        hi = min(RATE * (g0 + 1) + C0, max(g0 + LA, LB * g0 - LC), B + DIST * BB)
        assert hi <= g0 + B and 0 <= hi - n_iss <= RATE
        n_iss = hi
    assert n_iss == B + DIST * BB and 10 <= W2AT <= 15

    def tr(c):
        return jnp.swapaxes(c, 2, 3).reshape(B, nhp, 2 * Dh, Sk)

    any_spec = pl.BlockSpec(memory_space=pl.ANY)
    return pl.pallas_call(
        functools.partial(_kernel, scale=Dh ** -0.5 * LOG2E, nhp=nhp, nb=B),
        in_specs=[any_spec] * 10,
        out_specs=any_spec,
        out_shape=jax.ShapeDtypeStruct((B, Sq, 2 * D), A_x.dtype),
        scratch_shapes=[pltpu.VMEM((B, Sq, 2 * D), f32),
                        pltpu.VMEM((B, 2, Sq, D), bf16),
                        pltpu.VMEM((4 * 15 * 128, 128), bf16),
                        pltpu.VMEM((B, 4, 2 * Dh, Sk), bf16),
                        pltpu.VMEM((B, Sq, 2 * D), bf16),
                        pltpu.VMEM((2 * BB * Sq, 6 * 128), u32),
                        pltpu.VMEM((2 * BB * Sq // 4, 6 * 128), u32),
                        pltpu.VMEM((B * 2 * Sq // 4, XCW * 128), u32),
                        pltpu.VMEM((4 * 64, WCW * 128), u32),
                        pltpu.VMEM((4 * 64, WCW * 128), u32),
                        pltpu.SemaphoreType.DMA((B + 4,)),
                        pltpu.SemaphoreType.DMA((B,)),
                        pltpu.SemaphoreType.DMA((4,)),
                        pltpu.SemaphoreType.DMA(())],
        compiler_params=pltpu.CompilerParams(
            disable_bounds_checks=True,
            vmem_limit_bytes=110 * 1024 * 1024),
    )(A_x, tr(A_k_cache), tr(A_v_cache), A_wq, A_wo, B_x, tr(B_k_cache), tr(B_v_cache), B_wq, B_wo)
```

```python
import functools

import jax
import jax.numpy as jnp
from jax import lax
import jax.experimental.pallas as pl
import jax.experimental.pallas.tpu as pltpu

bf16 = jnp.bfloat16
f32 = jnp.float32
u32 = jnp.uint32
NT = (((1,), (1,)), ((), ()))
LOG2E = 1.4426950408889634

BB = 4
DIST = 2
C0, RATE, LA, LB, LC = 2, 2, 6, 2, 6
W2AT = 11
XCW, WCW = 32, 40

PAT = (
    "qa@0,qb@0,qa@1,qb@1,qa@2,s00@0,s01@0,s10@0,qb@2,s11@0,m0@0,t0@0,s00@1,qa@3,s01@1,t1@0,s10@1,qb@3,m1@0,"
    "s11@1,m0@1,t0@1,s00@2,qa@4,s01@2,m1@1,t1@1,s10@2,oa@0,s11@2,qa@5,m0@2,ob@0,t0@2,s00@3,qb@4,s01@3,t1@2,"
    "m1@2,s10@3,oa@1,qb@5,s11@3,m0@3,t0@3,ob@1,s00@4,oa@2,qa@6,s01@4,m1@3,t1@3,s10@4,s11@4,m0@4,t0@4,s00@5,"
    "ob@2,qb@6,qa@7,s01@5,m1@4,t1@4,s10@5,oa@3,qb@7,s11@5,m0@5,t0@5,ob@3,s00@6,oa@4,s01@6,s10@6,m1@5,t1@5,"
    "s11@6,m0@6,t0@6,ob@4,s00@7,s01@7,m1@6,t1@6,s10@7,oa@5,s11@7,m0@7,t0@7,ob@5,m1@7,t1@7,oa@6,ob@6,oa@7,"
    "ob@7")
SPAT = (
    "qa@0,qb@0,qa@1,s00@0,s10@0,s11@0,s01@0,qb@1,m1@0,m0@0,t0@0,s00@1,t1@0,s10@1,s01@1,s11@1,oa@0,m0@1,m1@1,"
    "t0@1,t1@1,ob@0,oa@1,ob@1")
LPAT = (
    "qa@0,qb@0,qa@1,qb@1,qa@2,s00@0,s01@0,s10@0,qb@2,s11@0,m0@0,s10@1,t0@0,s00@1,qa@3,s01@1,t1@0,qb@3,m1@0,"
    "s11@1,m0@1,t0@1,s00@2,qa@4,s01@2,m1@1,t1@1,s10@2,oa@0,s11@2,m0@2,ob@0,t0@2,s00@3,qa@5,qb@4,s01@3,t1@2,"
    "m1@2,s10@3,oa@1,qb@5,s11@3,m0@3,t0@3,ob@1,s00@4,qa@6,oa@2,s01@4,m1@3,t1@3,s10@4,s11@4,m0@4,t0@4,s00@5,"
    "ob@2,qb@6,qa@7,s01@5,m1@4,t1@4,s10@5,oa@3,qb@7,s11@5,m0@5,t0@5,ob@3,s00@6,oa@4,s01@6,s10@6,m1@5,t1@5,"
    "s11@6,m0@6,t0@6,ob@4,s00@7,s01@7,m1@6,t1@6,s10@7,oa@5,s11@7,m0@7,t0@7,ob@5,m1@7,t1@7,oa@6,ob@6,oa@7,"
    "ob@7")
QORD = (
    "16.9.24.21.19.1.15.18.22.17.20.12.3.2.4.5.23.7.6.14.8.0.10.11.13/"
    "9.16.24.21.19.1.12.15.18.22.6.20.3.2.4.5.23.7.17.8.14.0.10.11.13/"
    "9.16.24.21.19.1.15.18.22.17.20.12.3.2.4.5.23.7.6.8.14.0.10.11.13/"
    "9.16.24.21.19.1.15.18.22.17.20.12.3.2.4.5.23.7.6.8.14.0.10.11.13/"
    "9.16.24.21.19.1.15.18.22.17.20.12.3.2.4.5.23.7.6.8.14.0.10.11.13/"
    "9.16.24.21.19.15.1.18.22.17.20.12.3.2.4.5.23.7.6.8.14.0.10.11.13/"
    "9.16.24.21.19.1.15.18.22.17.20.12.2.3.4.5.23.7.6.8.14.0.10.11.13/"
    "9.16.24.21.19.1.15.18.22.17.20.12.3.2.4.5.23.7.6.8.14.0.10.11.13")
OORD = (
    "0.6.1.5.3.2.8.9.4.24.12.11.14.10.16.19.13.15.17.18.20.22.21.23.7/"
    "0.6.1.5.3.2.8.9.4.24.12.11.14.10.16.19.13.15.17.18.20.22.21.23.7/"
    "0.6.1.5.3.2.8.9.4.24.12.11.14.10.16.19.13.15.17.18.20.22.21.23.7/"
    "0.6.1.5.3.2.8.9.4.24.12.11.14.10.16.19.13.15.17.18.20.22.21.7.23/"
    "0.6.1.5.3.2.8.9.4.10.24.12.11.14.20.19.13.15.17.18.16.22.21.23.7/"
    "0.6.1.5.3.2.8.9.4.24.12.11.14.10.16.19.13.15.17.22.18.20.21.23.7/"
    "0.6.1.5.3.2.8.9.4.24.12.11.14.10.16.19.13.15.17.18.20.22.21.23.7/"
    "7.23.21.22.20.18.17.15.13.19.16.10.14.11.12.24.4.9.8.2.3.5.1.6.0")
SQORD = "3.16.24.15.18.7.20.21.9.10.22.1.23.6.12.0.2.14.8.17.13.11.4.5.19"
SOORD = "4.0.3.1.5.6.8.2.9.14.24.10.12.13.15.21.11.19.17.16.18.20.23.22.7"
LQORD = "9.16.24.21.19.1.15.20.18.22.17.23.12.3.2.4.7.6.8.5.14.0.10.11.13"
LOORD = "0.6.1.5.3.2.8.9.4.24.12.11.14.10.16.19.13.15.17.18.20.22.21.23.7"
STEADY = (PAT, QORD, OORD, 11, 10)
RAMP = (SPAT, SQORD, SOORD, 13, 13)
LAST = (LPAT, LQORD, LOORD, 11, 10)
PLO, PHI, SWLO, SWHI, SXLO, SXHI = 300, 520, 140, 920, 1500, 160

O_LHS_PROG = [
    (100, 4, 5, 1), (101, 0, 1, -1), (102, 3, 101, 1), (103, 2, 100, 1), (104, 0, 3, 1),
    (105, 2, 3, -1), (106, 0, 2, 1), (107, 2, 101, -1), (108, 3, 5, 1), (109, 1, 103, 1),
    (110, 2, 5, 1), (111, 3, 100, -1), (112, 5, 101, 1), (113, 4, 102, -1), (114, 0, 100, 1),
]
O_OUT_PROG = [
    (100, 5, 8, -1), (101, 3, 100, 1), (102, 2, 7, -1), (103, 0, 102, 1),
]
O_PRODS = [
    ((101, 1), [(2, 1), (5, 1), (10, -1), (12, 1)], [(102, 1)]),
    ((104, 1), [(3, 1)], [(100, -1)]),
    ((111, 1), [(0, 1), (3, 1)], [(5, 1)]),
    ((5, 1), [(5, 1), (10, -1)], [(5, -1), (103, 1)]),
    ((112, 1), [(5, 1), (10, -1), (12, 1)], [(103, -1)]),
    ((114, 1), [(0, 1), (3, 1), (5, 1)], [(101, 1)]),
    ((0, 1), [(0, 1), (5, 1)], [(0, 1), (101, -1)]),
    ((107, -1), [(10, 1), (12, -1)], [(0, -1)]),
    ((110, 1), [(12, 1)], [(0, 1), (2, 1)]),
    ((1, 1), [(2, 1), (7, 1)], [(2, 1), (4, -1)]),
    ((104, 1), [(1, 1), (2, 1), (4, 1), (7, 1), (9, 1)], [(4, 1)]),
    ((106, 1), [(1, 1)], [(1, 1), (4, -1)]),
    ((1, 1), [(6, 1)], [(1, 1), (3, -1)]),
    ((109, 1), [(6, 1), (8, 1)], [(3, 1)]),
    ((2, 1), [(1, 1), (11, -1)], [(1, -1), (6, 1)]),
    ((103, 1), [(6, 1), (8, 1), (13, -1)], [(3, -1), (6, 1)]),
    ((100, 1), [(0, 1), (3, 1), (5, 1), (13, 1)], [(3, -1), (8, 1)]),
    ((4, 1), [(8, 1), (13, -1)], [(6, -1), (8, 1)]),
    ((110, 1), [(6, 1), (8, 1), (11, -1), (13, -1), (14, -1)], [(6, -1)]),
    ((105, 1), [(1, 1), (14, 1)], [(4, 1), (6, -1)]),
    ((108, 1), [(14, 1)], [(6, -1), (9, 1)]),
    ((3, 1), [(4, 1), (14, -1)], [(4, -1), (9, 1)]),
    ((4, 1), [(9, 1)], [(7, -1), (9, 1)]),
    ((102, 1), [(2, 1), (7, 1), (9, 1)], [(4, -1), (7, 1)]),
    ((113, -1), [(7, 1), (9, 1)], [(7, -1)]),
]
Q_LHS_PROG = [
    (100, 3, 8, -1), (101, 0, 2, 1), (102, 7, 101, -1), (103, 5, 100, 1), (104, 4, 6, -1),
    (105, 4, 9, -1), (106, 7, 9, -1), (107, 0, 103, -1), (108, 6, 8, -1), (109, 5, 102, 1),
    (110, 1, 4, -1), (111, 5, 8, -1), (112, 6, 9, -1), (113, 4, 7, -1), (114, 2, 4, -1),
    (115, 1, 6, -1), (116, 2, 7, -1), (117, 1, 3, -1), (118, 3, 6, -1),
]
Q_OUT_PROG = [
    (100, 0, 3, 1), (101, 4, 5, 1), (102, 0, 1, -1), (103, 2, 101, 1), (104, 2, 5, 1),
    (105, 1, 100, -1),
]
Q_PRODS = [
    ((6, -1), [(6, 1), (8, 1), (11, -1), (13, -1), (14, -1)], [(104, 1)]),
    ((101, 1), [(12, 1)], [(104, 1)]),
    ((4, 1), [(1, 1), (2, 1), (4, 1), (7, 1), (9, 1)], [(100, 1)]),
    ((111, -1), [(3, 1)], [(100, 1)]),
    ((118, -1), [(6, 1), (8, 1), (13, -1)], [(103, 1)]),
    ((3, 1), [(6, 1), (8, 1)], [(1, 1), (103, 1)]),
    ((114, 1), [(2, 1), (7, 1)], [(1, 1)]),
    ((117, 1), [(6, 1)], [(1, 1)]),
    ((115, -1), [(1, 1), (11, -1)], [(2, 1)]),
    ((0, -1), [(10, 1), (12, -1)], [(2, -1), (102, 1)]),
    ((116, 1), [(2, 1), (5, 1), (10, -1), (12, 1)], [(102, 1)]),
    ((102, 1), [(5, 1), (10, -1), (12, 1)], [(5, 1), (102, 1)]),
    ((109, -1), [(5, 1), (10, -1)], [(5, 1)]),
    ((112, -1), [(14, 1)], [(3, 1), (5, 1)]),
    ((104, 1), [(1, 1), (14, 1)], [(2, 1), (3, -1)]),
    ((105, -1), [(4, 1), (14, -1)], [(3, 1)]),
    ((5, 1), [(0, 1), (3, 1)], [(3, 1), (101, -1)]),
    ((100, -1), [(0, 1), (3, 1), (5, 1), (13, 1)], [(101, 1)]),
    ((103, 1), [(0, 1), (3, 1), (5, 1)], [(0, 1), (101, 1)]),
    ((110, 1), [(1, 1)], [(0, 1), (2, 1)]),
    ((107, 1), [(0, 1), (5, 1)], [(0, 1)]),
    ((113, -1), [(2, 1), (7, 1), (9, 1)], [(105, -1)]),
    ((7, -1), [(7, 1), (9, 1)], [(4, -1), (105, -1)]),
    ((106, -1), [(9, 1)], [(4, 1)]),
    ((108, -1), [(8, 1), (13, -1)], [(4, 1)]),
]
NPROD = len(O_PRODS)


def _normalize(prods):
    out = []
    for (var, sgn), w, g in prods:
        sgn *= w[0][1]
        out.append((var, [(y, c * w[0][1]) for y, c in w], [(z, c * sgn) for z, c in g]))
    return out


def _positive_outputs(prods, prog):
    for flips in range(1 << 6):
        sg = [(-1 if (flips >> (r % 6)) & 1 else 1) for r in range(len(prods))]
        pos = {}
        for r, p in enumerate(prods):
            for z, c in p[2]:
                pos[z] = max(pos.get(z, -1), c * sg[r])
        for t, a, b, s in reversed(prog):
            st = pos.pop(t)
            pos[a] = max(pos.get(a, -1), st)
            pos[b] = max(pos.get(b, -1), st * s)
        if min(pos.values()) > 0:
            return sg
    raise AssertionError


O_PRODS = _normalize(O_PRODS)
Q_PRODS = _normalize(Q_PRODS)
W_FORMS = [p[1] for p in O_PRODS]
Q_SIGN = _positive_outputs(Q_PRODS, Q_OUT_PROG)
Q_PRODS = [(v, w, [(z, c * s) for z, c in g]) for (v, w, g), s in zip(Q_PRODS, Q_SIGN)]


def _make_lhs(block, prog):
    vals = {}

    def get(v):
        if v not in vals:
            vals[v] = block(v)
        return vals[v]

    for t, a, b, s in prog:
        vals[t] = get(a) + get(b) if s > 0 else get(a) - get(b)
    return get


def _acc_add(accs, z, sgn, m):
    if z not in accs:
        accs[z] = (sgn, m)
    else:
        s0, a = accs[z]
        accs[z] = (s0, a + m) if s0 == sgn else ((1, a - m) if s0 > 0 else (1, m - a))


def _bilinear_run(accs, prods, which, lhs_of, w_of, tick):
    for r in which:
        m = tick(jnp.dot(lhs_of(r), w_of(r), preferred_element_type=f32), 20)
        for z, c in prods[r][2]:
            _acc_add(accs, z, c, m)


def _bilinear_finish(accs, prog):
    for t, a, b, s in reversed(prog):
        st, v = accs.pop(t)
        _acc_add(accs, a, st, v)
        _acc_add(accs, b, st * s, v)
    return accs


def _mul(i, n):
    return i * n if isinstance(i, int) else pl.multiple_of(i * n, 16)


class _Packed:
    def __init__(self, ref):
        self.ref = ref

    @staticmethod
    def _rows(r):
        if isinstance(r, slice):
            return slice(r.start // 2, r.stop // 2)
        start, n = r
        if isinstance(start, int):
            return slice(start // 2, (start + n) // 2)
        return pl.ds(pl.multiple_of(lax.shift_right_logical(start, 1), 8), n // 2)

    def __getitem__(self, idx):
        return pltpu.bitcast(self.ref[self._rows(idx[0]), idx[1]], bf16)

    def __setitem__(self, idx, val):
        self.ref[self._rows(idx[0]), idx[1]] = pltpu.bitcast(val, u32)


def _q_operands(c):
    assert all(s > 0 for row in c for s, _ in row)
    (t0, t1, t2), (b0, b1, b2) = [[a for _, a in row] for row in c]
    lo = lax.broadcasted_iota(jnp.int32, t0.shape, 1) < 64
    return [[jnp.where(lo, t0, b0), jnp.where(lo, t1, t0 - b0), jnp.where(lo, b0 - t0, pltpu.roll(b1, 64, 1))],
            [jnp.where(lo, t2, b2), jnp.where(lo, pltpu.roll(t1, 64, 1), t2 - b2), jnp.where(lo, b2 - t2, b1)]]


def _scores_half(qh, kt, h, j, tick):
    k0, k1, k2 = (0, 64, 128) if h == 0 else (256, 320, 192)
    out = []
    for c in (2 * j, 2 * j + 1):
        cs = slice(c * 128, (c + 1) * 128)
        w = [kt[k0:k0 + 128, cs],
             jnp.concatenate([kt[k2:k2 + 64, cs], kt[k1:k1 + 64, cs]], axis=0),
             jnp.concatenate([kt[k0:k0 + 64, cs], kt[k2:k2 + 64, cs]], axis=0)]
        m = [tick(jnp.dot(qh[i], w[i], preferred_element_type=f32), 20) for i in range(3)]
        out.append(jnp.concatenate([m[0] + m[1], m[0] + m[2]], axis=0))
    return out


def _softmax(s):
    m = jnp.max(s, axis=1, keepdims=True)
    p = jnp.exp2(s - m)
    p0, p1, p2, p3 = (p[:, i * 128:(i + 1) * 128] for i in range(4))
    s01, s23 = p0 + p1, p2 + p3
    t = s01 + s23
    l = jnp.sum(t, axis=1, keepdims=True)
    r = pl.reciprocal(l, approx=True)
    r = r * (2.0 - l * r)
    return jnp.concatenate([s01, jnp.minimum(s23, t), p0, p2, p1, p3], axis=1).astype(bf16), r


def _pv_weights(vt, h, i):
    d0, d1, d2 = (0, 64, 128) if h == 0 else (256, 320, 192)

    def v(d, c):
        return vt[d:d + 64, c * 128:(c + 1) * 128]

    def f(d, c):
        return v(d, c).astype(f32)

    if i == 0:
        return jnp.concatenate([jnp.concatenate([v(d0, c), v(d1, c + 1)], axis=0) for c in (0, 2)], axis=1)
    if i == 1:
        w = [jnp.concatenate([f(d2, c), f(d1, c) - f(d1, c + 1)], axis=0) for c in (0, 2)]
    else:
        w = [jnp.concatenate([f(d0, c + 1) - f(d0, c), f(d2, c + 1)], axis=0) for c in (0, 2)]
    return jnp.concatenate(w, axis=1).astype(bf16)


def _kernel(ax, ak, av, awq, awo, bx, bk, bv, bwq, bwo, o_hbm,
            acc, xbuf, wbuf, kvbuf, obuf, pbuf, qbuf, xc32, wc0, wc1,
            kv_sem, x_sem, w_sem, o_sem, *, scale, nhp, nb):
    pbuf, qbuf, xc = (_Packed(r) for r in (pbuf, qbuf, xc32))
    wc = [_Packed(r) for r in (wc0, wc1)]
    sq = xbuf.shape[2]
    hq = sq // 2
    d = awq.shape[0]
    hw = kvbuf.shape[2]
    wrows = wbuf.shape[0] // 4
    ng = nhp * nb
    lg = nb.bit_length() - 1
    spb = nb // BB

    def kv_start(g):
        hp, b = (g >> lg) & (nhp - 1), g & (nb - 1)
        for i, src in enumerate((ak, av, bk, bv)):
            sem = kv_sem.at[jnp.where(g < nb, b, nb + (b >> 2))]
            pltpu.make_async_copy(src.at[b, hp], kvbuf.at[b, i], sem).start()

    def kv_wait(b):
        pltpu.make_async_copy(kvbuf.at[b], kvbuf.at[b], kv_sem.at[b]).wait()

    def kvg_start(g):
        hp, i4 = g >> lg, (g >> 2) & 3
        b = pl.multiple_of(i4 * BB, BB)
        for i, src in enumerate((ak, av, bk, bv)):
            pltpu.make_async_copy(src.at[pl.ds(b, BB), hp], kvbuf.at[pl.ds(b, BB), i], kv_sem.at[nb + i4]).start()

    def kvg_wait(i4):
        v = kvbuf.at[pl.ds(i4 * BB, BB)]
        pltpu.make_async_copy(v, v, kv_sem.at[nb + i4]).wait()

    def x_start(b, which=(0, 1)):
        for i, src in enumerate((ax, bx)):
            if i in which:
                pltpu.make_async_copy(src.at[b], xbuf.at[b, i], x_sem.at[b]).start()

    def x_wait(b):
        pltpu.make_async_copy(xbuf.at[b], xbuf.at[b], x_sem.at[b]).wait()

    def w_start(h, m):
        off = h * hw if isinstance(h, int) else pl.multiple_of(h * hw, 128)
        if m < 2:
            for c in range(hw // 128):
                pltpu.make_async_copy((awq, bwq)[m].at[:, pl.ds(off + c * 128, 128)],
                                      wbuf.at[pl.ds(m * wrows + c * d, d)], w_sem.at[m]).start()
        else:
            for c in range(d // 128):
                pltpu.make_async_copy((awo, bwo)[m - 2].at[pl.ds(off, hw), pl.ds(c * 128, 128)],
                                      wbuf.at[pl.ds(m * wrows + c * hw, hw)], w_sem.at[m]).start()

    def w_start_dyn(h, m, valid):
        for k in range(4):
            @pl.when(jnp.logical_and(m == k, valid))
            def _():
                w_start(h, k)

    def w_wait(m):
        v = wbuf.at[pl.ds(_mul(m, wrows), wrows)]
        pltpu.make_async_copy(v, v, w_sem.at[m]).wait()

    def prep_w(dst, msrc, mdst, row, nrows, zero=None, sub=0):
        whole = isinstance(row, int) and row == 0
        if isinstance(msrc, int):
            sa, sc = (5, 1) if msrc < 2 else (1, 3)
            off = [(msrc * 15 + (y // 5) * sa + (y % 5) * sc) * 128 + row * 16 for y in range(15)]
        else:
            sa, sc = jnp.where(msrc < 2, 5, 1), jnp.where(msrc < 2, 1, 3)
            off = [pl.multiple_of((msrc * 15 + (y // 5) * sa + (y % 5) * sc) * 128 + row * 16, 128 if whole else 64)
                   for y in range(15)]
        r16 = _mul(mdst * 8 + row, 16)
        if not isinstance(r16, int):
            r16 = pl.multiple_of(r16, 128 if whole else 64)
        for r, form in enumerate(W_FORMS):
            if len(form) == 1:
                val = wbuf[pl.ds(off[form[0][0]] + sub * 16, nrows * 16), :]
            else:
                val = None
                for y, c in form:
                    t = wbuf[pl.ds(off[y] + sub * 16, nrows * 16), :].astype(f32)
                    val = t if val is None else (val + t if c > 0 else val - t)
                val = val.astype(bf16)
            wc[dst][(r16 + sub * 16, nrows * 16), r * 128:(r + 1) * 128] = val
        if zero is not None:
            return lambda: wc[dst][(pl.multiple_of(r16 + zero * 16 + sub * 16, 16), 16), 0:128].astype(f32)[0:8]

    def prep_x(b, br, k0=0, k1=5, zero=None):
        get = _make_lhs(
            lambda z: xbuf[b, br, (z // 5) * hq + k0 * 16:(z // 5) * hq + k1 * 16,
                           (z % 5) * 128:(z % 5 + 1) * 128].astype(f32) * scale, Q_LHS_PROG)
        for r, p in enumerate(Q_PRODS):
            xc[(_mul(b * 2 + br, hq) + k0 * 16, (k1 - k0) * 16), r * 128:(r + 1) * 128] = (
                get(p[0]) * Q_SIGN[r]).astype(bf16)
        if zero is not None:
            c0 = (NPROD - 1) * 128
            return lambda: xc[(_mul(b * 2 + br + zero, hq) + k0 * 16, 16), c0:c0 + 128].astype(f32)[0:8]

    def body(g0, nbat, first, wpre, xpre, plan, cs, first_hp=False, last_hp=False):
        b0 = g0 & (nb - 1)
        pat, qord, oord, qsp, osp = plan
        sched = [(a.split("@")[0], int(a.split("@")[1])) for a in pat.split(",")]
        qord = [[int(i) for i in o.split(".")] for o in qord.split("/")]
        oord = [[int(i) for i in o.split(".")] for o in oord.split("/")]
        assert all(sched.index(("ob", u)) < sched.index(("ob", u + 1)) for u in range(0, 2 * nbat, 2))
        R, O, OT, QA, OA, SC, LH = {}, {}, {}, {}, {}, {}, {}
        lazy = {}
        pending = []
        clock = [0]

        def tick(o, cycles):
            t0 = clock[0]
            clock[0] += cycles
            groups = o.shape[0] // 8
            rows = None
            while pending and pending[0][0] <= clock[0]:
                due, emit = pending.pop(0)
                tok = emit()
                g = min(max((due - t0) * groups // cycles, 0), groups - 1)
                rows = rows or [o[8 * i:8 * i + 8] for i in range(groups)]
                rows[g] = jnp.minimum(rows[g], jnp.maximum(rows[g], tok()))
            return o if rows is None else jnp.concatenate(rows, axis=0)

        def later(delay, emit):
            pending.append((clock[0] + delay, emit))
            pending.sort(key=lambda e: e[0])

        def prow(u, h):
            return (2 * u + h) * sq

        def weights(m, prods):
            def w_of(r):
                s = W_FORMS.index(prods[r][1])
                return wc[cs][m * 128:(m + 1) * 128, s * 128:(s + 1) * 128]
            return w_of

        def q_(u, lo_, hi_):
            b, br = b0 + u // 2, u % 2

            def lhs_of(r):
                return xc[(_mul(b * 2 + br, hq), hq), r * 128:(r + 1) * 128]

            _bilinear_run(QA.setdefault(u, {}), Q_PRODS, qord[u % len(qord)][lo_:hi_], lhs_of, weights(br, Q_PRODS), tick)
            if hi_ == NPROD:
                fin = _bilinear_finish(QA[u], Q_OUT_PROG)

                def store_q():
                    c = [[fin[i * 3 + n] for n in range(3)] for i in range(2)]
                    for h, ops in enumerate(_q_operands(c)):
                        for i, a in enumerate(ops):
                            qbuf[u * hq:(u + 1) * hq, (3 * h + i) * 128:(3 * h + i + 1) * 128] = a.astype(bf16)

                lazy["q", u] = store_q

        def s_(u, h, j):
            b, br = b0 + u // 2, u % 2
            lazy.pop(("q", u), lambda: None)()
            qh = [qbuf[u * hq:(u + 1) * hq, (3 * h + i) * 128:(3 * h + i + 1) * 128] for i in range(3)]
            SC[u, h, j] = _scores_half(qh, kvbuf.at[b, 2 * br], h, j, tick)
            if j == 1:
                s = jnp.concatenate(SC[u, h, 0] + SC[u, h, 1], axis=1)

                def store_p():
                    p, R[u, h] = _softmax(s)
                    pbuf[prow(u, h):prow(u, h) + sq, :] = p

                lazy["p", u, h] = store_p

        def m_(u, h, half):
            lazy.pop(("p", u, h), lambda: None)()
            vt = kvbuf.at[b0 + u // 2 + (g0 >> 20) * half, 2 * (u % 2) + 1]
            r0 = prow(u, h) + half * hq
            res = [tick(lax.dot_general(pbuf[r0:r0 + hq, i * 256:(i + 1) * 256], _pv_weights(vt, h, i), NT,
                                        preferred_element_type=f32), 40) for i in range(3)]
            lo = lax.broadcasted_iota(jnp.int32, (hq, 128), 1) < 64
            r = R[u, h][half * hq:(half + 1) * hq]
            O[u, h, half] = (res[0] + jnp.where(lo, res[2], res[1])) * r
            OT[u, h, half] = jnp.where(lo, res[1], res[2]) * r

        def o_(u, lo_, hi_):
            b, br = b0 + u // 2, u % 2
            if lo_ == 0:
                lo = lax.broadcasted_iota(jnp.int32, (hq, 128), 1) < 64
                mid = [jnp.where(lo, OT[u, 0, i], OT[u, 1, i]) +
                       pltpu.roll(jnp.where(lo, OT[u, 1, i], OT[u, 0, i]), 64, 1) for i in range(2)]
                tiles = [[O[u, 0, i], mid[i], O[u, 1, i]] for i in range(2)]
                get = _make_lhs(lambda x: tiles[x // 3][x % 3], O_LHS_PROG)
                LH[u] = {p[0]: get(p[0]).astype(bf16) for p in O_PRODS}
            _bilinear_run(OA.setdefault(u, {}), O_PRODS, oord[u % len(oord)][lo_:hi_], lambda r: LH[u][O_PRODS[r][0]],
                          weights(2 + br, O_PRODS), tick)
            if hi_ < NPROD:
                return
            fin = _bilinear_finish(OA[u], O_OUT_PROG)
            for n in range(5):
                for i in range(2):
                    s, a = fin[i * 5 + n]
                    rows = slice(i * hq, (i + 1) * hq)
                    cols = slice(br * d + n * 128, br * d + (n + 1) * 128)
                    if first_hp:
                        new = a if s > 0 else -a
                    else:
                        new = acc[b, rows, cols] + a if s > 0 else acc[b, rows, cols] - a
                    if last_hp:
                        obuf[b, rows, cols] = new.astype(obuf.dtype)
                    else:
                        acc[b, rows, cols] = new
            if br == 1 and last_hp:
                pltpu.make_async_copy(obuf.at[b], o_hbm.at[b], o_sem).start()

        fns = {"qa": lambda u: q_(u, 0, qsp), "qb": lambda u: q_(u, qsp, NPROD),
               "oa": lambda u: o_(u, 0, osp), "ob": lambda u: o_(u, osp, NPROD),
               "s00": lambda u: s_(u, 0, 0), "s01": lambda u: s_(u, 0, 1),
               "s10": lambda u: s_(u, 1, 0), "s11": lambda u: s_(u, 1, 1),
               "m0": lambda u: m_(u, 0, 0), "m1": lambda u: m_(u, 1, 0),
               "t0": lambda u: m_(u, 0, 1), "t1": lambda u: m_(u, 1, 1)}
        for f in first:
            f()
        total = 2 * nbat * 1960
        lastq = max(i for i, it in enumerate(sched) if it[0][0] == "q")
        for k, f in enumerate(wpre):
            lo_, hi_ = (PLO, total - PHI) if nbat > 1 else (SWLO, SWHI)
            later(lo_ + k * (hi_ - lo_) // len(wpre), f)
        for i, item in enumerate(sched):
            fns[item[0]](item[1])
            if i == lastq:
                for k, f in enumerate(xpre):
                    later(SXLO + k * (total - SXHI - clock[0] - SXLO) // len(xpre), f)
        assert not pending and not lazy

    for k in range(4):
        w_start(0, k)
    x_start(0)
    kv_start(0)
    x_start(1)
    for g in range(1, C0):
        kv_start(g)
        x_start(g + 1)
    for m in range(4):
        w_wait(m)
        prep_w(0, m, m, 0, 8)
    x_wait(0)
    for br in range(2):
        prep_x(0, br)

    def issued(g):
        return jnp.minimum(jnp.minimum(RATE * (g + 1) + C0, jnp.maximum(g + LA, LB * g - LC)), nb + DIST * BB)

    def ramp(b0, carry):
        half = nb // 2
        m = (b0 - half) >> 1

        @pl.when(b0 + 1 < nb)
        def _():
            x_wait(b0 + 1)

        @pl.when(jnp.logical_and(b0 >= half, (b0 & 1) == 0))
        def _():
            w_wait(m)

        kv_wait(b0)

        hi = issued(b0)
        prev = jnp.where(b0 == 0, C0, issued(b0 - 1))

        def pf_x(k, w):
            @pl.when(jnp.logical_and(prev + k < hi, prev + k + 1 < nb))
            def _():
                x_start(prev + k + 1, (w,))

        def pf_kv(k):
            @pl.when(prev + k < hi)
            def _():
                kv_start(prev + k)

        def pf_w():
            w_start_dyn(jnp.where(b0 == W2AT, 2, 1), jnp.where(b0 == W2AT, 0, (b0 >> 1) - 1),
                        jnp.logical_or(b0 == W2AT, jnp.logical_and(b0 <= half, (b0 & 1) == 0)))

        first = [pf_w] + [functools.partial(pf_x, k, w) for k in range(RATE) for w in range(2)]
        first += [functools.partial(pf_kv, k) for k in range(RATE)]
        zero = b0 >> 20
        wpre = [functools.partial(prep_w, 1, jnp.where(b0 >= half, m, 3), jnp.maximum(m, 0), (b0 & 1) * 4, 1,
                                  zero, k) for k in range(4)]
        xpre = [functools.partial(prep_x, jnp.minimum(b0 + 1, nb - 1), br, k, k + 1, zero)
                for br in range(2) for k in range(5)]
        body(b0, 1, first, wpre, xpre, RAMP, 0, first_hp=True)
        return carry

    def step(par, last, hp, i, carry):
        g0 = hp * nb + i * BB

        if not last:
            w_wait(i)

        kvg_wait(i)

        if last:
            def pf_kv():
                @pl.when(g0 + DIST * BB < ng)
                def _():
                    kvg_start(g0 + DIST * BB)

            body(g0, BB, [pf_kv], [], [], LAST, par, last_hp=True)
        else:
            hn = jnp.where(i == 3, hp + 2, hp + 1)
            first = [lambda: w_start_dyn(hn, (i + 1) & 3, hn < nhp), functools.partial(kvg_start, g0 + DIST * BB)]
            wpre = [functools.partial(prep_w, 1 - par, i, i, 0, 1, i >> 20, k) for k in range(8)]
            body(g0, BB, first, wpre, [], STEADY, par)
        return carry

    def pair(t, carry):
        lax.fori_loop(jnp.where(t > 0, 0, spb), spb, functools.partial(step, 0, False, 2 * t), 0)
        lax.fori_loop(0, jnp.where(2 * t + 1 < nhp - 1, spb, 0), functools.partial(step, 1, False, 2 * t + 1), 0)
        return carry

    lax.fori_loop(0, nb, ramp, 0)
    lax.fori_loop(0, nhp // 2, pair, 0)
    lax.fori_loop(0, spb, functools.partial(step, 1, True, nhp - 1), 0)
    pltpu.make_async_copy(obuf, o_hbm, o_sem).wait()


@jax.jit
def pallas_concat_heads__gqa_block_cached__mha_block_cached__near_ridge_kernel(
    A_x: jax.Array,
    A_k_cache: jax.Array,
    A_v_cache: jax.Array,
    A_wq: jax.Array,
    A_wo: jax.Array,
    B_x: jax.Array,
    B_k_cache: jax.Array,
    B_v_cache: jax.Array,
    B_wq: jax.Array,
    B_wo: jax.Array,
):
    B, Sq, D = A_x.shape
    _, H, Sk, Dh = A_k_cache.shape
    nhp = H // 2
    assert (B, Sq, D, Sk, Dh) == (16, 160, 640, 512, 192) and A_wq.shape[1] == H * Dh
    assert nhp >= 4 and nhp & (nhp - 1) == 0 and B_k_cache.shape == A_k_cache.shape
    n_iss = C0
    for g0 in range(B):
        assert n_iss >= g0 + 2
        hi = min(RATE * (g0 + 1) + C0, max(g0 + LA, LB * g0 - LC), B + DIST * BB)
        assert hi <= g0 + B and 0 <= hi - n_iss <= RATE
        n_iss = hi
    assert n_iss == B + DIST * BB and 10 <= W2AT <= 15

    def tr(c):
        return jnp.swapaxes(c, 2, 3).reshape(B, nhp, 2 * Dh, Sk)

    any_spec = pl.BlockSpec(memory_space=pl.ANY)
    return pl.pallas_call(
        functools.partial(_kernel, scale=Dh ** -0.5 * LOG2E, nhp=nhp, nb=B),
        in_specs=[any_spec] * 10,
        out_specs=any_spec,
        out_shape=jax.ShapeDtypeStruct((B, Sq, 2 * D), A_x.dtype),
        scratch_shapes=[pltpu.VMEM((B, Sq, 2 * D), f32),
                        pltpu.VMEM((B, 2, Sq, D), bf16),
                        pltpu.VMEM((4 * 15 * 128, 128), bf16),
                        pltpu.VMEM((B, 4, 2 * Dh, Sk), bf16),
                        pltpu.VMEM((B, Sq, 2 * D), bf16),
                        pltpu.VMEM((2 * BB * Sq, 6 * 128), u32),
                        pltpu.VMEM((2 * BB * Sq // 4, 6 * 128), u32),
                        pltpu.VMEM((B * 2 * Sq // 4, XCW * 128), u32),
                        pltpu.VMEM((4 * 64, WCW * 128), u32),
                        pltpu.VMEM((4 * 64, WCW * 128), u32),
                        pltpu.SemaphoreType.DMA((B + 4,)),
                        pltpu.SemaphoreType.DMA((B,)),
                        pltpu.SemaphoreType.DMA((4,)),
                        pltpu.SemaphoreType.DMA(())],
        compiler_params=pltpu.CompilerParams(
            disable_bounds_checks=True,
            vmem_limit_bytes=110 * 1024 * 1024),
    )(A_x, tr(A_k_cache), tr(A_v_cache), A_wq, A_wo, B_x, tr(B_k_cache), tr(B_v_cache), B_wq, B_wo)
```
